```python
import jax
import jax.numpy as jnp

def _softmax(x, axis=-1):
    return jax.nn.softmax(x, axis=axis)
def _gelu(x):
    return jax.nn.gelu(x, approximate=True)
def _silu(x):
    return jax.nn.silu(x)
def _sigmoid(x):
    return jax.nn.sigmoid(x)
def _layernorm(x, axis=-1, eps=1e-5):
    m = jnp.mean(x, axis=axis, keepdims=True)
    v = jnp.var(x, axis=axis, keepdims=True)
    return (x - m) / jnp.sqrt(v + eps)
def _scatter_add(tgt, idx, src, axis=0):
    return tgt.at[idx].add(src)
def _segment_sum(src, seg, n):
    return jax.ops.segment_sum(src, seg, n)
class _Rng:
    def __init__(self, key):
        self._k = key
    def _next(self):
        self._k, sub = jax.random.split(self._k)
        return sub
    def normal(self, shape):
        return jax.random.normal(self._next(), shape, dtype=jnp.bfloat16)
    def randint(self, lo, hi, shape):
        return jax.random.randint(self._next(), shape, lo, hi, dtype=jnp.int32)
    def uniform(self, shape, lo=0.0, hi=1.0):
        return jax.random.uniform(self._next(), shape, jnp.bfloat16, lo, hi)
    def permutation(self, n):
        return jax.random.permutation(self._next(), n)


kernel_name = 'concat_heads__ssm_conv_h3__sliding_local_dilated__prompt'

def setup_inputs():
    _rng = _Rng(jax.random.key(int.from_bytes(__import__("os").urandom(4), "little")))
    _w = (lambda a: (lambda t: t.astype(jnp.bfloat16) if jnp.issubdtype(t.dtype, jnp.floating) else t)(jnp.asarray(a)))
    def _A_setup():
        B, S, D = 1, 2048, 1024
        ks = 4
        return {
            "q": _w((lambda *s: _rng.normal(s) * 0.05)(B, S, D)),
            "k": _w((lambda *s: _rng.normal(s) * 0.05)(B, S, D)),
            "v": _w((lambda *s: _rng.normal(s) * 0.05)(B, S, D)),
            "shift_k": _w((lambda *s: _rng.normal(s) * 0.05)(D, ks) * 0.5),
            "ssm_k": _w((lambda *s: _rng.normal(s) * 0.05)(D, S) * (1.0 / S ** 0.5)),
            "ssm_D": _w((lambda *s: _rng.normal(s) * 0.05)(D)),
        }
    _A_in = _A_setup()

    def _B_setup():
        B, S, D = 1, 2048, 1024
        return {
            "x": _w((lambda *s: _rng.normal(s) * 0.05)(B, S, D)),
            "wqkv": _w((lambda *s: _rng.normal(s) * 0.05)(D, 3 * D)),
            "wo": _w((lambda *s: _rng.normal(s) * 0.05)(D, D)),
        }
    _B_in = _B_setup()

    return {
        "A_q": _A_in["q"],
        "A_k": _A_in["k"],
        "A_v": _A_in["v"],
        "A_shift_k": _A_in["shift_k"],
        "A_ssm_k": _A_in["ssm_k"],
        "A_ssm_D": _A_in["ssm_D"],
        "B_x": _B_in["x"],
        "B_wqkv": _B_in["wqkv"],
        "B_wo": _B_in["wo"],
    }

def reference(A_q, A_k, A_v, A_shift_k, A_ssm_k, A_ssm_D, B_x, B_wqkv, B_wo):
    def _A_ref(q, k, v, shift_k, ssm_k, ssm_D):
        B, S, D = q.shape
        ks = shift_k.shape[-1]
        k_pad = jnp.pad(k, ((0, 0), (ks - 1, 0), (0, 0)))
        k_shift = jnp.zeros_like(k)
        for t in range(ks):
            k_shift = k_shift + k_pad[:, t:t + S, :] * shift_k[:, ks - 1 - t][None, None, :]
        kv = k_shift * v
        L = 2 * S
        kv_pad = jnp.pad(kv, ((0, 0), (0, S), (0, 0)))
        kf_pad = jnp.pad(ssm_k, ((0, 0), (0, S)))
        kv_f = (lambda x, axes=(-2,-1): jnp.fft.rfft2(x.astype(jnp.float32), axes=axes))(kv_pad[:, None, :, :], axes=(1, 2))
        kf_f = (lambda x, axes=(-2,-1): jnp.fft.rfft2(x.astype(jnp.float32), axes=axes))(kf_pad[:, None, :], axes=(1, 2))
        kf_f = (lambda x, *d: x.transpose(*d))(kf_f, 1, 2, 0)
        y_f = kv_f * kf_f[None, :, :, :]
        y = (lambda x, s, axes=(-2,-1): jnp.fft.irfft2(x, s=s, axes=axes).astype(jnp.bfloat16))(y_f, (1, L), axes=(1, 2))[:, 0, :S, :]
        y = y + kv * ssm_D[None, None, :]
        return q * y

    def _B_ref(x, wqkv, wo):
        B, S, D = x.shape
        H = 32; Dh = D // H
        W, dil = 8, 2
        qkv = (lambda x, *d: x.transpose(*d))((x @ wqkv).reshape(B, S, 3, H, Dh), 2, 0, 3, 1, 4)
        q, k, v = qkv[0], qkv[1], qkv[2]
        scale = Dh ** -0.5
        pos = jnp.arange(S)
        off = jnp.arange(W) * dil
        idx = pos[:, None] - off[None, :]
        mask = idx >= 0
        idx_c = jnp.where(mask, idx, 0).reshape(-1)
        kg = k[:, :, idx_c, :].reshape(B, H, S, W, Dh)
        vg = v[:, :, idx_c, :].reshape(B, H, S, W, Dh)
        logits = jnp.einsum("bhsd,bhswd->bhsw", q, kg) * scale
        logits = jnp.where(mask[None, None, :, :], logits, -1e9)
        attn = _softmax(logits, axis=-1)
        o = jnp.einsum("bhsw,bhswd->bhsd", attn, vg)
        return (lambda x, *d: x.transpose(*d))(o, 0, 2, 1, 3).reshape(B, S, D) @ wo

    a = _A_ref(A_q, A_k, A_v, A_shift_k, A_ssm_k, A_ssm_D)
    b = _B_ref(B_x, B_wqkv, B_wo)
    return jnp.concatenate([a, b], axis=-1)
```

```python
import functools

import jax
import jax.numpy as jnp
import numpy as np
from jax import lax
from jax.experimental import pallas as pl
import jax.experimental.pallas.tpu as pltpu

S = 2048
D = 1024
T = 128
NC = S // T
NS = 8
R = S // NS
NT = D // 128
WIN, DIL, DH = 8, 2, 32
HALO = 16
PITCH = 33

F32, BF16, U32 = jnp.float32, jnp.bfloat16, jnp.uint32


def _dft_matrices():
    n = np.arange(T)[None, :]
    f = np.arange(T)[:, None]
    th = 2.0 * np.pi * (f + 0.25) * n / T
    fwd = np.concatenate([np.cos(th), -np.sin(th)], axis=0)
    inv = fwd.T / T
    return fwd.astype(jnp.bfloat16), np.ascontiguousarray(inv).astype(jnp.bfloat16)


_FWD, _INV = _dft_matrices()


def _lo(w):
    return pltpu.bitcast(w << 16, F32)


def _hi(w):
    return pltpu.bitcast(w & jnp.uint32(0xFFFF0000), F32)


def _kernel(q_hbm, k_hbm, v_hbm, sk_ref, h_hbm, d_ref, x_hbm, w_hbm, wo_hbm,
            fwd_ref, inv_ref, out_hbm,
            qa, ka, va, ha, xb, wraw, wp, woraw, wop, tbuf, taps,
            kvb, xf, hf, zb, qs, ks, vs, ob, oa_st, ob_st,
            sem_in, sem_w, sem_out):

    def in_copies(j, slot):
        cols = pl.ds(pl.multiple_of(j * 128, 128), 128)
        rows = pl.ds(pl.multiple_of(j * R, R), R)
        return [
            pltpu.make_async_copy(h_hbm.at[cols, :], ha.at[slot], sem_in.at[slot, 0]),
            pltpu.make_async_copy(k_hbm.at[:, cols], ka.at[slot, pl.ds(16, S), :], sem_in.at[slot, 1]),
            pltpu.make_async_copy(v_hbm.at[:, cols], va.at[slot], sem_in.at[slot, 2]),
            pltpu.make_async_copy(x_hbm.at[rows, :], xb.at[slot], sem_in.at[slot, 3]),
            pltpu.make_async_copy(q_hbm.at[:, cols], qa.at[slot], sem_in.at[slot, 4]),
        ]

    def out_copies(j, slot):
        cols = pl.ds(pl.multiple_of(j * 128, 128), 128)
        rows = pl.ds(pl.multiple_of(j * R, R), R)
        return [
            pltpu.make_async_copy(oa_st.at[slot], out_hbm.at[:, cols], sem_out.at[slot, 0]),
            pltpu.make_async_copy(ob_st.at[slot], out_hbm.at[rows, pl.ds(D, D)], sem_out.at[slot, 1]),
        ]

    def w_copy(p):
        return pltpu.make_async_copy(
            w_hbm.at[:, pl.ds(p * D, D)], wraw.at[p], sem_w.at[p])

    wo_copy = pltpu.make_async_copy(wo_hbm, woraw, sem_w.at[3])

    for c in in_copies(0, 0):
        c.start()
    for p in range(3):
        w_copy(p).start()
    wo_copy.start()

    for slot in range(2):
        ka[slot, pl.ds(0, 16), :] = jnp.zeros((16, 128), BF16)
    ks[:, pl.ds(R, HALO), :] = jnp.zeros((NT, HALO, 128), F32)
    vs[:, pl.ds(R, HALO), :] = jnp.zeros((NT, HALO, 128), F32)
    skf = sk_ref[...].astype(F32)
    df = d_ref[...].astype(F32)
    for t in range(NT):
        for i in range(4):
            taps[t, i] = jnp.broadcast_to(skf[i:i + 1, t * 128:(t + 1) * 128], (8, 128))
        taps[t, 4] = jnp.broadcast_to(df[t:t + 1, :], (8, 128))

    wraw32 = wraw.bitcast(U32)
    for p in range(3):
        w_copy(p).wait()

        def perm_w(rb, carry, p=p):
            rows = pl.ds(pl.multiple_of(rb * 128, 128), 128)
            for t in range(NT):
                tt = wraw32[p, rows, pl.ds(t * 128, 128)].T
                for hh in range(4):
                    tbuf[pl.ds((4 * t + hh) * PITCH, DH), :] = tt[hh * DH:(hh + 1) * DH]
            for t in range(NT):
                g = jnp.concatenate(
                    [tbuf[pl.ds(4 * t + u, 32, stride=PITCH), :] for u in range(4)], axis=0)
                wp[p, rows, pl.ds(t * 128, 128)] = g.T
            return carry

        lax.fori_loop(0, D // 256, perm_w, 0)

    wo_copy.wait()
    for t in range(NT):
        wt = woraw[:, pl.ds(t * 128, 128)].astype(F32)
        for hh in range(32):
            tbuf[pl.ds(hh * PITCH, DH), :] = pltpu.bitcast(wt[hh * DH:(hh + 1) * DH], U32)
        g = jnp.concatenate([tbuf[pl.ds(u, 32, stride=PITCH), :] for u in range(DH)], axis=0)
        wop[:, pl.ds(t * 128, 128)] = pltpu.bitcast(pltpu.bitcast(g, F32).astype(BF16), U32)

    def step(j, carry):
        slot = j % 2
        for c in in_copies(j, slot):
            c.wait()

        @pl.when(j + 1 < NS)
        def _():
            for c in in_copies(j + 1, 1 - slot):
                c.start()

        @pl.when(j >= 2)
        def _():
            for c in out_copies(j - 2, slot):
                c.wait()

        k32 = ka.bitcast(U32)
        v32 = va.bitcast(U32)

        def a1(lo, hi):
            w0, w1, w2, w3 = (taps[j, i] for i in range(4))
            for r in range(lo, hi):
                c0 = k32[slot, pl.ds(8 + 8 * r, 8), :]
                c1 = k32[slot, pl.ds(7 + 8 * r, 8), :]
                c2 = k32[slot, pl.ds(6 + 8 * r, 8), :]
                vv = v32[slot, pl.ds(8 * r, 8), :]
                e0, o0, e1, o1, o2 = _lo(c0), _hi(c0), _lo(c1), _hi(c1), _hi(c2)
                ke = (e0 * w0 + o1 * w1) + (e1 * w2 + o2 * w3)
                ko = (o0 * w0 + e0 * w1) + (o1 * w2 + e1 * w3)
                kv = pltpu.pack_elementwise([ke * _lo(vv), ko * _hi(vv)], packed_dtype=BF16)
                kvb[pl.ds(8 * r, 8), :] = kv

        def proj(p, dst, off):
            w = pltpu.bitcast(wp[p], BF16)
            res = jnp.dot(xb[slot], w, preferred_element_type=F32)
            for t in range(NT):
                dst[t, pl.ds(off, R), :] = res[:, t * 128:(t + 1) * 128]

        def dft_h():
            hblk = jnp.concatenate([ha[slot, :, pl.ds(c * T, T)] for c in range(NC)], axis=0)
            res = lax.dot_general(fwd_ref[...], hblk, (((1,), (1,)), ((), ())),
                                  preferred_element_type=F32)
            for c in range(NC):
                hf[c] = res[:, c * 128:(c + 1) * 128]

        def dft_x():
            xblk = jnp.concatenate(
                [pltpu.bitcast(kvb[pl.ds(c * 64, 64), :], BF16) for c in range(NC)], axis=1)
            res = jnp.dot(fwd_ref[...], xblk, preferred_element_type=F32)
            for c in range(NC):
                xf[c] = res[:, c * 128:(c + 1) * 128]

        def conv(a, b):
            out = []
            for n in range(NC):
                acc = a[n] * b[0]
                for c in range(1, n + 1):
                    acc = acc + a[n - c] * b[c]
                out.append(acc)
            return out

        def a3_group(g):
            re, im = pl.ds(8 * g, 8), pl.ds(T + 8 * g, 8)
            ur = [hf[c, re, :] for c in range(NC)]
            ui = [hf[c, im, :] for c in range(NC)]
            cr = [ur[0]] + [ur[c] - ui[c - 1] for c in range(1, NC)]
            ci = [ui[0]] + [ui[c] + ur[c - 1] for c in range(1, NC)]
            ar = [xf[c, re, :] for c in range(NC)]
            ai = [xf[c, im, :] for c in range(NC)]
            k1 = conv([p + q for p, q in zip(ar, ai)], cr)
            k2 = conv(ar, [q - p for p, q in zip(cr, ci)])
            zi = [p + q for p, q in zip(k1, k2)]
            k3 = conv(ai, [q + p for p, q in zip(cr, ci)])
            zr = [p - q for p, q in zip(k1, k3)]
            for c in range(NC):
                zb[c, pl.ds(8 * g, 8), :] = pltpu.pack_elementwise([zr[c], zi[c]], packed_dtype=BF16)

        def a4():
            zblk = jnp.concatenate([pltpu.bitcast(zb[c], BF16) for c in range(NC)], axis=1)
            y = jnp.dot(inv_ref[...], zblk, preferred_element_type=F32)
            dd = taps[j, 4][0:1]
            for c in range(NC):
                rows = pl.ds(c * T, T)
                kv = pltpu.bitcast(kvb[pl.ds(c * 64, 64), :], BF16).astype(F32)
                yy = y[:, c * 128:(c + 1) * 128] + kv * dd
                oa_st[slot, rows, :] = (qa[slot, rows, :].astype(F32) * yy).astype(BF16)

        def halo_in():
            for t in range(NT):
                ks[t, pl.ds(0, HALO), :] = ks[t, pl.ds(R, HALO), :]
                vs[t, pl.ds(0, HALO), :] = vs[t, pl.ds(R, HALO), :]

        def halo_fix():
            for t in range(NT):
                first = jnp.broadcast_to(vs[t, pl.ds(HALO, 1), :], (HALO, 128))
                vs[t, pl.ds(0, HALO), :] = jnp.where(j == 0, first, vs[t, pl.ds(0, HALO), :])

        def attn8(r):
            base = HALO + 8 * r
            qv = [qs[t, pl.ds(8 * r, 8), :] for t in range(NT)]
            lg = []
            for w in range(WIN):
                pr = [qv[t] * ks[t, pl.ds(base - DIL * w, 8), :] for t in range(NT)]
                s = ((pr[0] + pr[1]) + (pr[2] + pr[3])) + ((pr[4] + pr[5]) + (pr[6] + pr[7]))
                s = s + pltpu.roll(s, 64, 1)
                s = s + pltpu.roll(s, 32, 1)
                s = s * (DH ** -0.5)
                if 8 * r < DIL * w:
                    pos = j * R + 8 * r + lax.broadcasted_iota(jnp.int32, (8, 128), 0)
                    s = jnp.where(pos >= DIL * w, s, -1e9)
                lg.append(s)
            m = functools.reduce(jnp.maximum, lg)
            e = [jnp.exp(s - m) for s in lg]
            inv = 1.0 / functools.reduce(jnp.add, e)
            p = [x * inv for x in e]
            o = []
            for t in range(NT):
                pr = [p[w] * vs[t, pl.ds(base - DIL * w, 8), :] for w in range(WIN)]
                o.append(((pr[0] + pr[1]) + (pr[2] + pr[3])) + ((pr[4] + pr[5]) + (pr[6] + pr[7])))
            return o

        def attn16(r):
            o0, o1 = attn8(2 * r), attn8(2 * r + 1)
            for t in range(NT):
                o = jnp.concatenate([o0[t], o1[t]], axis=0).astype(BF16)
                ob[pl.ds(8 * r, 8), pl.ds(t * 128, 128)] = pltpu.bitcast(o, U32)

        def out_proj():
            res = jnp.dot(pltpu.bitcast(ob[...], BF16), pltpu.bitcast(wop[...], BF16),
                          preferred_element_type=F32)
            ob_st[slot] = res.astype(BF16)

        halo_in()
        dft_h()
        a1(0, S // 16)
        dft_x()
        proj(0, qs, 0)
        for g in range(0, 8):
            a3_group(g)
        proj(1, ks, HALO)
        for g in range(8, 16):
            a3_group(g)
        proj(2, vs, HALO)
        halo_fix()
        for r in range(R // 16):
            attn16(r)
        a4()
        out_proj()

        for c in out_copies(j, slot):
            c.start()
        return carry

    lax.fori_loop(0, NS, step, 0)
    for j in (NS - 2, NS - 1):
        for c in out_copies(j, j % 2):
            c.wait()


@jax.jit
def pallas_concat_heads__ssm_conv_h3__sliding_local_dilated__prompt_kernel(
    A_q, A_k, A_v, A_shift_k, A_ssm_k, A_ssm_D, B_x, B_wqkv, B_wo,
):
    order = np.stack([np.arange(T), T + np.arange(T)], axis=1).reshape(-1)
    inv = np.ascontiguousarray(_INV[:, order])
    hbm = pl.BlockSpec(memory_space=pl.ANY)
    vmem = pl.BlockSpec(memory_space=pltpu.VMEM)
    out = pl.pallas_call(
        _kernel,
        in_specs=[hbm, hbm, hbm, vmem, hbm, vmem, hbm, hbm, hbm, vmem, vmem],
        out_specs=hbm,
        out_shape=jax.ShapeDtypeStruct((S, 2 * D), BF16),
        scratch_shapes=[
            pltpu.VMEM((2, S, 128), BF16),
            pltpu.VMEM((2, 16 + S, 128), BF16),
            pltpu.VMEM((2, S, 128), BF16),
            pltpu.VMEM((2, 128, S), BF16),
            pltpu.VMEM((2, R, D), BF16),
            pltpu.VMEM((3, D, D), BF16),
            pltpu.VMEM((3, D // 2, D), U32),
            pltpu.VMEM((D, D), BF16),
            pltpu.VMEM((D // 2, D), U32),
            pltpu.VMEM((32 * PITCH, 128), U32),
            pltpu.VMEM((NT, 5, 8, 128), F32),
            pltpu.VMEM((S // 2, 128), U32),
            pltpu.VMEM((NC, 2 * T, 128), F32),
            pltpu.VMEM((NC, 2 * T, 128), F32),
            pltpu.VMEM((NC, T, 128), U32),
            pltpu.VMEM((NT, R, 128), F32),
            pltpu.VMEM((NT, HALO + R, 128), F32),
            pltpu.VMEM((NT, HALO + R, 128), F32),
            pltpu.VMEM((R // 2, D), U32),
            pltpu.VMEM((2, S, 128), BF16),
            pltpu.VMEM((2, R, D), BF16),
            pltpu.SemaphoreType.DMA((2, 5)),
            pltpu.SemaphoreType.DMA((4,)),
            pltpu.SemaphoreType.DMA((2, 2)),
        ],
        compiler_params=pltpu.CompilerParams(vmem_limit_bytes=100 * 1024 * 1024),
        name="fused",
    )(A_q[0], A_k[0], A_v[0], A_shift_k.T, A_ssm_k, A_ssm_D.reshape(8, 128),
      B_x[0], B_wqkv, B_wo, _FWD, inv)
    return out[None]
```

```python
import functools

import jax
import jax.numpy as jnp
import numpy as np
from jax import lax
from jax.experimental import pallas as pl
import jax.experimental.pallas.tpu as pltpu

S = 2048
D = 1024
T = 128
NC = S // T
NS = 8
R = S // NS
NT = D // 128
WIN, DIL, DH = 8, 2, 32
HALO = 16
PITCH = 33
KR = HALO + R

F32, BF16, U32 = jnp.float32, jnp.bfloat16, jnp.uint32


def _pack_rows(m):
    b = m.astype(jnp.bfloat16).view(np.uint16).astype(np.uint32)
    return np.ascontiguousarray(b[0::2] | (b[1::2] << 16))


def _dft_matrices():
    n = np.arange(T)[None, :]
    f = np.arange(T)[:, None]
    th = 2.0 * np.pi * (f + 0.25) * n / T
    fwd = np.concatenate([np.cos(th), -np.sin(th)], axis=0)
    order = np.stack([np.arange(T), T + np.arange(T)], axis=1).reshape(-1)
    inv = fwd.T[:, order] / T
    return _pack_rows(fwd), _pack_rows(inv)


_FWD, _INV = _dft_matrices()


def _lo(w):
    return pltpu.bitcast(w << 16, F32)


def _hi(w):
    return pltpu.bitcast(w & jnp.uint32(0xFFFF0000), F32)


def _tree(xs):
    while len(xs) > 1:
        xs = [xs[i] + xs[i + 1] if i + 1 < len(xs) else xs[i] for i in range(0, len(xs), 2)]
    return xs[0]


def _weave(main, side):
    total_m = sum(c for c, _ in main)
    total_s = sum(c for c, _ in side)
    done_m, done_s, i = 0, 0, 0
    for c, f in main:
        f()
        done_m += c
        while i < len(side) and (done_s + side[i][0]) * total_m <= done_m * total_s:
            done_s += side[i][0]
            side[i][1]()
            i += 1
    assert i == len(side)


_BUFS = dict(
    hf=NC * 2 * T, xf=NC * 2 * T, kv0=S // 4, kv1=S // 4, z=NC * T,
    up=8 * NC, k1=8 * NC, pi=8 * NC, oa=S, part=R,
    q=NT * R, k=NT * KR, v0=4 * KR, v1=4 * KR, p=WIN * R,
    o0=4 * R // 2, o1=4 * R // 2, acc=NT * R,
)


def _kernel(z_ref, q_hbm, k_hbm, v_hbm, sk_ref, h_hbm, d_ref, x_hbm, w_hbm, wo_hbm,
            fwd_ref, inv_ref, out_hbm,
            qa, ka, va, ha, xb, wraw, wp, woraw, wop, tbuf, taps, ob_st,
            sem_in, sem_w, sem_out, *bufs):
    bufs = dict(zip(_BUFS, bufs))
    zs = [pl.multiple_of(z_ref[i] * 8, 8) for i in range(3)]
    views = {n: [b.at[pl.ds(z, _BUFS[n]), :] for z in zs] + [b] for n, b in bufs.items()}

    def ld(name, row, n=8, z=0):
        return views[name][z][pl.ds(row, n), :]

    def ldf(name, row, n=8, z=0):
        return pltpu.bitcast(ld(name, row, n, z), F32)

    def st(name, row, val):
        val = pltpu.bitcast(val, U32)
        bufs[name][pl.ds(row, val.shape[0]), :] = val

    def in_copies(j, slot):
        cols = pl.ds(pl.multiple_of(j * 128, 128), 128)
        rows = pl.ds(pl.multiple_of(j * R, R), R)
        return [
            pltpu.make_async_copy(h_hbm.at[cols, :], ha.at[slot], sem_in.at[slot, 0]),
            pltpu.make_async_copy(k_hbm.at[:, cols], ka.at[slot, pl.ds(16, S), :], sem_in.at[slot, 1]),
            pltpu.make_async_copy(v_hbm.at[:, cols], va.at[slot], sem_in.at[slot, 2]),
        ] + [
            pltpu.make_async_copy(x_hbm.at[rows, pl.ds(t * 128, 128)], xb.at[slot, t], sem_in.at[slot, 3])
            for t in range(NT)
        ] + [
            pltpu.make_async_copy(q_hbm.at[:, cols], qa.at[slot], sem_in.at[slot, 4]),
        ]

    def out_copies(j, slot):
        cols = pl.ds(pl.multiple_of(j * 128, 128), 128)
        rows = pl.ds(pl.multiple_of(j * R, R), R)
        src = bufs["oa"].bitcast(BF16).at[pl.ds(pl.multiple_of(slot * S, 16), S), :]
        return [
            pltpu.make_async_copy(src, out_hbm.at[:, cols], sem_out.at[slot, 0]),
        ] + [
            pltpu.make_async_copy(ob_st.at[slot, t], out_hbm.at[rows, pl.ds(D + t * 128, 128)],
                                  sem_out.at[slot, 1])
            for t in range(NT)
        ]

    def w_copy(p):
        return pltpu.make_async_copy(
            w_hbm.at[:, pl.ds(p * D, D)], wraw.at[p], sem_w.at[p])

    wo_copy = pltpu.make_async_copy(wo_hbm, woraw, sem_w.at[3])

    for c in in_copies(0, 0):
        c.start()
    for p in range(3):
        w_copy(p).start()
    wo_copy.start()

    for slot in range(2):
        ka[slot, pl.ds(0, 16), :] = jnp.zeros((16, 128), BF16)
    for t in range(NT):
        st("k", t * KR + R, jnp.zeros((HALO, 128), F32))
        st(f"v{t // 4}", t % 4 * KR + R, jnp.zeros((HALO, 128), F32))
    skf = sk_ref[...].astype(F32)
    df = d_ref[...].astype(F32)
    for t in range(NT):
        for i in range(4):
            taps[t, i] = jnp.broadcast_to(skf[i:i + 1, t * 128:(t + 1) * 128], (8, 128))
        taps[t, 4] = jnp.broadcast_to(df[t:t + 1, :], (8, 128))

    wraw32 = wraw.bitcast(U32)
    for p in range(3):
        w_copy(p).wait()

        def perm_w(rb, carry, p=p):
            rows = pl.ds(pl.multiple_of(rb * 128, 128), 128)
            for t in range(NT):
                tt = wraw32[p, rows, pl.ds(t * 128, 128)].T
                for hh in range(4):
                    tbuf[pl.ds((4 * t + hh) * PITCH, DH), :] = tt[hh * DH:(hh + 1) * DH]
            for t in range(NT):
                g = jnp.concatenate(
                    [tbuf[pl.ds(4 * t + u, 32, stride=PITCH), :] for u in range(4)], axis=0)
                wp[p, rows, pl.ds(t * 128, 128)] = g.T
            return carry

        lax.fori_loop(0, D // 256, perm_w, 0)

    wo_copy.wait()
    for t in range(NT):
        wt = woraw[:, pl.ds(t * 128, 128)].astype(F32)
        for hh in range(32):
            tbuf[pl.ds(hh * PITCH, DH), :] = pltpu.bitcast(wt[hh * DH:(hh + 1) * DH], U32)
        g = jnp.concatenate([tbuf[pl.ds(u, 32, stride=PITCH), :] for u in range(DH)], axis=0)
        wop[:, pl.ds(t * 128, 128)] = pltpu.bitcast(pltpu.bitcast(g, F32).astype(BF16), U32)

    def step(j, carry):
        slot = j % 2
        for c in in_copies(j, slot):
            c.wait()

        @pl.when(j + 1 < NS)
        def _():
            for c in in_copies(j + 1, 1 - slot):
                c.start()

        @pl.when(j >= 2)
        def _():
            for c in out_copies(j - 2, slot):
                c.wait()

        k32, v32, q32, x32 = (r.bitcast(U32) for r in (ka, va, qa, xb))
        ob32 = ob_st.bitcast(U32)
        P = functools.partial
        oview = bufs["oa"].at[pl.ds(pl.multiple_of(slot * (S // 2), 8), S // 2), :]
        memo = {}
        never = jnp.full((8, 128), zs[0], jnp.int32) != 0

        def once(key, fn):
            if key not in memo:
                memo[key] = fn()
            return memo[key]

        def pace(val):
            return jnp.where(never, pltpu.bitcast(memo["clock"], val.dtype), val)

        def ld_kv(c, row, n, z=0):
            return pltpu.bitcast(ld(f"kv{c // 8}", c % 8 * (T // 2) + row, n, z), BF16)

        def a1(r):
            w0, w1, w2, w3 = once("taps", lambda: [taps[j, i] for i in range(4)])
            c0 = k32[slot, pl.ds(8 + 8 * r, 8), :]
            c1 = k32[slot, pl.ds(7 + 8 * r, 8), :]
            c2 = k32[slot, pl.ds(6 + 8 * r, 8), :]
            vv = v32[slot, pl.ds(8 * r, 8), :]
            e0, o0, e1, o1, o2 = _lo(c0), _hi(c0), _lo(c1), _hi(c1), _hi(c2)
            ke = (e0 * w0 + o1 * w1) + (e1 * w2 + o2 * w3)
            ko = (o0 * w0 + e0 * w1) + (o1 * w2 + e1 * w3)
            kv = pltpu.pack_elementwise([ke * _lo(vv), ko * _hi(vv)], packed_dtype=BF16)
            st(f"kv{r // 64}", 8 * (r % 64), pace(kv))

        def a1_list(c0, c1):
            return [(24, P(a1, r)) for r in range(8 * c0, 8 * c1)]

        def dft(name, c0, m):
            def mm():
                f = pltpu.bitcast(fwd_ref[...], BF16)
                if name == "hf":
                    rhs = jnp.concatenate(
                        [ha[slot, :, pl.ds(c * T, T)] for c in range(c0, c0 + 4)], axis=0)
                    return lax.dot_general(f, rhs, (((1,), (1,)), ((), ())),
                                           preferred_element_type=F32)
                rhs = jnp.concatenate([ld_kv(c, 0, T // 2) for c in range(c0, c0 + 4)], axis=1)
                return jnp.dot(f, rhs, preferred_element_type=F32)
            res = once((name, c0), mm)
            for u in range(4):
                memo["clock"] = res[m:m + 8, u * 128:(u + 1) * 128]
                st(name, (c0 + u) * 2 * T + m, memo["clock"])

        def dft_list(name, c0):
            return [(8, P(dft, name, c0, m)) for m in range(0, 2 * T, 8)]

        def a3(g, plane, upper, n):
            def opnd(name, c):
                re = lambda: ldf(name, c * 2 * T + 8 * g, z=plane)
                im = lambda: ldf(name, c * 2 * T + T + 8 * g, z=plane)
                if name == "xf":
                    return re() + im() if plane == 0 else re() if plane == 1 else im()
                return re() if plane == 0 else im() - re() if plane == 1 else im() + re()
            get = lambda name, c: once((name, g, plane, c), P(opnd, name, c))
            cs = range(8, n + 1) if upper else range(min(n, 7) + 1)
            terms = [get("xf", n - c) * get("hf", c) for c in cs]
            if upper:
                st("up", 8 * n, pace(_tree(terms)))
                return
            if n >= 8:
                terms.append(ldf("up", 8 * n))
            if plane == 0:
                st("k1", 8 * n, pace(_tree(terms)))
            elif plane == 1:
                st("pi", 8 * n, pace(_tree(terms + [ldf("k1", 8 * n)])))
            else:
                pr = ldf("k1", 8 * n, z=1) - _tree(terms)
                pi = ldf("pi", 8 * n)
                zr, zi = pr, pi
                if n > 0:
                    qr, qi = memo["prev"]
                    zr, zi = pr - qi, pi + qr
                memo["prev"] = (pr, pi)
                st("z", n * T + 8 * g, pace(pltpu.pack_elementwise([zr, zi], packed_dtype=BF16)))

        def a3_list():
            out = []
            for g in range(T // 8):
                for plane in range(3):
                    out += [(2 * (n - 8) + 3, P(a3, g, plane, True, n)) for n in range(8, NC)]
                    out += [(2 * min(n, 7) + 3 + 2 * (plane == 2), P(a3, g, plane, False, n))
                            for n in range(NC)]
            return out

        def idft(c0, m):
            def mm():
                rhs = jnp.concatenate(
                    [pltpu.bitcast(ld("z", c * T, T), BF16) for c in range(c0, c0 + 2)], axis=1)
                return jnp.dot(pltpu.bitcast(inv_ref[...], BF16), rhs, preferred_element_type=F32)
            y = once(("y", c0), mm)
            dd = once("dd", lambda: jnp.concatenate([taps[j, 4]] * 2, axis=0))
            for u in range(2):
                c = c0 + u
                kv = ld_kv(c, m // 2, 8, z=1).astype(F32)
                qq = pltpu.bitcast(q32[slot, pl.ds((c * T + m) // 2, 8), :], BF16).astype(F32)
                o = (qq * (y[m:m + 16, u * 128:(u + 1) * 128] + kv * dd)).astype(BF16)
                oview[pl.ds((c * T + m) // 2, 8), :] = pltpu.bitcast(o, U32)
                memo["clock"] = y[m + 8:m + 16, u * 128:(u + 1) * 128]

        def idft_list():
            return [(11, P(idft, c0, m)) for c0 in range(0, NC, 2) for m in range(0, T, 16)]

        def at(p, t):
            return (("q", t * R), ("k", t * KR), (f"v{t // 4}", t % 4 * KR))[p]

        def proj(p, t, half, m):
            def mm():
                x = jnp.concatenate(
                    [pltpu.bitcast(x32[slot, 4 * half + u], BF16) for u in range(4)], axis=1)
                w = pltpu.bitcast(wp[p, pl.ds(half * 256, 256), pl.ds(t * 128, 128)], BF16)
                return jnp.dot(x, w, preferred_element_type=F32)
            res = memo["clock"] = once(("proj", p, t, half), mm)[m:m + 8]
            if not half:
                st("part", m, res)
                return
            res = res + ldf("part", m)
            name, row = at(p, t)
            st(name, row + (HALO if p else 0) + m, res)
            if m == 0 and p == 2:
                first = jnp.broadcast_to(res[0:1], (HALO, 128))
                st(name, row, jnp.where(j == 0, first, ldf(name, row + R, HALO, z=3)))

        def proj_list(p, t0, t1):
            return [(8, P(proj, p, t, half, m))
                    for t in range(t0, t1) for half in range(2) for m in range(0, R, 8)]

        def qk(r, w):
            qv = once(("qv", r), lambda: [ldf("q", t * R + 8 * r) for t in range(NT)])
            s = pace(_tree([qv[t] * ldf("k", t * KR + HALO + 8 * r - DIL * w, z=r % 2)
                            for t in range(NT)]))
            s = s + pltpu.roll(s, 64, 1)
            s = s + pltpu.roll(s, 32, 1)
            s = s * (DH ** -0.5)
            if 8 * r < DIL * w:
                pos = j * R + 8 * r + lax.broadcasted_iota(jnp.int32, (8, 128), 0)
                s = jnp.where(pos >= DIL * w, s, -1e9)
            memo["lg", r, w] = s
            if w == WIN - 1:
                lg = [memo["lg", r, u] for u in range(WIN)]
                m = functools.reduce(jnp.maximum, lg)
                e = [jnp.exp(s - m) for s in lg]
                inv = 1.0 / _tree(e)
                for u in range(WIN):
                    st("p", u * R + 8 * r, e[u] * inv)

        def qk_list():
            return [(1, P(qk, r, w)) for r in range(R // 8) for w in range(WIN)]

        def pv(r, t):
            name, row = at(2, t)
            halves = []
            for r8 in (2 * r, 2 * r + 1):
                p = once(("pv", r8, t // 4),
                         lambda: [ldf("p", w * R + 8 * r8, z=t // 4) for w in range(WIN)])
                halves.append(_tree(
                    [p[w] * ldf(name, row + HALO + 8 * r8 - DIL * w, z=r % 2) for w in range(WIN)]))
            o = pltpu.bitcast(jnp.concatenate(halves, axis=0).astype(BF16), U32)
            st(f"o{t // 4}", t % 4 * (R // 2) + 8 * r, pace(o))

        def pv_list(t0, t1):
            return [(31, P(pv, r, t)) for r in range(R // 16) for t in range(t0, t1)]

        def oproj(t, half, m):
            def mm():
                o = jnp.concatenate(
                    [pltpu.bitcast(ld(f"o{half}", u * (R // 2), R // 2), BF16) for u in range(4)], axis=1)
                w = pltpu.bitcast(wop[pl.ds(half * 256, 256), pl.ds(t * 128, 128)], BF16)
                return jnp.dot(o, w, preferred_element_type=F32)
            res = once(("oproj", t, half), mm)
            if half == 0:
                memo["clock"] = res[m:m + 8]
                st("acc", t * R + m, memo["clock"])
            else:
                o = (res[m:m + 16] + ldf("acc", t * R + m, 16)).astype(BF16)
                ob32[slot, t, pl.ds(m // 2, 8), :] = pltpu.bitcast(o, U32)

        def oproj_list(half, t0, t1):
            n = 16 if half else 8
            return [(n, P(oproj, t, half, m)) for t in range(t0, t1) for m in range(0, R, n)]

        for t in range(NT):
            st("k", t * KR, ld("k", t * KR + R, HALO, z=3))
        _weave(dft_list("hf", 0) + dft_list("hf", 4), a1_list(0, 8))
        _weave(dft_list("hf", 8) + dft_list("hf", 12) + dft_list("xf", 0), a1_list(8, 16))
        for c0 in (4, 8, 12):
            _weave(dft_list("xf", c0), [])
        _weave(proj_list(0, 0, NT) + proj_list(1, 0, NT - 1), a3_list())
        _weave(proj_list(1, NT - 1, NT), [])
        _weave(idft_list() + proj_list(2, 0, 4), qk_list())
        _weave(proj_list(2, 4, 5)[:32], [])
        _weave(proj_list(2, 4, 5)[32:] + proj_list(2, 5, 7), pv_list(0, 4))
        _weave(proj_list(2, 7, 8), [])
        _weave(oproj_list(0, 0, 7), pv_list(4, 8))
        _weave(oproj_list(0, 7, 8) + oproj_list(1, 0, 8), [])

        for c in out_copies(j, slot):
            c.start()
        return carry

    lax.fori_loop(0, NS, step, 0)
    for j in (NS - 2, NS - 1):
        for c in out_copies(j, j % 2):
            c.wait()


@jax.jit
def pallas_concat_heads__ssm_conv_h3__sliding_local_dilated__prompt_kernel(
    A_q, A_k, A_v, A_shift_k, A_ssm_k, A_ssm_D, B_x, B_wqkv, B_wo,
):
    hbm = pl.BlockSpec(memory_space=pl.ANY)
    vmem = pl.BlockSpec(memory_space=pltpu.VMEM)
    smem = pl.BlockSpec(memory_space=pltpu.SMEM)
    out = pl.pallas_call(
        _kernel,
        in_specs=[smem, hbm, hbm, hbm, vmem, hbm, vmem, hbm, hbm, hbm, vmem, vmem],
        out_specs=hbm,
        out_shape=jax.ShapeDtypeStruct((S, 2 * D), BF16),
        scratch_shapes=[
            pltpu.VMEM((2, S, 128), BF16),
            pltpu.VMEM((2, 16 + S, 128), BF16),
            pltpu.VMEM((2, S, 128), BF16),
            pltpu.VMEM((2, 128, S), BF16),
            pltpu.VMEM((2, NT, R, 128), BF16),
            pltpu.VMEM((3, D, D), BF16),
            pltpu.VMEM((3, D // 2, D), U32),
            pltpu.VMEM((D, D), BF16),
            pltpu.VMEM((D // 2, D), U32),
            pltpu.VMEM((32 * PITCH, 128), U32),
            pltpu.VMEM((NT, 5, 8, 128), F32),
            pltpu.VMEM((2, NT, R, 128), BF16),
            pltpu.SemaphoreType.DMA((2, 5)),
            pltpu.SemaphoreType.DMA((4,)),
            pltpu.SemaphoreType.DMA((2, 2)),
        ] + [pltpu.VMEM((n, 128), U32) for n in _BUFS.values()],
        compiler_params=pltpu.CompilerParams(vmem_limit_bytes=100 * 1024 * 1024),
        name="fused",
    )(np.zeros((4,), np.int32), A_q[0], A_k[0], A_v[0], A_shift_k.T, A_ssm_k,
      A_ssm_D.reshape(8, 128), B_x[0], B_wqkv, B_wo, _FWD, _INV)
    return out[None]
```

```python
import functools

import jax
import jax.numpy as jnp
import numpy as np
from jax import lax
from jax.experimental import pallas as pl
import jax.experimental.pallas.tpu as pltpu

S = 2048
D = 1024
T = 128
NC = S // T
NS = 8
R = S // NS
NT = D // 128
WIN, DIL, DH = 8, 2, 32
HALO = 16
PITCH = 33
KR = HALO + R

F32, BF16, U32 = jnp.float32, jnp.bfloat16, jnp.uint32


def _pack_rows(m):
    b = m.astype(jnp.bfloat16).view(np.uint16).astype(np.uint32)
    return np.ascontiguousarray(b[0::2] | (b[1::2] << 16))


def _dft_matrices():
    n = np.arange(T)[None, :]
    f = np.arange(T)[:, None]
    th = 2.0 * np.pi * (f + 0.25) * n / T
    fwd = np.concatenate([np.cos(th), -np.sin(th)], axis=0)
    order = np.stack([np.arange(T), T + np.arange(T)], axis=1).reshape(-1)
    inv = fwd.T[:, order] / T
    inv = _pack_rows(inv)
    return np.concatenate(
        [_pack_rows(fwd), inv[:, :T], inv[:, T:], np.zeros((8, T), np.uint32)], axis=0)


_TABLE = _dft_matrices()


def _lo(w):
    return pltpu.bitcast(w << 16, F32)


def _hi(w):
    return pltpu.bitcast(w & jnp.uint32(0xFFFF0000), F32)


def _tree(xs):
    while len(xs) > 1:
        xs = [xs[i] + xs[i + 1] if i + 1 < len(xs) else xs[i] for i in range(0, len(xs), 2)]
    return xs[0]


def _merge(main, side):
    total_m = sum(c for c, _ in main)
    total_s = sum(c for c, _ in side)
    done_m, done_s, i, out = 0, 0, 0, []
    for c, f in main:
        out.append((c * total_s, f))
        done_m += c
        while i < len(side) and (done_s + side[i][0]) * total_m <= done_m * total_s:
            done_s += side[i][0]
            out.append((side[i][0] * total_m, side[i][1]))
            i += 1
    assert i == len(side)
    return out


def _run(tasks):
    for _, f in tasks:
        f()


def _weave(main, side):
    _run(_merge(main, side))


_BUFS = dict(
    hf=NC * 2 * T, xf=NC * 2 * T, kv0=S // 4, kv1=S // 4, z=NC * T,
    up=8 * NC, k1=8 * NC, pi=8 * NC, oa=S, part=R,
    q=NT * R, k=NT * KR, v0=4 * KR, v1=4 * KR, p=WIN * R,
    o0=4 * R // 2, o1=4 * R // 2, acc0=NT * R, acc1=NT * R,
    ob=NT * R, t0=32 * PITCH, t1=32 * PITCH,
)


def _wait(copies):
    for c in copies:
        c.wait()


def _kernel(q_hbm, k_hbm, v_hbm, sk_hbm, h_hbm, d_hbm, x_hbm, w_hbm, wo_hbm, tab_hbm, out_hbm,
            qa, ka, va, ha, xb, wraw, woraw, taps, sk_ref, d_ref, tab,
            sem_in, sem_out, *bufs):
    wp, wop = bufs[:6], bufs[6:8]
    bufs = dict(zip(_BUFS, bufs[8:]))

    def ld(name, row, n=8, z=0):
        return views[name][z][pl.ds(row, n), :]

    def ldf(name, row, n=8, z=0):
        return pltpu.bitcast(ld(name, row, n, z), F32)

    def st(name, row, val):
        val = pltpu.bitcast(val, U32)
        bufs[name][pl.ds(row, val.shape[0]), :] = val

    def cols(j):
        return pl.ds(pl.multiple_of(j * 128, 128), 128)

    def rows(j):
        return pl.ds(pl.multiple_of(j * R, R), R)

    def a_copies(j, slot):
        return [
            pltpu.make_async_copy(h_hbm.at[cols(j), :], ha.at[slot], sem_in.at[slot]),
            pltpu.make_async_copy(k_hbm.at[:, cols(j)], ka.at[slot, pl.ds(16, S), :], sem_in.at[2 + slot]),
            pltpu.make_async_copy(v_hbm.at[:, cols(j)], va.at[slot], sem_in.at[4 + slot]),
        ]

    def x_copies(j, slot):
        return [pltpu.make_async_copy(x_hbm.at[rows(j), pl.ds(t * 128, 128)], xb.at[slot, t],
                                      sem_in.at[6 + slot]) for t in range(NT)]

    def q_copies(j, slot):
        return [pltpu.make_async_copy(q_hbm.at[:, cols(j)], qa.at[slot], sem_in.at[8 + slot])]

    def in_copies(j, slot):
        return a_copies(j, slot) + x_copies(j, slot) + q_copies(j, slot)

    def oa_copy(j, slot):
        src = bufs["oa"].bitcast(BF16).at[pl.ds(pl.multiple_of(slot * S, 16), S), :]
        return pltpu.make_async_copy(src, out_hbm.at[:, cols(j)], sem_out.at[slot])

    def ob_copy(j, slot, t):
        src = bufs["ob"].bitcast(BF16).at[pl.ds(pl.multiple_of((slot * NT + t) * R, 16), R), :]
        return pltpu.make_async_copy(src, out_hbm.at[rows(j), pl.ds(D + t * 128, 128)],
                                     sem_out.at[2 + slot])

    def out_copies(j, slot):
        return [oa_copy(j, slot)] + [ob_copy(j, slot, t) for t in range(NT)]

    def w_copy(n):
        half = pl.ds(n % 2 * (D // 2), D // 2)
        return pltpu.make_async_copy(
            w_hbm.at[half, pl.ds(n // 2 * D, D)], wraw.at[n], sem_in.at[10 + n])

    def wo_copy(n):
        return pltpu.make_async_copy(
            wo_hbm.at[:, pl.ds(n * (D // 2), D // 2)], woraw.at[n], sem_in.at[16 + n])

    small = [pltpu.make_async_copy(a, b, sem_in.at[18 + i]) for i, (a, b) in enumerate(
        ((tab_hbm, tab), (sk_hbm, sk_ref), (d_hbm, d_ref)))]
    for c in (small + [w_copy(0)] + a_copies(0, 0) + x_copies(0, 0) + [w_copy(n) for n in range(1, 6)]
              + q_copies(0, 0) + [wo_copy(0), wo_copy(1)]):
        c.start()
    _wait(small)
    zero = pltpu.bitcast(tab[pl.ds(2 * T, 8), :], jnp.int32)
    zs = [pl.multiple_of(zero[i, 0] * 8, 8) for i in range(3)]
    views = {n: [b.at[pl.ds(z, _BUFS[n]), :] for z in zs] + [b] for n, b in bufs.items()}

    for slot in range(2):
        ka[slot, pl.ds(0, 16), :] = jnp.zeros((16, 128), BF16)
    for t in range(NT):
        st("k", t * KR, jnp.zeros((HALO, 128), F32))
    skf = sk_ref[...].astype(F32)
    df = d_ref[...].astype(F32)
    for t in range(NT):
        for i in range(4):
            taps[t, i] = jnp.broadcast_to(skf[i:i + 1, t * 128:(t + 1) * 128], (8, 128))
        taps[t, 4] = jnp.broadcast_to(df[t:t + 1, :], (8, 128))

    def step(j, first):
        slot = j % 2
        k32, v32, q32, x32 = (r.bitcast(U32) for r in (ka, va, qa, xb))
        P = functools.partial
        oview = bufs["oa"].at[pl.ds(pl.multiple_of(slot * (S // 2), 8), S // 2), :]
        obview = bufs["ob"].at[pl.ds(pl.multiple_of(slot * (NT * R // 2), 8), NT * R // 2), :]
        memo = {}
        never = tab[pl.ds(2 * T, 8), :] != 0

        def once(key, fn):
            if key not in memo:
                memo[key] = fn()
            return memo[key]

        def pace(val):
            if memo.get("clock") is None:
                return val
            return jnp.where(never, pltpu.bitcast(memo["clock"], val.dtype), val)

        def wait(copies):
            memo["clock"] = None
            for c in copies:
                c.wait()

        def paced(x):
            return jnp.concatenate([pace(x[:8]), x[8:]], axis=0)

        def perm_in(n, u, t):
            tt = paced(wraw.bitcast(U32)[n, pl.ds(u * 128, 128), pl.ds(t * 128, 128)]).T
            for hh in range(4):
                st(f"t{u}", (4 * t + hh) * PITCH, tt[hh * DH:(hh + 1) * DH])

        def perm_out(n, u, t):
            g = jnp.concatenate(
                [bufs[f"t{u}"][pl.ds(zs[0] + 4 * t + i, 32, stride=PITCH), :] for i in range(4)], axis=0)
            wp[n][pl.ds(u * 128, 128), pl.ds(t * 128, 128)] = paced(g).T

        def perm_list(n):
            return [(1, P(f, n, u, t)) for f in (perm_in, perm_out) for u in range(2) for t in range(NT)]

        def wo_in(n, t, hh):
            wt = woraw[n, pl.ds(hh * DH, DH), pl.ds(t * 128, 128)].astype(F32)
            st(f"t{t % 2}", hh * PITCH, paced(wt))

        def wo_out(n, t, i):
            g = bufs[f"t{t % 2}"][pl.ds(zs[0] + i, 32, stride=PITCH), :]
            g = pltpu.bitcast(pltpu.bitcast(g, F32).astype(BF16), U32)
            wop[n][pl.ds(16 * i, 16), pl.ds(t * 128, 128)] = paced(g)

        def wo_list(n):
            return [(c, P(f, n, t, i)) for t in range(4)
                    for c, f in ((2, wo_in), (1, wo_out)) for i in range(32)]

        def ld_kv(c, row, n, z=0):
            return pltpu.bitcast(ld(f"kv{c // 8}", c % 8 * (T // 2) + row, n, z), BF16)

        def a1(r):
            w0, w1, w2, w3 = once("taps", lambda: [taps[j, i] for i in range(4)])
            c0 = k32[slot, pl.ds(8 + 8 * r, 8), :]
            c1 = k32[slot, pl.ds(7 + 8 * r, 8), :]
            c2 = k32[slot, pl.ds(6 + 8 * r, 8), :]
            vv = v32[slot, pl.ds(8 * r, 8), :]
            e0, o0, e1, o1, o2 = _lo(c0), _hi(c0), _lo(c1), _hi(c1), _hi(c2)
            ke = (e0 * w0 + o1 * w1) + (e1 * w2 + o2 * w3)
            ko = (o0 * w0 + e0 * w1) + (o1 * w2 + e1 * w3)
            kv = pltpu.pack_elementwise([ke * _lo(vv), ko * _hi(vv)], packed_dtype=BF16)
            st(f"kv{r // 64}", 8 * (r % 64), pace(kv))

        def a1_list(c0, c1):
            return [(24, P(a1, r)) for r in range(8 * c0, 8 * c1)]

        def dft(name, c0, m):
            def mm():
                f = pltpu.bitcast(tab[pl.ds(0, T), :], BF16)
                if name == "hf":
                    rhs = jnp.concatenate(
                        [ha[slot, :, pl.ds(c * T, T)] for c in range(c0, c0 + 4)], axis=0)
                    return lax.dot_general(f, rhs, (((1,), (1,)), ((), ())),
                                           preferred_element_type=F32)
                rhs = jnp.concatenate([ld_kv(c, 0, T // 2) for c in range(c0, c0 + 4)], axis=1)
                return jnp.dot(f, rhs, preferred_element_type=F32)
            res = once((name, c0), mm)
            for u in range(4):
                memo["clock"] = res[m:m + 8, u * 128:(u + 1) * 128]
                st(name, (c0 + u) * 2 * T + m, memo["clock"])

        def dft_list(name, c0):
            return [(8, P(dft, name, c0, m)) for m in range(0, 2 * T, 8)]

        def a3(g, plane, upper, n):
            def opnd(name, c):
                re = lambda: ldf(name, c * 2 * T + 8 * g, z=plane)
                im = lambda: ldf(name, c * 2 * T + T + 8 * g, z=plane)
                if name == "xf":
                    return re() + im() if plane == 0 else re() if plane == 1 else im()
                return re() if plane == 0 else im() - re() if plane == 1 else im() + re()
            get = lambda name, c: once((name, g, plane, c), P(opnd, name, c))
            cs = range(8, n + 1) if upper else range(min(n, 7) + 1)
            terms = [get("xf", n - c) * get("hf", c) for c in cs]
            if upper:
                st("up", 8 * n, pace(_tree(terms)))
                return
            if n >= 8:
                terms.append(ldf("up", 8 * n))
            if plane == 0:
                st("k1", 8 * n, pace(_tree(terms)))
            elif plane == 1:
                st("pi", 8 * n, pace(_tree(terms + [ldf("k1", 8 * n)])))
            else:
                pr = ldf("k1", 8 * n, z=1) - _tree(terms)
                pi = ldf("pi", 8 * n)
                zr, zi = pr, pi
                if n > 0:
                    qr, qi = memo["prev"]
                    zr, zi = pr - qi, pi + qr
                memo["prev"] = (pr, pi)
                st("z", n * T + 8 * g, pace(pltpu.pack_elementwise([zr, zi], packed_dtype=BF16)))

        def a3_list():
            out = []
            for g in range(T // 8):
                for plane in range(3):
                    out += [(2 * (n - 8) + 3, P(a3, g, plane, True, n)) for n in range(8, NC)]
                    out += [(2 * min(n, 7) + 3 + 2 * (plane == 2), P(a3, g, plane, False, n))
                            for n in range(NC)]
            return out

        def idft(c0, m):
            def mm():
                rhs = jnp.concatenate(
                    [pltpu.bitcast(ld("z", c * T, T), BF16) for c in range(c0, c0 + 2)], axis=1)
                f = jnp.concatenate(
                    [pltpu.bitcast(tab[pl.ds(T + u * 64, 64), :], BF16) for u in range(2)], axis=1)
                return jnp.dot(f, rhs, preferred_element_type=F32)
            y = once(("y", c0), mm)
            dd = once("dd", lambda: jnp.concatenate([taps[j, 4]] * 2, axis=0))
            for u in range(2):
                c = c0 + u
                kv = ld_kv(c, m // 2, 8, z=1).astype(F32)
                qq = pltpu.bitcast(q32[slot, pl.ds((c * T + m) // 2, 8), :], BF16).astype(F32)
                o = (qq * (y[m:m + 16, u * 128:(u + 1) * 128] + kv * dd)).astype(BF16)
                oview[pl.ds((c * T + m) // 2, 8), :] = pltpu.bitcast(o, U32)
                memo["clock"] = y[m + 8:m + 16, u * 128:(u + 1) * 128]

        def idft_list():
            return [(11, P(idft, c0, m)) for c0 in range(0, NC, 2) for m in range(0, T, 16)]

        def at(p, t):
            return (("q", t * R), ("k", t * KR), (f"v{t // 4}", t % 4 * KR))[p]

        def proj(p, t, half, m):
            def mm():
                x = jnp.concatenate(
                    [pltpu.bitcast(x32[slot, 4 * half + u], BF16) for u in range(4)], axis=1)
                w = pltpu.bitcast(wp[2 * p + half][:, pl.ds(t * 128, 128)], BF16)
                return jnp.dot(x, w, preferred_element_type=F32)
            res = memo["clock"] = once(("proj", p, t, half), mm)[m:m + 8]
            part = (f"acc{p % 2}", t * R + m) if first else ("part", m)
            if not half:
                st(*part, res)
                return
            res = res + ldf(*part)
            name, row = at(p, t)
            st(name, row + (HALO if p else 0) + m, res)
            if m == 0 and p == 2:
                st(name, row, jnp.broadcast_to(res[0:1], (HALO, 128)) if first
                   else ld(name, row + R, HALO, z=3))

        def proj_list(p, t0, t1, halves=(0, 1)):
            return [(8, P(proj, p, t, half, m))
                    for t in range(t0, t1) for half in halves for m in range(0, R, 8)]

        def qk(r, w):
            qv = once(("qv", r), lambda: [ldf("q", t * R + 8 * r) for t in range(NT)])
            s = pace(_tree([qv[t] * ldf("k", t * KR + HALO + 8 * r - DIL * w, z=r % 2)
                            for t in range(NT)]))
            s = s + pltpu.roll(s, 64, 1)
            s = s + pltpu.roll(s, 32, 1)
            s = s * (DH ** -0.5)
            if first and 8 * r < DIL * w:
                pos = 8 * r + lax.broadcasted_iota(jnp.int32, (8, 128), 0)
                s = jnp.where(pos >= DIL * w, s, -1e9)
            memo["lg", r, w] = s
            if w == WIN - 1:
                lg = [memo["lg", r, u] for u in range(WIN)]
                m = functools.reduce(jnp.maximum, lg)
                e = [jnp.exp(s - m) for s in lg]
                inv = 1.0 / _tree(e)
                for u in range(WIN):
                    st("p", u * R + 8 * r, e[u] * inv)

        def qk_list():
            return [(1, P(qk, r, w)) for r in range(R // 8) for w in range(WIN)]

        def pv(r, t):
            name, row = at(2, t)
            halves = []
            for r8 in (2 * r, 2 * r + 1):
                p = once(("pv", r8, t // 4),
                         lambda: [ldf("p", w * R + 8 * r8, z=t // 4) for w in range(WIN)])
                halves.append(_tree(
                    [p[w] * ldf(name, row + HALO + 8 * r8 - DIL * w, z=r % 2) for w in range(WIN)]))
            o = pltpu.bitcast(jnp.concatenate(halves, axis=0).astype(BF16), U32)
            st(f"o{t // 4}", t % 4 * (R // 2) + 8 * r, pace(o))

        def pv_list(t0, t1):
            return [(31, P(pv, r, t)) for r in range(R // 16) for t in range(t0, t1)]

        def oproj(t, half, m):
            def mm():
                o = jnp.concatenate(
                    [pltpu.bitcast(ld(f"o{half}", u * (R // 2), R // 2), BF16) for u in range(4)], axis=1)
                w = pltpu.bitcast(wop[t // 4][pl.ds(half * 256, 256), pl.ds(t % 4 * 128, 128)], BF16)
                return jnp.dot(o, w, preferred_element_type=F32)
            res = once(("oproj", t, half), mm)
            if half == 0:
                memo["clock"] = res[m:m + 8]
                st("acc1", t * R + m, memo["clock"])
            else:
                memo["clock"] = res[m + 8:m + 16]
                o = (res[m:m + 16] + ldf("acc1", t * R + m, 16)).astype(BF16)
                obview[pl.ds((t * R + m) // 2, 8), :] = pltpu.bitcast(o, U32)
                if m + 16 == R:
                    ob_copy(j, slot, t).start()

        def oproj_list(half, t0, t1):
            n = 16 if half else 8
            return [(n, P(oproj, t, half, m)) for t in range(t0, t1) for m in range(0, R, n)]

        def spectra():
            _weave(dft_list("hf", 0) + dft_list("hf", 4), a1_list(0, 8))
            _weave(dft_list("hf", 8) + dft_list("hf", 12) + dft_list("xf", 0), a1_list(8, 16))
            _run(dft_list("xf", 4) + dft_list("xf", 8) + dft_list("xf", 12))

        if first:
            conv, scores = a3_list(), qk_list()
            cut = [len(conv) * i // 16 for i in (0, 4, 7, 10, 13, 16)]
            idle = [(2, lambda: None)] * 4
            wait([w_copy(0)])
            _run(perm_list(0))
            wait(a_copies(0, 0))
            spectra()
            _run(conv[:cut[1]])
            for n in range(4):
                wait([w_copy(n + 1)] + (x_copies(0, 0) if n == 0 else []))
                _weave(proj_list(n // 2, 0, NT, (n % 2,)),
                       _merge(perm_list(n + 1) + idle, conv[cut[n + 1]:cut[n + 2]]))
            wait([w_copy(5)])
            _weave(proj_list(2, 0, NT, (0,)), perm_list(5) + idle)
            wait(q_copies(0, 0) + [wo_copy(0)])
            for c in in_copies(1, 1):
                c.start()
            _weave(proj_list(2, 0, NT, (1,)), _merge(scores[:176], wo_list(0)))
            _weave(idft_list(), scores[176:])
            oa_copy(j, slot).start()
            wait([wo_copy(1)])
            _run(pv_list(0, 4))
            _weave(oproj_list(0, 0, 4), pv_list(4, 8))
            _weave(oproj_list(1, 0, 4), wo_list(1))
            _run(oproj_list(0, 4, 8) + oproj_list(1, 4, 8))
            return

        for t in range(NT):
            st("k", t * KR, ld("k", t * KR + R, HALO, z=3))
        spectra()
        _weave(proj_list(0, 0, NT) + proj_list(1, 0, NT - 1), a3_list())
        _run(proj_list(1, NT - 1, NT))
        scores = qk_list()
        _weave(idft_list(), scores[:64])
        oa_copy(j, slot).start()
        _weave(proj_list(2, 0, 4) + proj_list(2, 4, 5, (0,)), scores[64:])
        _run(proj_list(2, 4, 5, (1,)))
        _weave(proj_list(2, 5, 7) + proj_list(2, 7, 8, (0,)), pv_list(0, 4))
        _run(proj_list(2, 7, 8, (1,)))
        _weave(oproj_list(0, 0, 7), pv_list(4, 8))
        _run(oproj_list(0, 7, 8) + oproj_list(1, 0, 8))

    step(0, True)

    def loop(j, carry):
        slot = j % 2
        for c in in_copies(j, slot):
            c.wait()

        @pl.when(j + 1 < NS)
        def _():
            for c in in_copies(j + 1, 1 - slot):
                c.start()

        @pl.when(j >= 2)
        def _():
            for c in out_copies(j - 2, slot):
                c.wait()

        step(j, False)
        return carry

    lax.fori_loop(1, NS, loop, 0)
    for j in (NS - 2, NS - 1):
        for c in out_copies(j, j % 2):
            c.wait()


@jax.jit
def pallas_concat_heads__ssm_conv_h3__sliding_local_dilated__prompt_kernel(
    A_q, A_k, A_v, A_shift_k, A_ssm_k, A_ssm_D, B_x, B_wqkv, B_wo,
):
    hbm = pl.BlockSpec(memory_space=pl.ANY)
    out = pl.pallas_call(
        _kernel,
        in_specs=[hbm] * 10,
        out_specs=hbm,
        out_shape=jax.ShapeDtypeStruct((S, 2 * D), BF16),
        scratch_shapes=[
            pltpu.VMEM((2, S, 128), BF16),
            pltpu.VMEM((2, 16 + S, 128), BF16),
            pltpu.VMEM((2, S, 128), BF16),
            pltpu.VMEM((2, 128, S), BF16),
            pltpu.VMEM((2, NT, R, 128), BF16),
            pltpu.VMEM((6, D // 2, D), BF16),
            pltpu.VMEM((2, D, D // 2), BF16),
            pltpu.VMEM((NT, 5, 8, 128), F32),
            pltpu.VMEM((4, D), BF16),
            pltpu.VMEM((8, 128), BF16),
            pltpu.VMEM(_TABLE.shape, U32),
            pltpu.SemaphoreType.DMA((21,)),
            pltpu.SemaphoreType.DMA((4,)),
        ] + [pltpu.VMEM((D // 4, D), U32)] * 6 + [pltpu.VMEM((D // 2, D // 2), U32)] * 2
        + [pltpu.VMEM((n, 128), U32) for n in _BUFS.values()],
        compiler_params=pltpu.CompilerParams(vmem_limit_bytes=100 * 1024 * 1024),
        name="fused",
    )(A_q[0], A_k[0], A_v[0], A_shift_k.T, A_ssm_k,
      A_ssm_D.reshape(8, 128), B_x[0], B_wqkv, B_wo, _TABLE)
    return out[None]
```

```python
import functools

import jax
import jax.numpy as jnp
import numpy as np
from jax import lax
from jax.experimental import pallas as pl
import jax.experimental.pallas.tpu as pltpu


S = 2048
D = 1024
T = 128
NC = S // T
NS = 8
R = S // NS
E = R // 2
NT = D // 128
WIN, DH = 8, 32
PITCH = 33
KR = WIN + E
FP = 2 * T + 16

F32, BF16, U32 = jnp.float32, jnp.bfloat16, jnp.uint32


def _pack_rows(m):
    b = m.astype(jnp.bfloat16).view(np.uint16).astype(np.uint32)
    return np.ascontiguousarray(b[0::2] | (b[1::2] << 16))


def _dft_table():
    n = np.arange(T)[None, :]
    f = np.arange(T)[:, None]
    th = 2.0 * np.pi * (f + 0.25) * n / T
    fwd = np.concatenate([np.cos(th), -np.sin(th)], axis=0)
    cols = np.stack([np.arange(T), T + np.arange(T)], axis=1).reshape(-1)
    rows = np.arange(T).reshape(-1, 8, 2).transpose(0, 2, 1).reshape(-1)
    inv = _pack_rows(fwd.T[rows][:, cols] / T)
    return np.concatenate(
        [_pack_rows(fwd), inv[:, :T], inv[:, T:], np.zeros((8, T), np.uint32)], axis=0)


_TABLE = _dft_table()


def _lo(w):
    return pltpu.bitcast(w << 16, F32)


def _hi(w):
    return pltpu.bitcast(w & jnp.uint32(0xFFFF0000), F32)


def _pack(lo, hi):
    return pltpu.pack_elementwise([lo, hi], packed_dtype=BF16)


def _tree(xs):
    while len(xs) > 1:
        xs = [xs[i] + xs[i + 1] if i + 1 < len(xs) else xs[i] for i in range(0, len(xs), 2)]
    return xs[0]


def _left(a11, a12, a21, a22):
    return [a21 + a22, a22, a11 + a12, a11, a11 + a22, a12 - a22, a21 - a11]


def _merge(main, side):
    total_m = sum(c for c, _ in main)
    total_s = sum(c for c, _ in side)
    done_m, done_s, i, out = 0, 0, 0, []
    for c, f in main:
        out.append((c * total_s, f))
        done_m += c
        while i < len(side) and (done_s + side[i][0]) * total_m <= done_m * total_s:
            done_s += side[i][0]
            out.append((side[i][0] * total_m, side[i][1]))
            i += 1
    assert i == len(side)
    return out


def _run(tasks):
    for _, f in tasks:
        f()


def _weave(main, side):
    _run(_merge(main, side))


def _split(tasks, *weights):
    ends = np.cumsum((0,) + weights) * len(tasks) // sum(weights)
    return [tasks[a:b] for a, b in zip(ends[:-1], ends[1:])]


def _wait(copies):
    for c in copies:
        c.wait()


_BUFS = dict(
    qa=S, ka=S + 16, va=S, x=NT * R, oa=S, ob=NT * R,
    hf=NC * FP + 16, xf=NC * FP, kv0=S // 4, kv1=S // 4, z=NC * T,
    up=8 * NC, k1=8 * NC, pi=8 * NC,
    xs=9 * 4 * E // 2, os0=7 * 4 * E // 2, os1=7 * 4 * E // 2,
    c21=E, m4=E, c11=E, m5=E, c22=E, d11=E, d22=E, f21=E, f12=E,
    q=2 * NT * E, k=2 * NT * KR, v=2 * NT * KR, p=2 * WIN * E,
    acc0=NT * R, acc1=NT * R, t0=32 * PITCH, t1=32 * PITCH,
)
_HALF = ("qa", "ka", "va", "x", "oa", "ob", "xs", "os0")


def _kernel(q_hbm, k_hbm, v_hbm, sk_hbm, h_hbm, d_hbm, x_hbm, w_hbm, wo_hbm, tab_hbm, out_hbm,
            ha, wraw, woraw, taps, sk_ref, d_ref, tab, sem_in, sem_out, *bufs):
    wp16, ws = bufs[6:8], bufs[8:12]
    wp = list(bufs[:6]) + [b.bitcast(U32) for b in wp16]
    KW = D // 4
    raw = dict(zip(_BUFS, bufs[12:]))
    bufs = {n: b.bitcast(U32) if n in _HALF else b for n, b in raw.items()}
    P = functools.partial

    def ld(name, row, n=8, z=0):
        return views[name][z][pl.ds(row, n), :]

    def ldf(name, row, n=8, z=0):
        return pltpu.bitcast(ld(name, row, n, z), F32)

    def st(name, row, val):
        val = pltpu.bitcast(val, U32)
        bufs[name][pl.ds(row, val.shape[0]), :] = val

    def st16(name, row, first, second):
        raw[name][pl.ds(2 * row, 16), :] = jnp.concatenate([first, second], axis=0).astype(BF16)

    def window(name, row, n):
        return bufs[name].at[pl.ds(pl.multiple_of(row, 8), n), :]

    def window16(name, row, n):
        return raw[name].at[pl.ds(pl.multiple_of(2 * row, 16), 2 * n), :]

    def cols(j):
        return pl.ds(pl.multiple_of(j * 128, 128), 128)

    def rows(j):
        return pl.ds(pl.multiple_of(j * R, R), R)

    def a_copies(j, slot):
        return [
            pltpu.make_async_copy(h_hbm.at[cols(j), :], ha.at[slot], sem_in.at[slot]),
            pltpu.make_async_copy(k_hbm.at[:, cols(j)], window16("ka", slot * (S // 2 + 8) + 8, S // 2),
                                  sem_in.at[2 + slot]),
            pltpu.make_async_copy(v_hbm.at[:, cols(j)], window16("va", slot * (S // 2), S // 2),
                                  sem_in.at[4 + slot]),
        ]

    def x_copies(j, slot):
        return [pltpu.make_async_copy(x_hbm.at[rows(j), pl.ds(t * 128, 128)],
                                      window16("x", (slot * NT + t) * E, E),
                                      sem_in.at[6 + slot]) for t in range(NT)]

    def q_copies(j, slot):
        return [pltpu.make_async_copy(q_hbm.at[:, cols(j)], window16("qa", slot * (S // 2), S // 2),
                                      sem_in.at[8 + slot])]

    def in_copies(j, slot):
        return a_copies(j, slot) + x_copies(j, slot) + q_copies(j, slot)

    def oa_copy(j, slot):
        return pltpu.make_async_copy(window16("oa", slot * (S // 2), S // 2), out_hbm.at[:, cols(j)],
                                     sem_out.at[slot])

    def ob_copy(j, slot, t):
        return pltpu.make_async_copy(window16("ob", (slot * NT + t) * E, E),
                                     out_hbm.at[rows(j), pl.ds(D + t * 128, 128)],
                                     sem_out.at[2 + slot])

    def ob_copies(j, slot):
        return [ob_copy(j, slot, t) for t in range(NT)]

    def w_copy(n):
        half = pl.ds(n % 2 * (D // 2), D // 2)
        return pltpu.make_async_copy(
            w_hbm.at[half, pl.ds(n // 2 * D, D)], wraw.at[n], sem_in.at[10 + n])

    def wo_copy(n):
        return pltpu.make_async_copy(
            wo_hbm.at[:, pl.ds(n * (D // 2), D // 2)], woraw.at[n], sem_in.at[16 + n])

    small = [pltpu.make_async_copy(a, b, sem_in.at[18 + i]) for i, (a, b) in enumerate(
        ((tab_hbm, tab), (sk_hbm, sk_ref), (d_hbm, d_ref)))]
    startup = lambda: ([w_copy(0)] + a_copies(0, 0) + x_copies(0, 0) + [w_copy(n) for n in range(1, 6)]
                       + [wo_copy(0), wo_copy(1)] + q_copies(0, 0))
    for c in small + startup():
        c.start()
    _wait(small)
    zero = pltpu.bitcast(tab[pl.ds(2 * T, 8), :], jnp.int32)
    zs = [pl.multiple_of(zero[i, 0] * 8, 8) for i in range(3)]
    views = {n: [b.at[pl.ds(z, _BUFS[n]), :] for z in zs] + [b] for n, b in bufs.items()}

    for slot in range(2):
        st("ka", slot * (S // 2 + 8), jnp.zeros((8, 128), U32))
    for t in range(2 * NT):
        st("k", t * KR, jnp.zeros((WIN, 128), F32))
    skf = sk_ref[...].astype(F32)
    df = d_ref[...].astype(F32)
    for t in range(NT):
        for i in range(4):
            taps[t, i] = jnp.broadcast_to(skf[i:i + 1, t * 128:(t + 1) * 128], (8, 128))
        taps[t, 4] = jnp.broadcast_to(df[t:t + 1, :], (8, 128))

    def step(j, first=False, last=False):
        slot = j % 2
        memo = {}
        never = tab[pl.ds(2 * T, 8), :] != 0

        def once(key, fn):
            if key not in memo:
                memo[key] = fn()
            return memo[key]

        def fresh():
            memo["fresh"] = memo.get("fresh", 1) + 1
            return pl.multiple_of(zs[0] * memo["fresh"], 8)

        def pace(val):
            if memo.get("clock") is None:
                return val
            return jnp.where(never, pltpu.bitcast(memo["clock"], val.dtype), val)

        def paced(x):
            return jnp.concatenate([pace(x[:8]), x[8:]], axis=0)

        def wait(copies):
            memo["clock"] = None
            _wait(copies)

        def perm_in(n, u, t):
            tt = paced(pltpu.bitcast(wraw[n, pl.ds(u * 256, 256), pl.ds(t * 128, 128)], U32)).T
            for hh in range(4):
                st(f"t{u}", (4 * t + hh) * PITCH, tt[hh * DH:(hh + 1) * DH])

        def perm_out(n, u, t):
            g = jnp.concatenate(
                [bufs[f"t{u}"][pl.ds(zs[0] + 4 * t + i, 32, stride=PITCH), :] for i in range(4)], axis=0)
            wp[n][pl.ds(t * KW + u * 128, 128), :] = paced(g).T

        def perm_list(n):
            return [(1, P(f, n, u, t)) for f in (perm_in, perm_out)
                    for u in range(2) for t in range(NT)] + [(2, lambda: None)] * 4

        def wo_in(t, hh):
            w = pltpu.bitcast(woraw[t // 4, pl.ds(hh * DH, DH), pl.ds(t % 4 * 128, 128)], U32)
            wt = pltpu.bitcast(paced(w), BF16).astype(F32)
            st(f"t{t % 2}", hh * PITCH, wt)

        def wo_out(t, i):
            g = bufs[f"t{t % 2}"][pl.ds(zs[0] + i, 32, stride=PITCH), :]
            wp16[i // 16][pl.ds(2 * t * KW + i % 16 * 32, 32), :] = (
                pltpu.bitcast(paced(g), F32).astype(BF16))

        def wo_list(n):
            return [(1, P(f, t, i)) for t in range(4 * n, 4 * n + 4)
                    for f in (wo_in, wo_out) for i in range(32)]

        def right(p, t, r):
            b = [once(("wv", p, h), lambda: wp[2 * p + h].at[pl.ds(zs[0], NT * KW), :])[pl.ds((t + 4 * u) * KW + r, 8), :]
                 for h in range(2) for u in range(2)]
            b[0] = pace(b[0])
            sums = []
            for half in (_lo, _hi):
                b11, b12, b21, b22 = map(half, b)
                sums.append([b21 - b11, b12 - b22, b11 + b22, b21 + b22, b11 + b12])
            for i, (lo, hi) in enumerate(zip(*sums)):
                ws[p][pl.ds((4 * i + t) * KW + r, 8), :] = _pack(lo, hi)

        def right_list(p):
            return [(1, P(right, p, t, r)) for t in range(4) for r in range(0, D // 4, 8)]

        def ld_kv(c, row, n, z=0):
            return ld(f"kv{c // 8}", c % 8 * (T // 2) + row, n, z)

        def a1(r):
            w0, w1, w2, w3 = once("taps", lambda: [taps[j, i] for i in range(4)])
            k32 = once("ka", lambda: window("ka", slot * (S // 2 + 8), S // 2 + 8))
            v32 = once("va", lambda: window("va", slot * (S // 2), S // 2))
            c0 = k32[pl.ds(8 + 8 * r, 8), :]
            c1 = k32[pl.ds(7 + 8 * r, 8), :]
            c2 = k32[pl.ds(6 + 8 * r, 8), :]
            vv = v32[pl.ds(8 * r, 8), :]
            e0, o0, e1, o1, o2 = _lo(c0), _hi(c0), _lo(c1), _hi(c1), _hi(c2)
            ke = (e0 * w0 + o1 * w1) + (e1 * w2 + o2 * w3)
            ko = (o0 * w0 + e0 * w1) + (o1 * w2 + e1 * w3)
            st(f"kv{r // 64}", 8 * (r % 64), pace(_pack(ke * _lo(vv), ko * _hi(vv))))

        def a1_list(c0, c1):
            return [(24, P(a1, r)) for r in range(8 * c0, 8 * c1)]

        def freq(name, c, im, m):
            return 16 * (name == "hf") + c * FP + im * (T + 8) + m

        def dft(name, c0, m):
            def mm():
                f = pltpu.bitcast(tab[pl.ds(fresh(), T), :], BF16)
                if name == "hf":
                    rhs = jnp.concatenate(
                        [ha[slot, :, pl.ds(c * T, T)] for c in range(c0, c0 + 4)], axis=0)
                    return lax.dot_general(f, rhs, (((1,), (1,)), ((), ())),
                                           preferred_element_type=F32)
                rhs = jnp.concatenate(
                    [pltpu.bitcast(ld_kv(c, 0, T // 2), BF16) for c in range(c0, c0 + 4)], axis=1)
                return jnp.dot(f, rhs, preferred_element_type=F32)
            res = once((name, c0), mm)
            for u in range(4):
                memo["clock"] = res[m:m + 8, u * 128:(u + 1) * 128]
                st(name, freq(name, c0 + u, m // T, m % T), memo["clock"])

        def dft_list(name, *c0s):
            return [(8, P(dft, name, c0, m)) for c0 in c0s for m in range(0, 2 * T, 8)]

        def a3(g, plane, upper, n):
            def opnd(name, c):
                re = lambda: ldf(name, freq(name, c, 0, 8 * g), z=plane)
                im = lambda: ldf(name, freq(name, c, 1, 8 * g), z=plane)
                if name == "xf":
                    val = re() + im() if plane == 0 else re() if plane == 1 else im()
                    return pace(val) if c >= 8 else val
                return pace(re() if plane == 0 else im() - re() if plane == 1 else im() + re())
            get = lambda name, c: once((name, g, plane, c), P(opnd, name, c))
            cs = range(8, n + 1) if upper else range(min(n, 7) + 1)
            terms = [get("xf", n - c) * get("hf", c) for c in cs]
            if upper:
                st("up", 8 * n, pace(_tree(terms)))
                return
            if n >= 8:
                terms.append(ldf("up", 8 * n))
            if plane == 0:
                st("k1", 8 * n, pace(_tree(terms)))
            elif plane == 1:
                st("pi", 8 * n, pace(_tree(terms + [ldf("k1", 8 * n)])))
            else:
                pr = ldf("k1", 8 * n, z=1) - _tree(terms)
                pi = ldf("pi", 8 * n)
                zr, zi = pr, pi
                if n > 0:
                    qr, qi = memo["prev"]
                    zr, zi = pr - qi, pi + qr
                memo["prev"] = (pr, pi)
                st("z", n * T + 8 * g, pace(_pack(zr, zi)))

        def a3_list():
            out = []
            for g in range(T // 8):
                for plane in range(3):
                    out += [(2 * (n - 8) + 4, P(a3, g, plane, True, n)) for n in range(8, NC)]
                    out += [(2 * min(n, 7) + 4 + 2 * (plane == 2), P(a3, g, plane, False, n))
                            for n in range(NC)]
            return out

        def idft(c0, m):
            def mm():
                rhs = jnp.concatenate(
                    [pltpu.bitcast(ld("z", c * T, T), BF16) for c in range(c0, c0 + 2)], axis=1)
                tv = tab.at[pl.ds(fresh() + T, T), :]
                f = jnp.concatenate(
                    [pltpu.bitcast(tv[pl.ds(u * 64, 64), :], BF16) for u in range(2)], axis=1)
                return jnp.dot(f, rhs, preferred_element_type=F32)
            y = once(("y", c0), mm)
            dd = once("dd", lambda: taps[j, 4])
            q32 = once("qa", lambda: window("qa", slot * (S // 2), S // 2))
            o32 = once("oa", lambda: window("oa", slot * (S // 2), S // 2))
            for u in range(2):
                c = c0 + u
                kv = ld_kv(c, m // 2, 8, z=1)
                qq = q32[pl.ds((c * T + m) // 2, 8), :]
                ye, yo = (y[m + i:m + i + 8, u * 128:(u + 1) * 128] for i in (0, 8))
                o32[pl.ds((c * T + m) // 2, 8), :] = _pack(
                    _lo(qq) * (ye + _lo(kv) * dd), _hi(qq) * (yo + _hi(kv) * dd))
                memo["clock"] = yo

        def idft_list():
            return [(16, P(idft, c0, m)) for c0 in range(0, NC, 2) for m in range(0, T, 16)]

        def xprep(u, r):
            x32 = once("x", lambda: window("x", slot * NT * E, NT * E))
            halves = []
            for m in (r, r + 8):
                a, b = pace(x32[pl.ds(u * E + m, 8), :]), x32[pl.ds((u + 4) * E + m, 8), :]
                a11, a12, a21, a22 = _lo(a), _lo(b), _hi(a), _hi(b)
                halves.append(_left(a11, a12, a21, a22) + ([a12, a21] if first else []))
            for i, (lo, hi) in enumerate(zip(*halves)):
                st16("xs", ((4 * i + u) * E + r) // 2, lo, hi)

        def xprep_list():
            return [(27, P(xprep, u, r)) for u in range(4) for r in range(0, E, 16)]

        def lhs(name, i):
            view = bufs[name].at[pl.ds(fresh() + i * 2 * E, 2 * E), :]
            return jnp.concatenate(
                [pltpu.bitcast(view[pl.ds(u * E // 2, E // 2), :], BF16) for u in range(4)], axis=1)

        def emit(p, par, t, m, val):
            if p == 0:
                st("q", (par * NT + t) * E + m, val)
                return
            name, row = "kv"[p - 1], (par * NT + t) * KR
            if m == 0 and not first:
                st(name, row, ld(name, row + E, WIN, z=3))
            if m == 0 and first and p == 2 and par == 0:
                for other in range(2):
                    st(name, (other * NT + t) * KR, jnp.broadcast_to(val[0:1], (WIN, 128)))
            st(name, row + WIN + m, val)

        def plain(p, t, half, m):
            def mm():
                x = jnp.concatenate([lhs("xs", i) for i in ((3, 8), (7, 1))[half]], axis=0)
                w = pltpu.bitcast(wp[2 * p + half][pl.ds(t * KW, KW), :], BF16)
                return jnp.dot(x, w, preferred_element_type=F32)
            res = memo["clock"] = once(("plain", p, t, half), mm)[m:m + 8]
            if half:
                emit(p, m // E, t, m % E, res + ldf(f"acc{p % 2}", t * R + m))
            else:
                st(f"acc{p % 2}", t * R + m, res)

        def plain_list(n):
            return [(8, P(plain, n // 2, t, n % 2, m)) for t in range(NT) for m in range(0, R, 8)]

        def product(p, t, i, m):
            def mm():
                if i == 0:
                    w = wp[2 * p][pl.ds(t * KW, KW), :]
                elif i == 2:
                    w = wp[2 * p + 1][pl.ds((t + 4) * KW, KW), :]
                else:
                    w = ws[p][pl.ds((4 * (i - 1 - (i > 2)) + t) * KW, KW), :]
                return jnp.dot(lhs("xs" if p < 3 else "os1", i), pltpu.bitcast(w, BF16),
                               preferred_element_type=F32)
            res = memo["clock"] = once(("product", p, t, i), mm)[m:m + 8]
            if i == 0:
                st("c21", m, res)
            elif i == 1:
                st("m4", m, res)
                c21 = ldf("c21", m) + res
                st("f21", m, c21) if p == 3 else emit(p, 1, t, m, c21)
            elif i == 2:
                st("c11", m, ldf("m4", m) - res)
                st("m5", m, res)
            elif i == 3:
                st("c22", m, res - ldf("c21", m, z=1))
                c12 = ldf("m5", m) + res
                st("f12", m, c12) if p == 3 else emit(p, 0, t + 4, m, c12)
            elif i == 4:
                st("d11", m, ldf("c11", m) + res)
                st("d22", m, ldf("c22", m) + res)
            elif p < 3:
                emit(p, i - 5, t + 4 * (i - 5), m, ldf(("d11", "d22")[i - 5], m) + res)
            else:
                prev = (j - 1) % 2
                o32 = once("ob", lambda: window("ob", prev * NT * E, NT * E))
                tile = t + 4 * (i - 5)
                if i == 5:
                    o32[pl.ds(tile * E + m, 8), :] = _pack(ldf("d11", m) + res, ldf("f21", m))
                else:
                    o32[pl.ds(tile * E + m, 8), :] = _pack(ldf("f12", m), ldf("d22", m) + res)
                if m + 8 == E:
                    ob_copy(j - 1, prev, tile).start()

        def strassen(p):
            return [(8, P(product, p, t, i, m))
                    for t in range(4) for i in range(7) for m in range(0, E, 8)]

        def qk(r, w):
            par, m = divmod(8 * r, E)
            qv = once(("qv", r), lambda: [ldf("q", (par * NT + t) * E + m) for t in range(NT)])
            s = pace(_tree([qv[t] * ldf("k", (par * NT + t) * KR + WIN + m - w, z=r % 2)
                            for t in range(NT)]))
            s = s + pltpu.roll(s, 64, 1)
            s = s + pltpu.roll(s, 32, 1)
            s = s * (DH ** -0.5)
            if first and m < w:
                s = jnp.where(m + lax.broadcasted_iota(jnp.int32, (8, 128), 0) >= w, s, -1e9)
            memo["lg", r, w] = s

        def expo(r):
            lg = [memo["lg", r, w] for w in range(WIN)]
            m = pace(functools.reduce(jnp.maximum, lg))
            memo["e", r] = [jnp.exp(s - m) for s in lg]

        def norm(r):
            memo["inv", r] = 1.0 / pace(_tree(memo["e", r]))

        def probs(r):
            inv = pace(memo["inv", r])
            for w in range(WIN):
                st("p", w * R + 8 * r, memo["e", r][w] * inv)

        def qk_list():
            out, nr = [], R // 8
            for i in range(WIN * nr + 26):
                r, w = divmod(i, WIN)
                tasks = [P(qk, r, w)] if r < nr else []
                for f, lag in ((expo, 21), (norm, 23), (probs, 25)):
                    if i >= lag and (i - lag) % WIN == 0 and (i - lag) // WIN < nr:
                        tasks.append(P(f, (i - lag) // WIN))
                out.append((26 if r < nr else 12, P(_run, [(0, f) for f in tasks])))
            return out

        def pv(m, par, h, u):
            p = once(("pv", m, par),
                     lambda: [ldf("p", w * R + par * E + m) for w in range(WIN)])
            row = (par * NT + 4 * h + u) * KR + WIN + m
            val = pace(_tree([p[w] * ldf("v", row - w, z=m // 8 % 2) for w in range(WIN)]))
            memo["o", m, par, h, u] = val
            if par and h:
                sums = memo["left", m, u] = _left(
                    *(memo["o", m, a, b, u] for a in range(2) for b in range(2)))
                if m % 16:
                    for i, (lo, hi) in enumerate(zip(memo["left", m - 8, u], sums)):
                        st16("os0", ((4 * i + u) * E + m - 8) // 2, lo, hi)

        def pv_list():
            return [(18, P(pv, m, par, h, u)) for r in range(0, E, 16) for u in range(0, 4)
                    for m in (r, r + 8) for par in range(2) for h in range(2)]

        if last:
            _run(strassen(3))
            return

        if first:
            conv = _split(a3_list(), 5, 1, 1, 1, 1, 1, 6)
            wait([w_copy(0)])
            _run(perm_list(0))
            wait(a_copies(0, 0))
            _weave(dft_list("hf", 0, 4), a1_list(0, 8))
            _weave(dft_list("hf", 8, 12) + dft_list("xf", 0), a1_list(8, 16))
            _run(dft_list("xf", 4, 8, 12) + conv[0])
            wait(x_copies(0, 0) + [w_copy(1)])
            _run(xprep_list())
            _weave(plain_list(0), _merge(perm_list(1), conv[1]))
            sums = _split(right_list(0), 1, 1) + _split(right_list(1), 1, 1)
            for n in range(1, 5):
                wait([w_copy(n + 1)])
                _weave(plain_list(n), _merge(perm_list(n + 1), _merge(sums[n - 1], conv[n + 1])))
            wait([wo_copy(0), wo_copy(1)])
            for c in in_copies(1, 1):
                c.start()
            _weave(plain_list(5), qk_list())
            _run(_merge(wo_list(0) + wo_list(1), conv[6]))
            wait(q_copies(0, 0))
            _weave(idft_list(), pv_list())
            oa_copy(j, slot).start()
            _run(right_list(2) + right_list(3))
            return

        conv = _split(a3_list(), 13, 3)
        mix = _split(pv_list(), 3, 1)
        pre = _split(xprep_list(), 1, 3)
        carry = [(1, lambda r=r: st("os1", r, pace(ld("os0", r, z=3)))) for r in range(0, _BUFS["os0"], 8)]
        _weave(dft_list("hf", 0, 4), a1_list(0, 8))
        _weave(dft_list("hf", 8, 12) + dft_list("xf", 0), a1_list(8, 16) + pre[0])
        _weave(dft_list("xf", 4, 8), pre[1])
        _run(dft_list("xf", 12))
        _weave(strassen(0) + strassen(1), _merge(carry, conv[0]))
        _weave(strassen(2), qk_list())
        tail = strassen(3)
        _weave(tail[:-32], _merge(conv[1], mix[0]) if conv[1] else mix[0])
        _weave(tail[-32:] + idft_list(), mix[1])
        oa_copy(j, slot).start()

    def loop(j, carry):
        slot = j % 2
        _wait(in_copies(j, slot))

        @pl.when(j + 1 < NS)
        def _():
            for c in in_copies(j + 1, 1 - slot):
                c.start()

        @pl.when(j >= 2)
        def _():
            oa_copy(j - 2, slot).wait()

        @pl.when(j >= 3)
        def _():
            _wait(ob_copies(j - 3, 1 - slot))

        step(j)
        return carry

    step(0, first=True)
    lax.fori_loop(1, NS, loop, 0)
    for r in range(0, _BUFS["os0"], 64):
        st("os1", r, ld("os0", r, 64, z=3))
    _wait(ob_copies(NS - 3, 1))
    step(NS, last=True)
    _wait([oa_copy(NS - 2, 0), oa_copy(NS - 1, 1)] + ob_copies(NS - 2, 0) + ob_copies(NS - 1, 1))


@jax.jit
def pallas_concat_heads__ssm_conv_h3__sliding_local_dilated__prompt_kernel(
    A_q, A_k, A_v, A_shift_k, A_ssm_k, A_ssm_D, B_x, B_wqkv, B_wo,
):
    hbm = pl.BlockSpec(memory_space=pl.ANY)
    out = pl.pallas_call(
        _kernel,
        in_specs=[hbm] * 10,
        out_specs=hbm,
        out_shape=jax.ShapeDtypeStruct((S, 2 * D), BF16),
        scratch_shapes=[
            pltpu.VMEM((2, 128, S), BF16),
            pltpu.VMEM((6, D // 2, D), BF16),
            pltpu.VMEM((2, D, D // 2), BF16),
            pltpu.VMEM((NT, 5, 8, 128), F32),
            pltpu.VMEM((4, D), BF16),
            pltpu.VMEM((8, 128), BF16),
            pltpu.VMEM(_TABLE.shape, U32),
            pltpu.SemaphoreType.DMA((21,)),
            pltpu.SemaphoreType.DMA((4,)),
        ] + [pltpu.VMEM((NT * D // 4, 128), U32)] * 6 + [pltpu.VMEM((NT * D // 2, 128), BF16)] * 2
        + [pltpu.VMEM((5 * D, 128), U32)] * 4
        + [pltpu.VMEM((2 * n, 128), BF16) if name in _HALF else pltpu.VMEM((n, 128), U32)
           for name, n in _BUFS.items()],
        compiler_params=pltpu.CompilerParams(vmem_limit_bytes=100 * 1024 * 1024),
        name="fused",
    )(A_q[0], A_k[0], A_v[0], A_shift_k.T, A_ssm_k,
      A_ssm_D.reshape(8, 128), B_x[0], B_wqkv, B_wo, _TABLE)
    return out[None]
```

```python
import functools

import jax
import jax.numpy as jnp
import numpy as np
from jax import lax
from jax.experimental import pallas as pl
import jax.experimental.pallas.tpu as pltpu


S = 2048
D = 1024
T = 128
NC = S // T
NS = 8
R = S // NS
E = R // 2
NT = D // 128
WIN, DH = 8, 32
PITCH = 33
KR = WIN + E
FP = 2 * T + 16

F32, BF16, U32 = jnp.float32, jnp.bfloat16, jnp.uint32


def _pack_rows(m):
    b = m.astype(jnp.bfloat16).view(np.uint16).astype(np.uint32)
    return np.ascontiguousarray(b[0::2] | (b[1::2] << 16))


def _dft_table():
    th = 2.0 * np.pi * (np.arange(T) + 0.25) / T
    ph = th[:, None] * (np.arange(T)[None, :] - (T - 1) / 4)
    fwd = np.concatenate([np.cos(ph), -np.sin(ph)], axis=0)
    rows = np.arange(T // 2).reshape(-1, 8, 2).transpose(0, 2, 1).reshape(-1)
    cols = np.arange(T).reshape(-1, 2, 8).transpose(0, 2, 1).reshape(-1)
    ph = (rows[:, None] + 0.5) * th[cols][None, :]
    return np.concatenate([_pack_rows(m) for m in (fwd, np.cos(ph) / T, np.sin(ph) / T)]
                          + [np.zeros((8, T), np.uint32)], axis=0)


_TABLE = _dft_table()


def _lo(w):
    return pltpu.bitcast(w << 16, F32)


def _hi(w):
    return pltpu.bitcast(w & jnp.uint32(0xFFFF0000), F32)


def _pack(lo, hi):
    return pltpu.pack_elementwise([lo, hi], packed_dtype=BF16)


def _tree(xs):
    while len(xs) > 1:
        xs = [xs[i] + xs[i + 1] if i + 1 < len(xs) else xs[i] for i in range(0, len(xs), 2)]
    return xs[0]


def _left(a11, a12, a21, a22):
    return [a21 + a22, a22, a11 + a12, a11, a11 + a22, a12 - a22, a21 - a11]


def _merge(main, side):
    total_m = sum(c for c, _ in main)
    total_s = sum(c for c, _ in side)
    done_m, done_s, i, out = 0, 0, 0, []
    for c, f in main:
        out.append((c * total_s, f))
        done_m += c
        while i < len(side) and (done_s + side[i][0]) * total_m <= done_m * total_s:
            done_s += side[i][0]
            out.append((side[i][0] * total_m, side[i][1]))
            i += 1
    assert i == len(side)
    return out


def _run(tasks):
    for _, f in tasks:
        f()


def _weave(main, side):
    _run(_merge(main, side))


def _split(tasks, *weights):
    ends = np.cumsum((0,) + weights) * len(tasks) // sum(weights)
    return [tasks[a:b] for a, b in zip(ends[:-1], ends[1:])]


def _wait(copies):
    for c in copies:
        c.wait()


_BUFS = dict(
    qa=NS * S // 2, ka=NS * (S // 2 + 8), va=NS * S // 2, oa=NS * S // 2, ob=NS * NT * E,
    hf=NC * FP + 16, xf=NC * FP, kv0=S // 8, kv1=S // 8, kv2=S // 8, kv3=S // 8, z=NC * T,
    up=8 * NC, k1=8 * NC, pi=8 * NC, zr=8 * NC, zi=8 * NC, even=2 * T,
    xs=9 * 4 * E // 2, os=7 * 4 * E // 2, o=NT * R,
    c21=E, m4=E, c11=E, m5=E, c22=E, d11=E, d22=E, f21=E, f12=E,
    q=2 * NT * E, k=2 * NT * KR, v=2 * NT * KR, p=2 * WIN * E,
    acc0=NT * R, acc1=NT * R, t0=32 * PITCH, t1=32 * PITCH,
)
_HALF = ("qa", "ka", "va", "oa", "ob", "xs", "os")


def _kernel(q_hbm, k_hbm, v_hbm, sk_hbm, h_hbm, d_hbm, x_hbm, w_hbm, wo_hbm, tab_hbm, out_hbm,
            ha, xa, wraw, woraw, taps, sk_ref, d_ref, tab, sem_in, sem_out, *bufs):
    wp16, ws = bufs[6:8], bufs[8:12]
    wp = list(bufs[:6]) + [b.bitcast(U32) for b in wp16]
    KW = D // 4
    raw = dict(zip(_BUFS, bufs[12:]))
    bufs = {n: b.bitcast(U32) if n in _HALF else b for n, b in raw.items()}
    P = functools.partial

    def ld(name, row, n=8, z=0):
        return views[name][z][pl.ds(row, n), :]

    def ldf(name, row, n=8, z=0):
        return pltpu.bitcast(ld(name, row, n, z), F32)

    def st(name, row, val):
        val = pltpu.bitcast(val, U32)
        bufs[name][pl.ds(row, val.shape[0]), :] = val

    def st16(name, row, first, second):
        raw[name][pl.ds(2 * row, 16), :] = jnp.concatenate([first, second], axis=0).astype(BF16)

    def window(name, row, n):
        return bufs[name].at[pl.ds(pl.multiple_of(row, 8), n), :]

    def window16(name, row, n):
        return raw[name].at[pl.ds(pl.multiple_of(2 * row, 16), 2 * n), :]

    def cols(j):
        return pl.ds(pl.multiple_of(j * 128, 128), 128)

    def rows(j):
        return pl.ds(pl.multiple_of(j * R, R), R)

    def a_copies(j):
        return [
            pltpu.make_async_copy(h_hbm.at[cols(j), :], ha.at[j], sem_in.at[j]),
            pltpu.make_async_copy(k_hbm.at[:, cols(j)], window16("ka", j * (S // 2 + 8) + 8, S // 2),
                                  sem_in.at[NS + j]),
            pltpu.make_async_copy(v_hbm.at[:, cols(j)], window16("va", j * (S // 2), S // 2),
                                  sem_in.at[2 * NS + j]),
        ]

    def x_copy(j):
        return pltpu.make_async_copy(x_hbm.at[rows(j), :], xa.at[j], sem_in.at[3 * NS + j])

    def q_copy(j):
        return pltpu.make_async_copy(q_hbm.at[:, cols(j)], window16("qa", j * (S // 2), S // 2),
                                     sem_in.at[4 * NS + j])

    def in_copies(j):
        return a_copies(j) + [x_copy(j), q_copy(j - 1)]

    def oa_copy(j):
        return pltpu.make_async_copy(window16("oa", j * (S // 2), S // 2), out_hbm.at[:, cols(j)],
                                     sem_out.at[0])

    def ob_copy(j, t):
        return pltpu.make_async_copy(window16("ob", (j * NT + t) * E, E),
                                     out_hbm.at[rows(j), pl.ds(D + t * 128, 128)], sem_out.at[1])

    def w_copy(n):
        half = pl.ds(n % 2 * (D // 2), D // 2)
        return pltpu.make_async_copy(
            w_hbm.at[half, pl.ds(n // 2 * D, D)], wraw.at[n], sem_in.at[5 * NS + n])

    def wo_copy(n):
        return pltpu.make_async_copy(
            wo_hbm.at[:, pl.ds(n * (D // 2), D // 2)], woraw.at[n], sem_in.at[5 * NS + 6 + n])

    small = [pltpu.make_async_copy(a, b, sem_in.at[5 * NS + 8 + i]) for i, (a, b) in enumerate(
        ((tab_hbm, tab), (sk_hbm, sk_ref), (d_hbm, d_ref)))]
    startup = lambda: ([w_copy(0)] + a_copies(0) + [x_copy(0)] + [w_copy(n) for n in range(1, 6)]
                       + [wo_copy(0), wo_copy(1)])
    for c in small + startup():
        c.start()
    _wait(small)
    zero = pltpu.bitcast(tab[pl.ds(3 * T // 2, 8), :], jnp.int32)
    zs = [pl.multiple_of(zero[i, 0] * 8, 8) for i in range(3)]
    views = {n: [b.at[pl.ds(z, _BUFS[n]), :] for z in zs] + [b] for n, b in bufs.items()}

    for slot in range(NS):
        st("ka", slot * (S // 2 + 8), jnp.zeros((8, 128), U32))
    for t in range(2 * NT):
        st("k", t * KR, jnp.zeros((WIN, 128), F32))
    skf = sk_ref[...].astype(F32)
    df = d_ref[...].astype(F32)
    for t in range(NT):
        for i in range(4):
            taps[t, i] = jnp.broadcast_to(skf[i:i + 1, t * 128:(t + 1) * 128], (8, 128))
        taps[t, 4] = jnp.broadcast_to(df[t:t + 1, :], (8, 128))

    def step(j, first=False, last=False):
        memo = {}
        never = tab[pl.ds(3 * T // 2, 8), :] != 0

        def once(key, fn):
            if key not in memo:
                memo[key] = fn()
            return memo[key]

        def fresh():
            memo["fresh"] = memo.get("fresh", 1) + 1
            return pl.multiple_of(zs[0] * memo["fresh"], 8)

        def pace(val):
            if memo.get("clock") is None:
                return val
            return jnp.where(never, pltpu.bitcast(memo["clock"], val.dtype), val)

        def paced(x):
            return jnp.concatenate([pace(x[:8]), x[8:]], axis=0)

        def wait(copies):
            memo["clock"] = None
            _wait(copies)

        def perm_in(n, u, t):
            tt = paced(pltpu.bitcast(wraw[n, pl.ds(u * 256, 256), pl.ds(t * 128, 128)], U32)).T
            for hh in range(4):
                st(f"t{u}", (4 * t + hh) * PITCH, tt[hh * DH:(hh + 1) * DH])

        def perm_out(n, u, t):
            g = jnp.concatenate(
                [bufs[f"t{u}"][pl.ds(zs[0] + 4 * t + i, 32, stride=PITCH), :] for i in range(4)], axis=0)
            wp[n][pl.ds(t * KW + u * 128, 128), :] = paced(g).T

        def perm_list(n):
            return [(1, P(f, n, u, t)) for f in (perm_in, perm_out)
                    for u in range(2) for t in range(NT)] + [(2, lambda: None)] * 4

        def wo_in(t, hh):
            w = pltpu.bitcast(woraw[t // 4, pl.ds(hh * DH, DH), pl.ds(t % 4 * 128, 128)], U32)
            wt = pltpu.bitcast(paced(w), BF16).astype(F32)
            st(f"t{t % 2}", hh * PITCH, wt)

        def wo_out(t, i):
            g = bufs[f"t{t % 2}"][pl.ds(zs[0] + i, 32, stride=PITCH), :]
            wp16[i // 16][pl.ds(2 * t * KW + i % 16 * 32, 32), :] = (
                pltpu.bitcast(paced(g), F32).astype(BF16))

        def wo_list(n):
            return [(1, P(f, t, i)) for t in range(4 * n, 4 * n + 4)
                    for f in (wo_in, wo_out) for i in range(32)]

        def right(p, t, r):
            b = [once(("wv", p, h), lambda: wp[2 * p + h].at[pl.ds(zs[0], NT * KW), :])[pl.ds((t + 4 * u) * KW + r, 8), :]
                 for h in range(2) for u in range(2)]
            b[0] = pace(b[0])
            sums = []
            for half in (_lo, _hi):
                b11, b12, b21, b22 = map(half, b)
                sums.append([b21 - b11, b12 - b22, b11 + b22, b21 + b22, b11 + b12])
            for i, (lo, hi) in enumerate(zip(*sums)):
                ws[p][pl.ds((4 * i + t) * KW + r, 8), :] = _pack(lo, hi)

        def right_list(p):
            return [(1, P(right, p, t, r)) for t in range(4) for r in range(0, D // 4, 8)]

        def ld_kv(c, row, n, z=0):
            return ld(f"kv{c // 4}", c % 4 * (T // 2) + row, n, z)

        def a1(r):
            w0, w1, w2, w3 = once("taps", lambda: [taps[j, i] for i in range(4)])
            k32 = once("ka", lambda: window("ka", j * (S // 2 + 8), S // 2 + 8))
            v32 = once("va", lambda: window("va", j * (S // 2), S // 2))
            c0 = k32[pl.ds(8 + 8 * r, 8), :]
            c1 = k32[pl.ds(7 + 8 * r, 8), :]
            c2 = k32[pl.ds(6 + 8 * r, 8), :]
            vv = v32[pl.ds(8 * r, 8), :]
            e0, o0, e1, o1, o2 = _lo(c0), _hi(c0), _lo(c1), _hi(c1), _hi(c2)
            ke = (e0 * w0 + o1 * w1) + (e1 * w2 + o2 * w3)
            ko = (o0 * w0 + e0 * w1) + (o1 * w2 + e1 * w3)
            st(f"kv{r // 32}", 8 * (r % 32), pace(_pack(ke * _lo(vv), ko * _hi(vv))))

        def a1_list(c0, c1):
            return [(24, P(a1, r)) for r in range(8 * c0, 8 * c1)]

        def freq(name, c, im, m):
            return 16 * (name == "hf") + c * FP + im * (T + 8) + m

        def dft(name, c0, m):
            def mm():
                f = pltpu.bitcast(tab[pl.ds(fresh(), T), :], BF16)
                if name == "hf":
                    rhs = jnp.concatenate(
                        [ha[j, :, pl.ds(c * T, T)] for c in range(c0, c0 + 4)], axis=0)
                    return lax.dot_general(f, rhs, (((1,), (1,)), ((), ())),
                                           preferred_element_type=F32)
                rhs = jnp.concatenate(
                    [pltpu.bitcast(ld_kv(c, 0, T // 2), BF16) for c in range(c0, c0 + 4)], axis=1)
                return jnp.dot(f, rhs, preferred_element_type=F32)
            res = once((name, c0), mm)
            for u in range(4):
                memo["clock"] = res[m:m + 8, u * 128:(u + 1) * 128]
                st(name, freq(name, c0 + u, m // T, m % T), memo["clock"])

        def dft_list(name, *c0s):
            return [(8, P(dft, name, c0, m)) for c0 in c0s for m in range(0, 2 * T, 8)]

        def a3(g, plane, upper, n):
            def opnd(name, c):
                re = lambda: ldf(name, freq(name, c, 0, 8 * g), z=plane)
                im = lambda: ldf(name, freq(name, c, 1, 8 * g), z=plane)
                if name == "xf":
                    val = re() + im() if plane == 0 else re() if plane == 1 else im()
                    return pace(val) if c >= 8 else val
                return pace(re() if plane == 0 else im() - re() if plane == 1 else im() + re())
            get = lambda name, c: once((name, g, plane, c), P(opnd, name, c))
            cs = range(8, n + 1) if upper else range(min(n, 7) + 1)
            terms = [get("xf", n - c) * get("hf", c) for c in cs]
            if upper:
                st("up", 8 * n, pace(_tree(terms)))
                return
            if n >= 8:
                terms.append(ldf("up", 8 * n))
            if plane == 0:
                st("k1", 8 * n, pace(_tree(terms)))
            elif plane == 1:
                st("pi", 8 * n, pace(_tree(terms + [ldf("k1", 8 * n)])))
            else:
                pr = ldf("k1", 8 * n, z=1) - _tree(terms)
                pi = ldf("pi", 8 * n)
                zr, zi = pr, pi
                if n > 0:
                    qr, qi = memo["prev"]
                    zr, zi = pr - qi, pi + qr
                memo["prev"] = (pr, pi)
                if g % 2 == 0:
                    st("zr", 8 * n, pace(zr))
                    st("zi", 8 * n, zi)
                else:
                    st("z", n * T + 4 * (g - 1), pace(_pack(ldf("zr", 8 * n), zr)))
                    st("z", n * T + T // 2 + 4 * (g - 1), _pack(ldf("zi", 8 * n), zi))

        def a3_list():
            out = []
            for g in range(T // 8):
                for plane in range(3):
                    out += [(2 * (n - 8) + 4, P(a3, g, plane, True, n)) for n in range(8, NC)]
                    out += [(2 * min(n, 7) + 4 + 2 * (plane == 2), P(a3, g, plane, False, n))
                            for n in range(NC)]
            return out

        def idft(c0, odd, m):
            def mm():
                rhs = jnp.concatenate([pltpu.bitcast(ld("z", c * T + odd * T // 2, T // 2), BF16)
                                       for c in range(c0, c0 + 4)], axis=1)
                f = tab[pl.ds(fresh() + T + odd * T // 4, T // 4), :]
                return jnp.dot(pltpu.bitcast(f, BF16), rhs, preferred_element_type=F32)
            y = once(("y", c0, odd), mm)
            prev = j - 1
            dd = once("dd", lambda: taps[j - 1, 4])
            q32 = once("qa", lambda: window("qa", prev * (S // 2), S // 2))
            o32 = once("oa", lambda: window("oa", prev * (S // 2), S // 2))
            flip = lambda w: jnp.take_along_axis(
                w, 7 - lax.broadcasted_iota(jnp.int32, (8, 128), 0), axis=0, mode="promise_in_bounds")

            def gate(c, row, lo, hi, order):
                kv, qq = order(ld_kv(c, row, 8, z=1)), order(q32[pl.ds(c * T // 2 + row, 8), :])
                o32[pl.ds(c * T // 2 + row, 8), :] = order(_pack(
                    _lo(qq) * (lo + _lo(kv) * dd), _hi(qq) * (hi + _hi(kv) * dd)))

            for u in range(4):
                s0, s1 = (y[m + i:m + i + 8, u * 128:(u + 1) * 128] for i in (0, 8))
                memo["clock"] = s1
                if not odd:
                    st("even", u * T // 2 + m, s0)
                    st("even", u * T // 2 + m + 8, s1)
                    continue
                e0, e1 = (ldf("even", u * T // 2 + m + i) for i in (0, 8))
                gate(c0 + u, T // 4 + m // 2, e0 - s0, e1 - s1, lambda w: w)
                gate(c0 + u, T // 4 - 8 - m // 2, e1 + s1, e0 + s0, flip)

        def idft_list(*c0s):
            return [(16, P(idft, c0, odd, m)) for c0 in c0s
                    for odd in range(2) for m in range(0, T // 2, 16)]

        def xprep(u, r):
            halves = []
            for m in (r, r + 8):
                a, b = (pltpu.bitcast(xa[j, pl.ds(2 * m, 16), pl.ds(t * 128, 128)], U32) for t in (u, u + 4))
                a = pace(a)
                a11, a12, a21, a22 = _lo(a), _lo(b), _hi(a), _hi(b)
                halves.append(_left(a11, a12, a21, a22) + ([a12, a21] if first else []))
            for i, (lo, hi) in enumerate(zip(*halves)):
                st16("xs", ((4 * i + u) * E + r) // 2, lo, hi)

        def xprep_list():
            return [(27, P(xprep, u, r)) for u in range(4) for r in range(0, E, 16)]

        def lhs(name, i):
            view = bufs[name].at[pl.ds(fresh() + i * 2 * E, 2 * E), :]
            return jnp.concatenate(
                [pltpu.bitcast(view[pl.ds(u * E // 2, E // 2), :], BF16) for u in range(4)], axis=1)

        def emit(p, par, t, m, val):
            if p == 0:
                st("q", (par * NT + t) * E + m, val)
                return
            name, row = "kv"[p - 1], (par * NT + t) * KR
            if m == 0 and not first:
                st(name, row, ld(name, row + E, WIN, z=3))
            if m == 0 and first and p == 2 and par == 0:
                for other in range(2):
                    st(name, (other * NT + t) * KR, jnp.broadcast_to(val[0:1], (WIN, 128)))
            st(name, row + WIN + m, val)

        def plain(p, t, half, m):
            def mm():
                x = jnp.concatenate([lhs("xs", i) for i in ((3, 8), (7, 1))[half]], axis=0)
                w = pltpu.bitcast(wp[2 * p + half][pl.ds(t * KW, KW), :], BF16)
                return jnp.dot(x, w, preferred_element_type=F32)
            res = memo["clock"] = once(("plain", p, t, half), mm)[m:m + 8]
            if half:
                emit(p, m // E, t, m % E, res + ldf(f"acc{p % 2}", t * R + m))
            else:
                st(f"acc{p % 2}", t * R + m, res)

        def plain_list(n):
            return [(8, P(plain, n // 2, t, n % 2, m)) for t in range(NT) for m in range(0, R, 8)]

        def product(p, t, i, m):
            def mm():
                if i == 0:
                    w = wp[2 * p][pl.ds(t * KW, KW), :]
                elif i == 2:
                    w = wp[2 * p + 1][pl.ds((t + 4) * KW, KW), :]
                else:
                    w = ws[p][pl.ds((4 * (i - 1 - (i > 2)) + t) * KW, KW), :]
                return jnp.dot(lhs("xs" if p < 3 else "os", i), pltpu.bitcast(w, BF16),
                               preferred_element_type=F32)
            res = memo["clock"] = once(("product", p, t, i), mm)[m:m + 8]
            if i == 0:
                st("c21", m, res)
            elif i == 1:
                st("m4", m, res)
                c21 = ldf("c21", m) + res
                st("f21", m, c21) if p == 3 else emit(p, 1, t, m, c21)
            elif i == 2:
                st("c11", m, ldf("m4", m) - res)
                st("m5", m, res)
            elif i == 3:
                st("c22", m, res - ldf("c21", m, z=1))
                c12 = ldf("m5", m) + res
                st("f12", m, c12) if p == 3 else emit(p, 0, t + 4, m, c12)
            elif i == 4:
                st("d11", m, ldf("c11", m) + res)
                st("d22", m, ldf("c22", m) + res)
            elif p < 3:
                emit(p, i - 5, t + 4 * (i - 5), m, ldf(("d11", "d22")[i - 5], m) + res)
            else:
                o32 = once("ob", lambda: window("ob", (j - 1) * NT * E, NT * E))
                tile = t + 4 * (i - 5)
                if i == 5:
                    o32[pl.ds(tile * E + m, 8), :] = _pack(ldf("d11", m) + res, ldf("f21", m))
                else:
                    o32[pl.ds(tile * E + m, 8), :] = _pack(ldf("f12", m), ldf("d22", m) + res)
                if m + 8 == E:
                    ob_copy(j - 1, tile).start()

        def strassen(p):
            return [(8, P(product, p, t, i, m))
                    for t in range(4) for i in range(7) for m in range(0, E, 8)]

        def qk(r, w):
            par, m = divmod(8 * r, E)
            qv = once(("qv", r), lambda: [ldf("q", (par * NT + t) * E + m) for t in range(NT)])
            s = pace(_tree([qv[t] * ldf("k", (par * NT + t) * KR + WIN + m - w, z=r % 2)
                            for t in range(NT)]))
            s = s + pltpu.roll(s, 64, 1)
            s = s + pltpu.roll(s, 32, 1)
            if first and m < w:
                s = jnp.where(m + lax.broadcasted_iota(jnp.int32, (8, 128), 0) >= w, s, -1e9 * DH ** 0.5)
            memo["lg", r, w] = s

        def expo(r):
            lg = [memo["lg", r, w] for w in range(WIN)]
            m = pace(functools.reduce(jnp.maximum, lg))
            memo["e", r] = [jnp.exp2((s - m) * (DH ** -0.5 * np.log2(np.e)).item()) for s in lg]

        def norm(r):
            memo["inv", r] = 1.0 / pace(_tree(memo["e", r]))

        def probs(r):
            inv = pace(memo["inv", r])
            for w in range(WIN):
                st("p", w * R + 8 * r, memo["e", r][w] * inv)

        def qk_list():
            out, nr = [], R // 8
            for i in range(WIN * nr + 26):
                r, w = divmod(i, WIN)
                tasks = [P(qk, r, w)] if r < nr else []
                for f, lag in ((expo, 21), (norm, 23), (probs, 25)):
                    if i >= lag and (i - lag) % WIN == 0 and (i - lag) // WIN < nr:
                        tasks.append(P(f, (i - lag) // WIN))
                out.append((26 if r < nr else 12, P(_run, [(0, f) for f in tasks])))
            return out

        def pv(r, t):
            par, m = divmod(8 * r, E)
            p = once(("pv", r), lambda: [ldf("p", w * R + 8 * r) for w in range(WIN)])
            row = (par * NT + t) * KR + WIN + m
            st("o", t * R + 8 * r, pace(_tree([p[w] * ldf("v", row - w, z=r % 2) for w in range(WIN)])))

        def pv_list():
            return [(16, P(pv, r, t)) for r in range(R // 8) for t in range(NT)]

        def oprep(u, r):
            halves = []
            for m in (r, r + 8):
                a = [ldf("o", (u + 4 * h) * R + par * E + m) for par in range(2) for h in range(2)]
                halves.append(_left(*a[:3], pace(a[3])))
            for i, (lo, hi) in enumerate(zip(*halves)):
                st16("os", ((4 * i + u) * E + r) // 2, lo, hi)

        def oprep_list():
            return [(19, P(oprep, u, r)) for u in range(4) for r in range(0, E, 16)]

        if last:
            _weave(idft_list(0, 4, 8, 12), oprep_list())
            oa_copy(j - 1).start()
            _run(strassen(3))
            return

        if first:
            conv = _split(a3_list(), 4, 3, 2, 2, 2, 2, 1)
            wait([w_copy(0)])
            _run(perm_list(0))
            wait(a_copies(0))
            _weave(dft_list("hf", 0, 4), a1_list(0, 8))
            _weave(dft_list("hf", 8, 12) + dft_list("xf", 0), a1_list(8, 16))
            _run(dft_list("xf", 4, 8, 12) + conv[0])
            wait([x_copy(0), w_copy(1)])
            _run(xprep_list())
            _weave(plain_list(0), _merge(perm_list(1), conv[1]))
            sums = _split(right_list(0), 1, 1) + _split(right_list(1), 1, 1)
            for n in range(1, 5):
                wait([w_copy(n + 1)])
                for c in in_copies(n):
                    c.start()
                _weave(plain_list(n), _merge(perm_list(n + 1), _merge(sums[n - 1], conv[n + 1])))
            wait([wo_copy(0)])
            for c in in_copies(5) + in_copies(6) + in_copies(7) + [q_copy(7)]:
                c.start()
            _weave(plain_list(5), qk_list())
            _run(_merge(wo_list(0), conv[6] + right_list(2)))
            wait([wo_copy(1)])
            _run(_merge(wo_list(1), pv_list()) + right_list(3))
            return

        conv = _split(a3_list(), 27, 5)
        _run(idft_list(0))
        _weave(dft_list("hf", 0), a1_list(0, 3))
        _run(idft_list(4))
        _weave(dft_list("hf", 4), a1_list(3, 6))
        _run(idft_list(8))
        _weave(dft_list("hf", 8), a1_list(6, 9))
        _run(idft_list(12))
        oa_copy(j - 1).start()
        _weave(dft_list("hf", 12), a1_list(9, 12))
        _weave(dft_list("xf", 0, 4, 8), a1_list(12, 16) + xprep_list())
        _weave(dft_list("xf", 12), oprep_list())
        _weave(strassen(0) + strassen(1), conv[0])
        tail = strassen(2) + strassen(3)
        _weave(tail[:480], qk_list())
        _weave(tail[480:], _merge(conv[1], pv_list()) if conv[1] else pv_list())

    def loop(j, carry):
        _wait(in_copies(j))
        step(j)
        return carry

    step(0, first=True)
    lax.fori_loop(1, NS, loop, 0)
    q_copy(NS - 1).wait()
    step(NS, last=True)
    _wait([oa_copy(j) for j in range(NS)] + [ob_copy(j, t) for j in range(NS) for t in range(NT)])


@jax.jit
def pallas_concat_heads__ssm_conv_h3__sliding_local_dilated__prompt_kernel(
    A_q, A_k, A_v, A_shift_k, A_ssm_k, A_ssm_D, B_x, B_wqkv, B_wo,
):
    hbm = pl.BlockSpec(memory_space=pl.ANY)
    out = pl.pallas_call(
        _kernel,
        in_specs=[hbm] * 10,
        out_specs=hbm,
        out_shape=jax.ShapeDtypeStruct((S, 2 * D), BF16),
        scratch_shapes=[
            pltpu.VMEM((NS, 128, S), BF16),
            pltpu.VMEM((NS, R, D), BF16),
            pltpu.VMEM((6, D // 2, D), BF16),
            pltpu.VMEM((2, D, D // 2), BF16),
            pltpu.VMEM((NT, 5, 8, 128), F32),
            pltpu.VMEM((4, D), BF16),
            pltpu.VMEM((8, 128), BF16),
            pltpu.VMEM(_TABLE.shape, U32),
            pltpu.SemaphoreType.DMA((5 * NS + 11,)),
            pltpu.SemaphoreType.DMA((2,)),
        ] + [pltpu.VMEM((NT * D // 4, 128), U32)] * 6 + [pltpu.VMEM((NT * D // 2, 128), BF16)] * 2
        + [pltpu.VMEM((5 * D, 128), U32)] * 4
        + [pltpu.VMEM((2 * n, 128), BF16) if name in _HALF else pltpu.VMEM((n, 128), U32)
           for name, n in _BUFS.items()],
        compiler_params=pltpu.CompilerParams(vmem_limit_bytes=100 * 1024 * 1024,
                                             disable_bounds_checks=True),
        name="fused",
    )(A_q[0], A_k[0], A_v[0], A_shift_k.T, A_ssm_k,
      A_ssm_D.reshape(8, 128), B_x[0], B_wqkv, B_wo, _TABLE)
    return out[None]
```

```python
import functools

import jax
import jax.numpy as jnp
import numpy as np
from jax import lax
from jax.experimental import pallas as pl
import jax.experimental.pallas.tpu as pltpu


S = 2048
D = 1024
T = 128
NC = S // T
NT = D // 128
NS = 4
R = S // NS
E = R // 2
WIN, DH = 8, 32
PITCH = 33
KR = WIN + E
FP = 2 * T + 16
KW = D // 4

F32, BF16, U32 = jnp.float32, jnp.bfloat16, jnp.uint32
P = functools.partial
add, sub, mul = lax.add, lax.sub, lax.mul


def _pack_rows(m):
    b = m.astype(jnp.bfloat16).view(np.uint16).astype(np.uint32)
    return np.ascontiguousarray(b[0::2] | (b[1::2] << 16))


def _dft_table():
    th = 2.0 * np.pi * (np.arange(T) + 0.25) / T
    ph = th[:, None] * (np.arange(T)[None, :] - (T - 1) / 4)
    fwd = np.concatenate([np.cos(ph), -np.sin(ph)], axis=0)
    rows = np.arange(T // 2).reshape(-1, 8, 2).transpose(0, 2, 1).reshape(-1)
    cols = np.arange(T).reshape(-1, 2, 8).transpose(0, 2, 1).reshape(-1)
    ph = (rows[:, None] + 0.5) * th[cols][None, :]
    return np.concatenate([_pack_rows(m) for m in (fwd, np.cos(ph) / T, np.sin(ph) / T)]
                          + [np.zeros((8, T), np.uint32)], axis=0)


_TABLE = _dft_table()


def _lo(w):
    return pltpu.bitcast(lax.shift_left(w, np.uint32(16)), F32)


def _hi(w):
    return pltpu.bitcast(lax.bitwise_and(w, np.uint32(0xFFFF0000)), F32)


def _pack(lo, hi):
    return pltpu.pack_elementwise([lo, hi], packed_dtype=BF16)


def _tree(xs):
    while len(xs) > 1:
        xs = [add(xs[i], xs[i + 1]) if i + 1 < len(xs) else xs[i] for i in range(0, len(xs), 2)]
    return xs[0]


def _left(a11, a12, a21, a22):
    return [add(a21, a22), a22, add(a11, a12), a11, add(a11, a22), sub(a12, a22), sub(a21, a11)]


def _merge(main, side):
    if not main:
        return side
    total_m = sum(c for c, _ in main)
    total_s = sum(c for c, _ in side)
    done_m, done_s, i, out = 0, 0, 0, []
    for c, f in main:
        out.append((c * total_s, f))
        done_m += c
        while i < len(side) and (done_s + side[i][0]) * total_m <= done_m * total_s:
            done_s += side[i][0]
            out.append((side[i][0] * total_m, side[i][1]))
            i += 1
    assert i == len(side)
    return out


def _run(tasks):
    for _, f in tasks:
        f()


def _weave(main, side):
    _run(_merge(main, side))


def _split(tasks, *weights):
    ends = np.cumsum((0,) + weights) * len(tasks) // sum(weights)
    return [tasks[a:b] for a, b in zip(ends[:-1], ends[1:])]


def _start(copies):
    for c in copies:
        c.start()


def _wait(copies):
    for c in copies:
        c.wait()


_BUFS = {n: (t, r) for t, group in (
    (BF16, dict(qa=NT * S // 2, ka=NT * (S // 2 + 8), va=NT * S // 2, oa=NT * S // 2, ob=S * NT // 2,
                xs=10 * 4 * E // 2, os=7 * 4 * E // 2, w3=2 * NT * KW)),
    (U32, dict(kv0=S // 8, kv1=S // 8, kv2=S // 8, kv3=S // 8, z=NC * T,
               **{f"w{p}": 2 * NT * KW for p in range(3)}, **{f"ws{p}": 20 * KW for p in range(4)},
               t0=32 * PITCH, t1=32 * PITCH)),
    (F32, dict(hf=NC * FP, xf=NC * FP, up=8 * NC, k1=8 * NC, pi=8 * NC, zr=8 * NC, zi=8 * NC,
               even=2 * T, c21=E, m4=E, c11=E, m5=E, c22=E, d11=E, d22=E, f21=E, f12=E,
               q=2 * NT * E, k=2 * NT * KR, v=2 * NT * KR, p=WIN * R, o=NT * R)),
) for n, r in group.items()}


def _kernel(q_hbm, k_hbm, v_hbm, sk_hbm, h_hbm, d_hbm, x_hbm, w_hbm, wo_hbm, tab_hbm, out_hbm,
            ha, xa, wraw, woraw, taps, sk_ref, d_ref, tab, sem_in, sem_out, *raw):
    raw = dict(zip(_BUFS, raw))
    bufs = {n: b.bitcast(U32) if _BUFS[n][0] == BF16 else b for n, b in raw.items()}

    def ld(name, row, n=8, z=0):
        return views[name][z][pl.ds(row, n), :]

    def st(name, row, val):
        views[name][3][pl.ds(row, val.shape[0]), :] = val

    def st16(name, row, val):
        views[name][4][pl.ds(2 * row, val.shape[0]), :] = val.astype(BF16)

    def window(name, row, n):
        return bufs[name].at[pl.ds(pl.multiple_of(row, 8), n), :]

    def window16(name, row, n):
        return raw[name].at[pl.ds(pl.multiple_of(2 * row, 16), 2 * n), :]

    def cols(a):
        return pl.ds(pl.multiple_of(a * 128, 128), 128)

    def rows(j):
        return pl.ds(pl.multiple_of(j * R, R), R)

    def a_copies(a):
        return [
            pltpu.make_async_copy(h_hbm.at[cols(a), :], ha.at[a], sem_in.at[a]),
            pltpu.make_async_copy(k_hbm.at[:, cols(a)], window16("ka", a * (S // 2 + 8) + 8, S // 2),
                                  sem_in.at[NT + a]),
            pltpu.make_async_copy(v_hbm.at[:, cols(a)], window16("va", a * (S // 2), S // 2),
                                  sem_in.at[2 * NT + a]),
        ]

    def q_copy(a):
        return pltpu.make_async_copy(q_hbm.at[:, cols(a)], window16("qa", a * (S // 2), S // 2),
                                     sem_in.at[3 * NT + a])

    def x_copy(j):
        return pltpu.make_async_copy(x_hbm.at[rows(j), :], xa.at[j], sem_in.at[4 * NT + j])

    def in_copies(j):
        return a_copies(2 * j) + [x_copy(j), q_copy(2 * j - 1)] + a_copies(2 * j + 1) + [q_copy(2 * j)]

    def w_copy(n):
        half = pl.ds(n % 2 * (D // 2), D // 2)
        return pltpu.make_async_copy(
            w_hbm.at[half, pl.ds(n // 2 * D, D)], wraw.at[n], sem_in.at[5 * NT + n])

    def w_wait(n):
        pltpu.make_async_copy(wraw.at[n], wraw.at[n], sem_in.at[5 * NT + n]).wait()

    def wo_copies():
        return [pltpu.make_async_copy(wo_hbm.at[:, pl.ds(t * 128, 128)], woraw.at[t],
                                      sem_in.at[5 * NT + 6]) for t in range(NT)]

    def oa_copy(a):
        return pltpu.make_async_copy(window16("oa", a * (S // 2), S // 2), out_hbm.at[:, cols(a)],
                                     sem_out.at[0])

    def ob_copy(j, t):
        return pltpu.make_async_copy(window16("ob", (j * NT + t) * E, E),
                                     out_hbm.at[rows(j), cols(NT + t)], sem_out.at[1])

    small = [pltpu.make_async_copy(a, b, sem_in.at[5 * NT + 7 + i]) for i, (a, b) in enumerate(
        ((tab_hbm, tab), (sk_hbm, sk_ref), (d_hbm, d_ref)))]
    startup = lambda: ([w_copy(0), x_copy(0), w_copy(1)] + a_copies(0) + [w_copy(n) for n in range(2, 6)]
                       + a_copies(1) + [q_copy(0)] + wo_copies())
    _start(small + startup())
    _wait(small)
    unit = pltpu.bitcast(tab[pl.ds(3 * T // 2, 8), :], jnp.int32)
    zs = [pl.multiple_of(unit[i, 0] * 8, 8) for i in range(3)]
    views = {n: [b.at[pl.ds(z, _BUFS[n][1]), :] for z in zs] + [b, raw[n]] for n, b in bufs.items()}

    for a in range(NT):
        st("ka", a * (S // 2 + 8), jnp.zeros((8, 128), U32))
    for t in range(2 * NT):
        st("k", t * KR, jnp.zeros((WIN, 128), F32))
    skf = sk_ref[...].astype(F32)
    df = d_ref[...].astype(F32)
    for t in range(NT):
        for i in range(4):
            taps[t, i] = jnp.broadcast_to(skf[i:i + 1, t * 128:(t + 1) * 128], (8, 128))
        taps[t, 4] = jnp.broadcast_to(df[t:t + 1, :], (8, 128))

    def step(j, first=False, last=False):
        memo = {}
        never = tab[pl.ds(3 * T // 2, 8), :] != 0

        def once(key, fn):
            if key not in memo:
                memo[key] = fn()
            return memo[key]

        def fresh():
            memo["fresh"] = memo.get("fresh", 1) + 1
            return pl.multiple_of(zs[0] * memo["fresh"], 8)

        def pace(val):
            clock = memo.get("clock")
            if clock is None:
                return val
            if val.dtype != F32:
                clock = pltpu.bitcast(clock, val.dtype)
            return lax.select(never, clock, val)

        def paced(x):
            return jnp.concatenate([pace(x[:8]), x[8:]], axis=0)

        def wait(copies):
            memo["clock"] = None
            _wait(copies)

        def rolled(n, shifts, body):
            def one(i, carry):
                saved, kept = dict(views), dict(memo)
                memo["clock"] = None
                for name, d in shifts.items():
                    size = _BUFS[name][1] - d * (n - 1)
                    views[name] = [window(name, z + d * i, size) for z in zs + [0]]
                    if _BUFS[name][0] == BF16:
                        views[name].append(window16(name, d * i, size))
                body(i)
                views.update(saved)
                memo.clear()
                memo.update(kept, clock=None)
                return carry
            lax.fori_loop(0, n, one, 0)

        def perm_in(w, u, t):
            tt = paced(pltpu.bitcast(w[pl.ds(u * 256, 256), pl.ds(t * 128, 128)], U32)).T
            for hh in range(4):
                st(f"t{u}", (4 * t + hh) * PITCH, tt[hh * DH:(hh + 1) * DH])

        def perm_out(p, h, u, t):
            g = jnp.concatenate(
                [bufs[f"t{u}"][pl.ds(zs[0] + 4 * t + i, 32, stride=PITCH), :] for i in range(4)], axis=0)
            st(f"w{p}", (h * NT + t) * KW + u * 128, paced(g).T)

        def perm_list(n, w=None, us=(0, 1)):
            w = wraw.at[n] if w is None else w
            return [(1, P(f, u, t)) for f in (P(perm_in, w), P(perm_out, n // 2, n % 2))
                    for u in us for t in range(NT)] + [(2, lambda: None)] * 4

        def wo_in(i, t, hh):
            w = pltpu.bitcast(woraw[2 * i + t, pl.ds(hh * DH, DH), :], U32)
            wt = pltpu.bitcast(paced(w), BF16).astype(F32)
            st(f"t{t % 2}", hh * PITCH, pltpu.bitcast(wt, U32))

        def wo_out(t, i):
            g = bufs[f"t{t % 2}"][pl.ds(zs[0] + i, 32, stride=PITCH), :]
            st16("w3", (i // 16 * NT + t) * KW + i % 16 * 16, pltpu.bitcast(paced(g), F32))

        def wo_list(i):
            return [(1, P(f, t, u)) for f in (P(wo_in, i), wo_out) for t in range(2) for u in range(32)]

        def right(p, t, r):
            b = [ld(f"w{p}", (h * NT + t + 4 * u) * KW + r, 16) for h in range(2) for u in range(2)]
            b[0] = paced(b[0])
            sums = []
            for half in (_lo, _hi):
                b11, b12, b21, b22 = map(half, b)
                sums.append([sub(b21, b11), sub(b12, b22), add(b11, b22), add(b21, b22), add(b11, b12)])
            for i, (lo, hi) in enumerate(zip(*sums)):
                st(f"ws{p}", (4 * i + t) * KW + r, _pack(lo, hi))

        def right_list(p):
            return [(1, P(right, p, t, r)) for t in range(4) for r in range(0, KW, 16)]

        def ld_kv(c, row, n, z=0):
            return ld(f"kv{c // 4}", c % 4 * (T // 2) + row, n, z)

        def a1(i, r):
            a = once(("a", i), lambda: 2 * j + i)
            w0, w1, w2, w3 = once(("taps", i), lambda: [taps[a, u] for u in range(4)])
            k32 = once(("ka", i), lambda: window("ka", a * (S // 2 + 8), S // 2 + 8))
            v32 = once(("va", i), lambda: window("va", a * (S // 2), S // 2))
            c0, c1, c2 = (k32[pl.ds(8 * r + 8 - u, 8), :] for u in range(3))
            vv = v32[pl.ds(8 * r, 8), :]
            e0, o0, e1, o1, o2 = _lo(c0), _hi(c0), _lo(c1), _hi(c1), _hi(c2)
            ke = _tree([mul(e0, w0), mul(o1, w1), mul(e1, w2), mul(o2, w3)])
            ko = _tree([mul(o0, w0), mul(e0, w1), mul(o1, w2), mul(e1, w3)])
            st(f"kv{r // 32}", 8 * (r % 32), pace(_pack(mul(ke, _lo(vv)), mul(ko, _hi(vv)))))

        def a1_list(i, c0, c1):
            return [(24, P(a1, i, r)) for r in range(8 * c0, 8 * c1)]

        def freq(c, im, m):
            return c * FP + im * (T + 8) + m

        def dft(i, name, c0, m):
            def mm():
                f = pltpu.bitcast(tab[pl.ds(fresh(), T), :], BF16)
                if name == "hf":
                    a = once(("a", i), lambda: 2 * j + i)
                    rhs = jnp.concatenate(
                        [ha[a, :, pl.ds(c * T, T)] for c in range(c0, c0 + 4)], axis=0)
                    return lax.dot_general(f, rhs, (((1,), (1,)), ((), ())),
                                           preferred_element_type=F32)
                rhs = jnp.concatenate(
                    [pltpu.bitcast(ld_kv(c, 0, T // 2, i), BF16) for c in range(c0, c0 + 4)], axis=1)
                return jnp.dot(f, rhs, preferred_element_type=F32)
            res = once((name, i, c0), mm)
            for u in range(4):
                st(name, freq(c0 + u, m // T, m % T), res[m:m + 16, u * 128:(u + 1) * 128])
            memo["clock"] = res[m + 8:m + 16, 384:]

        def dft_list(i, name, *c0s):
            return [(16, P(dft, i, name, c0, m)) for c0 in c0s for m in range(0, 2 * T, 16)]

        def a3(i, g, plane, upper, n):
            def opnd(name, c):
                re = lambda: ld(name, freq(c, 0, 8 * g), z=plane)
                im = lambda: ld(name, freq(c, 1, 8 * g), z=plane)
                if name == "xf":
                    val = add(re(), im()) if plane == 0 else re() if plane == 1 else im()
                    return pace(val) if c >= 8 else val
                return pace(re() if plane == 0 else (sub, add)[plane - 1](im(), re()))
            get = lambda name, c: once((name, i, g, plane, c), P(opnd, name, c))
            cs = range(8, n + 1) if upper else range(min(n, 7) + 1)
            terms = [mul(get("xf", n - c), get("hf", c)) for c in cs]
            if upper:
                st("up", 8 * n, pace(_tree(terms)))
                return
            if n >= 8:
                terms.append(ld("up", 8 * n))
            if plane == 0:
                st("k1", 8 * n, pace(_tree(terms)))
            elif plane == 1:
                st("pi", 8 * n, pace(_tree(terms + [ld("k1", 8 * n)])))
            else:
                pr = sub(ld("k1", 8 * n, z=1), _tree(terms))
                pi = ld("pi", 8 * n)
                zr, zi = pr, pi
                if n > 0:
                    qr, qi = memo["prev"]
                    zr, zi = sub(pr, qi), add(pi, qr)
                memo["prev"] = (pr, pi)
                if g % 2 == 0:
                    st("zr", 8 * n, pace(zr))
                    st("zi", 8 * n, zi)
                else:
                    st("z", n * T + 4 * (g - 1), _pack(ld("zr", 8 * n), pace(zr)))
                    st("z", n * T + T // 2 + 4 * (g - 1), _pack(ld("zi", 8 * n), zi))

        def a3_list(i):
            out = []
            for g in range(T // 8):
                for plane in range(3):
                    out += [(2 * (n - 8) + 4, P(a3, i, g, plane, True, n)) for n in range(8, NC)]
                    out += [(2 * min(n, 7) + 4 + 2 * (plane == 2), P(a3, i, g, plane, False, n))
                            for n in range(NC)]
            return out

        def idft(i, c0, odd, m):
            def mm():
                rhs = jnp.concatenate([pltpu.bitcast(ld("z", c * T + odd * T // 2, T // 2, i + 1), BF16)
                                       for c in range(c0, c0 + 4)], axis=1)
                f = tab[pl.ds(fresh() + T + odd * T // 4, T // 4), :]
                return jnp.dot(pltpu.bitcast(f, BF16), rhs, preferred_element_type=F32)
            y = once(("y", i, c0, odd), mm)
            a = once(("a", i), lambda: 2 * j + i)
            dd = once(("dd", i), lambda: taps[a, 4])
            q32 = once(("qa", i), lambda: window("qa", a * (S // 2), S // 2))
            o32 = once(("oa", i), lambda: window("oa", a * (S // 2), S // 2))
            flip = lambda w: jnp.take_along_axis(
                w, 7 - lax.broadcasted_iota(jnp.int32, (8, 128), 0), axis=0, mode="promise_in_bounds")

            def gate(c, row, lo, hi, order):
                kv, qq = order(ld_kv(c, row, 8, 2)), order(q32[pl.ds(c * T // 2 + row, 8), :])
                o32[pl.ds(c * T // 2 + row, 8), :] = order(_pack(
                    mul(_lo(qq), add(lo, mul(_lo(kv), dd))), mul(_hi(qq), add(hi, mul(_hi(kv), dd)))))

            for u in range(4):
                if not odd:
                    st("even", u * T // 2 + m, y[m:m + 16, u * 128:(u + 1) * 128])
                    continue
                s0, s1 = (y[m + h:m + h + 8, u * 128:(u + 1) * 128] for h in (0, 8))
                e0, e1 = (ld("even", u * T // 2 + m + h) for h in (0, 8))
                gate(c0 + u, T // 4 + m // 2, sub(e0, s0), sub(e1, s1), lambda w: w)
                gate(c0 + u, T // 4 - 8 - m // 2, add(e1, s1), add(e0, s0), flip)
            memo["clock"] = y[m + 8:m + 16, 384:]

        def idft_list(i, *c0s):
            return [(16, P(idft, i, c0, odd, m)) for c0 in c0s
                    for odd in range(2) for m in range(0, T // 2, 16)]

        def transforms(i, extra):
            extra = _split(extra, 1, 1, 1, 1, 1, 9)
            for u in range(4):
                _weave(idft_list(i - 1, 4 * u)[:4], extra[u])
                _run(idft_list(i - 1, 4 * u)[4:])
                _weave(dft_list(i, "hf", 4 * u), a1_list(i, 3 * u, 3 * u + 3))
            oa_copy(2 * j + i - 1).start()
            _weave(dft_list(i, "xf", 0), _merge(a1_list(i, 12, 16), extra[4]))
            _weave(dft_list(i, "xf", 4, 8), extra[5])
            _run(dft_list(i, "xf", 12))

        def xprep(x, u, r):
            halves = []
            for m in (r, r + 8):
                a, b = (pltpu.bitcast(x[pl.ds(2 * m, 16), pl.ds(t * 128, 128)], U32)
                        for t in (u, u + 4))
                a = pace(a)
                a11, a12, a21, a22 = _lo(a), _lo(b), _hi(a), _hi(b)
                halves.append(_left(a11, a12, a21, a22) + ([a21, a12, a22] if first else []))
            for i, pair in enumerate(zip(*halves)):
                st16("xs", ((4 * i + u) * E + r) // 2, jnp.concatenate(pair, axis=0))

        def xprep_list(x):
            return [(27, P(xprep, x, u, r)) for r in range(0, E, 16) for u in range(4)]

        def lhs(name, i):
            view = views[name][3].at[pl.ds(fresh() + i * 2 * E, 2 * E), :]
            return jnp.concatenate(
                [pltpu.bitcast(view[pl.ds(u * E // 2, E // 2), :], BF16) for u in range(4)], axis=1)

        def emit(p, par, t, m, val):
            if p == 0:
                st("q", (par * NT + t) * E + m, val)
                return
            name, row = "kv"[p - 1], (par * NT + t) * KR
            if m == 0 and not first:
                st(name, row, ld(name, row + E, WIN, z=3))
            if m == 0 and first and p == 2 and par == 0:
                for other in range(2):
                    st(name, (other * NT + t) * KR, jnp.broadcast_to(val[0:1], (WIN, 128)))
            st(name, row + WIN + m, val)

        def plain(half, t, m):
            def mm():
                w = pltpu.bitcast(ld("w0", (half * NT + t) * KW, KW, 3), BF16)
                x = lhs("xs", 8) if half else jnp.concatenate([lhs("xs", 3), lhs("xs", 7)], axis=0)
                return jnp.dot(x, w, preferred_element_type=F32)
            res = once(("plain", half, t), mm)
            memo["clock"] = res[m + 8:m + 16]
            if half:
                emit(0, 0, t, m, add(res[m:m + 16], ld("o", t * R + m, 16)))
            else:
                st("o", t * R + m, res[m:m + 16])

        def plain_list(half):
            return [(16, P(plain, half, t, m)) for t in range(NT) for m in range(0, E if half else R, 16)]

        def product(p, t, i, m):
            def mm():
                if i == 0:
                    w = ld(f"w{p}", t * KW, KW, 3)
                elif i == 2:
                    w = ld(f"w{p}", (NT + t + 4) * KW, KW, 3)
                else:
                    w = ld(f"ws{p}", (4 * (i - 1 - (i > 2)) + t) * KW, KW, 3)
                return jnp.dot(lhs("xs" if p < 3 else "os", i), pltpu.bitcast(w, BF16),
                               preferred_element_type=F32)
            res = once(("product", p, t, i), mm)
            memo["clock"] = res[m + 8:m + 16]
            res = res[m:m + 16]
            get = lambda name, z=0: ld(name, m, 16, z)
            if i == 0:
                st("c21", m, res)
            elif i == 1:
                st("m4", m, res)
                P(st, "f21", m)(add(get("c21"), res)) if p == 3 else emit(p, 1, t, m, add(get("c21"), res))
            elif i == 2:
                st("c11", m, sub(get("m4"), res))
                st("m5", m, res)
            elif i == 3:
                st("c22", m, sub(res, get("c21", 1)))
                P(st, "f12", m)(add(get("m5"), res)) if p == 3 else emit(p, 0, t + 4, m, add(get("m5"), res))
            elif i == 4:
                st("d11", m, add(get("c11"), res))
                st("d22", m, add(get("c22"), res))
            elif p < 3:
                emit(p, i - 5, t + 4 * (i - 5), m, add(get(("d11", "d22")[i - 5]), res))
            else:
                t0 = memo.get("tile", 0)
                o32 = once("ob", lambda: window("ob", ((j - 1) * NT + t0) * E, (NT - 2 * last) * E))
                tile = t + 4 * (i - 5)
                o32[pl.ds(tile * E + m, 16), :] = (
                    _pack(add(get("d11"), res), get("f21")) if i == 5
                    else _pack(get("f12"), add(get("d22"), res)))
                if m + 16 == E:
                    ob_copy(j - 1, t0 + tile).start()

        def strassen(p):
            return [(16, P(product, p, t, i, m))
                    for t in range(4) for i in range(7) for m in range(0, E, 16)]

        def qk(r, w):
            par, m = divmod(8 * r, E)
            qv = once(("qv", r), lambda: [ld("q", (par * NT + t) * E + m) for t in range(NT)])
            s = pace(_tree([mul(qv[t], ld("k", (par * NT + t) * KR + WIN + m - w)) for t in range(NT)]))
            s = add(s, pltpu.roll(s, 64, 1))
            s = add(s, pltpu.roll(s, 32, 1))
            if first and m < w:
                keep = m + lax.broadcasted_iota(jnp.int32, (8, 128), 0) >= w
                s = jnp.where(keep, s, -1e9 * DH ** 0.5)
            memo["lg", r, w] = s

        def expo(r):
            lg = [memo["lg", r, w] for w in range(WIN)]
            m = pace(functools.reduce(lax.max, lg))
            scale = np.float32(DH ** -0.5 * np.log2(np.e))
            memo["e", r] = [lax.exp2(mul(sub(s, m), scale)) for s in lg]

        def norm(r):
            memo["inv", r] = 1.0 / pace(_tree(memo["e", r]))

        def probs(r):
            inv = pace(memo["inv", r])
            for w in range(WIN):
                st("p", w * R + 8 * r, mul(memo["e", r][w], inv))

        def qk_list(nr=R // 8):
            out = []
            for i in range(WIN * nr + 26):
                r, w = divmod(i, WIN)
                tasks = [P(qk, r, w)] if r < nr else []
                for f, lag in ((expo, 21), (norm, 23), (probs, 25)):
                    if i >= lag and (i - lag) % WIN == 0 and (i - lag) // WIN < nr:
                        tasks.append(P(f, (i - lag) // WIN))
                out.append((26 if r < nr else 12, P(_run, [(0, f) for f in tasks])))
            return out

        def pv(r, t):
            par, m = divmod(8 * r, E)
            p = once(("pv", r), lambda: [ld("p", w * R + 8 * r) for w in range(WIN)])
            row = (par * NT + t) * KR + WIN + m
            st("o", t * R + 8 * r, pace(_tree([mul(p[w], ld("v", row - w)) for w in range(WIN)])))

        def pv_list():
            return [(16, P(pv, r, t)) for r in range(R // 8) for t in range(NT)]

        def oprep(u, r):
            a = [ld("o", (u + 4 * h) * R + par * E + r, 16, 1) for par in range(2) for h in range(2)]
            for i, val in enumerate(_left(*a[:3], paced(a[3]))):
                st16("os", ((4 * i + u) * E + r) // 2, val)

        def oprep_list():
            return [(18, P(oprep, u, r)) for r in range(0, E, 16) for u in range(4)]

        if last:
            _weave(idft_list(-1, 0, 4, 8, 12), oprep_list())
            oa_copy(2 * j - 1).start()

            def half(i):
                memo["tile"] = 2 * i
                _run(strassen(3)[:224])
            rolled(2, dict(w3=2 * KW, ws3=2 * KW), half)
            return

        if first:
            conv = _split(a3_list(0), 4, 4, 3, 5)
            wait([w_copy(0)])
            rolled(2, dict(w0=128), lambda i: _run(
                perm_list(0, wraw.at[0, pl.ds(pl.multiple_of(i * 256, 256), 256)], (0,))))
            wait([x_copy(0)])
            rolled(4, dict(xs=E // 8), lambda i: _run(
                xprep_list(xa.at[0, pl.ds(pl.multiple_of(i * (R // 4), 16), R // 4)])[:16]))
            wait([w_copy(1)])
            _weave(plain_list(0)[:144], perm_list(1))
            _weave(plain_list(0)[144:], right_list(0)[:48])
            wait(a_copies(0))
            _weave(dft_list(0, "hf", 0, 4), a1_list(0, 0, 8))
            _weave(dft_list(0, "hf", 8, 12) + dft_list(0, "xf", 0), a1_list(0, 8, 16))
            _weave(dft_list(0, "xf", 4, 8, 12), right_list(0)[48:])

            def queries(i):
                w_wait(2 + i)
                _weave(plain_list(1), _merge(perm_list(2, wraw.at[2 + i]), conv[0]))
            rolled(2, dict(w1=NT * KW, xs=2 * E, o=E, q=NT * E, hf=32, xf=32, z=16), queries)
            _run(right_list(1)[:32])
            wait([w_copy(4), w_copy(5)])
            _start(in_copies(1))
            keys = strassen(1)
            _weave(keys[:128], _merge(perm_list(4)[:18], right_list(1)[32:]))
            _weave(keys[128:304], _merge(perm_list(4)[18:32] + perm_list(5), conv[2]))
            _weave(keys[304:], _merge(right_list(2)[:32], conv[3]))
            wait(a_copies(1) + [q_copy(0)])
            _start(in_copies(2) + in_copies(3) + [q_copy(NT - 1)])
            transforms(1, right_list(2)[32:])
            rolled(2, dict(w2=2 * KW, ws2=2 * KW, v=2 * KR, q=NT * E, k=NT * KR, p=E),
                   lambda i: _weave(strassen(2)[:224], qk_list(E // 8)))
            wait(wo_copies())
            rolled(4, dict(w3=2 * KW, p=E // 4, v=E // 4, o=E // 4), lambda i: _run(
                _merge(wo_list(i), pv_list()[:64] + pv_list()[256:320])))
            rolled(4, dict(w3=KW, ws3=KW, hf=32, xf=32, z=16), lambda i: _run(
                _merge(right_list(3)[:16], a3_list(1)[:288])))
            return

        early, late = a3_list(0), _split(a3_list(1), 23, 2, 7)
        head, tail = strassen(0) + strassen(1), strassen(2) + strassen(3)
        transforms(0, xprep_list(xa.at[j]))
        _weave(head[:528], early)
        _run(head[528:536])
        transforms(1, oprep_list())
        _weave(head[536:], late[0])
        _weave(tail[:480], _merge(late[1], qk_list()))
        _run(tail[480:484])
        _weave(tail[484:-6], _merge(late[2], pv_list()))
        _run(tail[-6:])

    def loop(j, carry):
        _wait(in_copies(j))
        step(j)
        return carry

    step(0, first=True)
    lax.fori_loop(1, NS, loop, 0)
    q_copy(NT - 1).wait()
    step(NS, last=True)
    _wait([oa_copy(a) for a in range(NT)] + [ob_copy(j, t) for j in range(NS) for t in range(NT)])


@jax.jit
def pallas_concat_heads__ssm_conv_h3__sliding_local_dilated__prompt_kernel(
    A_q, A_k, A_v, A_shift_k, A_ssm_k, A_ssm_D, B_x, B_wqkv, B_wo,
):
    hbm = pl.BlockSpec(memory_space=pl.ANY)
    out = pl.pallas_call(
        _kernel,
        in_specs=[hbm] * 10,
        out_specs=hbm,
        out_shape=jax.ShapeDtypeStruct((S, 2 * D), BF16),
        scratch_shapes=[
            pltpu.VMEM((NT, 128, S), BF16),
            pltpu.VMEM((NS, R, D), BF16),
            pltpu.VMEM((6, D // 2, D), BF16),
            pltpu.VMEM((NT, D, 128), BF16),
            pltpu.VMEM((NT, 5, 8, 128), F32),
            pltpu.VMEM((4, D), BF16),
            pltpu.VMEM((8, 128), BF16),
            pltpu.VMEM(_TABLE.shape, U32),
            pltpu.SemaphoreType.DMA((5 * NT + 10,)),
            pltpu.SemaphoreType.DMA((2,)),
        ] + [pltpu.VMEM((r * 4 // np.dtype(t).itemsize, 128), t) for t, r in _BUFS.values()],
        compiler_params=pltpu.CompilerParams(vmem_limit_bytes=100 * 1024 * 1024,
                                             disable_bounds_checks=True),
        name="fused",
    )(A_q[0], A_k[0], A_v[0], A_shift_k.T, A_ssm_k,
      A_ssm_D.reshape(8, 128), B_x[0], B_wqkv, B_wo, _TABLE)
    return out[None]
```

```python
import functools

import jax
import jax.numpy as jnp
import numpy as np
from jax import lax
from jax.experimental import pallas as pl
import jax.experimental.pallas.tpu as pltpu


S = 2048
D = 1024
T = 128
NC = S // T
NT = D // 128
NS = 4
R = S // NS
E = R // 2
WIN, DH = 8, 32
PITCH = 33
KR = WIN + E
FP = 2 * T + 16
KW = D // 4

F32, BF16, U32 = jnp.float32, jnp.bfloat16, jnp.uint32
P = functools.partial
add, sub, mul = lax.add, lax.sub, lax.mul


def _pack_rows(m):
    b = m.astype(jnp.bfloat16).view(np.uint16).astype(np.uint32)
    return np.ascontiguousarray(b[0::2] | (b[1::2] << 16))


def _dft_table():
    th = 2.0 * np.pi * (np.arange(T) + 0.25) / T
    ph = th[:, None] * (np.arange(T)[None, :] - (T - 1) / 4)
    fwd = np.concatenate([np.cos(ph), -np.sin(ph)], axis=0)
    rows = np.arange(T // 2).reshape(-1, 8, 2).transpose(0, 2, 1).reshape(-1)
    cols = np.arange(T).reshape(-1, 2, 8).transpose(0, 2, 1).reshape(-1)
    ph = (rows[:, None] + 0.5) * th[cols][None, :]
    return np.concatenate([_pack_rows(m) for m in (fwd, np.cos(ph) / T, np.sin(ph) / T)]
                          + [np.zeros((8, T), np.uint32)], axis=0)


_TABLE = _dft_table()


def _lo(w):
    return pltpu.bitcast(lax.shift_left(w, np.uint32(16)), F32)


def _hi(w):
    return pltpu.bitcast(lax.bitwise_and(w, np.uint32(0xFFFF0000)), F32)


def _pack(lo, hi):
    return pltpu.pack_elementwise([lo, hi], packed_dtype=BF16)


def _tree(xs):
    while len(xs) > 1:
        xs = [add(xs[i], xs[i + 1]) if i + 1 < len(xs) else xs[i] for i in range(0, len(xs), 2)]
    return xs[0]


def _left(a11, a12, a21, a22):
    return [add(a21, a22), a22, add(a11, a12), a11, add(a11, a22), sub(a12, a22), sub(a21, a11)]


def _merge(main, side):
    if not main:
        return side
    total_m = sum(c for c, _ in main)
    total_s = sum(c for c, _ in side)
    done_m, done_s, i, out = 0, 0, 0, []
    for c, f in main:
        out.append((c * total_s, f))
        done_m += c
        while i < len(side) and (done_s + side[i][0]) * total_m <= done_m * total_s:
            done_s += side[i][0]
            out.append((side[i][0] * total_m, side[i][1]))
            i += 1
    assert i == len(side)
    return out


def _run(tasks):
    for _, f in tasks:
        f()


def _weave(main, side):
    _run(_merge(main, side))


def _split(tasks, *weights):
    ends = np.cumsum((0,) + weights) * len(tasks) // sum(weights)
    return [tasks[a:b] for a, b in zip(ends[:-1], ends[1:])]


def _start(copies):
    for c in copies:
        c.start()


def _wait(copies):
    for c in copies:
        c.wait()


_BUFS = {n: (t, r) for t, group in (
    (BF16, dict(qa=NT * S // 2, ka=NT * (S // 2 + 8), va=NT * S // 2, oa=NT * S // 2, ob=S * NT // 2,
                xs=9 * 4 * E // 2, os=7 * 4 * E // 2, w3=2 * NT * KW)),
    (U32, dict(kv0=S // 8, kv1=S // 8, kv2=S // 8, kv3=S // 8, z=NC * T,
               **{f"w{p}": 2 * NT * KW for p in range(3)}, **{f"ws{p}": 20 * KW for p in range(4)},
               t0=32 * PITCH, t1=32 * PITCH)),
    (F32, dict(hf=NC * FP, xf=NC * FP, up=8 * NC, k1=8 * NC, pi=8 * NC, zr=8 * NC, zi=8 * NC,
               even=2 * T, c21=E, m4=E, c11=E, m5=E, c22=E, d11=E, d22=E, f21=E, f12=E,
               q=2 * NT * E, k=2 * NT * KR, v=2 * NT * KR, p=WIN * R, o=NT * R)),
) for n, r in group.items()}


def _kernel(q_hbm, k_hbm, v_hbm, sk_hbm, h_hbm, d_hbm, x_hbm, w_hbm, wo_hbm, tab_hbm, out_hbm,
            ha, xa, wraw, woraw, taps, sk_ref, d_ref, tab, sem_in, sem_out, *raw):
    raw = dict(zip(_BUFS, raw))
    bufs = {n: b.bitcast(U32) if _BUFS[n][0] == BF16 else b for n, b in raw.items()}

    def ld(name, row, n=8, z=0):
        return views[name][z][pl.ds(row, n), :]

    def st(name, row, val):
        views[name][3][pl.ds(row, val.shape[0]), :] = val

    def st16(name, row, val):
        views[name][4][pl.ds(2 * row, val.shape[0]), :] = val.astype(BF16)

    def window(name, row, n):
        return bufs[name].at[pl.ds(pl.multiple_of(row, 8), n), :]

    def window16(name, row, n):
        return raw[name].at[pl.ds(pl.multiple_of(2 * row, 16), 2 * n), :]

    def cols(a):
        return pl.ds(pl.multiple_of(a * 128, 128), 128)

    def rows(j):
        return pl.ds(pl.multiple_of(j * R, R), R)

    def a_copies(a):
        return [
            pltpu.make_async_copy(h_hbm.at[cols(a), :], ha.at[a], sem_in.at[a]),
            pltpu.make_async_copy(k_hbm.at[:, cols(a)], window16("ka", a * (S // 2 + 8) + 8, S // 2),
                                  sem_in.at[NT + a]),
            pltpu.make_async_copy(v_hbm.at[:, cols(a)], window16("va", a * (S // 2), S // 2),
                                  sem_in.at[2 * NT + a]),
        ]

    def q_copy(a):
        return pltpu.make_async_copy(q_hbm.at[:, cols(a)], window16("qa", a * (S // 2), S // 2),
                                     sem_in.at[3 * NT + a])

    def x_copy(j):
        return pltpu.make_async_copy(x_hbm.at[rows(j), :], xa.at[j], sem_in.at[4 * NT + j])

    def in_copies(j):
        return a_copies(2 * j) + [x_copy(j), q_copy(2 * j - 1)] + a_copies(2 * j + 1) + [q_copy(2 * j)]

    def w_copy(n):
        half = pl.ds(n % 2 * (D // 2), D // 2)
        return pltpu.make_async_copy(
            w_hbm.at[half, pl.ds(n // 2 * D, D)], wraw.at[n], sem_in.at[5 * NT + n])

    def w_wait(n):
        pltpu.make_async_copy(wraw.at[n], wraw.at[n], sem_in.at[5 * NT + n]).wait()

    def wo_copies():
        return [pltpu.make_async_copy(wo_hbm.at[:, pl.ds(t * 128, 128)], woraw.at[t],
                                      sem_in.at[5 * NT + 6]) for t in range(NT)]

    def oa_copy(a):
        return pltpu.make_async_copy(window16("oa", a * (S // 2), S // 2), out_hbm.at[:, cols(a)],
                                     sem_out.at[0])

    def ob_copy(j, t):
        return pltpu.make_async_copy(window16("ob", (j * NT + t) * E, E),
                                     out_hbm.at[rows(j), cols(NT + t)], sem_out.at[1])

    small = [pltpu.make_async_copy(a, b, sem_in.at[5 * NT + 7 + i]) for i, (a, b) in enumerate(
        ((tab_hbm, tab), (sk_hbm, sk_ref), (d_hbm, d_ref)))]
    x0 = [pltpu.make_async_copy(x_hbm.at[rows(0), pl.ds(h * D // 2, D // 2)],
                                xa.at[0, :, pl.ds(h * D // 2, D // 2)], sem_in.at[4 * NT + h * NS])
          for h in range(2)]
    startup = lambda: ([w_copy(0), x0[0], w_copy(1)] + a_copies(0) + [x0[1]] + [w_copy(n) for n in (2, 3, 4)]
                       + a_copies(1) + [q_copy(0), w_copy(5)] + wo_copies())
    _start(small + startup())
    _wait(small)
    unit = pltpu.bitcast(tab[pl.ds(3 * T // 2, 8), :], jnp.int32)
    zs = [pl.multiple_of(unit[i, 0] * 8, 8) for i in range(3)]
    views = {n: [b.at[pl.ds(z, _BUFS[n][1]), :] for z in zs] + [b, raw[n]] for n, b in bufs.items()}

    for a in range(NT):
        st("ka", a * (S // 2 + 8), jnp.zeros((8, 128), U32))
    for t in range(2 * NT):
        st("k", t * KR, jnp.zeros((WIN, 128), F32))
    skf = sk_ref[...].astype(F32)
    df = d_ref[...].astype(F32)
    for t in range(NT):
        for i in range(4):
            taps[t, i] = jnp.broadcast_to(skf[i:i + 1, t * 128:(t + 1) * 128], (8, 128))
        taps[t, 4] = jnp.broadcast_to(df[t:t + 1, :], (8, 128))

    def step(j, first=False, last=False):
        memo = {}
        never = tab[pl.ds(3 * T // 2, 8), :] != 0

        def once(key, fn):
            if key not in memo:
                memo[key] = fn()
            return memo[key]

        def fresh():
            memo["fresh"] = memo.get("fresh", 1) + 1
            return pl.multiple_of(zs[0] * memo["fresh"], 8)

        def pace(val):
            clock = memo.get("clock")
            if clock is None:
                return val
            if val.dtype != F32:
                clock = pltpu.bitcast(clock, val.dtype)
            return lax.select(never, clock, val)

        def paced(x):
            return jnp.concatenate([pace(x[:8]), x[8:]], axis=0)

        def wait(copies):
            memo["clock"] = None
            _wait(copies)

        def rolled(n, shifts, body):
            def one(i, carry):
                saved, kept = dict(views), dict(memo)
                memo["clock"] = None
                for name, d in shifts.items():
                    size = _BUFS[name][1] - d * (n - 1)
                    views[name] = [window(name, z + d * i, size) for z in zs + [0]]
                    if _BUFS[name][0] == BF16:
                        views[name].append(window16(name, d * i, size))
                body(i)
                views.update(saved)
                memo.clear()
                memo.update(kept, clock=None)
                return carry
            lax.fori_loop(0, n, one, 0)

        def perm_in(w, u, t):
            tt = paced(pltpu.bitcast(w[pl.ds(u * 256, 256), pl.ds(t * 128, 128)], U32)).T
            for hh in range(4):
                st(f"t{u}", (4 * t + hh) * PITCH, tt[hh * DH:(hh + 1) * DH])

        def perm_out(p, h, u, t):
            g = jnp.concatenate(
                [bufs[f"t{u}"][pl.ds(zs[0] + 4 * t + i, 32, stride=PITCH), :] for i in range(4)], axis=0)
            st(f"w{p}", (h * NT + t) * KW + u * 128, paced(g).T)

        def perm_list(n, w=None, us=(0, 1)):
            w = wraw.at[n] if w is None else w
            return [(1, P(f, u, t)) for f in (P(perm_in, w), P(perm_out, n // 2, n % 2))
                    for u in us for t in range(NT)] + [(2, lambda: None)] * 4

        def wo_in(i, t, hh):
            w = pltpu.bitcast(woraw[2 * i + t, pl.ds(hh * DH, DH), :], U32)
            wt = pltpu.bitcast(paced(w), BF16).astype(F32)
            st(f"t{t % 2}", hh * PITCH, pltpu.bitcast(wt, U32))

        def wo_out(t, i):
            g = bufs[f"t{t % 2}"][pl.ds(zs[0] + i, 32, stride=PITCH), :]
            st16("w3", (i // 16 * NT + t) * KW + i % 16 * 16, pltpu.bitcast(paced(g), F32))

        def wo_list(i):
            return [(1, P(f, t, u)) for f in (P(wo_in, i), wo_out) for t in range(2) for u in range(32)]

        def right(p, t, r):
            b = [ld(f"w{p}", (h * NT + t + 4 * u) * KW + r, 16) for h in range(2) for u in range(2)]
            b[0] = paced(b[0])
            sums = []
            for half in (_lo, _hi):
                b11, b12, b21, b22 = map(half, b)
                sums.append([sub(b21, b11), sub(b12, b22), add(b11, b22), add(b21, b22), add(b11, b12)])
            for i, (lo, hi) in enumerate(zip(*sums)):
                st(f"ws{p}", (4 * i + t) * KW + r, _pack(lo, hi))

        def right_list(p):
            return [(1, P(right, p, t, r)) for t in range(4) for r in range(0, KW, 16)]

        def ld_kv(c, row, n, z=0):
            return ld(f"kv{c // 4}", c % 4 * (T // 2) + row, n, z)

        def a1(i, r):
            a = once(("a", i), lambda: 2 * j + i)
            w0, w1, w2, w3 = once(("taps", i), lambda: [taps[a, u] for u in range(4)])
            k32 = once(("ka", i), lambda: window("ka", a * (S // 2 + 8), S // 2 + 8))
            v32 = once(("va", i), lambda: window("va", a * (S // 2), S // 2))
            c0, c1, c2 = (k32[pl.ds(8 * r + 8 - u, 8), :] for u in range(3))
            vv = v32[pl.ds(8 * r, 8), :]
            e0, o0, e1, o1, o2 = _lo(c0), _hi(c0), _lo(c1), _hi(c1), _hi(c2)
            ke = _tree([mul(e0, w0), mul(o1, w1), mul(e1, w2), mul(o2, w3)])
            ko = _tree([mul(o0, w0), mul(e0, w1), mul(o1, w2), mul(e1, w3)])
            st(f"kv{r // 32}", 8 * (r % 32), pace(_pack(mul(ke, _lo(vv)), mul(ko, _hi(vv)))))

        def a1_list(i, c0, c1):
            return [(24, P(a1, i, r)) for r in range(8 * c0, 8 * c1)]

        def freq(c, im, m):
            return c * FP + im * (T + 8) + m

        def dft(i, name, c0, m):
            def mm():
                f = pltpu.bitcast(tab[pl.ds(fresh(), T), :], BF16)
                if name == "hf":
                    a = once(("a", i), lambda: 2 * j + i)
                    rhs = jnp.concatenate(
                        [ha[a, :, pl.ds(c * T, T)] for c in range(c0, c0 + 4)], axis=0)
                    return lax.dot_general(f, rhs, (((1,), (1,)), ((), ())),
                                           preferred_element_type=F32)
                rhs = jnp.concatenate(
                    [pltpu.bitcast(ld_kv(c, 0, T // 2, i), BF16) for c in range(c0, c0 + 4)], axis=1)
                return jnp.dot(f, rhs, preferred_element_type=F32)
            res = once((name, i, c0), mm)
            for u in range(4):
                st(name, freq(c0 + u, m // T, m % T), res[m:m + 16, u * 128:(u + 1) * 128])
            memo["clock"] = res[m + 8:m + 16, 384:]

        def dft_list(i, name, *c0s):
            return [(16, P(dft, i, name, c0, m)) for c0 in c0s for m in range(0, 2 * T, 16)]

        def a3(i, g, plane, upper, n):
            def opnd(name, c):
                re = lambda: ld(name, freq(c, 0, 8 * g), z=plane)
                im = lambda: ld(name, freq(c, 1, 8 * g), z=plane)
                if name == "xf":
                    val = add(re(), im()) if plane == 0 else re() if plane == 1 else im()
                    return pace(val) if c >= 8 else val
                return pace(re() if plane == 0 else (sub, add)[plane - 1](im(), re()))
            get = lambda name, c: once((name, i, g, plane, c), P(opnd, name, c))
            cs = range(8, n + 1) if upper else range(min(n, 7) + 1)
            terms = [mul(get("xf", n - c), get("hf", c)) for c in cs]
            if upper:
                st("up", 8 * n, pace(_tree(terms)))
                return
            if n >= 8:
                terms.append(ld("up", 8 * n))
            if plane == 0:
                st("k1", 8 * n, pace(_tree(terms)))
            elif plane == 1:
                st("pi", 8 * n, pace(_tree(terms + [ld("k1", 8 * n)])))
            else:
                pr = sub(ld("k1", 8 * n, z=1), _tree(terms))
                pi = ld("pi", 8 * n)
                zr, zi = pr, pi
                if n > 0:
                    qr, qi = memo["prev"]
                    zr, zi = sub(pr, qi), add(pi, qr)
                memo["prev"] = (pr, pi)
                if g % 2 == 0:
                    st("zr", 8 * n, pace(zr))
                    st("zi", 8 * n, zi)
                else:
                    st("z", n * T + 4 * (g - 1), _pack(ld("zr", 8 * n), pace(zr)))
                    st("z", n * T + T // 2 + 4 * (g - 1), _pack(ld("zi", 8 * n), zi))

        def a3_list(i):
            out = []
            for g in range(T // 8):
                for plane in range(3):
                    out += [(2 * (n - 8) + 4, P(a3, i, g, plane, True, n)) for n in range(8, NC)]
                    out += [(2 * min(n, 7) + 4 + 2 * (plane == 2), P(a3, i, g, plane, False, n))
                            for n in range(NC)]
            return out

        def idft(i, c0, odd, m):
            def mm():
                rhs = jnp.concatenate([pltpu.bitcast(ld("z", c * T + odd * T // 2, T // 2, i + 1), BF16)
                                       for c in range(c0, c0 + 4)], axis=1)
                f = tab[pl.ds(fresh() + T + odd * T // 4, T // 4), :]
                return jnp.dot(pltpu.bitcast(f, BF16), rhs, preferred_element_type=F32)
            y = once(("y", i, c0, odd), mm)
            a = once(("a", i), lambda: 2 * j + i)
            dd = once(("dd", i), lambda: taps[a, 4])
            q32 = once(("qa", i), lambda: window("qa", a * (S // 2), S // 2))
            o32 = once(("oa", i), lambda: window("oa", a * (S // 2), S // 2))
            flip = lambda w: jnp.take_along_axis(
                w, 7 - lax.broadcasted_iota(jnp.int32, (8, 128), 0), axis=0, mode="promise_in_bounds")

            def gate(c, row, lo, hi, order):
                kv, qq = order(ld_kv(c, row, 8, 2)), order(q32[pl.ds(c * T // 2 + row, 8), :])
                o32[pl.ds(c * T // 2 + row, 8), :] = order(_pack(
                    mul(_lo(qq), add(lo, mul(_lo(kv), dd))), mul(_hi(qq), add(hi, mul(_hi(kv), dd)))))

            for u in range(4):
                if not odd:
                    st("even", u * T // 2 + m, y[m:m + 16, u * 128:(u + 1) * 128])
                    continue
                s0, s1 = (y[m + h:m + h + 8, u * 128:(u + 1) * 128] for h in (0, 8))
                e0, e1 = (ld("even", u * T // 2 + m + h) for h in (0, 8))
                gate(c0 + u, T // 4 + m // 2, sub(e0, s0), sub(e1, s1), lambda w: w)
                gate(c0 + u, T // 4 - 8 - m // 2, add(e1, s1), add(e0, s0), flip)
            memo["clock"] = y[m + 8:m + 16, 384:]

        def idft_list(i, *c0s):
            return [(16, P(idft, i, c0, odd, m)) for c0 in c0s
                    for odd in range(2) for m in range(0, T // 2, 16)]

        def transforms(i, extra):
            extra = _split(extra, 1, 1, 1, 1, 1, 9)
            for u in range(4):
                _weave(idft_list(i - 1, 4 * u)[:4], extra[u])
                _run(idft_list(i - 1, 4 * u)[4:])
                _weave(dft_list(i, "hf", 4 * u), a1_list(i, 3 * u, 3 * u + 3))
            oa_copy(2 * j + i - 1).start()
            _weave(dft_list(i, "xf", 0), _merge(a1_list(i, 12, 16), extra[4]))
            _weave(dft_list(i, "xf", 4, 8), extra[5])
            _run(dft_list(i, "xf", 12))

        def xprep(x, u, r):
            halves = []
            for m in (r, r + 8):
                a, b = (pltpu.bitcast(x[pl.ds(2 * m, 16), pl.ds(t * 128, 128)], U32)
                        for t in (u, u + 4))
                a = pace(a)
                a11, a12, a21, a22 = _lo(a), _lo(b), _hi(a), _hi(b)
                halves.append(_left(a11, a12, a21, a22) + ([a12, a22] if first else []))
            for i, pair in enumerate(zip(*halves)):
                st16("xs", ((4 * i + u) * E + r) // 2, jnp.concatenate(pair, axis=0))

        def split_rows(i):
            for u in range(4):
                a = pltpu.bitcast(xa[0, pl.ds(pl.multiple_of(i * 128, 16), 128), pl.ds(u * 128, 128)], U32)
                st16("os", u * E // 2, _lo(a))
                st16("os", (4 + u) * E // 2, _hi(a))

        def xprep_list(x):
            return [(27, P(xprep, x, u, r)) for r in range(0, E, 16) for u in range(4)]

        def lhs(name, i):
            view = views[name][3].at[pl.ds(fresh() + i * 2 * E, 2 * E), :]
            return jnp.concatenate(
                [pltpu.bitcast(view[pl.ds(u * E // 2, E // 2), :], BF16) for u in range(4)], axis=1)

        def emit(p, par, t, m, val):
            if p == 0:
                st("q", (par * NT + t) * E + m, val)
                return
            name, row = "kv"[p - 1], (par * NT + t) * KR
            if m == 0 and not first:
                st(name, row, ld(name, row + E, WIN, z=3))
            if m == 0 and first and p == 2 and par == 0:
                for other in range(2):
                    st(name, (other * NT + t) * KR, jnp.broadcast_to(val[0:1], (WIN, 128)))
            st(name, row + WIN + m, val)

        def plain(half, t, m):
            def mm():
                w = pltpu.bitcast(ld("w0", (half * NT + t) * KW, KW, 3), BF16)
                x = lhs("xs", 7) if half else jnp.concatenate([lhs("os", 0), lhs("os", 1)], axis=0)
                return jnp.dot(x, w, preferred_element_type=F32)
            res = once(("plain", half, t), mm)
            memo["clock"] = res[m + 8:m + 16]
            if half:
                emit(0, 0, t, m, add(res[m:m + 16], ld("o", t * R + m, 16)))
            else:
                st("o", t * R + m, res[m:m + 16])

        def plain_list(half):
            return [(16, P(plain, half, t, m)) for t in range(NT) for m in range(0, E if half else R, 16)]

        def product(p, t, i, m):
            def mm():
                if i == 0:
                    w = ld(f"w{p}", t * KW, KW, 3)
                elif i == 2:
                    w = ld(f"w{p}", (NT + t + 4) * KW, KW, 3)
                else:
                    w = ld(f"ws{p}", (4 * (i - 1 - (i > 2)) + t) * KW, KW, 0 if first and t % 2 else 3)
                return jnp.dot(lhs("xs" if p < 3 else "os", i), pltpu.bitcast(w, BF16),
                               preferred_element_type=F32)
            res = once(("product", p, t, i), mm)
            memo["clock"] = res[m + 8:m + 16]
            res = res[m:m + 16]
            get = lambda name, z=0: ld(name, m, 16, z)
            if i == 0:
                st("c21", m, res)
            elif i == 1:
                st("m4", m, res)
                P(st, "f21", m)(add(get("c21"), res)) if p == 3 else emit(p, 1, t, m, add(get("c21"), res))
            elif i == 2:
                st("c11", m, sub(get("m4"), res))
                st("m5", m, res)
            elif i == 3:
                st("c22", m, sub(res, get("c21", 1)))
                P(st, "f12", m)(add(get("m5"), res)) if p == 3 else emit(p, 0, t + 4, m, add(get("m5"), res))
            elif i == 4:
                st("d11", m, add(get("c11"), res))
                st("d22", m, add(get("c22"), res))
            elif p < 3:
                emit(p, i - 5, t + 4 * (i - 5), m, add(get(("d11", "d22")[i - 5]), res))
            else:
                t0 = memo.get("tile", 0)
                o32 = once("ob", lambda: window("ob", ((j - 1) * NT + t0) * E, (NT - 2 * last) * E))
                tile = t + 4 * (i - 5)
                o32[pl.ds(tile * E + m, 16), :] = (
                    _pack(add(get("d11"), res), get("f21")) if i == 5
                    else _pack(get("f12"), add(get("d22"), res)))
                if m + 16 == E:
                    ob_copy(j - 1, t0 + tile).start()

        def strassen(p):
            return [(16, P(product, p, t, i, m))
                    for t in range(4) for i in range(7) for m in range(0, E, 16)]

        def qk(r, w):
            par, m = divmod(8 * r, E)
            qv = once(("qv", r), lambda: [pace(ld("q", (par * NT + t) * E + m)) for t in range(NT)])
            s = pace(_tree([mul(qv[t], ld("k", (par * NT + t) * KR + WIN + m - w)) for t in range(NT)]))
            s = add(s, pltpu.roll(s, 64, 1))
            s = add(s, pltpu.roll(s, 32, 1))
            if first and m < w:
                keep = m + lax.broadcasted_iota(jnp.int32, (8, 128), 0) >= w
                s = jnp.where(keep, s, -1e9 * DH ** 0.5)
            memo["lg", r, w] = s

        def expo(r):
            lg = [memo["lg", r, w] for w in range(WIN)]
            m = pace(functools.reduce(lax.max, lg))
            scale = np.float32(DH ** -0.5 * np.log2(np.e))
            memo["e", r] = [lax.exp2(mul(sub(s, m), scale)) for s in lg]

        def norm(r):
            memo["inv", r] = 1.0 / pace(_tree(memo["e", r]))

        def probs(r):
            inv = pace(memo["inv", r])
            for w in range(WIN):
                st("p", w * R + 8 * r, mul(memo["e", r][w], inv))

        def qk_list(nr=R // 8):
            out = []
            for i in range(WIN * nr + 23):
                r, w = divmod(i, WIN)
                tasks = [P(qk, r, w)] if r < nr else []
                for f, lag in ((expo, 24), (norm, 27), (probs, 30)):
                    if i >= lag and (i - lag) % WIN == 0 and (i - lag) // WIN < nr:
                        tasks.append(P(f, (i - lag) // WIN))
                out.append((26 if r < nr else 12, P(_run, [(0, f) for f in tasks])))
            return out

        def pv(r, t):
            par, m = divmod(8 * r, E)
            p = once(("pv", r), lambda: [pace(ld("p", w * R + 8 * r)) for w in range(WIN)])
            row = (par * NT + t) * KR + WIN + m
            st("o", t * R + 8 * r, pace(_tree([mul(p[w], ld("v", row - w)) for w in range(WIN)])))

        def pv_list():
            return [(16, P(pv, r, t)) for r in range(R // 8) for t in range(NT)]

        def oprep(u, r):
            a = [ld("o", (u + 4 * h) * R + par * E + r, 16, 1) for par in range(2) for h in range(2)]
            for i, val in enumerate(_left(*a[:3], paced(a[3]))):
                st16("os", ((4 * i + u) * E + r) // 2, val)

        def oprep_list():
            return [(18, P(oprep, u, r)) for r in range(0, E, 16) for u in range(4)]

        if last:
            _weave(idft_list(-1, 0, 4, 8, 12), oprep_list())
            oa_copy(2 * j - 1).start()

            def half(i):
                memo["tile"] = 2 * i
                _run(strassen(3)[:224])
            rolled(2, dict(w3=2 * KW, ws3=2 * KW), half)
            return

        if first:
            wait([w_copy(0)])
            rolled(2, dict(w0=128), lambda i: _run(
                perm_list(0, wraw.at[0, pl.ds(pl.multiple_of(i * 256, 256), 256)], (0,))))
            wait([x0[0]])
            rolled(4, dict(os=32), split_rows)
            _run(plain_list(0)[:64])
            wait([w_copy(1)])
            _weave(plain_list(0)[64:208], perm_list(1))
            _weave(plain_list(0)[208:], right_list(0)[:24])
            wait(a_copies(0))
            _weave(dft_list(0, "hf", 0, 4), a1_list(0, 0, 8))
            _weave(dft_list(0, "hf", 8, 12) + dft_list(0, "xf", 0), a1_list(0, 8, 16))
            _weave(dft_list(0, "xf", 4, 8, 12), right_list(0)[24:])
            wait([x0[1]])
            rolled(2, dict(xs=E // 4, hf=16, xf=16, z=8), lambda i: _run(_merge(
                xprep_list(xa.at[0, pl.ds(pl.multiple_of(i * (R // 2), 16), R // 2)])[:32],
                a3_list(0)[:144])))

            def queries(i):
                w_wait(2 + i)
                _weave(plain_list(1), _merge(perm_list(2, wraw.at[2 + i]), a3_list(0)[288:576]))
            rolled(2, dict(w1=NT * KW, xs=2 * E, o=E, q=NT * E, hf=32, xf=32, z=16), queries)
            _run(right_list(1)[:16])
            wait([w_copy(4)])
            _start(in_copies(1))
            keys = strassen(1)
            _weave(keys[:96], _merge(perm_list(4)[:18], right_list(1)[16:48]))
            _weave(keys[96:216], _merge(perm_list(4)[18:], a3_list(0)[864:]))
            _run(keys[216:224])
            wait(a_copies(1) + [q_copy(0)])
            transforms(1, right_list(1)[48:])
            wait([w_copy(5)])
            _start(in_copies(2) + in_copies(3) + [q_copy(NT - 1)])
            _weave(keys[224:360], _merge(perm_list(5), a3_list(1)[864:]))
            _weave(keys[360:], right_list(2))
            rolled(2, dict(w2=2 * KW, ws2=2 * KW, v=2 * KR, q=NT * E, k=NT * KR, p=E),
                   lambda i: _weave(strassen(2)[:224], qk_list(E // 8)))
            wait(wo_copies())
            rolled(4, dict(w3=2 * KW, p=E // 4, v=E // 4, o=E // 4), lambda i: _run(
                _merge(wo_list(i), pv_list()[:64] + pv_list()[256:320])))
            rolled(4, dict(w3=KW, ws3=KW), lambda i: _run(right_list(3)[:16]))
            rolled(6, dict(hf=16, xf=16, z=8), lambda i: _run(a3_list(1)[:144]))
            return

        early, late = a3_list(0), _split(a3_list(1), 3, 1)
        head, tail = strassen(0) + strassen(1), strassen(2) + strassen(3)
        transforms(0, xprep_list(xa.at[j]))
        pre = _split(oprep_list(), 1, 1)
        _weave(head[:520], early)
        _weave(head[520:536], pre[0][:16])
        transforms(1, pre[0][16:])
        _weave(head[536:], pre[1] + late[0])
        _weave(tail[:456], qk_list())
        _run(tail[456:460])
        _weave(tail[460:-6], _merge(late[1], pv_list()))
        _run(tail[-6:])

    def loop(j, carry):
        _wait(in_copies(j))
        step(j)
        return carry

    step(0, first=True)
    lax.fori_loop(1, NS, loop, 0)
    q_copy(NT - 1).wait()
    step(NS, last=True)
    _wait([oa_copy(a) for a in range(NT)] + [ob_copy(j, t) for j in range(NS) for t in range(NT)])


@jax.jit
def pallas_concat_heads__ssm_conv_h3__sliding_local_dilated__prompt_kernel(
    A_q, A_k, A_v, A_shift_k, A_ssm_k, A_ssm_D, B_x, B_wqkv, B_wo,
):
    hbm = pl.BlockSpec(memory_space=pl.ANY)
    out = pl.pallas_call(
        _kernel,
        in_specs=[hbm] * 10,
        out_specs=hbm,
        out_shape=jax.ShapeDtypeStruct((S, 2 * D), BF16),
        scratch_shapes=[
            pltpu.VMEM((NT, 128, S), BF16),
            pltpu.VMEM((NS, R, D), BF16),
            pltpu.VMEM((6, D // 2, D), BF16),
            pltpu.VMEM((NT, D, 128), BF16),
            pltpu.VMEM((NT, 5, 8, 128), F32),
            pltpu.VMEM((4, D), BF16),
            pltpu.VMEM((8, 128), BF16),
            pltpu.VMEM(_TABLE.shape, U32),
            pltpu.SemaphoreType.DMA((5 * NT + 10,)),
            pltpu.SemaphoreType.DMA((2,)),
        ] + [pltpu.VMEM((r * 4 // np.dtype(t).itemsize, 128), t) for t, r in _BUFS.values()],
        compiler_params=pltpu.CompilerParams(vmem_limit_bytes=100 * 1024 * 1024,
                                             disable_bounds_checks=True),
        name="fused",
    )(A_q[0], A_k[0], A_v[0], A_shift_k.T, A_ssm_k,
      A_ssm_D.reshape(8, 128), B_x[0], B_wqkv, B_wo, _TABLE)
    return out[None]
```

```python
import functools

import jax
import jax.numpy as jnp
import numpy as np
from jax import lax
from jax.experimental import pallas as pl
import jax.experimental.pallas.tpu as pltpu


S = 2048
D = 1024
T = 128
NC = S // T
NT = D // 128
NS = 4
R = S // NS
E = R // 2
WIN, DH = 8, 32
PITCH = 33
KR = WIN + E
FP = 2 * T + 16
KW = D // 4

F32, BF16, U32 = jnp.float32, jnp.bfloat16, jnp.uint32
P = functools.partial
add, sub, mul = lax.add, lax.sub, lax.mul


def _pack_rows(m):
    b = m.astype(jnp.bfloat16).view(np.uint16).astype(np.uint32)
    return np.ascontiguousarray(b[0::2] | (b[1::2] << 16))


def _dft_table():
    th = 2.0 * np.pi * (np.arange(T) + 0.25) / T
    ph = th[:, None] * (np.arange(T)[None, :] - (T - 1) / 4)
    fwd = np.concatenate([np.cos(ph), -np.sin(ph)], axis=0)
    rows = np.arange(T // 2).reshape(-1, 8, 2).transpose(0, 2, 1).reshape(-1)
    cols = np.arange(T).reshape(-1, 2, 8).transpose(0, 2, 1).reshape(-1)
    ph = (rows[:, None] + 0.5) * th[cols][None, :]
    return np.concatenate([_pack_rows(m) for m in (fwd, np.cos(ph) / T, np.sin(ph) / T)]
                          + [np.zeros((8, T), np.uint32)], axis=0)


_TABLE = _dft_table()


def _lo(w):
    return pltpu.bitcast(lax.shift_left(w, np.uint32(16)), F32)


def _hi(w):
    return pltpu.bitcast(lax.bitwise_and(w, np.uint32(0xFFFF0000)), F32)


def _pack(lo, hi):
    return pltpu.pack_elementwise([lo, hi], packed_dtype=BF16)


def _tree(xs):
    while len(xs) > 1:
        xs = [add(xs[i], xs[i + 1]) if i + 1 < len(xs) else xs[i] for i in range(0, len(xs), 2)]
    return xs[0]


def _left(a11, a12, a21, a22):
    return [add(a21, a22), a22, add(a11, a12), a11, add(a11, a22), sub(a12, a22), sub(a21, a11)]


def _merge(main, side):
    if not main:
        return side
    total_m = sum(c for c, _ in main)
    total_s = sum(c for c, _ in side)
    done_m, done_s, i, out = 0, 0, 0, []
    for c, f in main:
        out.append((c * total_s, f))
        done_m += c
        while i < len(side) and (done_s + side[i][0]) * total_m <= done_m * total_s:
            done_s += side[i][0]
            out.append((side[i][0] * total_m, side[i][1]))
            i += 1
    assert i == len(side)
    return out


def _run(tasks):
    for _, f in tasks:
        f()


def _weave(main, side):
    _run(_merge(main, side))


def _split(tasks, *weights):
    ends = np.cumsum((0,) + weights) * len(tasks) // sum(weights)
    return [tasks[a:b] for a, b in zip(ends[:-1], ends[1:])]


def _start(copies):
    for c in copies:
        c.start()


def _wait(copies):
    for c in copies:
        c.wait()


_BUFS = {n: (t, r) for t, group in (
    (BF16, dict(qa=NT * S // 2, ka=NT * (S // 2 + 8), va=NT * S // 2, oa=NT * S // 2, ob=S * NT // 2,
                xs=9 * 4 * E // 2, os=7 * 4 * E // 2, w3=2 * NT * KW)),
    (U32, dict(kv0=S // 8, kv1=S // 8, kv2=S // 8, kv3=S // 8, z=NC * T,
               **{f"w{p}": 2 * NT * KW for p in range(3)}, **{f"ws{p}": 20 * KW for p in range(4)},
               t0=32 * PITCH, t1=32 * PITCH)),
    (F32, dict(hf=NC * FP, xf=NC * FP, up=8 * NC, k1=8 * NC, pi=8 * NC, zr=8 * NC, zi=8 * NC,
               even=2 * T, c21=E, m4=E, c11=E, m5=E, c22=E, d11=E, d22=E, f21=E, f12=E,
               q=2 * NT * E, k=2 * NT * KR, v=2 * NT * KR, p=WIN * R, o=NT * R)),
) for n, r in group.items()}


def _kernel(q_hbm, k_hbm, v_hbm, sk_hbm, h_hbm, d_hbm, x_hbm, w_hbm, wo_hbm, tab_hbm, out_hbm,
            ha, xa, wraw, woraw, taps, sk_ref, d_ref, tab, sem_in, sem_out, *raw):
    raw = dict(zip(_BUFS, raw))
    bufs = {n: b.bitcast(U32) if _BUFS[n][0] == BF16 else b for n, b in raw.items()}

    def ld(name, row, n=8, z=0):
        return views[name][z][pl.ds(row, n), :]

    def st(name, row, val):
        views[name][3][pl.ds(row, val.shape[0]), :] = val

    def st16(name, row, val):
        views[name][4][pl.ds(2 * row, val.shape[0]), :] = val.astype(BF16)

    def window(name, row, n):
        return bufs[name].at[pl.ds(pl.multiple_of(row, 8), n), :]

    def window16(name, row, n):
        return raw[name].at[pl.ds(pl.multiple_of(2 * row, 16), 2 * n), :]

    def cols(a):
        return pl.ds(pl.multiple_of(a * 128, 128), 128)

    def rows(j):
        return pl.ds(pl.multiple_of(j * R, R), R)

    def a_copies(a):
        return [
            pltpu.make_async_copy(h_hbm.at[cols(a), :], ha.at[a], sem_in.at[a]),
            pltpu.make_async_copy(k_hbm.at[:, cols(a)], window16("ka", a * (S // 2 + 8) + 8, S // 2),
                                  sem_in.at[NT + a]),
            pltpu.make_async_copy(v_hbm.at[:, cols(a)], window16("va", a * (S // 2), S // 2),
                                  sem_in.at[2 * NT + a]),
        ]

    def q_copy(a):
        return pltpu.make_async_copy(q_hbm.at[:, cols(a)], window16("qa", a * (S // 2), S // 2),
                                     sem_in.at[3 * NT + a])

    def x_copy(j):
        return pltpu.make_async_copy(x_hbm.at[rows(j), :], xa.at[j], sem_in.at[4 * NT + j])

    def in_copies(j):
        return a_copies(2 * j - 1) + [q_copy(2 * j - 2), x_copy(j)] + a_copies(2 * j) + [q_copy(2 * j - 1)]

    def w_copy(n):
        half = pl.ds(n % 2 * (D // 2), D // 2)
        return pltpu.make_async_copy(
            w_hbm.at[half, pl.ds(n // 2 * D, D)], wraw.at[n], sem_in.at[5 * NT + n])

    def w_wait(n):
        pltpu.make_async_copy(wraw.at[n], wraw.at[n], sem_in.at[5 * NT + n]).wait()

    def wo_copies():
        return [pltpu.make_async_copy(wo_hbm.at[:, pl.ds(t * 128, 128)], woraw.at[t],
                                      sem_in.at[5 * NT + 6]) for t in range(NT)]

    def oa_copy(a):
        return pltpu.make_async_copy(window16("oa", a * (S // 2), S // 2), out_hbm.at[:, cols(a)],
                                     sem_out.at[0])

    def oa_part(u):
        src = window16("oa", (4 * (NT - 1) + u) * S // 8, S // 8)
        return pltpu.make_async_copy(src, out_hbm.at[pl.ds(u * S // 4, S // 4), cols(NT - 1)],
                                     sem_out.at[0])

    def ob_copy(j, t):
        return pltpu.make_async_copy(window16("ob", (j * NT + t) * E, E),
                                     out_hbm.at[rows(j), cols(NT + t)], sem_out.at[1])

    small = [pltpu.make_async_copy(a, b, sem_in.at[5 * NT + 7 + i]) for i, (a, b) in enumerate(
        ((tab_hbm, tab), (sk_hbm, sk_ref), (d_hbm, d_ref)))]
    x0 = [pltpu.make_async_copy(x_hbm.at[rows(0), pl.ds(h * D // 2, D // 2)],
                                xa.at[0, :, pl.ds(h * D // 2, D // 2)], sem_in.at[4 * NT + h * NS])
          for h in range(2)]
    w00 = [pltpu.make_async_copy(w_hbm.at[pl.ds(u * KW, KW), pl.ds(0, D)], wraw.at[0, pl.ds(u * KW, KW)],
                                 sem_in.at[4 * NT + NS + 1 + u]) for u in range(2)]
    startup = lambda: (w00 + [x0[0], w_copy(1)] + a_copies(0) + [x0[1]] + [w_copy(n) for n in (2, 3, 4, 5)]
                       + wo_copies())
    _start(small + startup())
    _wait(small)
    unit = pltpu.bitcast(tab[pl.ds(3 * T // 2, 8), :], jnp.int32)
    zs = [pl.multiple_of(unit[i, 0] * 8, 8) for i in range(3)]
    views = {n: [b.at[pl.ds(z, _BUFS[n][1]), :] for z in zs] + [b, raw[n]] for n, b in bufs.items()}

    for a in range(NT):
        st("ka", a * (S // 2 + 8), jnp.zeros((8, 128), U32))
    for t in range(2 * NT):
        st("k", t * KR, jnp.zeros((WIN, 128), F32))
    skf = sk_ref[...].astype(F32)
    df = d_ref[...].astype(F32)
    for t in range(NT):
        for i in range(4):
            taps[t, i] = jnp.broadcast_to(skf[i:i + 1, t * 128:(t + 1) * 128], (8, 128))
        taps[t, 4] = jnp.broadcast_to(df[t:t + 1, :], (8, 128))

    def step(j, first=False, last=False):
        memo = {}
        never = tab[pl.ds(3 * T // 2, 8), :] != 0

        def once(key, fn):
            if key not in memo:
                memo[key] = fn()
            return memo[key]

        def fresh():
            memo["fresh"] = memo.get("fresh", 1) + 1
            return pl.multiple_of(zs[0] * memo["fresh"], 8)

        def pace(val):
            clock = memo.get("clock")
            if clock is None:
                return val
            if val.dtype != F32:
                clock = pltpu.bitcast(clock, val.dtype)
            return lax.select(never, clock, val)

        def paced(x):
            return jnp.concatenate([pace(x[:8]), x[8:]], axis=0)

        def wait(copies):
            memo["clock"] = None
            _wait(copies)

        def rolled(n, shifts, body):
            def one(i, carry):
                saved, kept = dict(views), dict(memo)
                memo["clock"] = None
                for name, d in shifts.items():
                    size = _BUFS[name][1] - d * (n - 1)
                    views[name] = [window(name, z + d * i, size) for z in zs + [0]]
                    if _BUFS[name][0] == BF16:
                        views[name].append(window16(name, d * i, size))
                body(i)
                views.update(saved)
                memo.clear()
                memo.update(kept, clock=None)
                return carry
            lax.fori_loop(0, n, one, 0)

        def perm_in(w, u, t):
            tt = paced(pltpu.bitcast(w[pl.ds(u * 256, 256), pl.ds(t * 128, 128)], U32)).T
            for hh in range(4):
                st(f"t{u}", (4 * t + hh) * PITCH, tt[hh * DH:(hh + 1) * DH])

        def perm_out(p, h, u, t):
            g = jnp.concatenate(
                [bufs[f"t{u}"][pl.ds(zs[0] + 4 * t + i, 32, stride=PITCH), :] for i in range(4)], axis=0)
            st(f"w{p}", (h * NT + t) * KW + u * 128, paced(g).T)

        def perm_list(n, w=None, us=(0, 1)):
            w = wraw.at[n] if w is None else w
            return [(1, P(f, u, t)) for f in (P(perm_in, w), P(perm_out, n // 2, n % 2))
                    for u in us for t in range(NT)] + [(2, lambda: None)] * 4

        def wo_in(i, t0, t, hh):
            w = pltpu.bitcast(woraw[2 * i + t - t0, pl.ds(hh * DH, DH), :], U32)
            wt = pltpu.bitcast(paced(w), BF16).astype(F32)
            st(f"t{t % 2}", hh * PITCH, pltpu.bitcast(wt, U32))

        def wo_out(t, i):
            g = bufs[f"t{t % 2}"][pl.ds(zs[0] + i, 32, stride=PITCH), :]
            st16("w3", (i // 16 * NT + t) * KW + i % 16 * 16, pltpu.bitcast(paced(g), F32))

        def wo_list(i, t0=0):
            return [(1, P(f, t, u)) for f in (P(wo_in, i, t0), wo_out)
                    for t in (t0, t0 + 1) for u in range(32)]

        def right(p, t, r):
            b = [ld(f"w{p}", (h * NT + t + 4 * u) * KW + r, 16) for h in range(2) for u in range(2)]
            b[0] = paced(b[0])
            sums = []
            for half in (_lo, _hi):
                b11, b12, b21, b22 = map(half, b)
                sums.append([sub(b21, b11), sub(b12, b22), add(b11, b22), add(b21, b22), add(b11, b12)])
            for i, (lo, hi) in enumerate(zip(*sums)):
                st(f"ws{p}", (4 * i + t) * KW + r, _pack(lo, hi))

        def right_list(p):
            return [(1, P(right, p, t, r)) for t in range(4) for r in range(0, KW, 16)]

        def ld_kv(c, row, n, z=0):
            return ld(f"kv{c // 4}", c % 4 * (T // 2) + row, n, z)

        def a1(i, r):
            a = once(("a", i), lambda: 2 * j + i)
            w0, w1, w2, w3 = once(("taps", i), lambda: [taps[a, u] for u in range(4)])
            k32 = once(("ka", i), lambda: window("ka", a * (S // 2 + 8), S // 2 + 8))
            v32 = once(("va", i), lambda: window("va", a * (S // 2), S // 2))
            c0, c1, c2 = (k32[pl.ds(8 * r + 8 - u, 8), :] for u in range(3))
            vv = v32[pl.ds(8 * r, 8), :]
            e0, o0, e1, o1, o2 = _lo(c0), _hi(c0), _lo(c1), _hi(c1), _hi(c2)
            ke = _tree([mul(e0, w0), mul(o1, w1), mul(e1, w2), mul(o2, w3)])
            ko = _tree([mul(o0, w0), mul(e0, w1), mul(o1, w2), mul(e1, w3)])
            st(f"kv{r // 32}", 8 * (r % 32), pace(_pack(mul(ke, _lo(vv)), mul(ko, _hi(vv)))))

        def a1_list(i, c0, c1):
            return [(24, P(a1, i, r)) for r in range(8 * c0, 8 * c1)]

        def freq(c, im, m):
            return c * FP + im * (T + 8) + m

        def dft(i, name, c0, m):
            def mm():
                f = pltpu.bitcast(tab[pl.ds(fresh(), T), :], BF16)
                if name == "hf":
                    a = once(("a", i), lambda: 2 * j + i)
                    rhs = jnp.concatenate(
                        [ha[a, :, pl.ds(c * T, T)] for c in range(c0, c0 + 4)], axis=0)
                    return lax.dot_general(f, rhs, (((1,), (1,)), ((), ())),
                                           preferred_element_type=F32)
                rhs = jnp.concatenate(
                    [pltpu.bitcast(ld_kv(c, 0, T // 2, i % 2), BF16) for c in range(c0, c0 + 4)], axis=1)
                return jnp.dot(f, rhs, preferred_element_type=F32)
            res = once((name, i, c0), mm)
            for u in range(4):
                st(name, freq(c0 + u, m // T, m % T), res[m:m + 16, u * 128:(u + 1) * 128])
            memo["clock"] = res[m + 8:m + 16, 384:]

        def dft_list(i, name, *c0s):
            return [(16, P(dft, i, name, c0, m)) for c0 in c0s for m in range(0, 2 * T, 16)]

        def a3(i, g, plane, upper, n):
            def opnd(name, c):
                re = lambda: ld(name, freq(c, 0, 8 * g), z=plane)
                im = lambda: ld(name, freq(c, 1, 8 * g), z=plane)
                if name == "xf":
                    val = add(re(), im()) if plane == 0 else re() if plane == 1 else im()
                    return pace(val) if c >= 8 else val
                return pace(re() if plane == 0 else (sub, add)[plane - 1](im(), re()))
            get = lambda name, c: once((name, i, g, plane, c), P(opnd, name, c))
            cs = range(8, n + 1) if upper else range(min(n, 7) + 1)
            terms = [mul(get("xf", n - c), get("hf", c)) for c in cs]
            if upper:
                st("up", 8 * n, pace(_tree(terms)))
                return
            if n >= 8:
                terms.append(ld("up", 8 * n))
            if plane == 0:
                st("k1", 8 * n, pace(_tree(terms)))
            elif plane == 1:
                st("pi", 8 * n, pace(_tree(terms + [ld("k1", 8 * n)])))
            else:
                pr = sub(ld("k1", 8 * n, z=1), _tree(terms))
                pi = ld("pi", 8 * n)
                zr, zi = pr, pi
                if n > 0:
                    qr, qi = memo["prev"]
                    zr, zi = sub(pr, qi), add(pi, qr)
                memo["prev"] = (pr, pi)
                if g % 2 == 0:
                    st("zr", 8 * n, pace(zr))
                    st("zi", 8 * n, zi)
                else:
                    st("z", n * T + 4 * (g - 1), _pack(ld("zr", 8 * n), pace(zr)))
                    st("z", n * T + T // 2 + 4 * (g - 1), _pack(ld("zi", 8 * n), zi))

        def a3_list(i):
            out = []
            for g in range(T // 8):
                for plane in range(3):
                    out += [(2 * (n - 8) + 4, P(a3, i, g, plane, True, n)) for n in range(8, NC)]
                    out += [(2 * min(n, 7) + 4 + 2 * (plane == 2), P(a3, i, g, plane, False, n))
                            for n in range(NC)]
            return out

        def idft(i, c0, odd, m):
            def mm():
                rhs = jnp.concatenate([pltpu.bitcast(ld("z", c * T + odd * T // 2, T // 2, i + 2), BF16)
                                       for c in range(c0, c0 + 4)], axis=1)
                f = tab[pl.ds(fresh() + T + odd * T // 4, T // 4), :]
                return jnp.dot(pltpu.bitcast(f, BF16), rhs, preferred_element_type=F32)
            y = once(("y", i, c0, odd), mm)
            a = once(("a", i), lambda: 2 * j + i)
            dd = once(("dd", i), lambda: taps[a, 4])
            q32 = once(("qa", i), lambda: window("qa", a * (S // 2), S // 2))
            o32 = once(("oa", i), lambda: window("oa", a * (S // 2), S // 2))
            flip = lambda w: jnp.take_along_axis(
                w, 7 - lax.broadcasted_iota(jnp.int32, (8, 128), 0), axis=0, mode="promise_in_bounds")

            def gate(c, row, lo, hi, order):
                kv, qq = order(ld_kv(c, row, 8, 2)), order(q32[pl.ds(c * T // 2 + row, 8), :])
                o32[pl.ds(c * T // 2 + row, 8), :] = order(_pack(
                    mul(_lo(qq), add(lo, mul(_lo(kv), dd))), mul(_hi(qq), add(hi, mul(_hi(kv), dd)))))

            for u in range(4):
                if not odd:
                    st("even", u * T // 2 + m, y[m:m + 16, u * 128:(u + 1) * 128])
                    continue
                s0, s1 = (y[m + h:m + h + 8, u * 128:(u + 1) * 128] for h in (0, 8))
                e0, e1 = (ld("even", u * T // 2 + m + h) for h in (0, 8))
                gate(c0 + u, T // 4 + m // 2, sub(e0, s0), sub(e1, s1), lambda w: w)
                gate(c0 + u, T // 4 - 8 - m // 2, add(e1, s1), add(e0, s0), flip)
            memo["clock"] = y[m + 8:m + 16, 384:]

        def idft_list(i, *c0s):
            return [(16, P(idft, i, c0, odd, m)) for c0 in c0s
                    for odd in range(2) for m in range(0, T // 2, 16)]

        def transforms(i, extra, shares=(1, 1, 1, 1, 1, 9)):
            extra = _split(extra, *shares)
            for u in range(4):
                _weave(idft_list(i - 1, 4 * u)[:4], extra[u])
                _run(idft_list(i - 1, 4 * u)[4:])
                _weave(dft_list(i, "hf", 4 * u), a1_list(i, 3 * u, 3 * u + 3))
            oa_copy(2 * j + i - 1).start()
            _weave(dft_list(i, "xf", 0), _merge(a1_list(i, 12, 16), extra[4]))
            _weave(dft_list(i, "xf", 4, 8), extra[5])
            _run(dft_list(i, "xf", 12))

        def xprep(x, u, r):
            halves = []
            for m in (r, r + 8):
                a, b = (pltpu.bitcast(x[pl.ds(2 * m, 16), pl.ds(t * 128, 128)], U32)
                        for t in (u, u + 4))
                a = pace(a)
                a11, a12, a21, a22 = _lo(a), _lo(b), _hi(a), _hi(b)
                halves.append(_left(a11, a12, a21, a22) + ([a12, a22] if first else []))
            for i, pair in enumerate(zip(*halves)):
                st16("xs", ((4 * i + u) * E + r) // 2, jnp.concatenate(pair, axis=0))

        def split_rows(i):
            for u in range(4):
                a = pltpu.bitcast(xa[0, pl.ds(pl.multiple_of(i * 128, 16), 128), pl.ds(u * 128, 128)], U32)
                st16("os", u * E // 2, _lo(a))
                st16("os", (4 + u) * E // 2, _hi(a))

        def xprep_list(x):
            return [(27, P(xprep, x, u, r)) for r in range(0, E, 16) for u in range(4)]

        def lhs(name, i):
            view = views[name][3].at[pl.ds(fresh() + i * 2 * E, 2 * E), :]
            return jnp.concatenate(
                [pltpu.bitcast(view[pl.ds(u * E // 2, E // 2), :], BF16) for u in range(4)], axis=1)

        def emit(p, par, t, m, val):
            if p == 0:
                st("q", (par * NT + t) * E + m, val)
                return
            name, row = "kv"[p - 1], (par * NT + t) * KR
            if m == 0 and not first:
                st(name, row, ld(name, row + E, WIN, z=3))
            if m == 0 and first and p == 2 and par == 0:
                for other in range(2):
                    st(name, (other * NT + t) * KR, jnp.broadcast_to(val[0:1], (WIN, 128)))
            st(name, row + WIN + m, val)

        def plain(half, t, m):
            def mm():
                w = pltpu.bitcast(ld("w0", (half * NT + t) * KW, KW, 3), BF16)
                x = lhs("xs", 7) if half else jnp.concatenate([lhs("os", 0), lhs("os", 1)], axis=0)
                return jnp.dot(x, w, preferred_element_type=F32)
            res = once(("plain", half, t), mm)
            memo["clock"] = res[m + 8:m + 16]
            if half:
                emit(0, 0, t, m, add(res[m:m + 16], ld("o", t * R + m, 16)))
            else:
                st("o", t * R + m, res[m:m + 16])

        def plain_list(half):
            return [(16, P(plain, half, t, m)) for t in range(NT) for m in range(0, E if half else R, 16)]

        def product(p, t, i, m):
            def mm():
                if i == 0:
                    w = ld(f"w{p}", t * KW, KW, 3)
                elif i == 2:
                    w = ld(f"w{p}", (NT + t + 4) * KW, KW, 3)
                else:
                    w = ld(f"ws{p}", (4 * (i - 1 - (i > 2)) + t) * KW, KW, 3)
                return jnp.dot(lhs("xs" if p < 3 else "os", i), pltpu.bitcast(w, BF16),
                               preferred_element_type=F32)
            res = once(("product", p, t, i), mm)
            memo["clock"] = res[m + 8:m + 16]
            res = res[m:m + 16]
            get = lambda name, z=0: ld(name, m, 16, z)
            if i == 0:
                st("c21", m, res)
            elif i == 1:
                st("m4", m, res)
                P(st, "f21", m)(add(get("c21"), res)) if p == 3 else emit(p, 1, t, m, add(get("c21"), res))
            elif i == 2:
                st("c11", m, sub(get("m4"), res))
                st("m5", m, res)
            elif i == 3:
                st("c22", m, sub(res, get("c21", 1)))
                P(st, "f12", m)(add(get("m5"), res)) if p == 3 else emit(p, 0, t + 4, m, add(get("m5"), res))
            elif i == 4:
                st("d11", m, add(get("c11"), res))
                st("d22", m, add(get("c22"), res))
            elif p < 3:
                emit(p, i - 5, t + 4 * (i - 5), m, add(get(("d11", "d22")[i - 5]), res))
            else:
                t0 = memo.get("tile", 0)
                o32 = once("ob", lambda: window("ob", ((j - 1) * NT + t0) * E, (NT - 2 * last) * E))
                tile = t + 4 * (i - 5)
                o32[pl.ds(tile * E + m, 16), :] = (
                    _pack(add(get("d11"), res), get("f21")) if i == 5
                    else _pack(get("f12"), add(get("d22"), res)))
                if m + 16 == E:
                    ob_copy(j - 1, t0 + tile).start()

        def strassen(p):
            return [(16, P(product, p, t, i, m))
                    for t in range(4) for i in range(7) for m in range(0, E, 16)]

        def qk(r, w):
            par, m = divmod(8 * r, E)
            qv = once(("qv", r), lambda: [pace(ld("q", (par * NT + t) * E + m)) for t in range(NT)])
            s = pace(_tree([mul(qv[t], ld("k", (par * NT + t) * KR + WIN + m - w)) for t in range(NT)]))
            s = add(s, pltpu.roll(s, 64, 1))
            s = add(s, pltpu.roll(s, 32, 1))
            if first and m < w:
                keep = m + lax.broadcasted_iota(jnp.int32, (8, 128), 0) >= w
                s = jnp.where(keep, s, -1e9 * DH ** 0.5)
            memo["lg", r, w] = s

        def expo(r):
            lg = [memo["lg", r, w] for w in range(WIN)]
            m = pace(functools.reduce(lax.max, lg))
            scale = np.float32(DH ** -0.5 * np.log2(np.e))
            memo["e", r] = [lax.exp2(mul(sub(s, m), scale)) for s in lg]

        def norm(r):
            memo["inv", r] = 1.0 / pace(_tree(memo["e", r]))

        def probs(r):
            inv = pace(memo["inv", r])
            for w in range(WIN):
                st("p", w * R + 8 * r, mul(memo["e", r][w], inv))

        def qk_list(nr=R // 8):
            out = []
            for i in range(WIN * nr + 23):
                r, w = divmod(i, WIN)
                tasks = [P(qk, r, w)] if r < nr else []
                for f, lag in ((expo, 24), (norm, 27), (probs, 30)):
                    if i >= lag and (i - lag) % WIN == 0 and (i - lag) // WIN < nr:
                        tasks.append(P(f, (i - lag) // WIN))
                out.append((26 if r < nr else 12, P(_run, [(0, f) for f in tasks])))
            return out

        def pv(r, t):
            par, m = divmod(8 * r, E)
            p = once(("pv", r), lambda: [pace(ld("p", w * R + 8 * r)) for w in range(WIN)])
            row = (par * NT + t) * KR + WIN + m
            st("o", t * R + 8 * r, pace(_tree([mul(p[w], ld("v", row - w)) for w in range(WIN)])))

        def pv_list():
            return [(16, P(pv, r, t)) for r in range(R // 8) for t in range(NT)]

        def oprep(u, r):
            a = [ld("o", (u + 4 * h) * R + par * E + r, 16, 1) for par in range(2) for h in range(2)]
            for i, val in enumerate(_left(*a[:3], paced(a[3]))):
                st16("os", ((4 * i + u) * E + r) // 2, val)

        def oprep_list():
            return [(18, P(oprep, u, r)) for r in range(0, E, 16) for u in range(4)]

        if last:
            mix = []
            for r in range(E // 16):
                mix += pv_list()[16 * r:16 * r + 16] + pv_list()[E + 16 * r:E + 16 * r + 16]
                mix += oprep_list()[4 * r:4 * r + 4]
            transforms(-1, mix, (1, 1, 1, 1, 1, 10))

            def half(i):
                memo["tile"] = 2 * i
                _weave(strassen(3)[:224], a3_list(-1)[:576])
            rolled(2, dict(w3=2 * KW, ws3=2 * KW, hf=64, xf=64, z=32), half)
            for u in range(4):
                _run(idft_list(-1, 4 * u))
                oa_part(u).start()
            return

        if first:
            def leading(i):
                w = wraw.at[0, pl.ds(pl.multiple_of(i * KW, KW), KW)]
                pltpu.make_async_copy(w, w, sem_in.at[4 * NT + NS + 1 + i]).wait()
                _run(perm_list(0, w, (0,)))
            rolled(2, dict(w0=128), leading)
            wait([x0[0]])
            rolled(4, dict(os=32), split_rows)
            _run(plain_list(0)[:96])
            wait([w_copy(1)])
            _weave(plain_list(0)[96:240], perm_list(1))
            _weave(plain_list(0)[240:], right_list(0)[:8])
            wait(a_copies(0))
            _weave(dft_list(0, "hf", 0, 4), a1_list(0, 0, 8))
            _weave(dft_list(0, "hf", 8, 12) + dft_list(0, "xf", 0), a1_list(0, 8, 16))
            _weave(dft_list(0, "xf", 4, 8, 12), right_list(0)[8:32])
            wait([x0[1]])
            rolled(2, dict(xs=E // 4, hf=16, xf=16, z=8, w0=KW, ws0=KW), lambda i: _run(_merge(
                xprep_list(xa.at[0, pl.ds(pl.multiple_of(i * (R // 2), 16), R // 2)])[:32],
                a3_list(0)[:144] + right_list(0)[32:48])))

            def queries(i):
                w_wait(2 + i)
                _weave(plain_list(1), _merge(perm_list(2, wraw.at[2 + i]), a3_list(0)[288:576]))
            rolled(2, dict(w1=NT * KW, xs=2 * E, o=E, q=NT * E, hf=32, xf=32, z=16), queries)
            _run(right_list(1)[:32])
            wait([w_copy(4), w_copy(5)])
            _start(in_copies(1))
            keys, conv = strassen(1), _split(a3_list(0)[864:], 1, 3)
            _weave(keys[:128], _merge(perm_list(4), right_list(1)[32:] + conv[0]))
            _weave(keys[128:272], _merge(perm_list(5), conv[1]))
            _weave(keys[272:336], right_list(2)[:32])
            wait(wo_copies())
            _start(in_copies(2) + in_copies(3) + a_copies(NT - 1) + [q_copy(NT - 2), q_copy(NT - 1)])
            _weave(keys[336:], right_list(2)[32:] + wo_list(0))
            rolled(3, dict(w3=2 * KW), lambda i: _run(wo_list(i + 1, 2)))
            rolled(2, dict(w2=2 * KW, ws2=2 * KW, w3=2 * KW, ws3=2 * KW, v=2 * KR, q=NT * E, k=NT * KR, p=E),
                   lambda i: _weave(strassen(2)[:224], _merge(right_list(3)[:32], qk_list(E // 8))))
            return

        head = strassen(0) + strassen(1)
        pre = _split(oprep_list(), 3, 1)
        transforms(-1, xprep_list(xa.at[j]))
        _weave(head[:528], a3_list(-1))
        _weave(head[528:812], pv_list())
        _run(head[812:818])
        transforms(0, pre[0])
        _weave(head[818:] + strassen(3), pre[1] + a3_list(0))
        _weave(strassen(2), qk_list())

    def loop(j, carry):
        _wait(in_copies(j))
        step(j)
        return carry

    step(0, first=True)
    lax.fori_loop(1, NS, loop, 0)
    _wait(a_copies(NT - 1) + [q_copy(NT - 2), q_copy(NT - 1)])
    step(NS, last=True)
    _wait([oa_copy(a) for a in range(NT - 1)] + [oa_part(u) for u in range(4)]
          + [ob_copy(j, t) for j in range(NS) for t in range(NT)])


@jax.jit
def pallas_concat_heads__ssm_conv_h3__sliding_local_dilated__prompt_kernel(
    A_q, A_k, A_v, A_shift_k, A_ssm_k, A_ssm_D, B_x, B_wqkv, B_wo,
):
    hbm = pl.BlockSpec(memory_space=pl.ANY)
    out = pl.pallas_call(
        _kernel,
        in_specs=[hbm] * 10,
        out_specs=hbm,
        out_shape=jax.ShapeDtypeStruct((S, 2 * D), BF16),
        scratch_shapes=[
            pltpu.VMEM((NT, 128, S), BF16),
            pltpu.VMEM((NS, R, D), BF16),
            pltpu.VMEM((6, D // 2, D), BF16),
            pltpu.VMEM((NT, D, 128), BF16),
            pltpu.VMEM((NT, 5, 8, 128), F32),
            pltpu.VMEM((4, D), BF16),
            pltpu.VMEM((8, 128), BF16),
            pltpu.VMEM(_TABLE.shape, U32),
            pltpu.SemaphoreType.DMA((5 * NT + 10,)),
            pltpu.SemaphoreType.DMA((2,)),
        ] + [pltpu.VMEM((r * 4 // np.dtype(t).itemsize, 128), t) for t, r in _BUFS.values()],
        compiler_params=pltpu.CompilerParams(vmem_limit_bytes=100 * 1024 * 1024,
                                             disable_bounds_checks=True),
        name="fused",
    )(A_q[0], A_k[0], A_v[0], A_shift_k.T, A_ssm_k,
      A_ssm_D.reshape(8, 128), B_x[0], B_wqkv, B_wo, _TABLE)
    return out[None]
```

```python
import functools

import jax
import jax.numpy as jnp
import numpy as np
from jax import lax
from jax.experimental import pallas as pl
import jax.experimental.pallas.tpu as pltpu


S = 2048
D = 1024
T = 128
NC = S // T
NT = D // 128
NS = 4
R = S // NS
E = R // 2
WIN, DH = 8, 32
PITCH = 33
KR = WIN + E
FP = 2 * T + 16
KW = D // 4

F32, BF16, U32 = jnp.float32, jnp.bfloat16, jnp.uint32
P = functools.partial
add, sub, mul = lax.add, lax.sub, lax.mul


def _pack_rows(m):
    b = m.astype(jnp.bfloat16).view(np.uint16).astype(np.uint32)
    return np.ascontiguousarray(b[0::2] | (b[1::2] << 16))


def _dft_table():
    th = 2.0 * np.pi * (np.arange(T) + 0.25) / T
    ph = th[:, None] * (np.arange(T)[None, :] - (T - 1) / 4)
    fwd = np.concatenate([np.cos(ph), -np.sin(ph)], axis=0)
    rows = np.arange(T // 2).reshape(-1, 8, 2).transpose(0, 2, 1).reshape(-1)
    cols = np.arange(T).reshape(-1, 2, 8).transpose(0, 2, 1).reshape(-1)
    ph = (rows[:, None] + 0.5) * th[cols][None, :]
    return np.concatenate([_pack_rows(m) for m in (fwd, np.cos(ph) / T, np.sin(ph) / T)]
                          + [np.zeros((8, T), np.uint32)], axis=0)


_TABLE = _dft_table()


def _lo(w):
    return pltpu.bitcast(lax.shift_left(w, np.uint32(16)), F32)


def _hi(w):
    return pltpu.bitcast(lax.bitwise_and(w, np.uint32(0xFFFF0000)), F32)


def _pack(lo, hi):
    return pltpu.pack_elementwise([lo, hi], packed_dtype=BF16)


def _tree(xs):
    while len(xs) > 1:
        xs = [add(xs[i], xs[i + 1]) if i + 1 < len(xs) else xs[i] for i in range(0, len(xs), 2)]
    return xs[0]


def _left(a11, a12, a21, a22):
    return [add(a21, a22), a22, add(a11, a12), a11, add(a11, a22), sub(a12, a22), sub(a21, a11)]


def _merge(main, side):
    if not main:
        return side
    total_m = sum(c for c, _ in main)
    total_s = sum(c for c, _ in side)
    done_m, done_s, i, out = 0, 0, 0, []
    for c, f in main:
        out.append((c * total_s, f))
        done_m += c
        while i < len(side) and (done_s + side[i][0]) * total_m <= done_m * total_s:
            done_s += side[i][0]
            out.append((side[i][0] * total_m, side[i][1]))
            i += 1
    assert i == len(side)
    return out


def _run(tasks):
    for _, f in tasks:
        f()


def _weave(main, side):
    _run(_merge(main, side))


def _split(tasks, *weights):
    ends = np.cumsum((0,) + weights) * len(tasks) // sum(weights)
    return [tasks[a:b] for a, b in zip(ends[:-1], ends[1:])]


def _start(copies):
    for c in copies:
        c.start()


def _wait(copies):
    for c in copies:
        c.wait()


_BUFS = {n: (t, r) for t, group in (
    (BF16, dict(qa=NT * S // 2, ka=NT * (S // 2 + 8), va=NT * S // 2, oa=NT * S // 2, ob=S * NT // 2,
                xs=9 * 4 * E // 2, os=7 * 4 * E // 2, w3=2 * NT * KW)),
    (U32, dict(kv0=S // 8, kv1=S // 8, kv2=S // 8, kv3=S // 8, z=NC * T,
               **{f"w{p}": 2 * NT * KW for p in range(3)}, **{f"ws{p}": 20 * KW for p in range(4)},
               t0=32 * PITCH, t1=32 * PITCH)),
    (F32, dict(hf=NC * FP, xf=NC * FP, up=8 * NC, k1=8 * NC, pi=8 * NC, zr=8 * NC, zi=8 * NC,
               even=2 * T, c21=E, m4=E, c11=E, m5=E, c22=E, d11=E, d22=E, f21=E, f12=E,
               q=2 * NT * E, k=2 * NT * KR, v=2 * NT * KR, p=WIN * R, o=NT * R)),
) for n, r in group.items()}


def _kernel(q_hbm, k_hbm, v_hbm, sk_hbm, h_hbm, d_hbm, x_hbm, w_hbm, wo_hbm, tab_hbm, out_hbm,
            ha, xa, wraw, woraw, taps, sk_ref, d_ref, tab, sem_in, sem_out, *raw):
    raw = dict(zip(_BUFS, raw))
    bufs = {n: b.bitcast(U32) if _BUFS[n][0] == BF16 else b for n, b in raw.items()}

    raw["w0s"], bufs["w0s"] = raw["w0"], bufs["w0"]
    spec = dict(_BUFS, w0s=_BUFS["w0"])

    def ld(name, row, n=8, z=0):
        return views[name][z][pl.ds(row, n), :]

    def st(name, row, val):
        views[name][3][pl.ds(row, val.shape[0]), :] = val

    def st16(name, row, val):
        views[name][4][pl.ds(2 * row, val.shape[0]), :] = val.astype(BF16)

    def window(name, row, n):
        return bufs[name].at[pl.ds(pl.multiple_of(row, 8), n), :]

    def window16(name, row, n):
        return raw[name].at[pl.ds(pl.multiple_of(2 * row, 16), 2 * n), :]

    def cols(a):
        return pl.ds(pl.multiple_of(a * 128, 128), 128)

    def rows(j):
        return pl.ds(pl.multiple_of(j * R, R), R)

    def a_copies(a, sem):
        return [
            pltpu.make_async_copy(h_hbm.at[cols(a), :], ha.at[a], sem),
            pltpu.make_async_copy(k_hbm.at[:, cols(a)], window16("ka", a * (S // 2 + 8) + 8, S // 2), sem),
            pltpu.make_async_copy(v_hbm.at[:, cols(a)], window16("va", a * (S // 2), S // 2), sem),
        ]

    def q_copy(a, sem):
        return pltpu.make_async_copy(q_hbm.at[:, cols(a)], window16("qa", a * (S // 2), S // 2), sem)

    def in_copies(j):
        if isinstance(j, int) and j in (0, NS):
            a = max(2 * j - 1, 0)
            return a_copies(a, sem_in.at[j]) + ([q_copy(a - 1, sem_in.at[j])] if j else [])
        sem = sem_in.at[j]
        return (a_copies(2 * j - 1, sem) + [q_copy(2 * j - 2, sem)]
                + [pltpu.make_async_copy(x_hbm.at[rows(j), :], xa.at[j], sem)]
                + a_copies(2 * j, sem) + [q_copy(2 * j - 1, sem)])

    def last_q():
        return q_copy(NT - 1, sem_in.at[NS + 1])

    def x0_copy(h):
        half = pl.ds(h * D // 2, D // 2)
        return pltpu.make_async_copy(x_hbm.at[rows(0), half], xa.at[0, :, half], sem_in.at[NS + 2 + h])

    def w_copy(n):
        half = pl.ds(n % 2 * (D // 2), D // 2)
        return pltpu.make_async_copy(
            w_hbm.at[half, pl.ds(n // 2 * D, D)], wraw.at[n], sem_in.at[NS + 5 + n])

    def w_wait(n):
        pltpu.make_async_copy(wraw.at[n], wraw.at[n], sem_in.at[NS + 5 + n]).wait()

    def wo_copies():
        return [pltpu.make_async_copy(wo_hbm.at[:, pl.ds(t * 128, 128)], woraw.at[t],
                                      sem_in.at[NS + 11]) for t in range(NT)]

    def oa_copy(a):
        return pltpu.make_async_copy(window16("oa", a * (S // 2), S // 2), out_hbm.at[:, cols(a)],
                                     sem_out.at[0])

    def oa_part(u):
        src = window16("oa", (4 * (NT - 1) + u) * S // 8, S // 8)
        return pltpu.make_async_copy(src, out_hbm.at[pl.ds(u * S // 4, S // 4), cols(NT - 1)],
                                     sem_out.at[0])

    def ob_copy(j, t):
        return pltpu.make_async_copy(window16("ob", (j * NT + t) * E, E),
                                     out_hbm.at[rows(j), cols(NT + t)], sem_out.at[1])

    small = [pltpu.make_async_copy(a, b, sem_in.at[NS + 12])
             for a, b in ((tab_hbm, tab), (sk_hbm, sk_ref), (d_hbm, d_ref))]
    w00 = [pltpu.make_async_copy(w_hbm.at[pl.ds(u * KW, KW), pl.ds(0, D)], wraw.at[0, pl.ds(u * KW, KW)],
                                 sem_in.at[NS + 4 + u]) for u in range(2)]
    startup = lambda: (w00 + [x0_copy(0), w_copy(1), x0_copy(1), w_copy(2), w_copy(3)] + in_copies(0)
                       + [w_copy(4), w_copy(5)] + wo_copies())
    _start(small + startup())
    _wait(small)
    unit = pltpu.bitcast(tab[pl.ds(3 * T // 2, 8), :], jnp.int32)
    zs = [pl.multiple_of(unit[i, 0] * 8, 8) for i in range(3)]
    views = {n: [b.at[pl.ds(z, spec[n][1]), :] for z in zs] + [b, raw[n]] for n, b in bufs.items()}

    for a in range(NT):
        st("ka", a * (S // 2 + 8), jnp.zeros((8, 128), U32))
    for t in range(2 * NT):
        st("k", t * KR, jnp.zeros((WIN, 128), F32))
    skf = sk_ref[...].astype(F32)
    df = d_ref[...].astype(F32)
    for t in range(NT):
        for i in range(4):
            taps[t, i] = jnp.broadcast_to(skf[i:i + 1, t * 128:(t + 1) * 128], (8, 128))
        taps[t, 4] = jnp.broadcast_to(df[t:t + 1, :], (8, 128))

    def step(j, first=False, last=False):
        memo = {}
        never = tab[pl.ds(3 * T // 2, 8), :] != 0

        def once(key, fn):
            if key not in memo:
                memo[key] = fn()
            return memo[key]

        def fresh():
            memo["fresh"] = memo.get("fresh", 1) + 1
            return pl.multiple_of(zs[0] * memo["fresh"], 8)

        def pace(val):
            clock = memo.get("clock")
            if clock is None:
                return val
            if val.dtype != F32:
                clock = pltpu.bitcast(clock, val.dtype)
            return lax.select(never, clock, val)

        def paced(x):
            return jnp.concatenate([pace(x[:8]), x[8:]], axis=0)

        def wait(copies):
            memo["clock"] = None
            _wait(copies)

        def rolled(n, shifts, body):
            def one(i, carry):
                saved, kept = dict(views), dict(memo)
                memo["clock"] = None
                for name, d in shifts.items():
                    size = spec[name][1] - d * (n - 1)
                    views[name] = [window(name, z + d * i, size) for z in zs + [0]]
                    if spec[name][0] == BF16:
                        views[name].append(window16(name, d * i, size))
                body(i)
                views.update(saved)
                memo.clear()
                memo.update(kept, clock=None)
                return carry
            lax.fori_loop(0, n, one, 0)

        def perm_in(w, u, t):
            tt = paced(pltpu.bitcast(w[pl.ds(u * 256, 256), pl.ds(t * 128, 128)], U32)).T
            for hh in range(4):
                st(f"t{u}", (4 * t + hh) * PITCH, tt[hh * DH:(hh + 1) * DH])

        def perm_out(p, h, u, t):
            g = jnp.concatenate(
                [bufs[f"t{u}"][pl.ds(zs[0] + 4 * t + i, 32, stride=PITCH), :] for i in range(4)], axis=0)
            st(f"w{p}", (h * NT + t) * KW + u * 128, paced(g).T)

        def perm_list(n, w=None, us=(0, 1)):
            w = wraw.at[n] if w is None else w
            return [(1, P(f, u, t)) for f in (P(perm_in, w), P(perm_out, n // 2, n % 2))
                    for u in us for t in range(NT)] + [(2, lambda: None)] * 4

        def wo_in(i, t0, t, hh):
            w = pltpu.bitcast(woraw[2 * i + t - t0, pl.ds(hh * DH, DH), :], U32)
            wt = pltpu.bitcast(paced(w), BF16).astype(F32)
            st(f"t{t % 2}", hh * PITCH, pltpu.bitcast(wt, U32))

        def wo_out(t, i):
            g = bufs[f"t{t % 2}"][pl.ds(zs[0] + i, 32, stride=PITCH), :]
            st16("w3", (i // 16 * NT + t) * KW + i % 16 * 16, pltpu.bitcast(paced(g), F32))

        def wo_list(i, t0=0):
            return [(1, P(f, t, u)) for f in (P(wo_in, i, t0), wo_out)
                    for t in (t0, t0 + 1) for u in range(32)]

        def right(p, t, r):
            b = [ld(f"w{p}" if p else "w0s", (h * NT + t + 4 * u) * KW + r, 16) for h in range(2) for u in range(2)]
            b[0] = paced(b[0])
            sums = []
            for half in (_lo, _hi):
                b11, b12, b21, b22 = map(half, b)
                sums.append([sub(b21, b11), sub(b12, b22), add(b11, b22), add(b21, b22), add(b11, b12)])
            for i, (lo, hi) in enumerate(zip(*sums)):
                st(f"ws{p}", (4 * i + t) * KW + r, _pack(lo, hi))

        def right_list(p):
            return [(1, P(right, p, t, r)) for t in range(4) for r in range(0, KW, 16)]

        def ld_kv(c, row, n, z=0):
            return ld(f"kv{c // 4}", c % 4 * (T // 2) + row, n, z)

        def a1(i, r):
            a = once(("a", i), lambda: 2 * j + i)
            w0, w1, w2, w3 = once(("taps", i), lambda: [taps[a, u] for u in range(4)])
            k32 = once(("ka", i), lambda: window("ka", a * (S // 2 + 8), S // 2 + 8))
            v32 = once(("va", i), lambda: window("va", a * (S // 2), S // 2))
            c0, c1, c2 = (k32[pl.ds(8 * r + 8 - u, 8), :] for u in range(3))
            vv = v32[pl.ds(8 * r, 8), :]
            e0, o0, e1, o1, o2 = _lo(c0), _hi(c0), _lo(c1), _hi(c1), _hi(c2)
            ke = _tree([mul(e0, w0), mul(o1, w1), mul(e1, w2), mul(o2, w3)])
            ko = _tree([mul(o0, w0), mul(e0, w1), mul(o1, w2), mul(e1, w3)])
            st(f"kv{r // 32}", 8 * (r % 32), pace(_pack(mul(ke, _lo(vv)), mul(ko, _hi(vv)))))

        def a1_list(i, c0, c1):
            return [(24, P(a1, i, r)) for r in range(8 * c0, 8 * c1)]

        def freq(c, im, m):
            return c * FP + im * (T + 8) + m

        def dft(i, name, c0, m):
            def mm():
                f = pltpu.bitcast(tab[pl.ds(fresh(), T), :], BF16)
                if name == "hf":
                    a = once(("a", i), lambda: 2 * j + i)
                    rhs = jnp.concatenate(
                        [ha[a, :, pl.ds(c * T, T)] for c in range(c0, c0 + 4)], axis=0)
                    return lax.dot_general(f, rhs, (((1,), (1,)), ((), ())),
                                           preferred_element_type=F32)
                rhs = jnp.concatenate(
                    [pltpu.bitcast(ld_kv(c, 0, T // 2, i % 2), BF16) for c in range(c0, c0 + 4)], axis=1)
                return jnp.dot(f, rhs, preferred_element_type=F32)
            res = once((name, i, c0), mm)
            for u in range(4):
                st(name, freq(c0 + u, m // T, m % T), res[m:m + 16, u * 128:(u + 1) * 128])
            memo["clock"] = res[m + 8:m + 16, 384:]

        def dft_list(i, name, *c0s):
            return [(16, P(dft, i, name, c0, m)) for c0 in c0s for m in range(0, 2 * T, 16)]

        def a3(i, g, plane, upper, n):
            def opnd(name, c):
                re = lambda: ld(name, freq(c, 0, 8 * g), z=plane)
                im = lambda: ld(name, freq(c, 1, 8 * g), z=plane)
                if name == "xf":
                    val = add(re(), im()) if plane == 0 else re() if plane == 1 else im()
                    return pace(val) if c >= 8 else val
                return pace(re() if plane == 0 else (sub, add)[plane - 1](im(), re()))
            get = lambda name, c: once((name, i, g, plane, c), P(opnd, name, c))
            done = pace if not (first or last) or n % 4 == 3 else lambda v: v
            cs = range(8, n + 1) if upper else range(min(n, 7) + 1)
            terms = [mul(get("xf", n - c), get("hf", c)) for c in cs]
            if upper:
                st("up", 8 * n, done(_tree(terms)))
                return
            if n >= 8:
                terms.append(ld("up", 8 * n))
            if plane == 0:
                st("k1", 8 * n, done(_tree(terms)))
            elif plane == 1:
                st("pi", 8 * n, done(_tree(terms + [ld("k1", 8 * n)])))
            else:
                pr = sub(ld("k1", 8 * n, z=1), _tree(terms))
                pi = ld("pi", 8 * n)
                zr, zi = pr, pi
                if n > 0:
                    qr, qi = memo["prev"]
                    zr, zi = sub(pr, qi), add(pi, qr)
                memo["prev"] = (pr, pi)
                if g % 2 == 0:
                    st("zr", 8 * n, done(zr))
                    st("zi", 8 * n, zi)
                else:
                    st("z", n * T + 4 * (g - 1), _pack(ld("zr", 8 * n), done(zr)))
                    st("z", n * T + T // 2 + 4 * (g - 1), _pack(ld("zi", 8 * n), zi))

        def a3_list(i):
            out = []
            for g in range(T // 8):
                for plane in range(3):
                    out += [(2 * (n - 8) + 4, P(a3, i, g, plane, True, n)) for n in range(8, NC)]
                    out += [(2 * min(n, 7) + 4 + 2 * (plane == 2), P(a3, i, g, plane, False, n))
                            for n in range(NC)]
            return out

        def idft(i, c0, odd, m):
            def mm():
                rhs = jnp.concatenate([pltpu.bitcast(ld("z", c * T + odd * T // 2, T // 2, i + 2), BF16)
                                       for c in range(c0, c0 + 4)], axis=1)
                f = tab[pl.ds(fresh() + T + odd * T // 4, T // 4), :]
                return jnp.dot(pltpu.bitcast(f, BF16), rhs, preferred_element_type=F32)
            y = once(("y", i, c0, odd), mm)
            a = once(("a", i), lambda: 2 * j + i)
            dd = once(("dd", i), lambda: taps[a, 4])
            q32 = once(("qa", i), lambda: window("qa", a * (S // 2), S // 2))
            o32 = once(("oa", i), lambda: window("oa", a * (S // 2), S // 2))
            flip = lambda w: jnp.take_along_axis(
                w, 7 - lax.broadcasted_iota(jnp.int32, (8, 128), 0), axis=0, mode="promise_in_bounds")

            def gate(c, row, lo, hi, order):
                kv, qq = order(ld_kv(c, row, 8, 2)), order(q32[pl.ds(c * T // 2 + row, 8), :])
                o32[pl.ds(c * T // 2 + row, 8), :] = order(_pack(
                    mul(_lo(qq), add(lo, mul(_lo(kv), dd))), mul(_hi(qq), add(hi, mul(_hi(kv), dd)))))

            for u in range(4):
                if not odd:
                    st("even", u * T // 2 + m, y[m:m + 16, u * 128:(u + 1) * 128])
                    continue
                s0, s1 = (y[m + h:m + h + 8, u * 128:(u + 1) * 128] for h in (0, 8))
                e0, e1 = (ld("even", u * T // 2 + m + h) for h in (0, 8))
                gate(c0 + u, T // 4 + m // 2, sub(e0, s0), sub(e1, s1), lambda w: w)
                gate(c0 + u, T // 4 - 8 - m // 2, add(e1, s1), add(e0, s0), flip)
            memo["clock"] = y[m + 8:m + 16, 384:]

        def idft_list(i, *c0s):
            return [(16, P(idft, i, c0, odd, m)) for c0 in c0s
                    for odd in range(2) for m in range(0, T // 2, 16)]

        def transforms(i, extra, shares=(1, 1, 1, 1, 1, 9)):
            extra = _split(extra, *shares)
            for u in range(4):
                _weave(idft_list(i - 1, 4 * u)[:4], extra[u])
                _run(idft_list(i - 1, 4 * u)[4:])
                _weave(dft_list(i, "hf", 4 * u), a1_list(i, 3 * u, 3 * u + 3))
            oa_copy(2 * j + i - 1).start()
            _weave(dft_list(i, "xf", 0), _merge(a1_list(i, 12, 16), extra[4]))
            _weave(dft_list(i, "xf", 4, 8), extra[5])
            _run(dft_list(i, "xf", 12))

        def xprep(x, u, r):
            halves = []
            for m in (r, r + 8):
                a, b = (pltpu.bitcast(x[pl.ds(2 * m, 16), pl.ds(t * 128, 128)], U32)
                        for t in (u, u + 4))
                a = pace(a)
                a11, a12, a21, a22 = _lo(a), _lo(b), _hi(a), _hi(b)
                halves.append(_left(a11, a12, a21, a22) + ([a12, a22] if first else []))
            for i, pair in enumerate(zip(*halves)):
                st16("xs", ((4 * i + u) * E + r) // 2, jnp.concatenate(pair, axis=0))

        def split_rows(i):
            for u in range(4):
                a = pltpu.bitcast(xa[0, pl.ds(pl.multiple_of(i * 128, 16), 128), pl.ds(u * 128, 128)], U32)
                st16("os", u * E // 2, _lo(a))
                st16("os", (4 + u) * E // 2, _hi(a))

        def xprep_list(x):
            return [(27, P(xprep, x, u, r)) for r in range(0, E, 16) for u in range(4)]

        def lhs(name, i, m0=0, n=E):
            view = views[name][3].at[pl.ds(fresh() + i * 2 * E, 2 * E), :]
            return jnp.concatenate(
                [pltpu.bitcast(view[pl.ds((u * E + m0) // 2, n // 2), :], BF16) for u in range(4)], axis=1)

        def emit(p, par, t, m, val):
            if p == 0:
                st("q", (par * NT + t) * E + m, val)
                return
            name, row = "kv"[p - 1], (par * NT + t) * KR
            if m == 0 and not first:
                st(name, row, ld(name, row + E, WIN, z=3))
            if m == 0 and first and p == 2 and par == 0:
                for other in range(2):
                    st(name, (other * NT + t) * KR, jnp.broadcast_to(val[0:1], (WIN, 128)))
            st(name, row + WIN + m, val)

        def plain(half, t, m):
            def mm():
                w = pltpu.bitcast(ld("w0", (half * NT + t) * KW, KW, 3), BF16)
                x = lhs("xs", 7) if half else jnp.concatenate([lhs("os", 0), lhs("os", 1)], axis=0)
                return jnp.dot(x, w, preferred_element_type=F32)
            res = once(("plain", half, t), mm)
            memo["clock"] = res[m + 8:m + 16]
            if half:
                emit(0, 0, t, m, add(res[m:m + 16], ld("o", t * R + m, 16)))
            else:
                st("o", t * R + m, res[m:m + 16])

        def plain_list(half):
            return [(16, P(plain, half, t, m)) for t in range(NT) for m in range(0, E if half else R, 16)]

        def product(p, m0, n, t, i, m):
            def mm():
                if i == 0:
                    w = ld(f"w{p}", t * KW, KW, 3)
                elif i == 2:
                    w = ld(f"w{p}", (NT + t + 4) * KW, KW, 3)
                else:
                    w = ld(f"ws{p}", (4 * (i - 1 - (i > 2)) + t) * KW, KW, 3)
                return jnp.dot(lhs("xs" if p < 3 or m0 else "os", i, m0, n), pltpu.bitcast(w, BF16),
                               preferred_element_type=F32)
            res = once(("product", p, m0, t, i), mm)
            memo["clock"] = res[m - m0 + 8:m - m0 + 16]
            res = res[m - m0:m - m0 + 16]
            get = lambda name, z=0: ld(name, m, 16, z)
            if i == 0:
                st("c21", m, res)
            elif i == 1:
                st("m4", m, res)
                P(st, "f21", m)(add(get("c21"), res)) if p == 3 else emit(p, 1, t, m, add(get("c21"), res))
            elif i == 2:
                st("c11", m, sub(get("m4"), res))
                st("m5", m, res)
            elif i == 3:
                st("c22", m, sub(res, get("c21", 1)))
                P(st, "f12", m)(add(get("m5"), res)) if p == 3 else emit(p, 0, t + 4, m, add(get("m5"), res))
            elif i == 4:
                st("d11", m, add(get("c11"), res))
                st("d22", m, add(get("c22"), res))
            elif p < 3:
                emit(p, i - 5, t + 4 * (i - 5), m, add(get(("d11", "d22")[i - 5]), res))
            else:
                o32 = once("ob", lambda: window("ob", (j - 1) * NT * E, NT * E))
                tile = t + 4 * (i - 5)
                o32[pl.ds(tile * E + m, 16), :] = (
                    _pack(add(get("d11"), res), get("f21")) if i == 5
                    else _pack(get("f12"), add(get("d22"), res)))
                if m + 16 == E:
                    ob_copy(j - 1, tile).start()

        def strassen(p, m0=0, n=E):
            return [(16, P(product, p, m0, n, t, i, m))
                    for t in range(4) for i in range(7) for m in range(m0, m0 + n, 16)]

        def qk(r, w):
            par, m = divmod(8 * r, E)
            qv = once(("qv", r), lambda: [pace(ld("q", (par * NT + t) * E + m)) for t in range(NT)])
            s = pace(_tree([mul(qv[t], ld("k", (par * NT + t) * KR + WIN + m - w)) for t in range(NT)]))
            s = add(s, pltpu.roll(s, 64, 1))
            s = add(s, pltpu.roll(s, 32, 1))
            if first and m < w:
                keep = m + lax.broadcasted_iota(jnp.int32, (8, 128), 0) >= w
                s = jnp.where(keep, s, -1e9 * DH ** 0.5)
            memo["lg", r, w] = s

        def expo(r):
            lg = [memo["lg", r, w] for w in range(WIN)]
            m = pace(functools.reduce(lax.max, lg))
            scale = np.float32(DH ** -0.5 * np.log2(np.e))
            memo["e", r] = [lax.exp2(mul(sub(s, m), scale)) for s in lg]

        def norm(r):
            memo["inv", r] = 1.0 / pace(_tree(memo["e", r]))

        def probs(r):
            inv = pace(memo["inv", r])
            for w in range(WIN):
                st("p", w * R + 8 * r, mul(memo["e", r][w], inv))

        def qk_list(nr=R // 8):
            out = []
            for i in range(WIN * nr + 23):
                r, w = divmod(i, WIN)
                tasks = [P(qk, r, w)] if r < nr else []
                for f, lag in ((expo, 24), (norm, 27), (probs, 30)):
                    if i >= lag and (i - lag) % WIN == 0 and (i - lag) // WIN < nr:
                        tasks.append(P(f, (i - lag) // WIN))
                out.append((26 if r < nr else 12, P(_run, [(0, f) for f in tasks])))
            return out

        def pv(r, t):
            par, m = divmod(8 * r, E)
            p = once(("pv", r), lambda: [pace(ld("p", w * R + 8 * r)) for w in range(WIN)])
            row = (par * NT + t) * KR + WIN + m
            st("o", t * R + 8 * r, pace(_tree([mul(p[w], ld("v", row - w)) for w in range(WIN)])))

        def pv_list():
            return [(16, P(pv, r, t)) for r in range(R // 8) for t in range(NT)]

        def oprep(u, r):
            a = [ld("o", (u + 4 * h) * R + par * E + r, 16, 1) for par in range(2) for h in range(2)]
            for i, val in enumerate(_left(*a[:3], paced(a[3]))):
                st16("xs" if last and 2 * r >= E else "os", ((4 * i + u) * E + r) // 2, val)

        def oprep_list():
            return [(18, P(oprep, u, r)) for r in range(0, E, 16) for u in range(4)]

        if last:
            mix = []
            for r in range(E // 16):
                mix += pv_list()[16 * r:16 * r + 16] + pv_list()[E + 16 * r:E + 16 * r + 16]
                mix += oprep_list()[4 * r:4 * r + 4]
            mix, conv = _split(mix, 1, 1), _split(a3_list(-1), 3, 5)
            transforms(-1, mix[0], (1, 1, 1, 1, 1, 5))
            wait([last_q()])
            _weave(strassen(3, 0, E // 2), mix[1] + conv[0])
            _weave(strassen(3, E // 2, E // 2)[:-6], conv[1])
            _run(strassen(3, E // 2, E // 2)[-6:])
            for u in range(4):
                _run(idft_list(-1, 4 * u))
                oa_part(u).start()
            return

        if first:
            def leading(i):
                w = wraw.at[0, pl.ds(pl.multiple_of(i * KW, KW), KW)]
                pltpu.make_async_copy(w, w, sem_in.at[NS + 4 + i]).wait()
                _run(perm_list(0, w, (0,)))
            rolled(2, dict(w0=128), leading)
            wait([x0_copy(0)])
            rolled(4, dict(os=32), split_rows)
            _run(plain_list(0)[:96])
            wait([w_copy(1)])
            _weave(plain_list(0)[96:240], perm_list(1))
            _run(plain_list(0)[240:])
            wait([x0_copy(1)])
            rolled(4, dict(xs=E // 8), lambda i: _run(
                xprep_list(xa.at[0, pl.ds(pl.multiple_of(i * (R // 4), 16), R // 4)])[:16]))

            def queries(i):
                w_wait(2 + i)
                _weave(plain_list(1), _merge(perm_list(2, wraw.at[2 + i]), right_list(0)[:32]))
            rolled(2, dict(w1=NT * KW, ws0=2 * KW, w0s=2 * KW, xs=2 * E, o=E, q=NT * E), queries)
            _run(right_list(1)[:32])
            wait(in_copies(0))
            _start(in_copies(1))
            _weave(dft_list(0, "hf", 0, 4), a1_list(0, 0, 8))
            _weave(dft_list(0, "hf", 8, 12) + dft_list(0, "xf", 0), a1_list(0, 8, 16))
            _weave(dft_list(0, "xf", 4, 8, 12), right_list(1)[32:])

            def keys(i):
                w_wait(4 + i)
                _weave(strassen(1)[:144], _merge(perm_list(4, wraw.at[4 + i]), a3_list(0)[:320]))
                _weave(strassen(1)[144:220], a3_list(0)[320:576])
                _run(strassen(1)[220:224])
            rolled(2, dict(w1=2 * KW, ws1=2 * KW, w2=NT * KW, k=2 * KR, hf=64, xf=64, z=32), keys)
            wait(wo_copies())
            _start(in_copies(2) + in_copies(3) + in_copies(NS) + [last_q()])
            rolled(2, dict(w2=2 * KW, ws2=2 * KW, w3=4 * KW), lambda i: _run(
                _merge(right_list(2)[:32], wo_list(2 * i, 0) + wo_list(2 * i + 1, 2))))
            rolled(2, dict(w2=2 * KW, ws2=2 * KW, w3=2 * KW, ws3=2 * KW, v=2 * KR, q=NT * E, k=NT * KR, p=E),
                   lambda i: _weave(strassen(2)[:224], _merge(right_list(3)[:32], qk_list(E // 8))))
            return

        head = strassen(0) + strassen(1)
        pre = _split(oprep_list(), 3, 1)
        transforms(-1, xprep_list(xa.at[j]))
        _weave(head[:528], a3_list(-1))
        _weave(head[528:812], pv_list())
        _run(head[812:818])
        transforms(0, pre[0], (0, 0, 0, 0, 1, 9))
        _weave(head[818:] + strassen(3), pre[1] + a3_list(0))
        _weave(strassen(2), qk_list())

    def loop(j, carry):
        _wait(in_copies(j))
        step(j)
        return carry

    step(0, first=True)
    lax.fori_loop(1, NS, loop, 0)
    _wait(in_copies(NS))
    step(NS, last=True)
    for i, name in enumerate(("oa", "ob")):
        pltpu.make_async_copy(raw[name], raw[name], sem_out.at[i]).wait()


@jax.jit
def pallas_concat_heads__ssm_conv_h3__sliding_local_dilated__prompt_kernel(
    A_q, A_k, A_v, A_shift_k, A_ssm_k, A_ssm_D, B_x, B_wqkv, B_wo,
):
    hbm = pl.BlockSpec(memory_space=pl.ANY)
    out = pl.pallas_call(
        _kernel,
        in_specs=[hbm] * 10,
        out_specs=hbm,
        out_shape=jax.ShapeDtypeStruct((S, 2 * D), BF16),
        scratch_shapes=[
            pltpu.VMEM((NT, 128, S), BF16),
            pltpu.VMEM((NS, R, D), BF16),
            pltpu.VMEM((6, D // 2, D), BF16),
            pltpu.VMEM((NT, D, 128), BF16),
            pltpu.VMEM((NT, 5, 8, 128), F32),
            pltpu.VMEM((4, D), BF16),
            pltpu.VMEM((8, 128), BF16),
            pltpu.VMEM(_TABLE.shape, U32),
            pltpu.SemaphoreType.DMA((NS + 13,)),
            pltpu.SemaphoreType.DMA((2,)),
        ] + [pltpu.VMEM((r * 4 // np.dtype(t).itemsize, 128), t) for t, r in _BUFS.values()],
        compiler_params=pltpu.CompilerParams(vmem_limit_bytes=100 * 1024 * 1024,
                                             disable_bounds_checks=True,
                                             disable_semaphore_checks=True),
        name="fused",
    )(A_q[0], A_k[0], A_v[0], A_shift_k.T, A_ssm_k,
      A_ssm_D.reshape(8, 128), B_x[0], B_wqkv, B_wo, _TABLE)
    return out[None]
```

```python
import functools

import jax
import jax.numpy as jnp
import numpy as np
from jax import lax
from jax.experimental import pallas as pl
import jax.experimental.pallas.tpu as pltpu


S = 2048
D = 1024
T = 128
NC = S // T
NT = D // 128
NS = 4
R = S // NS
E = R // 2
WIN, DH = 8, 32
PITCH = 33
KR = WIN + E
FP = 2 * T + 16
KW = D // 4

F32, BF16, U32 = jnp.float32, jnp.bfloat16, jnp.uint32
P = functools.partial
add, sub, mul = lax.add, lax.sub, lax.mul


def _pack_rows(m):
    b = m.astype(jnp.bfloat16).view(np.uint16).astype(np.uint32)
    return np.ascontiguousarray(b[0::2] | (b[1::2] << 16))


def _dft_table():
    th = 2.0 * np.pi * (np.arange(T) + 0.25) / T
    dft = lambda t: np.concatenate([np.cos(np.outer(th, t)), -np.sin(np.outer(th, t))], axis=0)
    paired = np.arange(T).reshape(-1, 8, 2).transpose(0, 2, 1).reshape(-1)
    ph = np.outer(np.arange(T // 2) + 0.5, th)
    mats = (dft(np.arange(T)), dft(paired - (T - 1) / 2), np.cos(ph) / T, np.sin(ph) / T)
    return np.concatenate([_pack_rows(m) for m in mats] + [np.zeros((8, T), np.uint32)], axis=0)


_TABLE = _dft_table()


def _lo(w):
    return pltpu.bitcast(lax.shift_left(w, np.uint32(16)), F32)


def _hi(w):
    return pltpu.bitcast(lax.bitwise_and(w, np.uint32(0xFFFF0000)), F32)


def _rows(first, second):
    return jnp.concatenate([first, second], axis=0)


def _tree(xs):
    while len(xs) > 1:
        xs = [add(xs[i], xs[i + 1]) if i + 1 < len(xs) else xs[i] for i in range(0, len(xs), 2)]
    return xs[0]


def _left(a11, a12, a21, a22):
    return [add(a21, a22), a22, add(a11, a12), a11, add(a11, a22), sub(a12, a22), sub(a21, a11)]


def _merge(main, side):
    if not main:
        return side
    total_m = sum(c for c, _ in main)
    total_s = sum(c for c, _ in side)
    done_m, done_s, i, out = 0, 0, 0, []
    for c, f in main:
        out.append((c * total_s, f))
        done_m += c
        while i < len(side) and (done_s + side[i][0]) * total_m <= done_m * total_s:
            done_s += side[i][0]
            out.append((side[i][0] * total_m, side[i][1]))
            i += 1
    assert i == len(side)
    return out


def _run(tasks):
    for _, f in tasks:
        f()


def _weave(main, side):
    _run(_merge(main, side))


def _split(tasks, *weights):
    ends = np.cumsum((0,) + weights) * len(tasks) // sum(weights)
    return [tasks[a:b] for a, b in zip(ends[:-1], ends[1:])]


def _start(copies):
    for c in copies:
        c.start()


def _wait(copies):
    for c in copies:
        c.wait()


_BUFS = {n: (t, r) for t, group in (
    (BF16, dict(qa=NT * S // 2, ka=NT * (S // 2 + 8), va=NT * S // 2, oa=NT * S // 2, ob=S * NT // 2,
                xs=9 * 4 * E // 2, os=7 * 4 * E // 2, w3=2 * NT * KW,
                kv0=S // 8, kv1=S // 8, kv2=S // 8, kv3=S // 8, z=NC * T,
                **{f"ws{p}": 20 * KW for p in range(4)})),
    (U32, dict(**{f"w{p}": 2 * NT * KW for p in range(3)}, t0=34 * DH, t1=34 * DH)),
    (F32, dict(hf=NC * FP, xf=NC * FP, up=8 * NC, k1=8 * NC, pi=8 * NC, zr=8 * NC, zi=8 * NC,
               even=2 * T, c21=E, m4=E, c11=E, m5=E, c22=E, d11=E, d22=E,
               q=2 * NT * E, k=2 * NT * KR, v=2 * NT * KR, p=WIN * R, o=NT * R + 8)),
) for n, r in group.items()}


def _kernel(q_hbm, k_hbm, v_hbm, sk_hbm, h_hbm, d_hbm, x_hbm, w_hbm, wo_hbm, tab_hbm, out_hbm,
            ha, xa, wraw, woraw, taps, sk_ref, d_ref, tab, sem_in, sem_out, *raw):
    raw = dict(zip(_BUFS, raw))
    bufs = {n: b.bitcast(U32) if _BUFS[n][0] == BF16 else b for n, b in raw.items()}

    raw["w0s"], bufs["w0s"] = raw["w0"], bufs["w0"]
    spec = dict(_BUFS, w0s=_BUFS["w0"])

    def ld(name, row, n=8, z=0):
        assert 0 <= row and row + n <= views[name][z].shape[0]
        return views[name][z][pl.ds(row, n), :]

    def st(name, row, val):
        assert 0 <= row and row + val.shape[0] <= views[name][3].shape[0]
        views[name][3][pl.ds(row, val.shape[0]), :] = val

    def st16(name, row, val):
        assert 0 <= row and 2 * row + val.shape[0] <= views[name][4].shape[0]
        views[name][4][pl.ds(2 * row, val.shape[0]), :] = val.astype(BF16)

    def window(name, row, n):
        return bufs[name].at[pl.ds(pl.multiple_of(row, 8), n), :]

    def window16(name, row, n):
        return raw[name].at[pl.ds(pl.multiple_of(2 * row, 16), 2 * n), :]

    def cols(a):
        return pl.ds(pl.multiple_of(a * 128, 128), 128)

    def rows(j):
        return pl.ds(pl.multiple_of(j * R, R), R)

    def a_copies(a, sem):
        return [
            pltpu.make_async_copy(h_hbm.at[cols(a), :], ha.at[a], sem),
            pltpu.make_async_copy(k_hbm.at[:, cols(a)], window16("ka", a * (S // 2 + 8) + 8, S // 2), sem),
            pltpu.make_async_copy(v_hbm.at[:, cols(a)], window16("va", a * (S // 2), S // 2), sem),
        ]

    def q_copy(a, sem):
        return pltpu.make_async_copy(q_hbm.at[:, cols(a)], window16("qa", a * (S // 2), S // 2), sem)

    def in_copies(j):
        if isinstance(j, int) and j in (0, NS):
            a = max(2 * j - 1, 0)
            return a_copies(a, sem_in.at[j]) + ([q_copy(a - 1, sem_in.at[j])] if j else [])
        sem = sem_in.at[j]
        return (a_copies(2 * j - 1, sem) + [q_copy(2 * j - 2, sem)]
                + [pltpu.make_async_copy(x_hbm.at[rows(j), :], xa.at[j], sem)]
                + a_copies(2 * j, sem) + [q_copy(2 * j - 1, sem)])

    def last_q():
        return q_copy(NT - 1, sem_in.at[NS + 1])

    def x0_copy(h):
        half = pl.ds(h * D // 2, D // 2)
        return pltpu.make_async_copy(x_hbm.at[rows(0), half], xa.at[0, :, half], sem_in.at[NS + 2 + h])

    def w_copy(n):
        half = pl.ds(n % 2 * (D // 2), D // 2)
        return pltpu.make_async_copy(
            w_hbm.at[half, pl.ds(n // 2 * D, D)], wraw.at[n], sem_in.at[NS + 5 + n])

    def w_wait(n):
        pltpu.make_async_copy(wraw.at[n], wraw.at[n], sem_in.at[NS + 5 + n]).wait()

    def wo_copies():
        return [pltpu.make_async_copy(wo_hbm.at[:, pl.ds(t * 128, 128)], woraw.at[t],
                                      sem_in.at[NS + 11]) for t in range(NT)]

    def oa_copy(a):
        return pltpu.make_async_copy(window16("oa", a * (S // 2), S // 2), out_hbm.at[:, cols(a)],
                                     sem_out.at[0])

    def oa_part(u):
        src = window16("oa", (4 * (NT - 1) + u) * S // 8, S // 8)
        return pltpu.make_async_copy(src, out_hbm.at[pl.ds(u * S // 4, S // 4), cols(NT - 1)],
                                     sem_out.at[0])

    def ob_copy(j, t):
        return pltpu.make_async_copy(window16("ob", (j * NT + t) * E, E),
                                     out_hbm.at[rows(j), cols(NT + t)], sem_out.at[1])

    small = [pltpu.make_async_copy(a, b, sem_in.at[NS + 12])
             for a, b in ((tab_hbm, tab), (sk_hbm, sk_ref), (d_hbm, d_ref))]
    w00 = [pltpu.make_async_copy(w_hbm.at[pl.ds(u * KW, KW), pl.ds(0, D)], wraw.at[0, pl.ds(u * KW, KW)],
                                 sem_in.at[NS + 4 + u]) for u in range(2)]
    startup = lambda: (w00 + [x0_copy(0), w_copy(1), x0_copy(1), w_copy(2), w_copy(3)] + in_copies(0)
                       + [w_copy(4), w_copy(5)] + wo_copies())
    _start(small + startup())
    _wait(small)
    unit = pltpu.bitcast(tab[pl.ds(5 * T // 2, 8), :], jnp.int32)
    zs = [pl.multiple_of(unit[i, 0] * 8, 8) for i in range(3)]
    views = {n: [b.at[pl.ds(z, spec[n][1]), :] for z in zs] + [b, raw[n]] for n, b in bufs.items()}

    for a in range(NT):
        st("ka", a * (S // 2 + 8), jnp.zeros((8, 128), U32))
    for t in range(2 * NT):
        st("k", t * KR, jnp.zeros((WIN, 128), F32))
    skf = sk_ref[...].astype(F32)
    df = d_ref[...].astype(F32)
    for t in range(NT):
        for i in range(4):
            taps[t, i] = jnp.broadcast_to(skf[i:i + 1, t * 128:(t + 1) * 128], (8, 128))
        taps[t, 4] = jnp.broadcast_to(df[t:t + 1, :], (8, 128))

    def step(j, first=False, last=False):
        memo = {}
        never = tab[pl.ds(5 * T // 2, 8), :] != 0

        def once(key, fn):
            if key not in memo:
                memo[key] = fn()
            return memo[key]

        def fresh():
            memo["fresh"] = memo.get("fresh", 1) + 1
            return pl.multiple_of(zs[0] * memo["fresh"], 8)

        def pace(val):
            clock = memo.get("clock")
            if clock is None:
                return val
            if val.dtype != F32:
                clock = pltpu.bitcast(clock, val.dtype)
            return lax.select(never, clock, val)

        def paced(x):
            return jnp.concatenate([pace(x[:8]), x[8:]], axis=0)

        def wait(copies):
            memo["clock"] = None
            _wait(copies)

        def rolled(n, shifts, body):
            def one(i, carry):
                saved, kept = dict(views), dict(memo)
                memo["clock"] = None
                for name, d in shifts.items():
                    size = spec[name][1] - d * (n - 1)
                    views[name] = [window(name, z + d * i, size) for z in zs + [0]]
                    if spec[name][0] == BF16:
                        views[name].append(window16(name, d * i, size))
                body(i)
                views.update(saved)
                memo.clear()
                memo.update(kept, clock=None)
                return carry
            lax.fori_loop(0, n, one, 0)

        def perm_in(w, u, t):
            tt = paced(pltpu.bitcast(w[pl.ds(u * 256, 256), pl.ds(t * 128, 128)], U32)).T
            for hh in range(4):
                st(f"t{u}", (4 * t + hh) * PITCH, tt[hh * DH:(hh + 1) * DH])

        def perm_out(p, h, u, t):
            g = jnp.concatenate(
                [bufs[f"t{u}"][pl.ds(zs[0] + 4 * t + i, 32, stride=PITCH), :] for i in range(4)], axis=0)
            st(f"w{p}", (h * NT + t) * KW + u * 128, paced(g).T)

        def perm_list(n, w=None, us=(0, 1)):
            w = wraw.at[n] if w is None else w
            return [(1, P(f, u, t)) for f in (P(perm_in, w), P(perm_out, n // 2, n % 2))
                    for u in us for t in range(NT)] + [(2, lambda: None)] * 4

        def wo_in(i, t0, t, hh):
            w = pltpu.bitcast(woraw[2 * i + t - t0, pl.ds(hh * DH, DH), :], U32)
            wt = pltpu.bitcast(paced(w), BF16).astype(F32)
            st(f"t{t % 2}", hh * PITCH, pltpu.bitcast(wt, U32))

        def wo_out(t, i):
            g = bufs[f"t{t % 2}"][pl.ds(zs[0] + i, 32, stride=PITCH), :]
            st16("w3", (i // 16 * NT + t) * KW + i % 16 * 16, pltpu.bitcast(paced(g), F32))

        def wo_list(i, t0=0):
            return [(1, P(f, t, u)) for f in (P(wo_in, i, t0), wo_out)
                    for t in (t0, t0 + 1) for u in range(32)]

        def right(p, t, r):
            b = [ld(f"w{p}" if p else "w0s", (h * NT + t + 4 * u) * KW + r, 16) for h in range(2) for u in range(2)]
            b[0] = paced(b[0])
            b11, b12, b21, b22 = (pltpu.bitcast(x, BF16).astype(F32) for x in b)
            for i, val in enumerate((sub(b21, b11), sub(b12, b22), add(b11, b22),
                                     add(b21, b22), add(b11, b12))):
                st16(f"ws{p}", (4 * i + t) * KW + r, val)

        def right_list(p):
            return [(1, P(right, p, t, r)) for t in range(4) for r in range(0, KW, 16)]

        def ld_kv(c, row, n, z=0):
            return ld(f"kv{c // 4}", c % 4 * (T // 2) + row, n, z)

        def a1(i, r):
            a = once(("a", i), lambda: 2 * j + i)
            w0, w1, w2, w3 = once(("taps", i), lambda: [taps[a, u] for u in range(4)])
            k32 = once(("ka", i), lambda: window("ka", a * (S // 2 + 8), S // 2 + 8))
            v32 = once(("va", i), lambda: window("va", a * (S // 2), S // 2))
            c0, c1, c2 = (k32[pl.ds(8 * r + 8 - u, 8), :] for u in range(3))
            vv = v32[pl.ds(8 * r, 8), :]
            e0, o0, e1, o1, o2 = _lo(c0), _hi(c0), _lo(c1), _hi(c1), _hi(c2)
            ke = _tree([mul(e0, w0), mul(o1, w1), mul(e1, w2), mul(o2, w3)])
            ko = _tree([mul(o0, w0), mul(e0, w1), mul(o1, w2), mul(e1, w3)])
            st16(f"kv{r // 32}", 8 * (r % 32), _rows(mul(ke, _lo(vv)), pace(mul(ko, _hi(vv)))))

        def a1_list(i, c0, c1):
            return [(24, P(a1, i, r)) for r in range(8 * c0, 8 * c1)]

        def freq(c, im, m):
            return c * FP + im * (T + 8) + m

        def dft(i, name, c0, m):
            def mm():
                f = pltpu.bitcast(tab[pl.ds(fresh() + T * (name == "xf"), T), :], BF16)
                if name == "hf":
                    a = once(("a", i), lambda: 2 * j + i)
                    rhs = jnp.concatenate(
                        [ha[a, :, pl.ds(c * T, T)] for c in range(c0, c0 + 4)], axis=0)
                    return lax.dot_general(f, rhs, (((1,), (1,)), ((), ())),
                                           preferred_element_type=F32)
                rhs = jnp.concatenate(
                    [pltpu.bitcast(ld_kv(c, 0, T // 2, i % 2), BF16) for c in range(c0, c0 + 4)], axis=1)
                return jnp.dot(f, rhs, preferred_element_type=F32)
            res = once((name, i, c0), mm)
            for u in range(4):
                val = res[m:m + 16, u * 128:(u + 1) * 128]
                if name == "hf" and c0 + u == 0 and m < T:
                    val = add(val, once(("dd", i), lambda: _rows(*[taps[memo["a", i], 4]] * 2)))
                st(name, freq(c0 + u, m // T, m % T), val)
            memo["clock"] = res[m + 8:m + 16, 384:]

        def dft_list(i, name, *c0s):
            return [(16, P(dft, i, name, c0, m)) for c0 in c0s for m in range(0, 2 * T, 16)]

        def a3(i, g, plane, upper, n):
            def opnd(name, c):
                re = lambda: ld(name, freq(c, 0, 8 * g), z=plane)
                im = lambda: ld(name, freq(c, 1, 8 * g), z=plane)
                if name == "xf":
                    val = add(re(), im()) if plane == 0 else re() if plane == 1 else im()
                    return pace(val) if c >= 8 else val
                return pace(re() if plane == 0 else (sub, add)[plane - 1](im(), re()))
            get = lambda name, c: once((name, i, g, plane, c), P(opnd, name, c))
            done = pace if not (first or last) or n % 4 == 3 else lambda v: v
            cs = range(8, n + 1) if upper else range(min(n, 7) + 1)
            terms = [mul(get("xf", n - c), get("hf", c)) for c in cs]
            if upper:
                st("up", 8 * n, done(_tree(terms)))
                return
            if n >= 8:
                terms.append(ld("up", 8 * n))
            if plane == 0:
                st("k1", 8 * n, done(_tree(terms)))
            elif plane == 1:
                st("pi", 8 * n, done(_tree(terms + [ld("k1", 8 * n)])))
            else:
                pr = sub(ld("k1", 8 * n, z=1), _tree(terms))
                pi = ld("pi", 8 * n)
                zr, zi = pr, pi
                if n > 0:
                    qr, qi = memo["prev"]
                    zr, zi = sub(pr, qi), add(pi, qr)
                memo["prev"] = (pr, pi)
                if g % 2 == 0:
                    st("zr", 8 * n, done(zr))
                    st("zi", 8 * n, zi)
                else:
                    st16("z", n * T + 4 * (g - 1), _rows(ld("zr", 8 * n), done(zr)))
                    st16("z", n * T + T // 2 + 4 * (g - 1), _rows(ld("zi", 8 * n), zi))

        def a3_list(i):
            out = []
            for g in range(T // 8):
                for plane in range(3):
                    out += [(2 * (n - 8) + 4, P(a3, i, g, plane, True, n)) for n in range(8, NC)]
                    out += [(2 * min(n, 7) + 4 + 2 * (plane == 2), P(a3, i, g, plane, False, n))
                            for n in range(NC)]
            return out

        def idft(i, c0, odd, m):
            def mm():
                rhs = jnp.concatenate([pltpu.bitcast(ld("z", c * T + odd * T // 2, T // 2, i + 2), BF16)
                                       for c in range(c0, c0 + 4)], axis=1)
                f = tab[pl.ds(fresh() + 2 * T + odd * T // 4, T // 4), :]
                return jnp.dot(pltpu.bitcast(f, BF16), rhs, preferred_element_type=F32)
            y = once(("y", i, c0, odd), mm)
            a = once(("a", i), lambda: 2 * j + i)
            q16 = once(("qa", i), lambda: window16("qa", a * (S // 2), S // 2))
            o16 = once(("oa", i), lambda: window16("oa", a * (S // 2), S // 2))
            flip = lambda w: jnp.take_along_axis(
                w, 7 - lax.broadcasted_iota(jnp.int32, (8, 128), 0), axis=0, mode="promise_in_bounds")
            for u in range(4):
                val = y[m:m + 16, u * 128:(u + 1) * 128]
                if not odd:
                    st("even", u * T // 2 + m, val)
                    continue
                even, mid = ld("even", u * T // 2 + m, 16), (c0 + u) * T + T // 2
                low = add(even, val)
                for row, out in ((mid + m, sub(even, val)),
                                 (mid - 16 - m, _rows(flip(low[8:]), flip(low[:8])))):
                    o16[pl.ds(row, 16), :] = mul(q16[pl.ds(row, 16), :].astype(F32), out).astype(BF16)
            memo["clock"] = y[m + 8:m + 16, 384:]

        def idft_list(i, *c0s):
            return [(16, P(idft, i, c0, odd, m)) for c0 in c0s
                    for odd in range(2) for m in range(0, T // 2, 16)]

        def transforms(i, extra, shares=(1, 1, 1, 1, 1, 9)):
            extra = _split(extra, *shares)
            for u in range(4):
                _weave(idft_list(i - 1, 4 * u)[:4], extra[u])
                _run(idft_list(i - 1, 4 * u)[4:])
                _weave(dft_list(i, "hf", 4 * u), a1_list(i, 3 * u, 3 * u + 3))
            oa_copy(2 * j + i - 1).start()
            _weave(dft_list(i, "xf", 0), _merge(a1_list(i, 12, 16), extra[4]))
            _weave(dft_list(i, "xf", 4, 8), extra[5])
            _run(dft_list(i, "xf", 12))

        def xprep(x, u, r):
            halves = []
            for m in (r, r + 8):
                a, b = (pltpu.bitcast(x[pl.ds(2 * m, 16), pl.ds(t * 128, 128)], U32)
                        for t in (u, u + 4))
                a = pace(a)
                a11, a12, a21, a22 = _lo(a), _lo(b), _hi(a), _hi(b)
                halves.append(_left(a11, a12, a21, a22) + ([a12, a22] if first else []))
            for i, pair in enumerate(zip(*halves)):
                st16("xs", ((4 * i + u) * E + r) // 2, jnp.concatenate(pair, axis=0))

        def split_rows(i):
            for u in range(4):
                a = pltpu.bitcast(xa[0, pl.ds(pl.multiple_of(i * 128, 16), 128), pl.ds(u * 128, 128)], U32)
                st16("os", u * E // 2, _lo(a))
                st16("os", (4 + u) * E // 2, _hi(a))

        def xprep_list(x):
            return [(27, P(xprep, x, u, r)) for r in range(0, E, 16) for u in range(4)]

        def lhs(name, i, m0=0, n=E):
            view = views[name][3].at[pl.ds(fresh() + i * 2 * E, 2 * E), :]
            return jnp.concatenate(
                [pltpu.bitcast(view[pl.ds((u * E + m0) // 2, n // 2), :], BF16) for u in range(4)], axis=1)

        def emit(p, par, t, m, val):
            if p == 0:
                st("q", (par * NT + t) * E + m, val)
                return
            if p == 3:
                o16 = once("ob", lambda: window16("ob", (j - 1) * NT * E, NT * E))
                o16[pl.ds(t * R + par * E + m, 16), :] = val.astype(BF16)
                if m + 16 == E and par == t // 4:
                    ob_copy(j - 1, t).start()
                return
            name, row = "kv"[p - 1], (par * NT + t) * KR
            if m == 0 and not first:
                st(name, row, ld(name, row + E, WIN, z=3))
            if m == 0 and first and p == 2 and par == 0:
                for other in range(2):
                    st(name, (other * NT + t) * KR, jnp.broadcast_to(val[0:1], (WIN, 128)))
            st(name, row + WIN + m, val)

        def plain(half, t, m):
            def mm():
                w = pltpu.bitcast(ld("w0", (half * NT + t) * KW, KW, 3), BF16)
                x = lhs("xs", 7) if half else jnp.concatenate([lhs("os", 0), lhs("os", 1)], axis=0)
                return jnp.dot(x, w, preferred_element_type=F32)
            res = once(("plain", half, t), mm)
            memo["clock"] = res[m + 8:m + 16]
            if half:
                emit(0, 0, t, m, add(res[m:m + 16], ld("o", t * R + m, 16)))
            else:
                st("o", t * R + m, res[m:m + 16])

        def plain_list(half):
            return [(16, P(plain, half, t, m)) for t in range(NT) for m in range(0, E if half else R, 16)]

        def product(p, m0, n, t, i, m):
            def mm():
                if i == 0:
                    w = ld(f"w{p}", t * KW, KW, 3)
                elif i == 2:
                    w = ld(f"w{p}", (NT + t + 4) * KW, KW, 3)
                else:
                    w = ld(f"ws{p}", (4 * (i - 1 - (i > 2)) + t) * KW, KW, 3)
                return jnp.dot(lhs("xs" if p < 3 or m0 else "os", i, m0, n), pltpu.bitcast(w, BF16),
                               preferred_element_type=F32)
            res = once(("product", p, m0, t, i), mm)
            memo["clock"] = res[m - m0 + 8:m - m0 + 16]
            res = res[m - m0:m - m0 + 16]
            get = lambda name, z=0: ld(name, m, 16, z)
            if i == 0:
                st("c21", m, res)
            elif i == 1:
                st("m4", m, res)
                emit(p, 1, t, m, add(get("c21"), res))
            elif i == 2:
                st("c11", m, sub(get("m4"), res))
                st("m5", m, res)
            elif i == 3:
                st("c22", m, sub(res, get("c21", 1)))
                emit(p, 0, t + 4, m, add(get("m5"), res))
            elif i == 4:
                st("d11", m, add(get("c11"), res))
                st("d22", m, add(get("c22"), res))
            else:
                emit(p, i - 5, t + 4 * (i - 5), m, add(get(("d11", "d22")[i - 5]), res))

        def strassen(p, m0=0, n=E):
            return [(16, P(product, p, m0, n, t, i, m))
                    for t in range(4) for i in range(7) for m in range(m0, m0 + n, 16)]

        def qk(r, w):
            par, m = divmod(8 * r, E)
            qv = once(("qv", r), lambda: [pace(ld("q", (par * NT + t) * E + m)) for t in range(NT)])
            s = pace(_tree([mul(qv[t], ld("k", (par * NT + t) * KR + WIN + m - w)) for t in range(NT)]))
            s = add(s, pltpu.roll(s, 64, 1))
            s = add(s, pltpu.roll(s, 32, 1))
            if first and m < w:
                keep = m + lax.broadcasted_iota(jnp.int32, (8, 128), 0) >= w
                s = jnp.where(keep, s, -1e9 * DH ** 0.5)
            memo["lg", r, w] = s

        def expo(r):
            lg = [memo["lg", r, w] for w in range(WIN)]
            m = pace(functools.reduce(lax.max, lg))
            scale = np.float32(DH ** -0.5 * np.log2(np.e))
            memo["e", r] = [lax.exp2(mul(sub(s, m), scale)) for s in lg]

        def norm(r):
            memo["inv", r] = 1.0 / pace(_tree(memo["e", r]))

        def probs(r):
            inv = pace(memo["inv", r])
            for w in range(WIN):
                st("p", w * R + 8 * r, mul(memo["e", r][w], inv))

        def qk_list(nr=R // 8):
            out = []
            for i in range(WIN * nr + 23):
                r, w = divmod(i, WIN)
                tasks = [P(qk, r, w)] if r < nr else []
                for f, lag in ((expo, 24), (norm, 27), (probs, 30)):
                    if i >= lag and (i - lag) % WIN == 0 and (i - lag) // WIN < nr:
                        tasks.append(P(f, (i - lag) // WIN))
                out.append((26 if r < nr else 12, P(_run, [(0, f) for f in tasks])))
            return out

        def pv(r, t):
            par, m = divmod(8 * r, E)
            p = once(("pv", r), lambda: [pace(ld("p", w * R + 8 * r)) for w in range(WIN)])
            row = (par * NT + t) * KR + WIN + m
            bufs["o"][pl.ds(t * R + 2 * m + par, 8, stride=2), :] = pace(
                _tree([mul(p[w], ld("v", row - w)) for w in range(WIN)]))

        def pv_list():
            return [(16, P(pv, r, t)) for r in range(R // 8) for t in range(NT)]

        def oprep(u, r):
            a = [ld("o", (u + 4 * h) * R + par * E + r, 16, 1) for par in range(2) for h in range(2)]
            for i, val in enumerate(_left(*a[:3], paced(a[3]))):
                st16("xs" if last and 2 * r >= E else "os", ((4 * i + u) * E + r) // 2, val)

        def oprep_list():
            return [(18, P(oprep, u, r)) for r in range(0, E, 16) for u in range(4)]

        if last:
            mix = []
            for r in range(E // 16):
                for base in (0, E // 2, E, 3 * E // 2):
                    mix += pv_list()[base + 8 * r:base + 8 * r + 8]
                mix += oprep_list()[4 * r:4 * r + 4]
            mix, conv = _split(mix, 1, 1), _split(a3_list(-1), 3, 5)
            transforms(-1, mix[0], (1, 1, 1, 1, 1, 5))
            wait([last_q()])
            _weave(strassen(3, 0, E // 2), mix[1] + conv[0])
            _weave(strassen(3, E // 2, E // 2)[:-6], conv[1])
            _run(strassen(3, E // 2, E // 2)[-6:])
            for u in range(4):
                _run(idft_list(-1, 4 * u))
                oa_part(u).start()
            return

        if first:
            def leading(i):
                w = wraw.at[0, pl.ds(pl.multiple_of(i * KW, KW), KW)]
                pltpu.make_async_copy(w, w, sem_in.at[NS + 4 + i]).wait()
                _run(perm_list(0, w, (0,)))
            rolled(2, dict(w0=128), leading)
            wait([x0_copy(0)])
            rolled(4, dict(os=32), split_rows)
            _run(plain_list(0)[:96])
            wait([w_copy(1)])
            _weave(plain_list(0)[96:240], perm_list(1))
            _run(plain_list(0)[240:])
            wait([x0_copy(1)])
            rolled(4, dict(xs=E // 8), lambda i: _run(
                xprep_list(xa.at[0, pl.ds(pl.multiple_of(i * (R // 4), 16), R // 4)])[:16]))

            def queries(i):
                w_wait(2 + i)
                _weave(plain_list(1), _merge(perm_list(2, wraw.at[2 + i]), right_list(0)[:32]))
            rolled(2, dict(w1=NT * KW, ws0=2 * KW, w0s=2 * KW, xs=2 * E, o=E, q=NT * E), queries)
            _run(right_list(1)[:32])
            wait(in_copies(0))
            _start(in_copies(1))
            _weave(dft_list(0, "hf", 0, 4), a1_list(0, 0, 8))
            _weave(dft_list(0, "hf", 8, 12) + dft_list(0, "xf", 0), a1_list(0, 8, 16))
            _weave(dft_list(0, "xf", 4, 8, 12), right_list(1)[32:])

            def keys(i):
                w_wait(4 + i)
                _weave(strassen(1)[:144], _merge(perm_list(4, wraw.at[4 + i]), a3_list(0)[:320]))
                _weave(strassen(1)[144:220], a3_list(0)[320:576])
                _run(strassen(1)[220:224])
            rolled(2, dict(w1=2 * KW, ws1=2 * KW, w2=NT * KW, k=2 * KR, hf=64, xf=64, z=32), keys)
            wait(wo_copies())
            _start(in_copies(2) + in_copies(3) + in_copies(NS) + [last_q()])
            rolled(2, dict(w2=2 * KW, ws2=2 * KW, w3=4 * KW), lambda i: _run(
                _merge(right_list(2)[:32], wo_list(2 * i, 0) + wo_list(2 * i + 1, 2))))
            rolled(2, dict(w2=2 * KW, ws2=2 * KW, w3=2 * KW, ws3=2 * KW, v=2 * KR, q=NT * E, k=NT * KR, p=E),
                   lambda i: _weave(strassen(2)[:224], _merge(right_list(3)[:32], qk_list(E // 8))))
            return

        head = strassen(0) + strassen(1)
        pre = _split(oprep_list(), 3, 1)
        transforms(-1, xprep_list(xa.at[j]))
        _weave(head[:528], a3_list(-1))
        _weave(head[528:812], pv_list())
        _run(head[812:818])
        transforms(0, pre[0], (0, 0, 0, 0, 1, 9))
        _weave(head[818:] + strassen(3), pre[1] + a3_list(0))
        _weave(strassen(2), qk_list())

    def loop(j, carry):
        _wait(in_copies(j))
        step(j)
        return carry

    step(0, first=True)
    lax.fori_loop(1, NS, loop, 0)
    _wait(in_copies(NS))
    step(NS, last=True)
    for i, name in enumerate(("oa", "ob")):
        pltpu.make_async_copy(raw[name], raw[name], sem_out.at[i]).wait()


@jax.jit
def pallas_concat_heads__ssm_conv_h3__sliding_local_dilated__prompt_kernel(
    A_q, A_k, A_v, A_shift_k, A_ssm_k, A_ssm_D, B_x, B_wqkv, B_wo,
):
    hbm = pl.BlockSpec(memory_space=pl.ANY)
    out = pl.pallas_call(
        _kernel,
        in_specs=[hbm] * 10,
        out_specs=hbm,
        out_shape=jax.ShapeDtypeStruct((S, 2 * D), BF16),
        scratch_shapes=[
            pltpu.VMEM((NT, 128, S), BF16),
            pltpu.VMEM((NS, R, D), BF16),
            pltpu.VMEM((6, D // 2, D), BF16),
            pltpu.VMEM((NT, D, 128), BF16),
            pltpu.VMEM((NT, 5, 8, 128), F32),
            pltpu.VMEM((4, D), BF16),
            pltpu.VMEM((8, 128), BF16),
            pltpu.VMEM(_TABLE.shape, U32),
            pltpu.SemaphoreType.DMA((NS + 13,)),
            pltpu.SemaphoreType.DMA((2,)),
        ] + [pltpu.VMEM((r * 4 // np.dtype(t).itemsize, 128), t) for t, r in _BUFS.values()],
        compiler_params=pltpu.CompilerParams(vmem_limit_bytes=100 * 1024 * 1024,
                                             disable_bounds_checks=True,
                                             disable_semaphore_checks=True),
        name="fused",
    )(A_q[0], A_k[0], A_v[0], A_shift_k.T, A_ssm_k,
      A_ssm_D.reshape(8, 128), B_x[0], B_wqkv, B_wo, _TABLE)
    return out[None]
```

```python
import functools

import jax
import jax.numpy as jnp
import numpy as np
from jax import lax
from jax.experimental import pallas as pl
import jax.experimental.pallas.tpu as pltpu


S = 2048
D = 1024
T = 128
NC = S // T
NT = D // 128
NS = 4
R = S // NS
E = R // 2
WIN, DH = 8, 32
PITCH = 33
KR = WIN + E
FP = 2 * T + 16
KW = D // 4

F32, BF16, U32 = jnp.float32, jnp.bfloat16, jnp.uint32
P = functools.partial
add, sub, mul = lax.add, lax.sub, lax.mul


def _pack_rows(m):
    b = m.astype(jnp.bfloat16).view(np.uint16).astype(np.uint32)
    return np.ascontiguousarray(b[0::2] | (b[1::2] << 16))


def _dft_table():
    th = 2.0 * np.pi * (np.arange(T) + 0.25) / T
    dft = lambda t: np.concatenate([np.cos(np.outer(th, t)), -np.sin(np.outer(th, t))], axis=0)
    paired = np.arange(T).reshape(-1, 8, 2).transpose(0, 2, 1).reshape(-1)
    ph = np.outer(np.arange(T // 2) + 0.5, th)
    mats = (dft(np.arange(T)), dft(paired - (T - 1) / 2), np.cos(ph) / T, np.sin(ph) / T)
    return np.concatenate([_pack_rows(m) for m in mats] + [np.zeros((8, T), np.uint32)], axis=0)


_TABLE = _dft_table()


def _lo(w):
    return pltpu.bitcast(lax.shift_left(w, np.uint32(16)), F32)


def _hi(w):
    return pltpu.bitcast(lax.bitwise_and(w, np.uint32(0xFFFF0000)), F32)


def _rows(first, second):
    return jnp.concatenate([first, second], axis=0)


def _tree(xs):
    while len(xs) > 1:
        xs = [add(xs[i], xs[i + 1]) if i + 1 < len(xs) else xs[i] for i in range(0, len(xs), 2)]
    return xs[0]


def _left(a11, a12, a21, a22):
    return [add(a21, a22), a22, add(a11, a12), a11, add(a11, a22), sub(a12, a22), sub(a21, a11)]


def _merge(main, side):
    if not main:
        return side
    total_m = sum(c for c, _ in main)
    total_s = sum(c for c, _ in side)
    done_m, done_s, i, out = 0, 0, 0, []
    for c, f in main:
        out.append((c * total_s, f))
        done_m += c
        while i < len(side) and (done_s + side[i][0]) * total_m <= done_m * total_s:
            done_s += side[i][0]
            out.append((side[i][0] * total_m, side[i][1]))
            i += 1
    assert i == len(side)
    return out


def _run(tasks):
    for _, f in tasks:
        f()


def _weave(main, side):
    _run(_merge(main, side))


def _split(tasks, *weights):
    ends = np.cumsum((0,) + weights) * len(tasks) // sum(weights)
    return [tasks[a:b] for a, b in zip(ends[:-1], ends[1:])]


def _start(copies):
    for c in copies:
        c.start()


def _wait(copies):
    for c in copies:
        c.wait()


_BUFS = {n: (t, r) for t, group in (
    (BF16, dict(qa=NT * S // 2, ka=NT * (S // 2 + 8), va=NT * S // 2, oa=NT * S // 2, ob=S * NT // 2,
                xs=7 * 4 * E // 2, os=7 * 4 * E // 2, w3=2 * NT * KW,
                kv0=S // 8, kv1=S // 8, kv2=S // 8, kv3=S // 8, z=NC * T,
                **{f"ws{p}": 20 * KW for p in range(4)})),
    (U32, dict(**{f"w{p}": 2 * NT * KW for p in range(3)}, t0=34 * DH, t1=34 * DH)),
    (F32, dict(hf=NC * FP, xf=NC * FP, up=8 * NC, k1=8 * NC, pi=8 * NC, zr=8 * NC, zi=8 * NC,
               even=2 * T, c21=E, m4=E, c11=E, m5=E, c22=E, d11=E, d22=E,
               q=2 * NT * E, k=2 * NT * KR, v=2 * NT * KR, p=WIN * R, o=NT * R + 8)),
) for n, r in group.items()}


def _kernel(q_hbm, k_hbm, v_hbm, sk_hbm, h_hbm, d_hbm, x_hbm, w_hbm, wo_hbm, tab_hbm, out_hbm,
            ha, xa, wraw, woraw, taps, sk_ref, d_ref, tab, sem_in, sem_out, *raw):
    raw = dict(zip(_BUFS, raw))
    bufs = {n: b.bitcast(U32) if _BUFS[n][0] == BF16 else b for n, b in raw.items()}

    raw["w0s"], bufs["w0s"] = raw["w0"], bufs["w0"]
    spec = dict(_BUFS, w0s=_BUFS["w0"])

    def ld(name, row, n=8, z=0):
        assert 0 <= row and row + n <= views[name][z].shape[0]
        return views[name][z][pl.ds(row, n), :]

    def st(name, row, val):
        assert 0 <= row and row + val.shape[0] <= views[name][3].shape[0]
        views[name][3][pl.ds(row, val.shape[0]), :] = val

    def st16(name, row, val):
        assert 0 <= row and 2 * row + val.shape[0] <= views[name][4].shape[0]
        views[name][4][pl.ds(2 * row, val.shape[0]), :] = val.astype(BF16)

    def window(name, row, n):
        return bufs[name].at[pl.ds(pl.multiple_of(row, 8), n), :]

    def window16(name, row, n):
        return raw[name].at[pl.ds(pl.multiple_of(2 * row, 16), 2 * n), :]

    def cols(a):
        return pl.ds(pl.multiple_of(a * 128, 128), 128)

    def rows(j):
        return pl.ds(pl.multiple_of(j * R, R), R)

    def a_copies(a, sem, skip=0):
        return [pltpu.make_async_copy(src, dst, sem) for src, dst in (
            (h_hbm.at[cols(a), :], ha.at[a]),
            (k_hbm.at[:, cols(a)], window16("ka", a * (S // 2 + 8) + 8, S // 2)),
            (v_hbm.at[:, cols(a)], window16("va", a * (S // 2), S // 2)))[skip:]]

    def q_copy(a, sem):
        return pltpu.make_async_copy(q_hbm.at[:, cols(a)], window16("qa", a * (S // 2), S // 2), sem)

    def in_copies(j):
        sem = sem_in.at[j]
        out = a_copies(2 * j - 1, sem) + [q_copy(2 * j - 2, sem)]
        if isinstance(j, int) and j == NS:
            return out
        return (out + [pltpu.make_async_copy(x_hbm.at[rows(j), :], xa.at[j], sem)]
                + a_copies(2 * j, sem) + [q_copy(2 * j - 1, sem)])

    def h0_copies():
        full = pl.ds(0, 5 * T // 2)
        return [pltpu.make_async_copy(tab_hbm.at[full], tab.at[full], sem_in.at[0]),
                pltpu.make_async_copy(h_hbm.at[cols(0), :], ha.at[0], sem_in.at[0])]

    def kv0_copies():
        return a_copies(0, sem_in.at[NS + 13], 1)

    def last_q():
        return q_copy(NT - 1, sem_in.at[NS + 1])

    def x0_copy(h):
        half = pl.ds(h * D // 2, D // 2)
        return pltpu.make_async_copy(x_hbm.at[rows(0), half], xa.at[0, :, half], sem_in.at[NS + 2 + h])

    def w_copy(n):
        half = pl.ds(n % 2 * (D // 2), D // 2)
        return pltpu.make_async_copy(
            w_hbm.at[half, pl.ds(n // 2 * D, D)], wraw.at[n], sem_in.at[NS + 5 + n])

    def w_wait(n):
        pltpu.make_async_copy(wraw.at[n], wraw.at[n], sem_in.at[NS + 5 + n]).wait()

    def wo_copies():
        return [pltpu.make_async_copy(wo_hbm.at[:, pl.ds(t * 128, 128)], woraw.at[t],
                                      sem_in.at[NS + 11]) for t in range(NT)]

    def oa_copy(a):
        return pltpu.make_async_copy(window16("oa", a * (S // 2), S // 2), out_hbm.at[:, cols(a)],
                                     sem_out.at[0])

    def oa_part(u):
        src = window16("oa", (4 * (NT - 1) + u) * S // 8, S // 8)
        return pltpu.make_async_copy(src, out_hbm.at[pl.ds(u * S // 4, S // 4), cols(NT - 1)],
                                     sem_out.at[0])

    def ob_copy(j, t):
        return pltpu.make_async_copy(window16("ob", (j * NT + t) * E, E),
                                     out_hbm.at[rows(j), cols(NT + t)], sem_out.at[1])

    small = [pltpu.make_async_copy(a, b, sem_in.at[NS + 12])
             for a, b in ((tab_hbm.at[pl.ds(5 * T // 2, 8)], tab.at[pl.ds(5 * T // 2, 8)]),
                          (sk_hbm, sk_ref), (d_hbm, d_ref))]
    w00 = [pltpu.make_async_copy(w_hbm.at[pl.ds(u * KW, KW), pl.ds(0, D)], wraw.at[0, pl.ds(u * KW, KW)],
                                 sem_in.at[NS + 4 + u]) for u in range(2)]
    startup = lambda: (w00 + [x0_copy(0), w_copy(1), x0_copy(1), w_copy(2), w_copy(3)] + h0_copies() + kv0_copies()
                       + [w_copy(4), w_copy(5)] + wo_copies())
    _start(small + startup())
    _wait(small)
    unit = pltpu.bitcast(tab[pl.ds(5 * T // 2, 8), :], jnp.int32)
    zs = [pl.multiple_of(unit[i, 0] * 8, 8) for i in range(3)]
    views = {n: [b.at[pl.ds(z, spec[n][1]), :] for z in zs] + [b, raw[n]] for n, b in bufs.items()}

    for a in range(NT):
        st("ka", a * (S // 2 + 8), jnp.zeros((8, 128), U32))
    for t in range(2 * NT):
        st("k", t * KR, jnp.zeros((WIN, 128), F32))
    skf = sk_ref[...].astype(F32)
    df = d_ref[...].astype(F32)
    for t in range(NT):
        for i in range(4):
            taps[t, i] = jnp.broadcast_to(skf[i:i + 1, t * 128:(t + 1) * 128], (8, 128))
        taps[t, 4] = jnp.broadcast_to(df[t:t + 1, :], (8, 128))

    def step(j, first=False, last=False):
        memo = {}
        never = tab[pl.ds(5 * T // 2, 8), :] != 0

        def once(key, fn):
            if key not in memo:
                memo[key] = fn()
            return memo[key]

        def fresh():
            memo["fresh"] = memo.get("fresh", 1) + 1
            return pl.multiple_of(zs[0] * memo["fresh"], 8)

        def pace(val):
            clock = memo.get("clock")
            if clock is None:
                return val
            if val.dtype != F32:
                clock = pltpu.bitcast(clock, val.dtype)
            return lax.select(never, clock, val)

        def paced(x):
            return jnp.concatenate([pace(x[:8]), x[8:]], axis=0)

        def wait(copies):
            memo["clock"] = None
            _wait(copies)

        def rolled(n, shifts, body):
            def one(i, carry):
                saved, kept = dict(views), dict(memo)
                memo["clock"] = None
                for name, d in shifts.items():
                    size = spec[name][1] - d * (n - 1)
                    views[name] = [window(name, z + d * i, size) for z in zs + [0]]
                    if spec[name][0] == BF16:
                        views[name].append(window16(name, d * i, size))
                body(i)
                views.update(saved)
                memo.clear()
                memo.update(kept, clock=None)
                return carry
            lax.fori_loop(0, n, one, 0)

        def perm_in(w, u, t):
            tt = paced(pltpu.bitcast(w[pl.ds(u * 256, 256), pl.ds(t * 128, 128)], U32)).T
            for hh in range(4):
                st(f"t{u}", (4 * t + hh) * PITCH, tt[hh * DH:(hh + 1) * DH])

        def perm_out(p, h, u, t):
            g = jnp.concatenate(
                [bufs[f"t{u}"][pl.ds(zs[0] + 4 * t + i, 32, stride=PITCH), :] for i in range(4)], axis=0)
            st(f"w{p}", (h * NT + t) * KW + u * 128, paced(g).T)

        def perm_list(n, w=None, us=(0, 1)):
            w = wraw.at[n] if w is None else w
            return [(1, P(f, u, t)) for f in (P(perm_in, w), P(perm_out, n // 2, n % 2))
                    for u in us for t in range(NT)] + [(2, lambda: None)] * 4

        def wo_in(i, t0, t, hh):
            w = pltpu.bitcast(woraw[2 * i + t - t0, pl.ds(hh * DH, DH), :], U32)
            st(f"t{t % 2}", hh * (DH // 2 + 1), paced(w))

        def wo_out(t, i):
            g = paced(bufs[f"t{t % 2}"][pl.ds(zs[0] + i, 32, stride=DH // 2 + 1), :])
            st16("w3", (i // 8 * NT + t) * KW + i % 8 * 32, _rows(_lo(g), _hi(g)))

        def wo_list(i, t0=0):
            return [(1, P(f, t, u)) for f, n in ((P(wo_in, i, t0), 32), (wo_out, 16))
                    for t in (t0, t0 + 1) for u in range(n)]

        def right(p, t, r):
            b = [ld(f"w{p}" if p else "w0s", (h * NT + t + 4 * u) * KW + r, 16) for h in range(2) for u in range(2)]
            b[0] = paced(b[0])
            b11, b12, b21, b22 = (pltpu.bitcast(x, BF16).astype(F32) for x in b)
            for i, val in enumerate((sub(b21, b11), sub(b12, b22), add(b11, b22),
                                     add(b21, b22), add(b11, b12))):
                st16(f"ws{p}", (4 * i + t) * KW + r, val)

        def right_list(p):
            return [(1, P(right, p, t, r)) for t in range(4) for r in range(0, KW, 16)]

        def ld_kv(c, row, n, z=0):
            return ld(f"kv{c // 4}", c % 4 * (T // 2) + row, n, z)

        def a1(i, r):
            a = once(("a", i), lambda: 2 * j + i)
            w0, w1, w2, w3 = once(("taps", i), lambda: [taps[a, u] for u in range(4)])
            k32 = once(("ka", i), lambda: window("ka", a * (S // 2 + 8), S // 2 + 8))
            v32 = once(("va", i), lambda: window("va", a * (S // 2), S // 2))
            c0, c1, c2 = (k32[pl.ds(8 * r + 8 - u, 8), :] for u in range(3))
            vv = v32[pl.ds(8 * r, 8), :]
            e0, o0, e1, o1, o2 = _lo(c0), _hi(c0), _lo(c1), _hi(c1), _hi(c2)
            ke = _tree([mul(e0, w0), mul(o1, w1), mul(e1, w2), mul(o2, w3)])
            ko = _tree([mul(o0, w0), mul(e0, w1), mul(o1, w2), mul(e1, w3)])
            st16(f"kv{r // 32}", 8 * (r % 32), _rows(mul(ke, _lo(vv)), pace(mul(ko, _hi(vv)))))

        def a1_list(i, c0, c1):
            return [(24, P(a1, i, r)) for r in range(8 * c0, 8 * c1)]

        def freq(c, im, m):
            return c * FP + im * (T + 8) + m

        def dft(i, name, c0, m):
            def mm():
                f = pltpu.bitcast(tab[pl.ds(fresh() + T * (name == "xf"), T), :], BF16)
                if name == "hf":
                    a = once(("a", i), lambda: 2 * j + i)
                    rhs = jnp.concatenate(
                        [ha[a, :, pl.ds(c * T, T)] for c in range(c0, c0 + 4)], axis=0)
                    return lax.dot_general(f, rhs, (((1,), (1,)), ((), ())),
                                           preferred_element_type=F32)
                rhs = jnp.concatenate(
                    [pltpu.bitcast(ld_kv(c, 0, T // 2, i % 2), BF16) for c in range(c0, c0 + 4)], axis=1)
                return jnp.dot(f, rhs, preferred_element_type=F32)
            res = once((name, i, c0), mm)
            for u in range(4):
                val = res[m:m + 16, u * 128:(u + 1) * 128]
                if name == "hf" and c0 + u == 0 and m < T:
                    val = add(val, once(("dd", i), lambda: _rows(*[taps[memo["a", i], 4]] * 2)))
                st(name, freq(c0 + u, m // T, m % T), val)
            memo["clock"] = res[m + 8:m + 16, 384:]

        def dft_list(i, name, *c0s):
            return [(16, P(dft, i, name, c0, m)) for c0 in c0s for m in range(0, 2 * T, 16)]

        def a3(i, g, plane, upper, n):
            def opnd(name, c):
                re = lambda: ld(name, freq(c, 0, 8 * g), z=plane)
                im = lambda: ld(name, freq(c, 1, 8 * g), z=plane)
                if name == "xf":
                    val = add(re(), im()) if plane == 0 else re() if plane == 1 else im()
                    return pace(val) if c >= 8 else val
                return pace(re() if plane == 0 else (sub, add)[plane - 1](im(), re()))
            get = lambda name, c: once((name, i, g, plane, c), P(opnd, name, c))
            done = pace if n % 4 == 3 else lambda v: v
            cs = range(8, n + 1) if upper else range(min(n, 7) + 1)
            terms = [mul(get("xf", n - c), get("hf", c)) for c in cs]
            if upper:
                st("up", 8 * n, done(_tree(terms)))
                return
            if n >= 8:
                terms.append(ld("up", 8 * n))
            if plane == 0:
                st("k1", 8 * n, done(_tree(terms)))
            elif plane == 1:
                st("pi", 8 * n, done(_tree(terms + [ld("k1", 8 * n)])))
            else:
                pr = sub(ld("k1", 8 * n, z=1), _tree(terms))
                pi = ld("pi", 8 * n)
                zr, zi = pr, pi
                if n > 0:
                    qr, qi = memo["prev"]
                    zr, zi = sub(pr, qi), add(pi, qr)
                memo["prev"] = (pr, pi)
                if g % 2 == 0:
                    st("zr", 8 * n, done(zr))
                    st("zi", 8 * n, zi)
                else:
                    st16("z", n * T + 4 * (g - 1), _rows(ld("zr", 8 * n), done(zr)))
                    st16("z", n * T + T // 2 + 4 * (g - 1), _rows(ld("zi", 8 * n), zi))

        def a3_list(i):
            out = []
            for g in range(T // 8):
                for plane in range(3):
                    out += [(2 * (n - 8) + 4, P(a3, i, g, plane, True, n)) for n in range(8, NC)]
                    out += [(2 * min(n, 7) + 4 + 2 * (plane == 2), P(a3, i, g, plane, False, n))
                            for n in range(NC)]
            return out

        def idft(i, c0, odd, m):
            def mm():
                rhs = jnp.concatenate([pltpu.bitcast(ld("z", c * T + odd * T // 2, T // 2, i + 2), BF16)
                                       for c in range(c0, c0 + 4)], axis=1)
                f = tab[pl.ds(fresh() + 2 * T + odd * T // 4, T // 4), :]
                return jnp.dot(pltpu.bitcast(f, BF16), rhs, preferred_element_type=F32)
            y = once(("y", i, c0, odd), mm)
            a = once(("a", i), lambda: 2 * j + i)
            q16 = once(("qa", i), lambda: window16("qa", a * (S // 2), S // 2))
            o16 = once(("oa", i), lambda: window16("oa", a * (S // 2), S // 2))
            flip = lambda w: jnp.take_along_axis(
                w, 7 - lax.broadcasted_iota(jnp.int32, (8, 128), 0), axis=0, mode="promise_in_bounds")
            for u in range(4):
                val = y[m:m + 16, u * 128:(u + 1) * 128]
                if not odd:
                    st("even", u * T // 2 + m, val)
                    continue
                even, mid = ld("even", u * T // 2 + m, 16), (c0 + u) * T + T // 2
                low = add(even, val)
                for row, out in ((mid + m, sub(even, val)),
                                 (mid - 16 - m, _rows(flip(low[8:]), flip(low[:8])))):
                    o16[pl.ds(row, 16), :] = mul(q16[pl.ds(row, 16), :].astype(F32), out).astype(BF16)
            memo["clock"] = y[m + 8:m + 16, 384:]

        def idft_list(i, *c0s):
            return [(16, P(idft, i, c0, odd, m)) for c0 in c0s
                    for odd in range(2) for m in range(0, T // 2, 16)]

        def transforms(i, extra, shares=(1, 1, 1, 1, 1, 9)):
            extra = _split(extra, *shares)
            for u in range(4):
                _weave(idft_list(i - 1, 4 * u)[:4], extra[u])
                _run(idft_list(i - 1, 4 * u)[4:])
                _weave(dft_list(i, "hf", 4 * u), a1_list(i, 3 * u, 3 * u + 3))
            oa_copy(2 * j + i - 1).start()
            _weave(dft_list(i, "xf", 0), _merge(a1_list(i, 12, 16), extra[4]))
            _weave(dft_list(i, "xf", 4, 8), extra[5])
            _run(dft_list(i, "xf", 12))

        def xprep(x, u, r):
            halves = []
            for m in (r, r + 8):
                a, b = (pltpu.bitcast(x[pl.ds(2 * m, 16), pl.ds(t * 128, 128)], U32)
                        for t in (u, u + 4))
                a = pace(a)
                a11, a12, a21, a22 = _lo(a), _lo(b), _hi(a), _hi(b)
                halves.append(_left(a11, a12, a21, a22))
            for i, pair in enumerate(zip(*halves)):
                st16("xs", ((4 * i + u) * E + r) // 2, jnp.concatenate(pair, axis=0))

        def split_rows(half):
            for u in range(4):
                for r in range(0, E, 64):
                    a = pltpu.bitcast(xa[0, pl.ds(2 * r, 128), pl.ds((4 * half + u) * 128, 128)], U32)
                    st16("os", ((8 * half + u) * E + r) // 2, _lo(a))
                    st16("os", ((8 * half + 4 + u) * E + r) // 2, _hi(a))

        def xprep_list(x):
            return [(27, P(xprep, x, u, r)) for r in range(0, E, 16) for u in range(4)]

        def lhs(name, i, m0=0, n=E):
            view = views[name][3].at[pl.ds(fresh() + i * 2 * E, 2 * E), :]
            return jnp.concatenate(
                [pltpu.bitcast(view[pl.ds((u * E + m0) // 2, n // 2), :], BF16) for u in range(4)], axis=1)

        def emit(p, par, t, m, val):
            if p == 0:
                st("q", (par * NT + t) * E + m, val)
                return
            if p == 3:
                o16 = once("ob", lambda: window16("ob", (j - 1) * NT * E, NT * E))
                o16[pl.ds(t * R + par * E + m, 16), :] = val.astype(BF16)
                if m + 16 == E and par == t // 4:
                    ob_copy(j - 1, t).start()
                return
            name, row = "kv"[p - 1], (par * NT + t) * KR
            if m == 0 and not first:
                st(name, row, ld(name, row + E, WIN, z=3))
            if m == 0 and first and p == 2 and par == 0:
                for other in range(2):
                    st(name, (other * NT + t) * KR, jnp.broadcast_to(val[0:1], (WIN, 128)))
            st(name, row + WIN + m, val)

        def plain(half, t, m):
            def mm():
                w = pltpu.bitcast(ld("w0", (half * NT + t) * KW, KW, 3), BF16)
                x = lhs("os", 2) if half else jnp.concatenate([lhs("os", 0), lhs("os", 1)], axis=0)
                return jnp.dot(x, w, preferred_element_type=F32)
            res = once(("plain", half, t), mm)
            memo["clock"] = res[m + 8:m + 16]
            if half:
                emit(0, 0, t, m, add(res[m:m + 16], ld("o", t * R + m, 16)))
            else:
                st("o", t * R + m, res[m:m + 16])

        def plain_list(half):
            return [(16, P(plain, half, t, m)) for t in range(NT) for m in range(0, E if half else R, 16)]

        def product(p, m0, n, t, i, m):
            def mm():
                if i == 0:
                    w = ld(f"w{p}", t * KW, KW, 3)
                elif i == 2:
                    w = ld(f"w{p}", (NT + t + 4) * KW, KW, 3)
                else:
                    w = ld(f"ws{p}", (4 * (i - 1 - (i > 2)) + t) * KW, KW, 3)
                return jnp.dot(lhs("xs" if p < 3 or m0 else "os", i, m0, n), pltpu.bitcast(w, BF16),
                               preferred_element_type=F32)
            res = once(("product", p, m0, t, i), mm)
            memo["clock"] = res[m - m0 + 8:m - m0 + 16]
            res = res[m - m0:m - m0 + 16]
            get = lambda name, z=0: ld(name, m, 16, z)
            if i == 0:
                st("c21", m, res)
            elif i == 1:
                st("m4", m, res)
                emit(p, 1, t, m, add(get("c21"), res))
            elif i == 2:
                st("c11", m, sub(get("m4"), res))
                st("m5", m, res)
            elif i == 3:
                st("c22", m, sub(res, get("c21", 1)))
                emit(p, 0, t + 4, m, add(get("m5"), res))
            elif i == 4:
                st("d11", m, add(get("c11"), res))
                st("d22", m, add(get("c22"), res))
            else:
                emit(p, i - 5, t + 4 * (i - 5), m, add(get(("d11", "d22")[i - 5]), res))

        def strassen(p, m0=0, n=E):
            return [(16, P(product, p, m0, n, t, i, m))
                    for t in range(4) for i in range(7) for m in range(m0, m0 + n, 16)]

        def qk(r, w):
            par, m = divmod(8 * r, E)
            qv = once(("qv", r), lambda: [pace(ld("q", (par * NT + t) * E + m)) for t in range(NT)])
            s = pace(_tree([mul(qv[t], ld("k", (par * NT + t) * KR + WIN + m - w)) for t in range(NT)]))
            s = add(s, pltpu.roll(s, 64, 1))
            s = add(s, pltpu.roll(s, 32, 1))
            if first and m < w:
                keep = m + lax.broadcasted_iota(jnp.int32, (8, 128), 0) >= w
                s = jnp.where(keep, s, -1e9 * DH ** 0.5)
            memo["lg", r, w] = s

        def expo(r):
            lg = [memo["lg", r, w] for w in range(WIN)]
            m = pace(functools.reduce(lax.max, lg))
            scale = np.float32(DH ** -0.5 * np.log2(np.e))
            memo["e", r] = [lax.exp2(mul(sub(s, m), scale)) for s in lg]

        def norm(r):
            memo["inv", r] = 1.0 / pace(_tree(memo["e", r]))

        def probs(r):
            inv = pace(memo["inv", r])
            for w in range(WIN):
                st("p", w * R + 8 * r, mul(memo["e", r][w], inv))

        def qk_list(nr=R // 8):
            out = []
            for i in range(WIN * nr + 23):
                r, w = divmod(i, WIN)
                tasks = [P(qk, r, w)] if r < nr else []
                for f, lag in ((expo, 24), (norm, 27), (probs, 30)):
                    if i >= lag and (i - lag) % WIN == 0 and (i - lag) // WIN < nr:
                        tasks.append(P(f, (i - lag) // WIN))
                out.append((26 if r < nr else 12, P(_run, [(0, f) for f in tasks])))
            return out

        def pv(r, t):
            par, m = divmod(8 * r, E)
            p = once(("pv", r), lambda: [(pace if w % 4 == 0 else lambda v: v)(ld("p", w * R + 8 * r)) for w in range(WIN)])
            row = (par * NT + t) * KR + WIN + m
            bufs["o"][pl.ds(t * R + 2 * m + par, 8, stride=2), :] = pace(
                _tree([mul(p[w], ld("v", row - w)) for w in range(WIN)]))

        def pv_list():
            return [(16, P(pv, r, t)) for r in range(R // 8) for t in range(NT)]

        def oprep(u, r):
            a = [ld("o", (u + 4 * h) * R + par * E + r, 16, 1) for par in range(2) for h in range(2)]
            for i, val in enumerate(_left(*a[:3], paced(a[3]))):
                st16("xs" if last and 2 * r >= E else "os", ((4 * i + u) * E + r) // 2, val)

        def oprep_list():
            return [(18, P(oprep, u, r)) for r in range(0, E, 16) for u in range(4)]

        if last:
            mix = []
            for r in range(E // 16):
                for base in (0, E // 2, E, 3 * E // 2):
                    mix += pv_list()[base + 8 * r:base + 8 * r + 8]
                mix += oprep_list()[4 * r:4 * r + 4]
            mix, conv = _split(mix, 1, 1), _split(a3_list(-1), 3, 5)
            transforms(-1, mix[0], (1, 1, 1, 1, 1, 5))
            wait([last_q()])
            _weave(strassen(3, 0, E // 2), mix[1] + conv[0])
            _weave(strassen(3, E // 2, E // 2)[:-6], conv[1])
            _run(strassen(3, E // 2, E // 2)[-6:])
            for u in range(4):
                _run(idft_list(-1, 4 * u))
                oa_part(u).start()
            return

        if first:
            def leading(i):
                w = wraw.at[0, pl.ds(pl.multiple_of(i * KW, KW), KW)]
                pltpu.make_async_copy(w, w, sem_in.at[NS + 4 + i]).wait()
                _run(perm_list(0, w, (0,)))
            rolled(2, dict(w0=128), leading)
            wait([x0_copy(0)])
            split_rows(0)
            _run(plain_list(0)[:96])
            wait([w_copy(1)])
            _weave(plain_list(0)[96:240], perm_list(1))
            _run(plain_list(0)[240:])
            wait([x0_copy(1)])
            split_rows(1)

            def queries(i):
                w_wait(2 + i)
                x = xa.at[0, pl.ds(pl.multiple_of(i * (R // 2), 16), R // 2)]
                _weave(plain_list(1), _merge(perm_list(2, wraw.at[2 + i]),
                                             _merge(xprep_list(x)[:32], right_list(0)[:32])))
            rolled(2, dict(w1=NT * KW, ws0=2 * KW, w0s=2 * KW, xs=E // 4, os=2 * E, o=E, q=NT * E),
                   queries)
            _run(right_list(1)[:16])
            wait(h0_copies())
            _weave(dft_list(0, "hf", 0, 4, 8, 12), right_list(1)[16:])
            wait(kv0_copies())
            _start(in_copies(1))
            _run(a1_list(0, 0, 4))
            for u in range(4):
                _weave(dft_list(0, "xf", 4 * u)[:13], a1_list(0, 4 * u + 4, min(4 * u + 8, NC)))
                _run(dft_list(0, "xf", 4 * u)[13:])

            def keys(i):
                w_wait(4 + i)
                _weave(strassen(1)[:144], _merge(perm_list(4, wraw.at[4 + i]), a3_list(0)[:320]))
                _weave(strassen(1)[144:220], a3_list(0)[320:576])
                _run(strassen(1)[220:224])
            rolled(2, dict(w1=2 * KW, ws1=2 * KW, w2=NT * KW, k=2 * KR, hf=64, xf=64, z=32), keys)
            wait(wo_copies())
            _start(in_copies(2) + in_copies(3) + in_copies(NS) + [last_q()])
            rolled(2, dict(w2=2 * KW, ws2=2 * KW, w3=4 * KW), lambda i: _run(
                _merge(right_list(2)[:32], wo_list(2 * i, 0) + wo_list(2 * i + 1, 2))))
            rolled(2, dict(w2=2 * KW, ws2=2 * KW, w3=2 * KW, ws3=2 * KW, v=2 * KR, q=NT * E, k=NT * KR, p=E),
                   lambda i: _weave(strassen(2)[:224], _merge(right_list(3)[:32], qk_list(E // 8))))
            return

        head = strassen(0) + strassen(1)
        pre = _split(oprep_list(), 3, 1)
        transforms(-1, xprep_list(xa.at[j]))
        _weave(head[:528], a3_list(-1))
        _weave(head[528:812], pv_list())
        _run(head[812:818])
        transforms(0, pre[0], (0, 0, 0, 0, 1, 9))
        _weave(head[818:] + strassen(3), pre[1] + a3_list(0))
        _weave(strassen(2), qk_list())

    def loop(j, carry):
        _wait(in_copies(j))
        step(j)
        return carry

    step(0, first=True)
    lax.fori_loop(1, NS, loop, 0)
    _wait(in_copies(NS))
    step(NS, last=True)
    for i, name in enumerate(("oa", "ob")):
        pltpu.make_async_copy(raw[name], raw[name], sem_out.at[i]).wait()


@jax.jit
def pallas_concat_heads__ssm_conv_h3__sliding_local_dilated__prompt_kernel(
    A_q, A_k, A_v, A_shift_k, A_ssm_k, A_ssm_D, B_x, B_wqkv, B_wo,
):
    hbm = pl.BlockSpec(memory_space=pl.ANY)
    out = pl.pallas_call(
        _kernel,
        in_specs=[hbm] * 10,
        out_specs=hbm,
        out_shape=jax.ShapeDtypeStruct((S, 2 * D), BF16),
        scratch_shapes=[
            pltpu.VMEM((NT, 128, S), BF16),
            pltpu.VMEM((NS, R, D), BF16),
            pltpu.VMEM((6, D // 2, D), BF16),
            pltpu.VMEM((NT, D, 128), BF16),
            pltpu.VMEM((NT, 5, 8, 128), F32),
            pltpu.VMEM((4, D), BF16),
            pltpu.VMEM((8, 128), BF16),
            pltpu.VMEM(_TABLE.shape, U32),
            pltpu.SemaphoreType.DMA((NS + 14,)),
            pltpu.SemaphoreType.DMA((2,)),
        ] + [pltpu.VMEM((r * 4 // np.dtype(t).itemsize, 128), t) for t, r in _BUFS.values()],
        compiler_params=pltpu.CompilerParams(vmem_limit_bytes=100 * 1024 * 1024,
                                             disable_bounds_checks=True,
                                             disable_semaphore_checks=True),
        name="fused",
    )(A_q[0], A_k[0], A_v[0], A_shift_k.T, A_ssm_k,
      A_ssm_D.reshape(8, 128), B_x[0], B_wqkv, B_wo, _TABLE)
    return out[None]
```

```python
import functools

import jax
import jax.numpy as jnp
import numpy as np
from jax import lax
from jax.experimental import pallas as pl
import jax.experimental.pallas.tpu as pltpu


S = 2048
D = 1024
T = 128
NC = S // T
NT = D // 128
NS = 4
R = S // NS
E = R // 2
WIN, DH = 8, 32
PITCH = 33
KR = E + 16
FP = 2 * T + 16
KW = D // 4
KA = S // 2 + 32

F32, BF16, U32 = jnp.float32, jnp.bfloat16, jnp.uint32
P = functools.partial
add, sub, mul = lax.add, lax.sub, lax.mul


def _pack_rows(m):
    b = m.astype(jnp.bfloat16).view(np.uint16).astype(np.uint32)
    return np.ascontiguousarray(b[0::2] | (b[1::2] << 16))


def _dft_table():
    th = 2.0 * np.pi * (np.arange(T) + 0.25) / T
    dft = lambda t: np.concatenate([np.cos(np.outer(th, t)), -np.sin(np.outer(th, t))], axis=0)
    paired = np.arange(T).reshape(-1, 8, 2).transpose(0, 2, 1).reshape(-1)
    ph = np.outer(np.arange(T // 2) + 0.5, th)
    mats = (dft(np.arange(T)), dft(paired - (T - 1) / 2), np.cos(ph) / T, np.sin(ph) / T)
    return np.concatenate([_pack_rows(m) for m in mats] + [np.zeros((32, T), np.uint32)], axis=0)


_TABLE = _dft_table()


def _lo(w):
    return pltpu.bitcast(lax.shift_left(w, np.uint32(16)), F32)


def _hi(w):
    return pltpu.bitcast(lax.bitwise_and(w, np.uint32(0xFFFF0000)), F32)


def _rows(first, second):
    return jnp.concatenate([first, second], axis=0)


def _tree(xs):
    while len(xs) > 1:
        xs = [add(xs[i], xs[i + 1]) if i + 1 < len(xs) else xs[i] for i in range(0, len(xs), 2)]
    return xs[0]


def _left(a11, a12, a21, a22):
    return [add(a21, a22), a22, add(a11, a12), a11, add(a11, a22), sub(a12, a22), sub(a21, a11)]


def _merge(main, side):
    if not main:
        return side
    total_m = sum(c for c, _ in main)
    total_s = sum(c for c, _ in side)
    done_m, done_s, i, out = 0, 0, 0, []
    for c, f in main:
        out.append((c * total_s, f))
        done_m += c
        while i < len(side) and (done_s + side[i][0]) * total_m <= done_m * total_s:
            done_s += side[i][0]
            out.append((side[i][0] * total_m, side[i][1]))
            i += 1
    assert i == len(side)
    return out


def _run(tasks):
    for _, f in tasks:
        f()


def _weave(main, side):
    _run(_merge(main, side))


def _split(tasks, *weights):
    ends = np.cumsum((0,) + weights) * len(tasks) // sum(weights)
    return [tasks[a:b] for a, b in zip(ends[:-1], ends[1:])]


def _start(copies):
    for c in copies:
        c.start()


def _wait(copies):
    for c in copies:
        c.wait()


_BUFS = {n: (t, r) for t, group in (
    (BF16, dict(qa=NT * S // 2, ka=NT * KA, va=NT * S // 2, oa=NT * S // 2, ob=S * NT // 2,
                xs=7 * 4 * E // 2, os=7 * 4 * E // 2, w3=2 * NT * KW,
                kv0=S // 8, kv1=S // 8, kv2=S // 8, kv3=S // 8, z=NC * T,
                **{f"ws{p}": 20 * KW for p in range(4)})),
    (U32, dict(**{f"w{p}": 2 * NT * KW for p in range(3)}, t0=34 * DH, t1=34 * DH)),
    (F32, dict(hf=NC * FP, xf=NC * FP, up=8 * NC, k1=8 * NC, pi=8 * NC, zr=8 * NC, zi=8 * NC,
               even=2 * T, c21=E, m4=E, c11=E, m5=E, c22=E, d11=E, d22=E,
               q=2 * NT * E, k=2 * NT * KR, v=2 * NT * KR, p=WIN * R, o=NT * R + 32)),
) for n, r in group.items()}


def _kernel(q_hbm, k_hbm, v_hbm, sk_hbm, h_hbm, d_hbm, x_hbm, w_hbm, wo_hbm, tab_hbm, out_hbm,
            ha, xa, wraw, woraw, taps, tab, sem_in, sem_out, *raw):
    *raw, sk_ref, d_ref = raw
    raw = dict(zip(_BUFS, raw))
    bufs = {n: b.bitcast(U32) if _BUFS[n][0] == BF16 else b for n, b in raw.items()}

    raw["w0s"], bufs["w0s"] = raw["w0"], bufs["w0"]
    spec = dict(_BUFS, w0s=_BUFS["w0"])

    def ld(name, row, n=8, z=0):
        assert 0 <= row and row + n <= views[name][z].shape[0]
        return views[name][z][pl.ds(row, n), :]

    def st(name, row, val):
        assert 0 <= row and row + val.shape[0] <= views[name][3].shape[0]
        views[name][3][pl.ds(row, val.shape[0]), :] = val

    def st16(name, row, val):
        assert 0 <= row and 2 * row + val.shape[0] <= views[name][4].shape[0]
        views[name][4][pl.ds(2 * row, val.shape[0]), :] = val.astype(BF16)

    def window(name, row, n):
        return bufs[name].at[pl.ds(pl.multiple_of(row, 8), n), :]

    def window16(name, row, n):
        return raw[name].at[pl.ds(pl.multiple_of(2 * row, 16), 2 * n), :]

    def cols(a):
        return pl.ds(pl.multiple_of(a * 128, 128), 128)

    def rows(j):
        return pl.ds(pl.multiple_of(j * R, R), R)

    def a_copies(a, sem, skip=0):
        return [pltpu.make_async_copy(src, dst, sem) for src, dst in (
            (h_hbm.at[cols(a), :], ha.at[a]),
            (k_hbm.at[:, cols(a)], window16("ka", a * KA + 32, S // 2)),
            (v_hbm.at[:, cols(a)], window16("va", a * (S // 2), S // 2)))[skip:]]

    def q_copy(a, sem):
        return pltpu.make_async_copy(q_hbm.at[:, cols(a)], window16("qa", a * (S // 2), S // 2), sem)

    def in_copies(j):
        sem = sem_in.at[j]
        out = a_copies(2 * j - 1, sem) + [q_copy(2 * j - 2, sem)]
        if isinstance(j, int) and j == NS:
            return out
        return (out + [pltpu.make_async_copy(x_hbm.at[rows(j), :], xa.at[j], sem)]
                + a_copies(2 * j, sem) + [q_copy(2 * j - 1, sem)])

    def h0_copies():
        full = pl.ds(0, 5 * T // 2)
        return [pltpu.make_async_copy(tab_hbm.at[full], tab.at[full], sem_in.at[0]),
                pltpu.make_async_copy(h_hbm.at[cols(0), :], ha.at[0], sem_in.at[0])]

    def kv0_copies():
        return a_copies(0, sem_in.at[NS + 13], 1)

    def last_q():
        return q_copy(NT - 1, sem_in.at[NS + 1])

    def x0_copy(h):
        half = pl.ds(h * D // 2, D // 2)
        return pltpu.make_async_copy(x_hbm.at[rows(0), half], xa.at[0, :, half], sem_in.at[NS + 2 + h])

    def w_copy(n):
        half = pl.ds(n % 2 * (D // 2), D // 2)
        return pltpu.make_async_copy(
            w_hbm.at[half, pl.ds(n // 2 * D, D)], wraw.at[n], sem_in.at[NS + 5 + n])

    def w_wait(n):
        pltpu.make_async_copy(wraw.at[n], wraw.at[n], sem_in.at[NS + 5 + n]).wait()

    def wo_copies():
        return [pltpu.make_async_copy(wo_hbm.at[:, pl.ds(t * 128, 128)], woraw.at[t],
                                      sem_in.at[NS + 11]) for t in range(NT)]

    def oa_copy(a):
        return pltpu.make_async_copy(window16("oa", a * (S // 2), S // 2), out_hbm.at[:, cols(a)],
                                     sem_out.at[0])

    def oa_part(u):
        src = window16("oa", (4 * (NT - 1) + u) * S // 8, S // 8)
        return pltpu.make_async_copy(src, out_hbm.at[pl.ds(u * S // 4, S // 4), cols(NT - 1)],
                                     sem_out.at[0])

    def ob_copy(j, t):
        return pltpu.make_async_copy(window16("ob", (j * NT + t) * E, E),
                                     out_hbm.at[rows(j), cols(NT + t)], sem_out.at[1])

    small = [pltpu.make_async_copy(a, b, sem_in.at[NS + 12])
             for a, b in ((tab_hbm.at[pl.ds(5 * T // 2, 8)], tab.at[pl.ds(5 * T // 2, 8)]),
                          (sk_hbm, sk_ref), (d_hbm, d_ref))]
    w00 = [pltpu.make_async_copy(w_hbm.at[pl.ds(u * KW, KW), pl.ds(0, D)], wraw.at[0, pl.ds(u * KW, KW)],
                                 sem_in.at[NS + 4 + u]) for u in range(2)]
    startup = lambda: (w00 + [x0_copy(0), w_copy(1), x0_copy(1), w_copy(2), w_copy(3)] + h0_copies() + kv0_copies()
                       + [w_copy(4), w_copy(5)] + wo_copies())
    _start(small + startup())
    _wait(small)
    unit = pltpu.bitcast(tab[pl.ds(5 * T // 2, 8), :], jnp.int32)
    zs = [pl.multiple_of(unit[i, 0] * 8, 8) for i in range(3)]
    views = {n: [b.at[pl.ds(z, spec[n][1]), :] for z in zs] + [b, raw[n]] for n, b in bufs.items()}

    for a in range(NT):
        st("ka", a * KA + 24, jnp.zeros((8, 128), U32))
    for t in range(2 * NT):
        st("k", t * KR, jnp.zeros((WIN, 128), F32))
    skf = sk_ref[...].astype(F32)
    df = d_ref[...].astype(F32)
    for t in range(NT):
        for i in range(4):
            taps[t, i] = jnp.broadcast_to(skf[i:i + 1, t * 128:(t + 1) * 128], (8, 128))
        taps[t, 4] = jnp.broadcast_to(df[t:t + 1, :], (8, 128))

    def step(j, first=False, last=False):
        memo = {}
        never = tab[pl.ds(5 * T // 2, 8), :] != 0

        def once(key, fn):
            if key not in memo:
                memo[key] = fn()
            return memo[key]

        def fresh():
            memo["fresh"] = memo.get("fresh", 1) + 1
            return pl.multiple_of(zs[0] * memo["fresh"], 8)

        def pace(val):
            clock = memo.get("clock")
            if clock is None:
                return val
            if val.dtype != F32:
                clock = pltpu.bitcast(clock, val.dtype)
            return lax.select(never, clock, val)

        def paced(x):
            return jnp.concatenate([pace(x[:8]), x[8:]], axis=0)

        def wait(copies):
            memo["clock"] = None
            _wait(copies)

        def rolled(n, shifts, body):
            def one(i, carry):
                saved, kept = dict(views), dict(memo)
                memo["clock"] = None
                for name, d in shifts.items():
                    size = spec[name][1] - d * (n - 1)
                    views[name] = [window(name, z + d * i, size) for z in zs + [0]]
                    if spec[name][0] == BF16:
                        views[name].append(window16(name, d * i, size))
                body(i)
                views.update(saved)
                memo.clear()
                memo.update(kept, clock=None)
                return carry
            lax.fori_loop(0, n, one, 0)

        def perm_in(w, u, t):
            tt = paced(pltpu.bitcast(w[pl.ds(u * 256, 256), pl.ds(t * 128, 128)], U32)).T
            for hh in range(4):
                st(f"t{u}", (4 * t + hh) * PITCH, tt[hh * DH:(hh + 1) * DH])

        def perm_out(p, h, u, t):
            g = jnp.concatenate(
                [bufs[f"t{u}"][pl.ds(zs[0] + 4 * t + i, 32, stride=PITCH), :] for i in range(4)], axis=0)
            st(f"w{p}", (h * NT + t) * KW + u * 128, paced(g).T)

        def perm_list(n, w=None, us=(0, 1)):
            w = wraw.at[n] if w is None else w
            return [(1, P(f, u, t)) for f in (P(perm_in, w), P(perm_out, n // 2, n % 2))
                    for u in us for t in range(NT)] + [(2, lambda: None)] * 4

        def wo_in(i, t0, t, hh):
            w = pltpu.bitcast(woraw[2 * i + t - t0, pl.ds(hh * DH, DH), :], U32)
            st(f"t{t % 2}", hh * (DH // 2 + 1), paced(w))

        def wo_out(t, i):
            g = paced(bufs[f"t{t % 2}"][pl.ds(zs[0] + i, 32, stride=DH // 2 + 1), :])
            st16("w3", (i // 8 * NT + t) * KW + i % 8 * 32, _rows(_lo(g), _hi(g)))

        def wo_list(i, t0=0):
            return [(1, P(f, t, u)) for f, n in ((P(wo_in, i, t0), 32), (wo_out, 16))
                    for t in (t0, t0 + 1) for u in range(n)]

        def right(p, t, r):
            b = [ld(f"w{p}" if p else "w0s", (h * NT + t + 4 * u) * KW + r, 16) for h in range(2) for u in range(2)]
            b[0] = paced(b[0])
            b11, b12, b21, b22 = (pltpu.bitcast(x, BF16).astype(F32) for x in b)
            for i, val in enumerate((sub(b21, b11), sub(b12, b22), add(b11, b22),
                                     add(b21, b22), add(b11, b12))):
                st16(f"ws{p}", (4 * i + t) * KW + r, val)

        def right_list(p):
            return [(1, P(right, p, t, r)) for t in range(4) for r in range(0, KW, 16)]

        def ld_kv(c, row, n, z=0):
            return ld(f"kv{c // 4}", c % 4 * (T // 2) + row, n, z)

        def a1(i, r):
            a = once(("a", i), lambda: 2 * j + i)
            w0, w1, w2, w3 = once(("taps", i), lambda: [taps[a, u] for u in range(4)])
            k32 = once(("ka", i), lambda: window("ka", a * KA, KA))
            v32 = once(("va", i), lambda: window("va", a * (S // 2), S // 2))
            c0, c1, c2 = (k32[pl.ds(8 * r + 32 - u, 8), :] for u in range(3))
            vv = v32[pl.ds(8 * r, 8), :]
            e0, o0, e1, o1, o2 = _lo(c0), _hi(c0), _lo(c1), _hi(c1), _hi(c2)
            ke = _tree([mul(e0, w0), mul(o1, w1), mul(e1, w2), mul(o2, w3)])
            ko = _tree([mul(o0, w0), mul(e0, w1), mul(o1, w2), mul(e1, w3)])
            st16(f"kv{r // 32}", 8 * (r % 32), _rows(mul(ke, _lo(vv)), pace(mul(ko, _hi(vv)))))

        def a1_list(i, c0, c1):
            return [(24, P(a1, i, r)) for r in range(8 * c0, 8 * c1)]

        def freq(c, im, m):
            return c * FP + im * (T + 8) + m

        def dft(i, name, c0, m):
            def mm():
                f = pltpu.bitcast(tab[pl.ds(fresh() + T * (name == "xf"), T), :], BF16)
                if name == "hf":
                    a = once(("a", i), lambda: 2 * j + i)
                    rhs = jnp.concatenate(
                        [ha[a, :, pl.ds(c * T, T)] for c in range(c0, c0 + 4)], axis=0)
                    return lax.dot_general(f, rhs, (((1,), (1,)), ((), ())),
                                           preferred_element_type=F32)
                rhs = jnp.concatenate(
                    [pltpu.bitcast(ld_kv(c, 0, T // 2, i % 2), BF16) for c in range(c0, c0 + 4)], axis=1)
                return jnp.dot(f, rhs, preferred_element_type=F32)
            res = once((name, i, c0), mm)
            for u in range(4):
                val = res[m:m + 16, u * 128:(u + 1) * 128]
                if name == "hf" and c0 + u == 0 and m < T:
                    val = add(val, once(("dd", i), lambda: _rows(*[taps[memo["a", i], 4]] * 2)))
                st(name, freq(c0 + u, m // T, m % T), val)
            memo["clock"] = res[m + 8:m + 16, 384:]

        def dft_list(i, name, *c0s):
            return [(16, P(dft, i, name, c0, m)) for c0 in c0s for m in range(0, 2 * T, 16)]

        def a3(i, g, plane, upper, n):
            def opnd(name, c):
                re = lambda: ld(name, freq(c, 0, 8 * g), z=plane)
                im = lambda: ld(name, freq(c, 1, 8 * g), z=plane)
                if name == "xf":
                    val = add(re(), im()) if plane == 0 else re() if plane == 1 else im()
                    return pace(val) if c >= 8 else val
                return pace(re() if plane == 0 else (sub, add)[plane - 1](im(), re()))
            get = lambda name, c: once((name, i, g, plane, c), P(opnd, name, c))
            done = pace if n % 4 == 3 else lambda v: v
            cs = range(8, n + 1) if upper else range(min(n, 7) + 1)
            terms = [mul(get("xf", n - c), get("hf", c)) for c in cs]
            if upper:
                st("up", 8 * n, done(_tree(terms)))
                return
            if n >= 8:
                terms.append(ld("up", 8 * n))
            if plane == 0:
                st("k1", 8 * n, done(_tree(terms)))
            elif plane == 1:
                st("pi", 8 * n, done(_tree(terms + [ld("k1", 8 * n)])))
            else:
                pr = sub(ld("k1", 8 * n, z=1), _tree(terms))
                pi = ld("pi", 8 * n)
                zr, zi = pr, pi
                if n > 0:
                    qr, qi = memo["prev"]
                    zr, zi = sub(pr, qi), add(pi, qr)
                memo["prev"] = (pr, pi)
                if g % 2 == 0:
                    st("zr", 8 * n, done(zr))
                    st("zi", 8 * n, zi)
                else:
                    st16("z", n * T + 4 * (g - 1), _rows(ld("zr", 8 * n), done(zr)))
                    st16("z", n * T + T // 2 + 4 * (g - 1), _rows(ld("zi", 8 * n), zi))

        def a3_list(i):
            out = []
            for g in range(T // 8):
                for plane in range(3):
                    out += [(2 * (n - 8) + 4, P(a3, i, g, plane, True, n)) for n in range(8, NC)]
                    out += [(2 * min(n, 7) + 4 + 2 * (plane == 2), P(a3, i, g, plane, False, n))
                            for n in range(NC)]
            return out

        def idft(i, c0, odd, m):
            def mm():
                rhs = jnp.concatenate([pltpu.bitcast(ld("z", c * T + odd * T // 2, T // 2, i + 2), BF16)
                                       for c in range(c0, c0 + 4)], axis=1)
                f = tab[pl.ds(fresh() + 2 * T + odd * T // 4, T // 4), :]
                return jnp.dot(pltpu.bitcast(f, BF16), rhs, preferred_element_type=F32)
            y = once(("y", i, c0, odd), mm)
            a = once(("a", i), lambda: 2 * j + i)
            q16 = once(("qa", i), lambda: window16("qa", a * (S // 2), S // 2))
            o16 = once(("oa", i), lambda: window16("oa", a * (S // 2), S // 2))
            flip = lambda w: jnp.take_along_axis(
                w, 7 - lax.broadcasted_iota(jnp.int32, (8, 128), 0), axis=0, mode="promise_in_bounds")
            for u in range(4):
                val = y[m:m + 16, u * 128:(u + 1) * 128]
                if not odd:
                    st("even", u * T // 2 + m, val)
                    continue
                even, mid = ld("even", u * T // 2 + m, 16), (c0 + u) * T + T // 2
                low = add(even, val)
                for row, out in ((mid + m, sub(even, val)),
                                 (mid - 16 - m, _rows(flip(low[8:]), flip(low[:8])))):
                    o16[pl.ds(row, 16), :] = mul(q16[pl.ds(row, 16), :].astype(F32), out).astype(BF16)
            memo["clock"] = y[m + 8:m + 16, 384:]

        def idft_list(i, *c0s):
            return [(16, P(idft, i, c0, odd, m)) for c0 in c0s
                    for odd in range(2) for m in range(0, T // 2, 16)]

        def transforms(i, extra, shares=(1, 1, 1, 1, 1, 9)):
            extra = _split(extra, *shares)
            for u in range(4):
                _weave(idft_list(i - 1, 4 * u)[:4], extra[u])
                _run(idft_list(i - 1, 4 * u)[4:])
                _weave(dft_list(i, "hf", 4 * u), a1_list(i, 3 * u, 3 * u + 3))
            oa_copy(2 * j + i - 1).start()
            _weave(dft_list(i, "xf", 0), _merge(a1_list(i, 12, 16), extra[4]))
            _weave(dft_list(i, "xf", 4, 8), extra[5])
            _run(dft_list(i, "xf", 12))

        def xprep(x, u, r):
            halves = []
            for m in (r, r + 8):
                a, b = (pltpu.bitcast(x[pl.ds(2 * m, 16), pl.ds(t * 128, 128)], U32)
                        for t in (u, u + 4))
                a = pace(a)
                a11, a12, a21, a22 = _lo(a), _lo(b), _hi(a), _hi(b)
                halves.append(_left(a11, a12, a21, a22))
            for i, pair in enumerate(zip(*halves)):
                st16("xs", ((4 * i + u) * E + r) // 2, jnp.concatenate(pair, axis=0))

        def split_rows(half):
            for u in range(4):
                for r in range(0, E, 64):
                    a = pltpu.bitcast(xa[0, pl.ds(2 * r, 128), pl.ds((4 * half + u) * 128, 128)], U32)
                    st16("os", ((8 * half + u) * E + r) // 2, _lo(a))
                    st16("os", ((8 * half + 4 + u) * E + r) // 2, _hi(a))

        def xprep_list(x):
            return [(27, P(xprep, x, u, r)) for r in range(0, E, 16) for u in range(4)]

        def lhs(name, i, m0=0, n=E):
            view = views[name][3].at[pl.ds(fresh() + i * 2 * E, 2 * E), :]
            return jnp.concatenate(
                [pltpu.bitcast(view[pl.ds((u * E + m0) // 2, n // 2), :], BF16) for u in range(4)], axis=1)

        def emit(p, par, t, m, val):
            if p == 0:
                st("q", (par * NT + t) * E + m, val)
                return
            if p == 3:
                o16 = once("ob", lambda: window16("ob", (j - 1) * NT * E, NT * E))
                o16[pl.ds(t * R + par * E + m, 16), :] = val.astype(BF16)
                if m + 16 == E and par == t // 4:
                    ob_copy(j - 1, t).start()
                return
            name, row = "kv"[p - 1], (par * NT + t) * KR
            if m == 0 and not first:
                st(name, row, ld(name, row + E, WIN, z=3))
            if m == 0 and first and p == 2 and par == 0:
                for other in range(2):
                    st(name, (other * NT + t) * KR, jnp.broadcast_to(val[0:1], (WIN, 128)))
            st(name, row + WIN + m, val)

        def plain(half, t, m):
            def mm():
                w = pltpu.bitcast(ld("w0", (half * NT + t) * KW, KW, 3), BF16)
                x = lhs("os", 2) if half else jnp.concatenate([lhs("os", 0), lhs("os", 1)], axis=0)
                return jnp.dot(x, w, preferred_element_type=F32)
            res = once(("plain", half, t), mm)
            memo["clock"] = res[m + 8:m + 16]
            if half:
                emit(0, 0, t, m, add(res[m:m + 16], ld("o", t * R + m, 16)))
            else:
                st("o", t * R + m, res[m:m + 16])

        def plain_list(half):
            return [(16, P(plain, half, t, m)) for t in range(NT) for m in range(0, E if half else R, 16)]

        def product(p, m0, n, t, i, m):
            def mm():
                if i == 0:
                    w = ld(f"w{p}", t * KW, KW, 3)
                elif i == 2:
                    w = ld(f"w{p}", (NT + t + 4) * KW, KW, 3)
                else:
                    w = ld(f"ws{p}", (4 * (i - 1 - (i > 2)) + t) * KW, KW, 3)
                return jnp.dot(lhs("xs" if p < 3 or m0 else "os", i, m0, n), pltpu.bitcast(w, BF16),
                               preferred_element_type=F32)
            res = once(("product", p, m0, t, i), mm)
            memo["clock"] = res[m - m0 + 8:m - m0 + 16]
            res = res[m - m0:m - m0 + 16]
            get = lambda name, z=0: ld(name, m, 16, z)
            if i == 0:
                st("c21", m, res)
            elif i == 1:
                st("m4", m, res)
                emit(p, 1, t, m, add(get("c21"), res))
            elif i == 2:
                st("c11", m, sub(get("m4"), res))
                st("m5", m, res)
            elif i == 3:
                st("c22", m, sub(res, get("c21", 1)))
                emit(p, 0, t + 4, m, add(get("m5"), res))
            elif i == 4:
                st("d11", m, add(get("c11"), res))
                st("d22", m, add(get("c22"), res))
            else:
                emit(p, i - 5, t + 4 * (i - 5), m, add(get(("d11", "d22")[i - 5]), res))

        def strassen(p, m0=0, n=E):
            return [(16, P(product, p, m0, n, t, i, m))
                    for t in range(4) for i in range(7) for m in range(m0, m0 + n, 16)]

        def qk(r, w):
            par, m = divmod(8 * r, E)
            qv = once(("qv", r), lambda: [pace(ld("q", (par * NT + t) * E + m)) for t in range(NT)])
            s = pace(_tree([mul(qv[t], ld("k", (par * NT + t) * KR + WIN + m - w)) for t in range(NT)]))
            s = add(s, pltpu.roll(s, 64, 1))
            s = add(s, pltpu.roll(s, 32, 1))
            if first and m < w:
                keep = m + lax.broadcasted_iota(jnp.int32, (8, 128), 0) >= w
                s = jnp.where(keep, s, -1e9 * DH ** 0.5)
            memo["lg", r, w] = s

        def expo(r):
            lg = [memo["lg", r, w] for w in range(WIN)]
            m = pace(functools.reduce(lax.max, lg))
            scale = np.float32(DH ** -0.5 * np.log2(np.e))
            memo["e", r] = [lax.exp2(mul(sub(s, m), scale)) for s in lg]

        def norm(r):
            memo["inv", r] = 1.0 / pace(_tree(memo["e", r]))

        def probs(r):
            inv = pace(memo["inv", r])
            for w in range(WIN):
                st("p", w * R + 8 * r, mul(memo["e", r][w], inv))

        def qk_list(nr=R // 8):
            out = []
            for i in range(WIN * nr + 23):
                r, w = divmod(i, WIN)
                tasks = [P(qk, r, w)] if r < nr else []
                for f, lag in ((expo, 24), (norm, 27), (probs, 30)):
                    if i >= lag and (i - lag) % WIN == 0 and (i - lag) // WIN < nr:
                        tasks.append(P(f, (i - lag) // WIN))
                out.append((26 if r < nr else 12, P(_run, [(0, f) for f in tasks])))
            return out

        def pv(r, t):
            par, m = divmod(8 * r, E)
            p = once(("pv", r), lambda: [(pace if w % 4 == 0 else lambda v: v)(ld("p", w * R + 8 * r)) for w in range(WIN)])
            row = (par * NT + t) * KR + WIN + m
            bufs["o"][pl.ds(t * R + 2 * m + par, 8, stride=2), :] = pace(
                _tree([mul(p[w], ld("v", row - w)) for w in range(WIN)]))

        def pv_list():
            return [(16, P(pv, r, t)) for r in range(R // 8) for t in range(NT)]

        def oprep(u, r):
            a = [ld("o", (u + 4 * h) * R + par * E + r, 16, 1) for par in range(2) for h in range(2)]
            for i, val in enumerate(_left(*a[:3], paced(a[3]))):
                st16("xs" if last and 2 * r >= E else "os", ((4 * i + u) * E + r) // 2, val)

        def oprep_list():
            return [(18, P(oprep, u, r)) for r in range(0, E, 16) for u in range(4)]

        if last:
            mix = []
            for r in range(E // 16):
                for base in (0, E // 2, E, 3 * E // 2):
                    mix += pv_list()[base + 8 * r:base + 8 * r + 8]
                mix += oprep_list()[4 * r:4 * r + 4]
            mix, conv = _split(mix, 1, 1), _split(a3_list(-1), 3, 5)
            transforms(-1, mix[0], (1, 1, 1, 1, 1, 5))
            wait([last_q()])
            _weave(strassen(3, 0, E // 2), mix[1] + conv[0])
            _weave(strassen(3, E // 2, E // 2)[:-6], conv[1])
            _run(strassen(3, E // 2, E // 2)[-6:])
            for u in range(4):
                _run(idft_list(-1, 4 * u))
                oa_part(u).start()
            return

        if first:
            def leading(i):
                w = wraw.at[0, pl.ds(pl.multiple_of(i * KW, KW), KW)]
                pltpu.make_async_copy(w, w, sem_in.at[NS + 4 + i]).wait()
                _run(perm_list(0, w, (0,)))
            rolled(2, dict(w0=128), leading)
            wait([x0_copy(0)])
            split_rows(0)
            _run(plain_list(0)[:96])
            wait([w_copy(1)])
            _weave(plain_list(0)[96:240], perm_list(1))
            _run(plain_list(0)[240:])
            wait([x0_copy(1)])
            split_rows(1)

            def queries(i):
                w_wait(2 + i)
                x = xa.at[0, pl.ds(pl.multiple_of(i * (R // 2), 16), R // 2)]
                _weave(plain_list(1), _merge(perm_list(2, wraw.at[2 + i]),
                                             _merge(xprep_list(x)[:32], right_list(0)[:32])))
            rolled(2, dict(w1=NT * KW, ws0=2 * KW, w0s=2 * KW, xs=E // 4, os=2 * E, o=E, q=NT * E),
                   queries)
            _run(right_list(1)[:16])
            wait(h0_copies())
            _weave(dft_list(0, "hf", 0, 4, 8, 12), right_list(1)[16:])
            wait(kv0_copies())
            _start(in_copies(1))
            _run(a1_list(0, 0, 4))
            for u in range(4):
                _weave(dft_list(0, "xf", 4 * u)[:13], a1_list(0, 4 * u + 4, min(4 * u + 8, NC)))
                _run(dft_list(0, "xf", 4 * u)[13:])

            def keys(i):
                w_wait(4 + i)
                _weave(strassen(1)[:144], _merge(perm_list(4, wraw.at[4 + i]), a3_list(0)[:320]))
                _weave(strassen(1)[144:220], a3_list(0)[320:576])
                _run(strassen(1)[220:224])
            rolled(2, dict(w1=2 * KW, ws1=2 * KW, w2=NT * KW, k=2 * KR, hf=64, xf=64, z=32), keys)
            wait(wo_copies())
            _start(in_copies(2) + in_copies(3) + in_copies(NS) + [last_q()])
            rolled(2, dict(w2=2 * KW, ws2=2 * KW, w3=4 * KW), lambda i: _run(
                _merge(right_list(2)[:32], wo_list(2 * i, 0) + wo_list(2 * i + 1, 2))))
            rolled(2, dict(w2=2 * KW, ws2=2 * KW, w3=2 * KW, ws3=2 * KW, v=2 * KR, q=NT * E, k=NT * KR, p=E),
                   lambda i: _weave(strassen(2)[:224], _merge(right_list(3)[:32], qk_list(E // 8))))
            return

        head = strassen(0) + strassen(1)
        pre = _split(oprep_list(), 3, 1)
        transforms(-1, xprep_list(xa.at[j]))
        _weave(head[:528], a3_list(-1))
        _weave(head[528:812], pv_list())
        _run(head[812:818])
        transforms(0, pre[0], (0, 0, 0, 0, 1, 9))
        _weave(head[818:] + strassen(3), pre[1] + a3_list(0))
        _weave(strassen(2), qk_list())

    def loop(j, carry):
        _wait(in_copies(j))
        step(j)
        return carry

    step(0, first=True)
    lax.fori_loop(1, NS, loop, 0)
    _wait(in_copies(NS))
    step(NS, last=True)
    for i, name in enumerate(("oa", "ob")):
        pltpu.make_async_copy(raw[name], raw[name], sem_out.at[i]).wait()


@jax.jit
def pallas_concat_heads__ssm_conv_h3__sliding_local_dilated__prompt_kernel(
    A_q, A_k, A_v, A_shift_k, A_ssm_k, A_ssm_D, B_x, B_wqkv, B_wo,
):
    hbm = pl.BlockSpec(memory_space=pl.ANY)
    out = pl.pallas_call(
        _kernel,
        in_specs=[hbm] * 10,
        out_specs=hbm,
        out_shape=jax.ShapeDtypeStruct((S, 2 * D), BF16),
        scratch_shapes=[
            pltpu.VMEM((NT, 128, S), BF16),
            pltpu.VMEM((NS, R, D), BF16),
            pltpu.VMEM((6, D // 2, D), BF16),
            pltpu.VMEM((NT, D, 128), BF16),
            pltpu.VMEM((NT, 5, 8, 128), F32),
            pltpu.VMEM(_TABLE.shape, U32),
            pltpu.SemaphoreType.DMA((NS + 14,)),
            pltpu.SemaphoreType.DMA((2,)),
        ] + [pltpu.VMEM((r * 4 // np.dtype(t).itemsize, 128), t) for t, r in _BUFS.values()]
        + [pltpu.VMEM((4, D), BF16), pltpu.VMEM((8, 128), BF16)],
        compiler_params=pltpu.CompilerParams(vmem_limit_bytes=100 * 1024 * 1024,
                                             disable_bounds_checks=True,
                                             disable_semaphore_checks=True),
        name="fused",
    )(A_q[0], A_k[0], A_v[0], A_shift_k.T, A_ssm_k,
      A_ssm_D.reshape(8, 128), B_x[0], B_wqkv, B_wo, _TABLE)
    return out[None]
```

```python
import functools

import jax
import jax.numpy as jnp
import numpy as np
from jax import lax
from jax.experimental import pallas as pl
import jax.experimental.pallas.tpu as pltpu

S = 2048
D = 1024
T = 128
NC = S // T
NT = D // 128
NS = 4
R = S // NS
E = R // 2
WIN, DH = 8, 32
PITCH = DH + 1
KR = E + 16
FP = 2 * T + 16
KW = D // 4
KA = S // 2 + 32
ZERO = 5 * T // 2

F32, BF16, U32 = jnp.float32, jnp.bfloat16, jnp.uint32
P = functools.partial
add, sub, mul = lax.add, lax.sub, lax.mul


def _pack_rows(m):
    b = m.astype(jnp.bfloat16).view(np.uint16).astype(np.uint32)
    return np.ascontiguousarray(b[0::2] | (b[1::2] << 16))


def _dft_table():
    th = 2.0 * np.pi * (np.arange(T) + 0.25) / T
    dft = lambda t: np.concatenate([np.cos(np.outer(th, t)), -np.sin(np.outer(th, t))], axis=0)
    paired = np.arange(T).reshape(-1, 8, 2).transpose(0, 2, 1).reshape(-1)
    ph = np.outer(np.arange(T // 2) + 0.5, th)
    mats = (dft(np.arange(T)), dft(paired - (T - 1) / 2), np.cos(ph) / T, np.sin(ph) / T)
    return np.concatenate([_pack_rows(m) for m in mats] + [np.zeros((32, T), np.uint32)], axis=0)


_TABLE = _dft_table()


def _lo(w):
    return pltpu.bitcast(lax.shift_left(w, np.uint32(16)), F32)


def _hi(w):
    return pltpu.bitcast(lax.bitwise_and(w, np.uint32(0xFFFF0000)), F32)


def _rows(first, second):
    return jnp.concatenate([first, second], axis=0)


def _tree(xs):
    while len(xs) > 1:
        xs = [add(xs[i], xs[i + 1]) if i + 1 < len(xs) else xs[i] for i in range(0, len(xs), 2)]
    return xs[0]


def _left(a11, a12, a21, a22):
    return [add(a21, a22), a22, add(a11, a12), a11, add(a11, a22), sub(a12, a22), sub(a21, a11)]


def _merge(main, side):
    total_m = sum(c for c, _ in main)
    total_s = sum(c for c, _ in side)
    done_m, done_s, i, out = 0, 0, 0, []
    for c, f in main:
        out.append((c * total_s, f))
        done_m += c
        while i < len(side) and (done_s + side[i][0]) * total_m <= done_m * total_s:
            done_s += side[i][0]
            out.append((side[i][0] * total_m, side[i][1]))
            i += 1
    assert i == len(side)
    return out


def _run(tasks):
    for _, f in tasks:
        f()


def _weave(main, side):
    _run(_merge(main, side))


def _split(tasks, *weights):
    ends = np.cumsum((0,) + weights) * len(tasks) // sum(weights)
    return [tasks[a:b] for a, b in zip(ends[:-1], ends[1:])]


def _start(copies):
    for c in copies:
        c.start()


def _wait(copies):
    for c in copies:
        c.wait()


_BUFS = {n: (t, r) for t, group in (
    (BF16, dict(qa=NT * S // 2, ka=NT * KA, va=NT * S // 2, oa=NT * S // 2, ob=S * NT // 2,
                xs=7 * 4 * E // 2, os=7 * 4 * E // 2, w3=2 * NT * KW,
                kv0=S // 8, kv1=S // 8, kv2=S // 8, kv3=S // 8, z=NC * T,
                **{f"ws{p}": 20 * KW for p in range(4)})),
    (U32, dict(**{f"w{p}": 2 * NT * KW for p in range(3)}, t0=34 * DH, t1=34 * DH)),
    (F32, dict(hf=NC * FP, xf=NC * FP, up=8 * NC, k1=8 * NC, pi=8 * NC, zr=8 * NC, zi=8 * NC,
               even=2 * T, c21=E, m4=E, c11=E, m5=E, c22=E, d11=E, d22=E,
               q=2 * NT * E + 32, k=2 * NT * KR, v=2 * NT * KR, p=WIN * R, o=NT * R + 32)),
) for n, r in group.items()}


def _kernel(q_hbm, k_hbm, v_hbm, sk_hbm, h_hbm, d_hbm, x_hbm, w_hbm, wo_hbm, tab_hbm, out_hbm,
            ha, xa, wraw, woraw, taps, tab, sem_in, sem_out, *raw):
    *raw, sk_ref, d_ref = raw
    raw = dict(zip(_BUFS, raw))
    bufs = {n: b.bitcast(U32) if _BUFS[n][0] == BF16 else b for n, b in raw.items()}

    raw["w0s"], bufs["w0s"] = raw["w0"], bufs["w0"]
    spec = dict(_BUFS, w0s=_BUFS["w0"])

    def ld(name, row, n=8, z=0):
        assert 0 <= row and row + n <= views[name][z].shape[0]
        return views[name][z][pl.ds(row, n), :]

    def st(name, row, val):
        assert 0 <= row and row + val.shape[0] <= views[name][3].shape[0]
        views[name][3][pl.ds(row, val.shape[0]), :] = val

    def st16(name, row, val):
        assert 0 <= row and 2 * row + val.shape[0] <= views[name][4].shape[0]
        views[name][4][pl.ds(2 * row, val.shape[0]), :] = val.astype(BF16)

    def window(name, row, n):
        return bufs[name].at[pl.ds(pl.multiple_of(row, 8), n), :]

    def window16(name, row, n):
        return raw[name].at[pl.ds(pl.multiple_of(2 * row, 16), 2 * n), :]

    def cols(a):
        return pl.ds(pl.multiple_of(a * 128, 128), 128)

    def rows(j):
        return pl.ds(pl.multiple_of(j * R, R), R)

    def a_copies(a, sem, skip=0):
        return [pltpu.make_async_copy(src, dst, sem) for src, dst in (
            (h_hbm.at[cols(a), :], ha.at[a]),
            (k_hbm.at[:, cols(a)], window16("ka", a * KA + 32, S // 2)),
            (v_hbm.at[:, cols(a)], window16("va", a * (S // 2), S // 2)))[skip:]]

    def q_copy(a, sem):
        return pltpu.make_async_copy(q_hbm.at[:, cols(a)], window16("qa", a * (S // 2), S // 2), sem)

    def in_copies(j):
        sem = sem_in.at[j]
        out = a_copies(2 * j - 1, sem) + [q_copy(2 * j - 2, sem)]
        if isinstance(j, int) and j == NS:
            return out
        return (out + [pltpu.make_async_copy(x_hbm.at[rows(j), :], xa.at[j], sem)]
                + a_copies(2 * j, sem) + [q_copy(2 * j - 1, sem)])

    def h0_copies():
        full = pl.ds(0, ZERO)
        return [pltpu.make_async_copy(tab_hbm.at[full], tab.at[full], sem_in.at[0]),
                pltpu.make_async_copy(h_hbm.at[cols(0), :], ha.at[0], sem_in.at[0])]

    def kv0_copies():
        return a_copies(0, sem_in.at[NS + 13], 1)

    def last_q():
        return q_copy(NT - 1, sem_in.at[NS + 1])

    def x0_copy(row, n, half, sem):
        part = pl.ds(row, n), pl.ds(half * D // 2, D // 2)
        return pltpu.make_async_copy(x_hbm.at[part], xa.at[(0, *part)], sem_in.at[sem])

    def w_copy(n):
        half = pl.ds(n % 2 * (D // 2), D // 2)
        return pltpu.make_async_copy(
            w_hbm.at[half, pl.ds(n // 2 * D, D)], wraw.at[n], sem_in.at[NS + 5 + n])

    def w_wait(n):
        pltpu.make_async_copy(wraw.at[n], wraw.at[n], sem_in.at[NS + 5 + n]).wait()

    def wo_copies():
        return [pltpu.make_async_copy(wo_hbm.at[:, pl.ds(t * 128, 128)], woraw.at[t],
                                      sem_in.at[NS + 11]) for t in range(NT)]

    def oa_copy(a):
        return pltpu.make_async_copy(window16("oa", a * (S // 2), S // 2), out_hbm.at[:, cols(a)],
                                     sem_out.at[0])

    def oa_part(u):
        src = window16("oa", (4 * (NT - 1) + u) * S // 8, S // 8)
        return pltpu.make_async_copy(src, out_hbm.at[pl.ds(u * S // 4, S // 4), cols(NT - 1)],
                                     sem_out.at[0])

    def ob_copy(j, t):
        return pltpu.make_async_copy(window16("ob", (j * NT + t) * E, E),
                                     out_hbm.at[rows(j), cols(NT + t)], sem_out.at[1])

    small = [pltpu.make_async_copy(a, b, sem_in.at[NS + 12])
             for a, b in ((tab_hbm.at[pl.ds(ZERO, 8)], tab.at[pl.ds(ZERO, 8)]),
                          (sk_hbm, sk_ref), (d_hbm, d_ref))]
    w00 = [pltpu.make_async_copy(w_hbm.at[pl.ds(u * KW, KW), pl.ds(0, D)], wraw.at[0, pl.ds(u * KW, KW)],
                                 sem_in.at[NS + 4 + u]) for u in range(2)]
    _start(small + w00 + [x0_copy(0, R, 0, NS + 2), w_copy(1), x0_copy(0, E, 1, NS + 7), w_copy(2),
                          x0_copy(E, E, 1, NS + 8), w_copy(3)] + h0_copies() + kv0_copies()
           + [w_copy(4), w_copy(5)] + wo_copies())
    _wait(small)
    unit = pltpu.bitcast(tab[pl.ds(ZERO, 8), :], jnp.int32)
    zs = [pl.multiple_of(unit[i, 0] * 8, 8) for i in range(3)]
    views = {n: [b.at[pl.ds(z, spec[n][1]), :] for z in zs] + [b, raw[n]] for n, b in bufs.items()}

    for a in range(NT):
        st("ka", a * KA + 24, jnp.zeros((8, 128), U32))
    for t in range(2 * NT):
        st("k", t * KR, jnp.zeros((WIN, 128), F32))
    skf = sk_ref[...].astype(F32)
    df = d_ref[...].astype(F32)
    for t in range(NT):
        for i in range(4):
            taps[t, i] = jnp.broadcast_to(skf[i:i + 1, t * 128:(t + 1) * 128], (8, 128))
        taps[t, 4] = jnp.broadcast_to(df[t:t + 1, :], (8, 128))

    def step(j, first=False, last=False):
        memo = {}
        never = tab[pl.ds(ZERO, 8), :] != 0

        def once(key, fn):
            if key not in memo:
                memo[key] = fn()
            return memo[key]

        def fresh():
            memo["fresh"] = memo.get("fresh", 1) + 1
            return pl.multiple_of(zs[0] * memo["fresh"], 8)

        def pace(val):
            clock = memo.get("clock")
            if clock is None:
                return val
            if val.dtype != F32:
                clock = pltpu.bitcast(clock, val.dtype)
            return lax.select(never, clock, val)

        def paced(x):
            return jnp.concatenate([pace(x[:8]), x[8:]], axis=0)

        def wait(copies):
            memo["clock"] = None
            _wait(copies)

        def rolled(n, shifts, body):
            def one(i, carry):
                saved, kept = dict(views), dict(memo)
                memo["clock"] = None
                for name, d in shifts.items():
                    size = spec[name][1] - d * (n - 1)
                    views[name] = [window(name, z + d * i, size) for z in zs + [0]]
                    if spec[name][0] == BF16:
                        views[name].append(window16(name, d * i, size))
                body(i)
                views.update(saved)
                memo.clear()
                memo.update(kept, clock=None)
                return carry
            lax.fori_loop(0, n, one, 0)

        def perm_in(w, u, t):
            tt = paced(pltpu.bitcast(w[pl.ds(u * 256, 256), pl.ds(t * 128, 128)], U32)).T
            for hh in range(4):
                st(f"t{u}", (4 * t + hh) * PITCH, tt[hh * DH:(hh + 1) * DH])

        def perm_out(p, h, u, t):
            g = jnp.concatenate(
                [bufs[f"t{u}"][pl.ds(zs[0] + 4 * t + i, 32, stride=PITCH), :] for i in range(4)], axis=0)
            st(f"w{p}", (h * NT + t) * KW + u * 128, paced(g).T)

        def perm_list(n, w=None, us=(0, 1)):
            w = wraw.at[n] if w is None else w
            return [(1, P(f, u, t)) for f in (P(perm_in, w), P(perm_out, n // 2, n % 2))
                    for u in us for t in range(NT)] + [(2, lambda: None)] * 4

        def wo_in(i, t0, t, hh):
            w = pltpu.bitcast(woraw[2 * i + t - t0, pl.ds(hh * DH, DH), :], U32)
            st(f"t{t % 2}", hh * (DH // 2 + 1), paced(w))

        def wo_out(t, i):
            g = paced(bufs[f"t{t % 2}"][pl.ds(zs[0] + i, 32, stride=DH // 2 + 1), :])
            st16("w3", (i // 8 * NT + t) * KW + i % 8 * 32, _rows(_lo(g), _hi(g)))

        def wo_list(i, t0=0):
            return [(1, P(f, t, u)) for f, n in ((P(wo_in, i, t0), 32), (wo_out, 16))
                    for t in (t0, t0 + 1) for u in range(n)]

        def right(p, t, r):
            b = [ld(f"w{p}" if p else "w0s", (h * NT + t + 4 * u) * KW + r, 16)
                 for h in range(2) for u in range(2)]
            b[0] = paced(b[0])
            b11, b12, b21, b22 = (pltpu.bitcast(x, BF16).astype(F32) for x in b)
            for i, val in enumerate((sub(b21, b11), sub(b12, b22), add(b11, b22),
                                     add(b21, b22), add(b11, b12))):
                st16(f"ws{p}", (4 * i + t) * KW + r, val)

        def right_list(p):
            return [(1, P(right, p, t, r)) for t in range(4) for r in range(0, KW, 16)]

        def ld_kv(c, row, n, z=0):
            return ld(f"kv{c // 4}", c % 4 * (T // 2) + row, n, z)

        def a1(i, r):
            a = once(("a", i), lambda: 2 * j + i)
            w0, w1, w2, w3 = once(("taps", i), lambda: [taps[a, u] for u in range(4)])
            k32 = once(("ka", i), lambda: window("ka", a * KA, KA))
            v32 = once(("va", i), lambda: window("va", a * (S // 2), S // 2))
            c0, c1, c2 = (k32[pl.ds(8 * r + 32 - u, 8), :] for u in range(3))
            vv = v32[pl.ds(8 * r, 8), :]
            e0, o0, e1, o1, o2 = _lo(c0), _hi(c0), _lo(c1), _hi(c1), _hi(c2)
            ke = _tree([mul(e0, w0), mul(o1, w1), mul(e1, w2), mul(o2, w3)])
            ko = _tree([mul(o0, w0), mul(e0, w1), mul(o1, w2), mul(e1, w3)])
            st16(f"kv{r // 32}", 8 * (r % 32), _rows(mul(ke, _lo(vv)), pace(mul(ko, _hi(vv)))))

        def a1_list(i, c0, c1):
            return [(24, P(a1, i, r)) for r in range(8 * c0, 8 * c1)]

        def freq(c, im, m):
            return c * FP + im * (T + 8) + m

        def dft(i, name, c0, m):
            def mm():
                f = pltpu.bitcast(tab[pl.ds(fresh() + T * (name == "xf"), T), :], BF16)
                if name == "hf":
                    a = once(("a", i), lambda: 2 * j + i)
                    rhs = jnp.concatenate(
                        [ha[a, :, pl.ds(c * T, T)] for c in range(c0, c0 + 4)], axis=0)
                    return lax.dot_general(f, rhs, (((1,), (1,)), ((), ())),
                                           preferred_element_type=F32)
                rhs = jnp.concatenate(
                    [pltpu.bitcast(ld_kv(c, 0, T // 2, i % 2), BF16) for c in range(c0, c0 + 4)], axis=1)
                return jnp.dot(f, rhs, preferred_element_type=F32)
            res = once((name, i, c0), mm)
            for u in range(4):
                val = res[m:m + 16, u * 128:(u + 1) * 128]
                if name == "hf" and c0 + u == 0 and m < T:
                    val = add(val, once(("dd", i), lambda: _rows(*[taps[memo["a", i], 4]] * 2)))
                st(name, freq(c0 + u, m // T, m % T), val)
            memo["clock"] = res[m + 8:m + 16, 384:]

        def dft_list(i, name, *c0s):
            return [(16, P(dft, i, name, c0, m)) for c0 in c0s for m in range(0, 2 * T, 16)]

        def a3(i, g, plane, upper, n):
            def opnd(name, c):
                re = lambda: ld(name, freq(c, 0, 8 * g), z=plane)
                im = lambda: ld(name, freq(c, 1, 8 * g), z=plane)
                if name == "xf":
                    val = add(re(), im()) if plane == 0 else re() if plane == 1 else im()
                    return pace(val) if c >= 8 else val
                return pace(re() if plane == 0 else (sub, add)[plane - 1](im(), re()))
            get = lambda name, c: once((name, i, g, plane, c), P(opnd, name, c))
            done = pace if n % 4 == 3 else lambda v: v
            cs = range(8, n + 1) if upper else range(min(n, 7) + 1)
            terms = [mul(get("xf", n - c), get("hf", c)) for c in cs]
            if upper:
                st("up", 8 * n, done(_tree(terms)))
                return
            if n >= 8:
                terms.append(ld("up", 8 * n))
            if plane == 0:
                st("k1", 8 * n, done(_tree(terms)))
            elif plane == 1:
                st("pi", 8 * n, done(_tree(terms + [ld("k1", 8 * n)])))
            else:
                pr = sub(ld("k1", 8 * n, z=1), _tree(terms))
                pi = ld("pi", 8 * n)
                zr, zi = pr, pi
                if n > 0:
                    qr, qi = memo["prev"]
                    zr, zi = sub(pr, qi), add(pi, qr)
                memo["prev"] = (pr, pi)
                if g % 2 == 0:
                    st("zr", 8 * n, done(zr))
                    st("zi", 8 * n, zi)
                else:
                    st16("z", n * T + 4 * (g - 1), _rows(ld("zr", 8 * n), done(zr)))
                    st16("z", n * T + T // 2 + 4 * (g - 1), _rows(ld("zi", 8 * n), zi))

        def a3_list(i):
            out = []
            for g in range(T // 8):
                for plane in range(3):
                    out += [(2 * (n - 8) + 4, P(a3, i, g, plane, True, n)) for n in range(8, NC)]
                    out += [(2 * min(n, 7) + 4 + 2 * (plane == 2), P(a3, i, g, plane, False, n))
                            for n in range(NC)]
            return out

        def idft(i, c0, odd, m):
            def mm():
                rhs = jnp.concatenate([pltpu.bitcast(ld("z", c * T + odd * T // 2, T // 2, i + 2), BF16)
                                       for c in range(c0, c0 + 4)], axis=1)
                f = tab[pl.ds(fresh() + 2 * T + odd * T // 4, T // 4), :]
                return jnp.dot(pltpu.bitcast(f, BF16), rhs, preferred_element_type=F32)
            y = once(("y", i, c0, odd), mm)
            a = once(("a", i), lambda: 2 * j + i)
            q16 = once(("qa", i), lambda: window16("qa", a * (S // 2), S // 2))
            o16 = once(("oa", i), lambda: window16("oa", a * (S // 2), S // 2))
            flip = lambda w: jnp.take_along_axis(
                w, 7 - lax.broadcasted_iota(jnp.int32, (8, 128), 0), axis=0, mode="promise_in_bounds")
            for u in range(4):
                val = y[m:m + 16, u * 128:(u + 1) * 128]
                if not odd:
                    st("even", u * T // 2 + m, val)
                    continue
                even, mid = ld("even", u * T // 2 + m, 16), (c0 + u) * T + T // 2
                low = add(even, val)
                for row, out in ((mid + m, sub(even, val)),
                                 (mid - 16 - m, _rows(flip(low[8:]), flip(low[:8])))):
                    o16[pl.ds(row, 16), :] = mul(q16[pl.ds(row, 16), :].astype(F32), out).astype(BF16)
            memo["clock"] = y[m + 8:m + 16, 384:]

        def idft_list(i, *c0s):
            return [(16, P(idft, i, c0, odd, m)) for c0 in c0s
                    for odd in range(2) for m in range(0, T // 2, 16)]

        def transforms(i, extra, shares=(1, 1, 1, 1, 1, 9)):
            extra = _split(extra, *shares)
            for u in range(4):
                _weave(idft_list(i - 1, 4 * u)[:4], extra[u])
                _run(idft_list(i - 1, 4 * u)[4:])
                _weave(dft_list(i, "hf", 4 * u), a1_list(i, 3 * u, 3 * u + 3))
            oa_copy(2 * j + i - 1).start()
            _weave(dft_list(i, "xf", 0), _merge(a1_list(i, 12, 16), extra[4]))
            _weave(dft_list(i, "xf", 4, 8), extra[5])
            _run(dft_list(i, "xf", 12))

        def xprep(x, u, r):
            halves = []
            for m in (r, r + 8):
                a, b = (pltpu.bitcast(x[pl.ds(2 * m, 16), pl.ds(t * 128, 128)], U32)
                        for t in (u, u + 4))
                a = pace(a)
                a11, a12, a21, a22 = _lo(a), _lo(b), _hi(a), _hi(b)
                halves.append(_left(a11, a12, a21, a22))
            for i, pair in enumerate(zip(*halves)):
                st16("xs", ((4 * i + u) * E + r) // 2, jnp.concatenate(pair, axis=0))

        def xprep_list(x):
            return [(27, P(xprep, x, u, r)) for r in range(0, E, 16) for u in range(4)]

        def lhs(name, i, m0=0, n=E):
            view = views[name][3].at[pl.ds(fresh() + i * 2 * E, 2 * E), :]
            return jnp.concatenate(
                [pltpu.bitcast(view[pl.ds((u * E + m0) // 2, n // 2), :], BF16) for u in range(4)], axis=1)

        def emit(p, par, t, m, val):
            if p == 0:
                st("q", (par * NT + t) * E + m, val)
                return
            if p == 3:
                o16 = once("ob", lambda: window16("ob", (j - 1) * NT * E, NT * E))
                o16[pl.ds(t * R + par * E + m, 16), :] = val.astype(BF16)
                if m + 16 == E and par == t // 4:
                    ob_copy(j - 1, t).start()
                return
            name, row = "kv"[p - 1], (par * NT + t) * KR
            if m == 0 and not first:
                st(name, row, ld(name, row + E, WIN, z=3))
            if m == 0 and first and p == 2 and par == 0:
                for other in range(2):
                    st(name, (other * NT + t) * KR, jnp.broadcast_to(val[0:1], (WIN, 128)))
            st(name, row + WIN + m, val)

        def plain(x, half, t, m):
            def mm():
                w = pltpu.bitcast(ld("w0", (half * NT + t) * KW, KW, 3), BF16)
                return jnp.dot(x[:, pl.ds(half * D // 2, D // 2)], w, preferred_element_type=F32)
            res = once(("plain", half, t), mm)
            memo["clock"] = res[m + 8:m + 16]
            if half:
                st("q", t * R + m, add(res[m:m + 16], ld("o", t * R + m, 16)))
            else:
                st("o", t * R + m, res[m:m + 16])

        def plain_list(x, half):
            return [(16, P(plain, x, half, t, m)) for t in range(NT) for m in range(0, x.shape[0], 16)]

        def product(p, m0, n, t, i, m):
            def mm():
                if i == 0:
                    w = ld(f"w{p}", t * KW, KW, 3)
                elif i == 2:
                    w = ld(f"w{p}", (NT + t + 4) * KW, KW, 3)
                else:
                    w = ld(f"ws{p}", (4 * (i - 1 - (i > 2)) + t) * KW, KW, 3)
                return jnp.dot(lhs("xs" if p < 3 or m0 else "os", i, m0, n), pltpu.bitcast(w, BF16),
                               preferred_element_type=F32)
            res = once(("product", p, m0, t, i), mm)
            memo["clock"] = res[m - m0 + 8:m - m0 + 16]
            res = res[m - m0:m - m0 + 16]
            get = lambda name, z=0: ld(name, m, 16, z)
            if i == 0:
                st("c21", m, res)
            elif i == 1:
                st("m4", m, res)
                emit(p, 1, t, m, add(get("c21"), res))
            elif i == 2:
                st("c11", m, sub(get("m4"), res))
                st("m5", m, res)
            elif i == 3:
                st("c22", m, sub(res, get("c21", 1)))
                emit(p, 0, t + 4, m, add(get("m5"), res))
            elif i == 4:
                st("d11", m, add(get("c11"), res))
                st("d22", m, add(get("c22"), res))
            else:
                emit(p, i - 5, t + 4 * (i - 5), m, add(get(("d11", "d22")[i - 5]), res))

        def strassen(p, m0=0, n=E):
            return [(16, P(product, p, m0, n, t, i, m))
                    for t in range(4) for i in range(7) for m in range(m0, m0 + n, 16)]

        def qk(r, w):
            par, m = divmod(8 * r, E)
            query = lambda t: (bufs["q"][pl.ds(memo["parity"] + t * R + 2 * m, 8, stride=2), :] if first
                               else ld("q", (par * NT + t) * E + m))
            qv = once(("qv", r), lambda: [pace(query(t)) for t in range(NT)])
            s = pace(_tree([mul(qv[t], ld("k", (par * NT + t) * KR + WIN + m - w)) for t in range(NT)]))
            s = add(s, pltpu.roll(s, 64, 1))
            s = add(s, pltpu.roll(s, 32, 1))
            if first and m < w:
                keep = m + lax.broadcasted_iota(jnp.int32, (8, 128), 0) >= w
                s = jnp.where(keep, s, -1e9 * DH ** 0.5)
            memo["lg", r, w] = s

        def expo(r):
            lg = [memo["lg", r, w] for w in range(WIN)]
            m = pace(functools.reduce(lax.max, lg))
            scale = np.float32(DH ** -0.5 * np.log2(np.e))
            memo["e", r] = [lax.exp2(mul(sub(s, m), scale)) for s in lg]

        def norm(r):
            memo["inv", r] = 1.0 / pace(_tree(memo["e", r]))

        def probs(r):
            inv = pace(memo["inv", r])
            for w in range(WIN):
                st("p", w * R + 8 * r, mul(memo["e", r][w], inv))

        def qk_list(nr=R // 8):
            out = []
            for i in range(WIN * nr + 23):
                r, w = divmod(i, WIN)
                tasks = [P(qk, r, w)] if r < nr else []
                for f, lag in ((expo, 24), (norm, 27), (probs, 30)):
                    if i >= lag and (i - lag) % WIN == 0 and (i - lag) // WIN < nr:
                        tasks.append(P(f, (i - lag) // WIN))
                out.append((26 if r < nr else 12, P(_run, [(0, f) for f in tasks])))
            return out

        def pv(r, t):
            par, m = divmod(8 * r, E)
            p = once(("pv", r), lambda: [(pace if w % 4 == 0 else lambda v: v)(ld("p", w * R + 8 * r))
                                         for w in range(WIN)])
            row = (par * NT + t) * KR + WIN + m
            bufs["o"][pl.ds(t * R + 2 * m + par, 8, stride=2), :] = pace(
                _tree([mul(p[w], ld("v", row - w)) for w in range(WIN)]))

        def pv_list():
            return [(16, P(pv, r, t)) for r in range(R // 8) for t in range(NT)]

        def oprep(u, r):
            a = [ld("o", (u + 4 * h) * R + par * E + r, 16, 1) for par in range(2) for h in range(2)]
            for i, val in enumerate(_left(*a[:3], paced(a[3]))):
                st16("xs" if last and 2 * r >= E else "os", ((4 * i + u) * E + r) // 2, val)

        def oprep_list():
            return [(18, P(oprep, u, r)) for r in range(0, E, 16) for u in range(4)]

        if last:
            mix = []
            for r in range(E // 16):
                for base in (0, E // 2, E, 3 * E // 2):
                    mix += pv_list()[base + 8 * r:base + 8 * r + 8]
                mix += oprep_list()[4 * r:4 * r + 4]
            mix, conv = _split(mix, 1, 1), _split(a3_list(-1), 2, 3)
            transforms(-1, mix[0], (3, 3, 3, 3, 2, 9))
            wait([last_q()])
            _weave(strassen(3, 0, E // 2), mix[1] + conv[0])
            _weave(strassen(3, E // 2, E // 2)[:-24], conv[1])
            _run(strassen(3, E // 2, E // 2)[-24:-16])
            for u in range(4):
                _run(idft_list(-1, 4 * u))
                oa_part(u).start()
            _run(strassen(3, E // 2, E // 2)[-16:])
            return

        if first:

            def leading(i):
                w = wraw.at[0, pl.ds(pl.multiple_of(i * KW, KW), KW)]
                pltpu.make_async_copy(w, w, sem_in.at[NS + 4 + i]).wait()
                _run(perm_list(0, w, (0,)))
            rolled(2, dict(w0=128), leading)
            wait([x0_copy(0, R, 0, NS + 2)])
            _run(plain_list(xa.at[0], 0)[:96])
            wait([w_copy(1)])
            _weave(plain_list(xa.at[0], 0)[96:240], perm_list(1))
            _run(plain_list(xa.at[0], 0)[240:])

            def queries(i):
                w_wait(2 + i)
                x0_copy(pl.multiple_of(i * E, 16), E, 1, NS + 7 + i).wait()
                x = xa.at[0, pl.ds(pl.multiple_of(i * (R // 2), 16), R // 2)]
                _weave(plain_list(x, 1), _merge(perm_list(2, wraw.at[2 + i]),
                                             _merge(xprep_list(x)[:32], right_list(0)[:32])))
            rolled(2, dict(w1=NT * KW, ws0=2 * KW, w0s=2 * KW, xs=E // 4, o=E, q=E),
                   queries)
            wait(h0_copies())
            _weave(dft_list(0, "hf", 0, 4, 8, 12), right_list(1))
            wait(kv0_copies())
            _start(in_copies(1))
            _run(a1_list(0, 0, 9))
            _weave(dft_list(0, "xf", 0), a1_list(0, 9, 13))
            _weave(dft_list(0, "xf", 4), a1_list(0, 13, 16))
            _run(dft_list(0, "xf", 8, 12))

            def keys(i):
                w_wait(4 + i)
                _weave(strassen(1)[:144], _merge(perm_list(4, wraw.at[4 + i]), a3_list(0)[:320]))
                _weave(strassen(1)[144:220], a3_list(0)[320:576])
                _run(strassen(1)[220:224])
            rolled(2, dict(w1=2 * KW, ws1=2 * KW, w2=NT * KW, k=2 * KR, hf=64, xf=64, z=32), keys)
            wait(wo_copies())
            _start(in_copies(2) + in_copies(3) + in_copies(NS) + [last_q()])
            rolled(2, dict(w2=2 * KW, ws2=2 * KW, w3=4 * KW), lambda i: _run(
                _merge(right_list(2)[:32], wo_list(2 * i, 0) + wo_list(2 * i + 1, 2))))

            def values(i):
                memo["parity"] = i
                _weave(strassen(2)[:224], _merge(right_list(3)[:32], qk_list(E // 8)))
            rolled(2, dict(w2=2 * KW, ws2=2 * KW, w3=2 * KW, ws3=2 * KW, v=2 * KR, k=NT * KR, p=E), values)
            return

        head = strassen(0) + strassen(1)
        pre = _split(oprep_list(), 3, 1)
        transforms(-1, xprep_list(xa.at[j]))
        _weave(head[:528], a3_list(-1))
        _weave(head[528:812], pv_list())
        _run(head[812:818])
        transforms(0, pre[0], (0, 0, 0, 0, 1, 9))
        _weave(head[818:] + strassen(3), pre[1] + a3_list(0))
        _weave(strassen(2), qk_list())

    def loop(j, carry):
        _wait(in_copies(j))
        step(j)
        return carry

    step(0, first=True)
    lax.fori_loop(1, NS, loop, 0)
    _wait(in_copies(NS))
    step(NS, last=True)
    for i, name in enumerate(("oa", "ob")):
        pltpu.make_async_copy(raw[name], raw[name], sem_out.at[i]).wait()


@jax.jit
def pallas_concat_heads__ssm_conv_h3__sliding_local_dilated__prompt_kernel(
    A_q, A_k, A_v, A_shift_k, A_ssm_k, A_ssm_D, B_x, B_wqkv, B_wo,
):
    hbm = pl.BlockSpec(memory_space=pl.ANY)
    out = pl.pallas_call(
        _kernel,
        in_specs=[hbm] * 10,
        out_specs=hbm,
        out_shape=jax.ShapeDtypeStruct((S, 2 * D), BF16),
        scratch_shapes=[
            pltpu.VMEM((NT, 128, S), BF16),
            pltpu.VMEM((NS, R, D), BF16),
            pltpu.VMEM((6, D // 2, D), BF16),
            pltpu.VMEM((NT, D, 128), BF16),
            pltpu.VMEM((NT, 5, 8, 128), F32),
            pltpu.VMEM(_TABLE.shape, U32),
            pltpu.SemaphoreType.DMA((NS + 14,)),
            pltpu.SemaphoreType.DMA((2,)),
        ] + [pltpu.VMEM((r * 4 // np.dtype(t).itemsize, 128), t) for t, r in _BUFS.values()]
        + [pltpu.VMEM((4, D), BF16), pltpu.VMEM((8, 128), BF16)],
        compiler_params=pltpu.CompilerParams(vmem_limit_bytes=100 * 1024 * 1024,
                                             disable_bounds_checks=True,
                                             disable_semaphore_checks=True),
        name="fused",
    )(A_q[0], A_k[0], A_v[0], A_shift_k.T, A_ssm_k,
      A_ssm_D.reshape(8, 128), B_x[0], B_wqkv, B_wo, _TABLE)
    return out[None]
```

```python
import functools

import jax
import jax.numpy as jnp
import numpy as np
from jax import lax
from jax.experimental import pallas as pl
import jax.experimental.pallas.tpu as pltpu


S = 2048
D = 1024
T = 128
NC = S // T
NT = D // 128
NS = 4
R = S // NS
E = R // 2
WIN, DH = 8, 32
PITCH = 33
WP = 33
KR = E + 16
FP = 2 * T + 16
KW = D // 4
KA = S // 2 + 32

F32, BF16, U32 = jnp.float32, jnp.bfloat16, jnp.uint32
P = functools.partial
add, sub, mul = lax.add, lax.sub, lax.mul


def _pack_rows(m):
    b = m.astype(jnp.bfloat16).view(np.uint16).astype(np.uint32)
    return np.ascontiguousarray(b[0::2] | (b[1::2] << 16))


def _dft_table():
    th = 2.0 * np.pi * (np.arange(T) + 0.25) / T
    dft = lambda t: np.concatenate([np.cos(np.outer(th, t)), -np.sin(np.outer(th, t))], axis=0)
    paired = np.arange(T).reshape(-1, 8, 2).transpose(0, 2, 1).reshape(-1)
    ph = np.outer(np.arange(T // 2) + 0.5, th)
    mats = (dft(np.arange(T)), dft(paired - (T - 1) / 2), np.cos(ph) / T, np.sin(ph) / T)
    return np.concatenate([_pack_rows(m) for m in mats] + [np.zeros((32, T), np.uint32)], axis=0)


_TABLE = _dft_table()


def _lo(w):
    return pltpu.bitcast(lax.shift_left(w, np.uint32(16)), F32)


def _hi(w):
    return pltpu.bitcast(lax.bitwise_and(w, np.uint32(0xFFFF0000)), F32)


def _rows(first, second):
    return jnp.concatenate([first, second], axis=0)


def _tree(xs):
    while len(xs) > 1:
        xs = [add(xs[i], xs[i + 1]) if i + 1 < len(xs) else xs[i] for i in range(0, len(xs), 2)]
    return xs[0]


def _left(a11, a12, a21, a22):
    return [add(a21, a22), a22, add(a11, a12), a11, add(a11, a22), sub(a12, a22), sub(a21, a11)]


def _merge(main, side):
    if not main:
        return side
    total_m = sum(c for c, _ in main)
    total_s = sum(c for c, _ in side)
    done_m, done_s, i, out = 0, 0, 0, []
    for c, f in main:
        out.append((c * total_s, f))
        done_m += c
        while i < len(side) and (done_s + side[i][0]) * total_m <= done_m * total_s:
            done_s += side[i][0]
            out.append((side[i][0] * total_m, side[i][1]))
            i += 1
    assert i == len(side)
    return out


def _zip(main, side):
    cost = {id(f): c for c, f in main + side}
    return [(cost[id(f)], f) for _, f in _merge(main, side)]


def _run(tasks):
    for _, f in tasks:
        f()


def _weave(main, side):
    _run(_merge(main, side))


def _split(tasks, *weights):
    ends = np.cumsum((0,) + weights) * len(tasks) // sum(weights)
    return [tasks[a:b] for a, b in zip(ends[:-1], ends[1:])]


def _start(copies):
    for c in copies:
        c.start()


def _wait(copies):
    for c in copies:
        c.wait()


_BUFS = {n: (t, r) for t, group in (
    (BF16, dict(qa=NT * S // 2, ka=NT * KA, va=NT * S // 2, oa=NT * S // 2, ob=S * NT // 2,
                xs=7 * 4 * E // 2, **{f'os{i}': 7 * E // 2 for i in range(7)}, wt3=35 * KW, wt2=35 * KW, xt=35 * E // 2, w3=NT * KW,
                kv0=S // 8, kv1=S // 8, kv2=S // 8, kv3=S // 8, z=NC * T,
                **{f"ws{p}": 20 * KW for p in range(4)})),
    (U32, dict(**{f"w{p}": 2 * NT * KW for p in range(3)}, t0=34 * DH, t1=34 * DH, wp=4 * WP * DH)),
    (F32, dict(hf=NC * FP, xf=NC * FP, up=8 * NC, k1=8 * NC, pi=8 * NC, zr=8 * NC, zi=8 * NC,
               even=2 * T, **{n + '1': 4 * E for n in 'abcde'}, **{n + '2': E for n in 'abcde'},
               q=2 * NT * E + 32, k=2 * NT * KR, v=2 * NT * KR, p=WIN * R, o=NT * R + 32)),
) for n, r in group.items()}


def _kernel(q_hbm, k_hbm, v_hbm, sk_hbm, h_hbm, d_hbm, x_hbm, w_hbm, wo_hbm, tab_hbm, out_hbm,
            ha, xa, wraw, taps, tab, sem_in, sem_out, *raw):
    *raw, sk_ref, d_ref = raw
    raw = dict(zip(_BUFS, raw))
    bufs = {n: b.bitcast(U32) if _BUFS[n][0] == BF16 else b for n, b in raw.items()}

    spec = _BUFS

    def ld(name, row, n=8, z=0):
        assert 0 <= row and row + n <= views[name][z].shape[0]
        return views[name][z][pl.ds(row, n), :]

    def st(name, row, val):
        assert 0 <= row and row + val.shape[0] <= views[name][3].shape[0]
        views[name][3][pl.ds(row, val.shape[0]), :] = val

    def st16(name, row, val):
        assert 0 <= row and 2 * row + val.shape[0] <= views[name][4].shape[0]
        views[name][4][pl.ds(2 * row, val.shape[0]), :] = val.astype(BF16)

    def window(name, row, n):
        return bufs[name].at[pl.ds(pl.multiple_of(row, 8), n), :]

    def window16(name, row, n):
        return raw[name].at[pl.ds(pl.multiple_of(2 * row, 16), 2 * n), :]

    def cols(a):
        return pl.ds(pl.multiple_of(a * 128, 128), 128)

    def rows(j):
        return pl.ds(pl.multiple_of(j * R, R), R)

    def a_copies(a, sem, skip=0):
        return [pltpu.make_async_copy(src, dst, sem) for src, dst in (
            (h_hbm.at[cols(a), :], ha.at[a]),
            (k_hbm.at[:, cols(a)], window16("ka", a * KA + 32, S // 2)),
            (v_hbm.at[:, cols(a)], window16("va", a * (S // 2), S // 2)))[skip:]]

    def q_copy(a, sem):
        return pltpu.make_async_copy(q_hbm.at[:, cols(a)], window16("qa", a * (S // 2), S // 2), sem)

    def in_copies(j):
        sem = sem_in.at[j]
        out = a_copies(2 * j - 1, sem) + [q_copy(2 * j - 2, sem)]
        if isinstance(j, int) and j == NS:
            return out
        return (out + [pltpu.make_async_copy(x_hbm.at[rows(j), :], xa.at[j], sem)]
                + a_copies(2 * j, sem) + [q_copy(2 * j - 1, sem)])

    def h0_copies():
        full = pl.ds(0, 5 * T // 2)
        return [pltpu.make_async_copy(tab_hbm.at[full], tab.at[full], sem_in.at[0]),
                pltpu.make_async_copy(h_hbm.at[cols(0), :], ha.at[0], sem_in.at[0])]

    def kv0_copies():
        return a_copies(0, sem_in.at[NS + 14], 1)

    def last_q():
        return q_copy(NT - 1, sem_in.at[NS + 1])

    def x0_copy(half, sem):
        part = pl.ds(0, R), pl.ds(half * D // 2, D // 2)
        return pltpu.make_async_copy(x_hbm.at[part], xa.at[(0, *part)], sem_in.at[sem])

    def w_copy(n):
        half = pl.ds(n % 2 * (D // 2), D // 2)
        return pltpu.make_async_copy(
            w_hbm.at[half, pl.ds(n // 2 * D, D)], wraw.at[n], sem_in.at[NS + 5 + n])

    def w_wait(n):
        pltpu.make_async_copy(wraw.at[n], wraw.at[n], sem_in.at[NS + 5 + n]).wait()

    def wo_copy(n):
        return pltpu.make_async_copy(wo_hbm.at[pl.ds(n * D // 2, D // 2), :], wraw.at[6 + n],
                                     sem_in.at[NS + 11 + n])

    def oa_copy(a):
        return pltpu.make_async_copy(window16("oa", a * (S // 2), S // 2), out_hbm.at[:, cols(a)],
                                     sem_out.at[0])

    def oa_part(u):
        src = window16("oa", (4 * (NT - 1) + u) * S // 8, S // 8)
        return pltpu.make_async_copy(src, out_hbm.at[pl.ds(u * S // 4, S // 4), cols(NT - 1)],
                                     sem_out.at[0])

    def ob_copy(j, t):
        return pltpu.make_async_copy(window16("ob", (j * NT + t) * E, E),
                                     out_hbm.at[rows(j), cols(NT + t)], sem_out.at[1])

    small = [pltpu.make_async_copy(a, b, sem_in.at[NS + 13])
             for a, b in ((tab_hbm.at[pl.ds(5 * T // 2, 8)], tab.at[pl.ds(5 * T // 2, 8)]),
                          (sk_hbm, sk_ref), (d_hbm, d_ref))]
    w00 = [pltpu.make_async_copy(w_hbm.at[pl.ds(u * KW, KW), pl.ds(0, D)], wraw.at[0, pl.ds(u * KW, KW)],
                                 sem_in.at[NS + 4 + u]) for u in range(2)]
    startup = lambda: (w00 + [x0_copy(0, NS + 2), w_copy(1), x0_copy(1, 0)] + h0_copies() + kv0_copies()
                       + [w_copy(2), w_copy(3), wo_copy(0), w_copy(4), wo_copy(1), w_copy(5)])
    _start(small + startup())
    _wait(small)
    unit = pltpu.bitcast(tab[pl.ds(5 * T // 2, 8), :], jnp.int32)
    zs = [pl.multiple_of(unit[i, 0] * 8, 8) for i in range(3)]
    views = {n: [b.at[pl.ds(z, spec[n][1]), :] for z in zs] + [b, raw[n]] for n, b in bufs.items()}

    for a in range(NT):
        st("ka", a * KA + 24, jnp.zeros((8, 128), U32))
    for t in range(2 * NT):
        st("k", t * KR, jnp.zeros((WIN, 128), F32))
    skf = sk_ref[...].astype(F32)
    df = d_ref[...].astype(F32)
    for t in range(NT):
        for i in range(4):
            taps[t, i] = jnp.broadcast_to(skf[i:i + 1, t * 128:(t + 1) * 128], (8, 128))
        taps[t, 4] = jnp.broadcast_to(df[t:t + 1, :], (8, 128))

    def step(j, first=False, last=False):
        memo = {}
        never = tab[pl.ds(5 * T // 2, 8), :] != 0

        def once(key, fn):
            if key not in memo:
                memo[key] = fn()
            return memo[key]

        def fresh():
            memo["fresh"] = memo.get("fresh", 1) + 1
            return pl.multiple_of(zs[0] * memo["fresh"], 8)

        def pace(val):
            clock = memo.get("clock")
            if clock is None:
                return val
            if val.dtype != F32:
                clock = pltpu.bitcast(clock, val.dtype)
            return lax.select(never, clock, val)

        def paced(x):
            return jnp.concatenate([pace(x[:8]), x[8:]], axis=0)

        def wait(copies):
            memo["clock"] = None
            _wait(copies)

        def rolled(n, shifts, body):
            def one(i, carry):
                saved, kept = dict(views), dict(memo)
                memo["clock"] = None
                for name, d in shifts.items():
                    size = spec[name][1] - d * (n - 1)
                    views[name] = [window(name, z + d * i, size) for z in zs + [0]]
                    if spec[name][0] == BF16:
                        views[name].append(window16(name, d * i, size))
                body(i)
                views.update(saved)
                memo.clear()
                memo.update(kept, clock=None)
                return carry
            lax.fori_loop(0, n, one, 0)

        def perm_in(w, u, t):
            tt = paced(pltpu.bitcast(w[pl.ds(u * 256, 256), pl.ds(t * 128, 128)], U32)).T
            for hh in range(4):
                st(f"t{u}", (4 * t + hh) * PITCH, tt[hh * DH:(hh + 1) * DH])

        def perm_out(p, h, u, t):
            g = jnp.concatenate(
                [bufs[f"t{u}"][pl.ds(zs[0] + 4 * t + i, 32, stride=PITCH), :] for i in range(4)], axis=0)
            st(f"w{p}", (h * NT + t) * KW + u * 128, paced(g).T)

        def perm_list(n, w=None, us=(0, 1)):
            w = wraw.at[n] if w is None else w
            return [(1, P(f, u, t)) for f in (P(perm_in, w), P(perm_out, n // 2, n % 2))
                    for u in us for t in range(NT)] + [(2, lambda: None)] * 4

        def wo_in(w, t, hh):
            w = pltpu.bitcast(w[pl.ds(hh * DH, DH), pl.ds(t * 128, 128)], U32)
            st("wp", (16 * t + hh) * WP, _rows(pace(w[:8]), pace(w[8:])))

        def wo_list(w):
            return [(4, P(wo_in, w, t, hh)) for t in range(NT) for hh in range(16)]

        LEFT = ((2, add, 3), (3,), (0, add, 1), (0,), (0, add, 3), (1, sub, 3), (2, sub, 0))
        RIGHT = ((0,), (2, sub, 0), (3,), (1, sub, 3), (0, add, 3), (2, add, 3), (0, add, 1))

        def wo_out(t, dh):
            b = [bufs["wp"][pl.ds(zs[dh % 2] + 16 * (t + n % 2 * 4) * WP + n // 2 * 8 + dh // 2, 16, stride=WP), :]
                 for n in range(4)]
            b = [(_lo, _hi)[dh % 2](w) for w in [paced(b[0])] + b[1:]]
            for i, (b0, *rest) in enumerate(RIGHT):
                name, n = ("ws3", 4 * (i - 1 - (i > 2))) if rest else ("w3", i * 2)
                st16(name, (n + t) * KW + 16 * dh, rest[0](b[b0], b[rest[1]]) if rest else b[b0])

        def wo_out_list():
            return [(26, P(wo_out, t, dh)) for t in range(4) for dh in range(16)]

        def right2(p, r, i):
            u, m = divmod(r, KW // 2)
            w = [factor(p, i, u + c % 2 * 2, c // 2 * KW // 2 + m, 8, 1) for c in range(4)]
            w[0], w[3] = pace(w[0]), pace(w[3])
            b = [pltpu.bitcast(x, BF16).astype(F32) for x in w]
            for k in (1, 3, 4, 5, 6):
                st16(f"wt{p}", (5 * i + k - 1 - (k > 2)) * KW + r, RIGHT[k][1](b[RIGHT[k][0]], b[RIGHT[k][2]]))

        def right2_list(p, step):
            return [(25, P(right2, p, r, i)) for i in ORDER for r in range(0, 16 * step, step)]

        def right(p, t, r):
            b = [ld(f"w{p}", (h * NT + t + 4 * u) * KW + r, 16) for h in range(2) for u in range(2)]
            mask = 1 if p else 9
            b = [_rows(pace(x[:8]), pace(x[8:])) if mask >> c & 1 else x for c, x in enumerate(b)]
            b11, b12, b21, b22 = (pltpu.bitcast(x, BF16).astype(F32) for x in b)
            for i, val in enumerate((sub(b21, b11), sub(b12, b22), add(b11, b22),
                                     add(b21, b22), add(b11, b12))):
                st16(f"ws{p}", (4 * i + t) * KW + r, val)

        def right_list(p):
            return [(1, P(right, p, t, r)) for t in range(4) for r in range(0, KW, 16)]

        def ld_kv(c, row, n, z=0):
            return ld(f"kv{c // 4}", c % 4 * (T // 2) + row, n, z)

        def a1(i, r):
            a = once(("a", i), lambda: 2 * j + i)
            w0, w1, w2, w3 = once(("taps", i), lambda: [taps[a, u] for u in range(4)])
            k32 = once(("ka", i), lambda: window("ka", a * KA, KA))
            v32 = once(("va", i), lambda: window("va", a * (S // 2), S // 2))
            c0, c1, c2 = (k32[pl.ds(8 * r + 32 - u, 8), :] for u in range(3))
            vv = v32[pl.ds(8 * r, 8), :]
            e0, o0, e1, o1, o2 = _lo(c0), _hi(c0), _lo(c1), _hi(c1), _hi(c2)
            ke = _tree([mul(e0, w0), mul(o1, w1), mul(e1, w2), mul(o2, w3)])
            ko = _tree([mul(o0, w0), mul(e0, w1), mul(o1, w2), mul(e1, w3)])
            st16(f"kv{r // 32}", 8 * (r % 32), _rows(mul(ke, _lo(vv)), pace(mul(ko, _hi(vv)))))

        def a1_list(i, c0, c1):
            return [(24, P(a1, i, r)) for r in range(8 * c0, 8 * c1)]

        def freq(c, im, m):
            return c * FP + im * (T + 8) + m

        def dft(i, name, c0, m):
            def mm():
                f = pltpu.bitcast(tab[pl.ds(fresh() + T * (name == "xf"), T), :], BF16)
                if name == "hf":
                    a = once(("a", i), lambda: 2 * j + i)
                    rhs = jnp.concatenate(
                        [ha[a, :, pl.ds(c * T, T)] for c in range(c0, c0 + 4)], axis=0)
                    return lax.dot_general(f, rhs, (((1,), (1,)), ((), ())),
                                           preferred_element_type=F32)
                rhs = jnp.concatenate(
                    [pltpu.bitcast(ld_kv(c, 0, T // 2, i % 2), BF16) for c in range(c0, c0 + 4)], axis=1)
                return jnp.dot(f, rhs, preferred_element_type=F32)
            res = once((name, i, c0), mm)
            for u in range(4):
                val = res[m:m + 16, u * 128:(u + 1) * 128]
                if name == "hf" and c0 + u == 0 and m < T:
                    val = add(val, once(("dd", i), lambda: _rows(*[taps[memo["a", i], 4]] * 2)))
                st(name, freq(c0 + u, m // T, m % T), val)
            memo["clock"] = res[m + 8:m + 16, 384:]

        def dft_list(i, name, *c0s):
            return [(16, P(dft, i, name, c0, m)) for c0 in c0s for m in range(0, 2 * T, 16)]

        def a3(i, g, plane, upper, n):
            def opnd(name, c):
                re = lambda: ld(name, freq(c, 0, 8 * g), z=plane)
                im = lambda: ld(name, freq(c, 1, 8 * g), z=plane)
                if name == "xf":
                    val = add(re(), im()) if plane == 0 else re() if plane == 1 else im()
                    return pace(val) if c >= 8 else val
                return pace(re() if plane == 0 else (sub, add)[plane - 1](im(), re()))
            get = lambda name, c: once((name, i, g, plane, c), P(opnd, name, c))
            done = pace if n % 4 == 3 else lambda v: v
            cs = range(8, n + 1) if upper else range(min(n, 7) + 1)
            terms = [mul(get("xf", n - c), get("hf", c)) for c in cs]
            if upper:
                st("up", 8 * n, done(_tree(terms)))
                return
            if n >= 8:
                terms.append(ld("up", 8 * n))
            if plane == 0:
                st("k1", 8 * n, done(_tree(terms)))
            elif plane == 1:
                st("pi", 8 * n, done(_tree(terms + [ld("k1", 8 * n)])))
            else:
                pr = sub(ld("k1", 8 * n, z=1), _tree(terms))
                pi = ld("pi", 8 * n)
                zr, zi = pr, pi
                if n > 0:
                    qr, qi = memo["prev"]
                    zr, zi = sub(pr, qi), add(pi, qr)
                memo["prev"] = (pr, pi)
                if g % 2 == 0:
                    st("zr", 8 * n, done(zr))
                    st("zi", 8 * n, zi)
                else:
                    st16("z", n * T + 4 * (g - 1), _rows(ld("zr", 8 * n), done(zr)))
                    st16("z", n * T + T // 2 + 4 * (g - 1), _rows(ld("zi", 8 * n), zi))

        def a3_list(i):
            out = []
            for g in range(T // 8):
                for plane in range(3):
                    out += [(2 * (n - 8) + 4, P(a3, i, g, plane, True, n)) for n in range(8, NC)]
                    out += [(2 * min(n, 7) + 4 + 2 * (plane == 2), P(a3, i, g, plane, False, n))
                            for n in range(NC)]
            return out

        def idft(i, c0, odd, m):
            def mm():
                rhs = jnp.concatenate([pltpu.bitcast(ld("z", c * T + odd * T // 2, T // 2, i + 2), BF16)
                                       for c in range(c0, c0 + 4)], axis=1)
                f = tab[pl.ds(fresh() + 2 * T + odd * T // 4, T // 4), :]
                return jnp.dot(pltpu.bitcast(f, BF16), rhs, preferred_element_type=F32)
            y = once(("y", i, c0, odd), mm)
            a = once(("a", i), lambda: 2 * j + i)
            q16 = once(("qa", i), lambda: window16("qa", a * (S // 2), S // 2))
            o16 = once(("oa", i), lambda: window16("oa", a * (S // 2), S // 2))
            flip = lambda w: jnp.take_along_axis(
                w, 7 - lax.broadcasted_iota(jnp.int32, (8, 128), 0), axis=0, mode="promise_in_bounds")
            for u in range(4):
                val = y[m:m + 16, u * 128:(u + 1) * 128]
                if not odd:
                    st("even", u * T // 2 + m, val)
                    continue
                even, mid = ld("even", u * T // 2 + m, 16), (c0 + u) * T + T // 2
                low = add(even, val)
                for row, out in ((mid + m, sub(even, val)),
                                 (mid - 16 - m, _rows(flip(low[8:]), flip(low[:8])))):
                    o16[pl.ds(row, 16), :] = mul(q16[pl.ds(row, 16), :].astype(F32), out).astype(BF16)
            memo["clock"] = y[m + 8:m + 16, 384:]

        def idft_list(i, *c0s):
            return [(16, P(idft, i, c0, odd, m)) for c0 in c0s
                    for odd in range(2) for m in range(0, T // 2, 16)]

        def transforms(i, extra, shares=(1, 1, 1, 1, 1, 9)):
            extra = _split(extra, *shares)
            for u in range(4):
                _weave(idft_list(i - 1, 4 * u)[:4], extra[u])
                _run(idft_list(i - 1, 4 * u)[4:])
                _weave(dft_list(i, "hf", 4 * u), a1_list(i, 3 * u, 3 * u + 3))
            oa_copy(2 * j + i - 1).start()
            _weave(dft_list(i, "xf", 0), _merge(a1_list(i, 12, 16), extra[4]))
            _weave(dft_list(i, "xf", 4, 8), extra[5])
            _run(dft_list(i, "xf", 12))

        def xprep(x, u, r):
            halves = []
            for m in (r, r + 8):
                a, b = (pltpu.bitcast(x[pl.ds(2 * m, 16), pl.ds(t * 128, 128)], U32)
                        for t in (u, u + 4))
                a = pace(a)
                a11, a12, a21, a22 = _lo(a), _lo(b), _hi(a), _hi(b)
                halves.append(_left(a11, a12, a21, a22))
            for i, pair in enumerate(zip(*halves)):
                st16("xs", ((4 * i + u) * E + r) // 2, jnp.concatenate(pair, axis=0))

        def xprep_list(x):
            return [(27, P(xprep, x, u, r)) for r in range(0, E, 16) for u in range(4)]

        def lhs(name, i, m0=0, n=E):
            view = views[name][3].at[pl.ds(fresh() + i * 2 * E, 2 * E), :]
            return jnp.concatenate(
                [pltpu.bitcast(view[pl.ds((u * E + m0) // 2, n // 2), :], BF16) for u in range(4)], axis=1)

        def emit(p, par, t, m, val, start=0, end=E):
            if p == 0:
                st("q", (par * NT + t) * E + m, val)
                return
            if p == 3:
                o16 = once("ob", lambda: window16("ob", (j - 1) * NT * E, NT * E))
                o16[pl.ds(t * R + par * E + m, 16), :] = val.astype(BF16)
                if m + 16 == end and par == t // 4:
                    ob_copy(j - 1, t).start()
                return
            name, row = "kv"[p - 1], (par * NT + t) * KR
            if m == start and not first:
                st(name, row, ld(name, row + E, WIN, z=3))
            if m == 0 and first and p == 2 and par == 0:
                for other in range(2):
                    st(name, (other * NT + t) * KR, jnp.broadcast_to(val[0:1], (WIN, 128)))
            st(name, row + WIN + m, val)

        def plain(x, half, t, m):
            def mm():
                w = pltpu.bitcast(ld("w0", (half * NT + t) * KW, KW, 3), BF16)
                return jnp.dot(x[:, pl.ds(half * D // 2, D // 2)], w, preferred_element_type=F32)
            res = once(("plain", half, t), mm)
            memo["clock"] = res[m + 8:m + 16]
            if half:
                st("q", t * R + m, add(res[m:m + 16], ld("o", t * R + m, 16)))
            else:
                st("o", t * R + m, res[m:m + 16])

        def plain_list(x, half):
            return [(16, P(plain, x, half, t, m)) for t in range(NT) for m in range(0, x.shape[0], 16)]

        def combine(level, i, row, res, out):
            get = lambda name, z=0: ld(name + level, row, 16, z)
            if i % 2 == 0 and i < 6:
                st("abc"[i // 2] + level, row, res)
            elif i == 1:
                st("d" + level, row, sub(res, get("b")))
                out(1, 0, add(get("a"), res))
            elif i == 3:
                st("e" + level, row, sub(res, get("a", 1)))
                out(0, 1, add(get("b", 1), res))
            else:
                out(i - 5, i - 5, add(add(get("de"[i - 5]), get("c", i - 5)), res))

        def factor(p, i, t, r=0, n=KW, z=3):
            if i in (0, 2):
                return ld(f"w{p}", (t + (4 if p == 3 else NT + 4) * i // 2) * KW + r, n, z)
            return ld(f"ws{p}", (4 * (i - 1 - (i > 2)) + t) * KW + r, n, z)

        def product(p, m0, n, t, i, m):
            res = once(("product", p, m0, t, i), lambda: jnp.dot(
                lhs(*(("xs", i) if p < 3 or m0 else (f"os{i}", 0)), m0, n), pltpu.bitcast(factor(p, i, t), BF16),
                preferred_element_type=F32))
            memo["clock"] = res[m - m0 + 8:m - m0 + 16]
            combine("1", i, t * E + m, res[m - m0:m - m0 + 16],
                    lambda par, h, val: emit(p, par, t + 4 * h, m, val))

        ORDER = (0, 2, 1, 4, 5, 3, 6)

        def strassen(p, m0=0, n=E):
            return [(16, P(product, p, m0, n, t, i, m))
                    for t in range(4) for i in ORDER for m in range(m0, m0 + n, 16)]

        def product2(p, i, k, m):
            def mm():
                if p == 3:
                    name, rows = f"os{i}", [(k * 2 + u) * E // 4 for u in range(2)]
                elif k in (1, 3):
                    name, rows = "xs", [(4 * i + u + 2 * (k == 1)) * E // 2 + (k == 1) * E // 4 for u in range(2)]
                else:
                    name, rows = "xt", [((5 * i + k // 2 + (k > 4) * (k - 4 - (k > 5))) * 2 + u) * E // 4 for u in range(2)]
                view = views[name][3].at[pl.ds(fresh(), spec[name][1]), :]
                x = jnp.concatenate([pltpu.bitcast(view[pl.ds(row, E // 4), :], BF16) for row in rows], axis=1)
                if k in (0, 2):
                    w = [factor(p, i, k + u, k * KW // 4, KW // 2) for u in range(2)]
                else:
                    w = [ld(f"wt{p}", ((5 * i + k - 1 - (k > 2)) * 2 + u) * KW // 2, KW // 2, 3) for u in range(2)]
                return jnp.dot(x, jnp.concatenate([pltpu.bitcast(v, BF16) for v in w], axis=1),
                               preferred_element_type=F32)
            res = once(("product2", p, i, k), mm)
            memo["clock"] = res[m + 8:m + 16, 128:]

            def out(u, r2, c2, val):
                t, row = 2 * c2 + u, r2 * E // 2 + m
                combine("1", i, t * E + row, val, lambda par, h, v: emit(
                    p, par, t + 4 * h, row, v, (1 - c2) * E // 2, (1 + c2) * E // 2))
            for u in range(2):
                combine("2", k, u * E // 2 + m, res[m:m + 16, u * 128:(u + 1) * 128], P(out, u))

        def strassen2(p):
            return [(16, P(product2, p, i, k, m))
                    for i in ORDER for k in ORDER for m in range(0, E // 2, 16)]

        def xprep2(x, u, r, i):
            def blk(b):
                w = once(("x", u, r, b % 2), lambda: [pltpu.bitcast(
                    x[pl.ds(c // 2 * E + 2 * r, 32), pl.ds((u + c % 2 * 2 + b % 2 * 4) * 128, 128)], U32)
                    for c in range(4)])
                return [(_lo, _hi)[b // 2](v) for v in w]
            b0, *rest = LEFT[i]
            a = list(once(("left", u, r, b0), P(blk, b0)))
            a[0], a[3] = paced(a[0]), paced(a[3])
            if rest:
                a = list(map(rest[0], a, once(("left", u, r, rest[1]), P(blk, rest[1]))))
            for n, k in enumerate((0, 2, 4, 5, 6)):
                st16("xt", ((5 * i + n) * 2 + u) * E // 4 + r // 2, LEFT[k][1](a[LEFT[k][0]], a[LEFT[k][2]]))

        def xprep2_list(x):
            return [(c, P(xprep2, x, u, r, i)) for r in range(0, E // 2, 16) for u in range(2)
                    for i, c in ((1, 25), (0, 33), (6, 33), (4, 25), (3, 17), (5, 33), (2, 25))]

        def oprep2(i, u, r):
            view = once(("oprep", i), lambda: bufs["o"].at[pl.ds(fresh(), spec["o"][1]), :])
            blk = lambda b, c: view[pl.ds(
                (u + 2 * (c % 2) + 4 * (b % 2)) * R + b // 2 * E + c // 2 * E // 2 + r, 16), :]
            b0, *rest = LEFT[i]
            a = [blk(b0, c) for c in range(4)]
            a[3] = paced(a[3])
            a[0] = paced(a[0])
            if rest:
                a = [rest[0](x, blk(rest[1], c)) for c, x in enumerate(a)]
            for k, val in enumerate(_left(*a)):
                st16(f"os{i}", (k * 2 + u) * E // 4 + r // 2, val)

        def oprep2_list():
            return [(19 + 8 * (len(LEFT[i]) > 1), P(oprep2, i, u, r))
                    for i in ORDER for r in range(0, E // 2, 16) for u in range(2)]

        def qk(r, w):
            par, m = divmod(8 * r, E)
            query = lambda t: (bufs["q"][pl.ds(memo["parity"] + t * R + 2 * m, 8, stride=2), :] if first
                               else ld("q", (par * NT + t) * E + m))
            qv = once(("qv", r), lambda: [pace(query(t)) for t in range(NT)])
            s = pace(_tree([mul(qv[t], ld("k", (par * NT + t) * KR + WIN + m - w)) for t in range(NT)]))
            s = add(s, pltpu.roll(s, 64, 1))
            s = add(s, pltpu.roll(s, 32, 1))
            if first and m < w:
                keep = m + lax.broadcasted_iota(jnp.int32, (8, 128), 0) >= w
                s = jnp.where(keep, s, -1e9 * DH ** 0.5)
            memo["lg", r, w] = s

        def expo(r):
            lg = [memo["lg", r, w] for w in range(WIN)]
            m = pace(functools.reduce(lax.max, lg))
            scale = np.float32(DH ** -0.5 * np.log2(np.e))
            memo["e", r] = [lax.exp2(mul(sub(s, m), scale)) for s in lg]

        def norm(r):
            total = pace(_tree(memo["e", r]))
            memo["inv", r] = total, pl.reciprocal(total, approx=True)

        def probs(r):
            total, inv = memo["inv", r]
            inv = pace(inv)
            inv = mul(inv, sub(np.float32(2), mul(total, inv)))
            for w in range(WIN):
                st("p", w * R + 8 * r, mul(memo["e", r][w], inv))

        def qk_list(nr=R // 8):
            out, q0, q1 = [], 26 if first else 24, 3
            for i in range(WIN * nr + q0 + 2 * q1 - 7):
                r, w = divmod(i, WIN)
                tasks = [P(qk, r, w)] if r < nr else []
                for f, lag in ((expo, q0), (norm, q0 + q1), (probs, q0 + 2 * q1)):
                    if i >= lag and (i - lag) % WIN == 0 and (i - lag) // WIN < nr:
                        tasks.append(P(f, (i - lag) // WIN))
                out.append((26 if r < nr else 12, P(_run, [(0, f) for f in tasks])))
            return out

        def pv(r, t):
            par, m = divmod(8 * r, E)
            p = once(("pv", r), lambda: [(pace if w % 4 == 0 else lambda v: v)(ld("p", w * R + 8 * r)) for w in range(WIN)])
            row = (par * NT + t) * KR + WIN + m
            bufs["o"][pl.ds(t * R + 2 * m + par, 8, stride=2), :] = pace(
                _tree([mul(p[w], ld("v", row - w)) for w in range(WIN)]))

        def pv_list():
            return [(16, P(pv, r, t)) for r in range(R // 8) for t in range(NT)]

        def oprep(u, r):
            a = [ld("o", (u + 4 * h) * R + par * E + r, 16, 1) for par in range(2) for h in range(2)]
            for i, val in enumerate(_left(*a[:3], paced(a[3]))):
                if last and 2 * r >= E:
                    st16("xs", ((4 * i + u) * E + r) // 2, val)
                else:
                    st16(f"os{i}", (u * E + r) // 2, val)

        def oprep_list():
            return [(18, P(oprep, u, r)) for r in range(0, E, 16) for u in range(4)]

        if last:
            mix = []
            for r in range(E // 16):
                for base in (0, E // 2, E, 3 * E // 2):
                    mix += pv_list()[base + 8 * r:base + 8 * r + 8]
                mix += oprep_list()[4 * r:4 * r + 4]
            mix, conv = _split(mix, 1, 1), _split(a3_list(-1), 2, 3)
            transforms(-1, mix[0], (3, 3, 3, 3, 2, 9))
            wait([last_q()])
            _weave(strassen(3, 0, E // 2), mix[1] + conv[0])
            _weave(strassen(3, E // 2, E // 2)[:-24], conv[1])
            _run(strassen(3, E // 2, E // 2)[-24:-16])
            for u in range(4):
                _run(idft_list(-1, 4 * u))
                oa_part(u).start()
            _run(strassen(3, E // 2, E // 2)[-16:])
            return

        if first:
            def leading(i):
                w = wraw.at[0, pl.ds(pl.multiple_of(i * KW, KW), KW)]
                pltpu.make_async_copy(w, w, sem_in.at[NS + 4 + i]).wait()
                _run(perm_list(0, w, (0,)))
            rolled(2, dict(w0=128), leading)
            wait([x0_copy(0, NS + 2)])
            main, a0, a1_, a2 = plain_list(xa.at[0], 0), 96, 186, 250
            _run(main[:a0])
            wait([w_copy(1)])
            _weave(main[a0:a1_], perm_list(1))
            _weave(main[a1_:a2], right_list(0))
            _run(main[a2:])
            wait([x0_copy(1, 0)] + h0_copies())
            main = plain_list(xa.at[0], 1)
            _weave(dft_list(0, "hf", 0, 4, 8, 12) + main[:26], xprep_list(xa.at[0]))
            _run(main[26:32])
            wait(kv0_copies())
            _start(in_copies(1))
            _weave(main[32:64], a1_list(0, 0, 8))
            _weave(dft_list(0, "xf", 0), a1_list(0, 8, 12))
            _weave(dft_list(0, "xf", 4), a1_list(0, 12, 16))
            _run(dft_list(0, "xf", 8, 12))

            def queries(i):
                w_wait(2 + i)
                _weave(main[64:64 + 90], _merge(perm_list(2, wraw.at[2 + i]), a3_list(0)[:288]))
                _run(main[64 + 90:160])
            rolled(2, dict(w1=NT * KW, w0=3 * KW, o=3 * R, q=3 * R, hf=32, xf=32, z=16), queries)

            def keys(i):
                k0, k1, kr, g0, g1 = 112, 220, 26, 9, 3
                conv = a3_list(0)[576:864]
                main = strassen(1)[:224]
                main = main[:32] + main[112:144] + main[32:112] + main[144:]
                w_wait(6 + i)
                _weave(main[:kr], right_list(1)[:32])
                _weave(main[kr:k0], _zip(wo_list(wraw.at[6 + i]), conv[:24 * g1]) + _zip(conv[24 * g1:24 * g0], wo_out_list()))
                memo["clock"] = None
                w_wait(4 + i)
                _weave(main[k0:k1], _merge(perm_list(4, wraw.at[4 + i]), _zip(right2_list(3, 16), conv[24 * g0:])))
                _run(main[k1:])
            rolled(2, dict(w1=2 * KW, ws1=2 * KW, w2=NT * KW, k=2 * KR, hf=32, xf=32, z=16,
                           w3=8, ws3=8, wt3=8), keys)
            _start(in_copies(2) + in_copies(3) + in_copies(NS) + [last_q()])

            def values(i):
                memo["parity"] = i
                main, v0 = strassen(2)[:112] + strassen(2)[224:336], 26
                vm = 1
                if vm & 1:
                    main = main[:32] + main[112:144] + main[32:112] + main[144:]
                _weave(main[:v0], right_list(2)[:16] + right_list(2)[32:48])
                if vm & 2:
                    _weave(main[v0:], qk_list(E // 8))
                elif vm & 4:
                    _weave(main[v0:60], right2_list(2, 8)[:56])
                    _weave(main[60:], _merge(qk_list(E // 8), right2_list(2, 8)[56:]))
                else:
                    _weave(main[v0:], _merge(right2_list(2, 8), qk_list(E // 8)))
            rolled(2, dict(w2=KW, ws2=KW, wt2=KW // 2, v=KR, k=NT * KR, p=E), values)
            return

        head = strassen(0) + strassen(1)
        two = True
        pre = _split(oprep2_list(), 2, 2, 3) if two else _split(oprep_list(), 3, 1, 0)
        transforms(-1, xprep_list(xa.at[j]))
        _weave(head[:420], a3_list(-1))
        _weave(head[420:515], xprep2_list(xa.at[j]))
        _weave(head[515:770], pv_list())
        _run(head[770:770 + 6])
        transforms(0, pre[0], (0, 0, 0, 0, 1, 9))
        if two:
            conv = _split(a3_list(0), 1, 1)
            _weave(head[770 + 6:] + strassen2(3), pre[1] + _zip(conv[0], pre[2]) + conv[1])
        else:
            _weave(head[818:] + strassen(3), pre[1] + a3_list(0))
        _weave(strassen2(2) if True else strassen(2), qk_list())

    def loop(j, carry):
        _wait(in_copies(j))
        step(j)
        return carry

    step(0, first=True)
    lax.fori_loop(1, NS, loop, 0)
    _wait(in_copies(NS))
    step(NS, last=True)
    for i, name in enumerate(("oa", "ob")):
        pltpu.make_async_copy(raw[name], raw[name], sem_out.at[i]).wait()


@jax.jit
def pallas_concat_heads__ssm_conv_h3__sliding_local_dilated__prompt_kernel(
    A_q, A_k, A_v, A_shift_k, A_ssm_k, A_ssm_D, B_x, B_wqkv, B_wo,
):
    hbm = pl.BlockSpec(memory_space=pl.ANY)
    out = pl.pallas_call(
        _kernel,
        in_specs=[hbm] * 10,
        out_specs=hbm,
        out_shape=jax.ShapeDtypeStruct((S, 2 * D), BF16),
        scratch_shapes=[
            pltpu.VMEM((NT, 128, S), BF16),
            pltpu.VMEM((NS, R, D), BF16),
            pltpu.VMEM((8, D // 2, D), BF16),
            pltpu.VMEM((NT, 5, 8, 128), F32),
            pltpu.VMEM(_TABLE.shape, U32),
            pltpu.SemaphoreType.DMA((NS + 15,)),
            pltpu.SemaphoreType.DMA((2,)),
        ] + [pltpu.VMEM((r * 4 // np.dtype(t).itemsize, 128), t) for t, r in _BUFS.values()]
        + [pltpu.VMEM((4, D), BF16), pltpu.VMEM((8, 128), BF16)],
        compiler_params=pltpu.CompilerParams(vmem_limit_bytes=100 * 1024 * 1024,
                                             disable_bounds_checks=True,
                                             disable_semaphore_checks=True),
        name="fused",
    )(A_q[0], A_k[0], A_v[0], A_shift_k.T, A_ssm_k,
      A_ssm_D.reshape(8, 128), B_x[0], B_wqkv, B_wo, _TABLE)
    return out[None]
```

```python
import functools

import jax
import jax.numpy as jnp
import numpy as np
from jax import lax
from jax.experimental import pallas as pl
import jax.experimental.pallas.tpu as pltpu


S = 2048
D = 1024
T = 128
NC = S // T
NT = D // 128
NS = 4
R0 = 512
R = (S - R0) // NS
E0, E, HS = R0 // 2, R // 2, S // 2
WIN, DH = 8, 32
LOG2E = float(np.log2(np.e))
PITCH = 33
WP = 33
KR, KL = HS + 16, E0 + 16
FP = 2 * T + 16
KW = D // 4
KA = S // 2 + 32

F32, BF16, U32 = jnp.float32, jnp.bfloat16, jnp.uint32
P = functools.partial
add, sub, mul = lax.add, lax.sub, lax.mul


def _pack_rows(m):
    b = m.astype(jnp.bfloat16).view(np.uint16).astype(np.uint32)
    return np.ascontiguousarray(b[0::2] | (b[1::2] << 16))


def _dft_table():
    th = 2.0 * np.pi * (np.arange(T) + 0.25) / T
    dft = lambda t: np.concatenate([np.cos(np.outer(th, t)), -np.sin(np.outer(th, t))], axis=0)
    paired = np.arange(T).reshape(-1, 8, 2).transpose(0, 2, 1).reshape(-1)
    ph = np.outer(np.arange(T // 2) + 0.5, th)
    mats = (dft(np.arange(T)), dft(paired - (T - 1) / 2), np.cos(ph) / T, np.sin(ph) / T)
    return np.concatenate([_pack_rows(m) for m in mats] + [np.zeros((32, T), np.uint32)], axis=0)


_TABLE = _dft_table()


def _lo(w):
    return pltpu.bitcast(lax.shift_left(w, np.uint32(16)), F32)


def _hi(w):
    return pltpu.bitcast(lax.bitwise_and(w, np.uint32(0xFFFF0000)), F32)


def _rows(first, second):
    return jnp.concatenate([first, second], axis=0)


def _tree(xs):
    while len(xs) > 1:
        xs = [add(xs[i], xs[i + 1]) if i + 1 < len(xs) else xs[i] for i in range(0, len(xs), 2)]
    return xs[0]


def _left(a11, a12, a21, a22):
    return [add(a21, a22), a22, add(a11, a12), a11, add(a11, a22), sub(a12, a22), sub(a21, a11)]


def _merge(main, side):
    if not main:
        return side
    total_m = sum(c for c, _ in main)
    total_s = sum(c for c, _ in side)
    done_m, done_s, i, out = 0, 0, 0, []
    for c, f in main:
        out.append((c * total_s, f))
        done_m += c
        while i < len(side) and (done_s + side[i][0]) * total_m <= done_m * total_s:
            done_s += side[i][0]
            out.append((side[i][0] * total_m, side[i][1]))
            i += 1
    assert i == len(side)
    return out


def _zip(main, side):
    cost = {id(f): c for c, f in main + side}
    return [(cost[id(f)], f) for _, f in _merge(main, side)]


def _run(tasks):
    for _, f in tasks:
        f()


def _weave(main, side):
    _run(_merge(main, side))


def _split(tasks, *weights):
    ends = np.cumsum((0,) + weights) * len(tasks) // sum(weights)
    return [tasks[a:b] for a, b in zip(ends[:-1], ends[1:])]


def _start(copies):
    for c in copies:
        c.start()


def _wait(copies):
    for c in copies:
        c.wait()


_BUFS = {n: (t, r) for t, group in (
    (BF16, dict(qa=NT * HS, ka=NT * KA, va=NT * HS, oa=NT * HS, ob=NT * HS,
                xs=14 * E0, xt=35 * E0 // 2, **{f"os{i}": 7 * E0 // 2 for i in range(7)},
                kv0=S // 8, kv1=S // 8, kv2=S // 8, kv3=S // 8, z=NC * T, w3=NT * KW, xu=14 * E0,
                **{f"ws{p}": 20 * KW for p in range(4)}, wt0=20 * KW, wt2=35 * KW, wt3=35 * KW)),
    (U32, dict(**{f"w{p}": 2 * NT * KW for p in range(3)}, t0=34 * DH, t1=34 * DH, wp=4 * WP * DH)),
    (F32, dict(hf=NC * FP, xf=NC * FP, up=8 * NC, k1=8 * NC, pi=8 * NC, zr=8 * NC, zi=8 * NC,
               even=2 * T, pair=8 * WIN, quad=8 * WIN, **{n + "1": 4 * E0 for n in "abcde"}, **{n + "2": E0 for n in "abcde"},
               q=NT * R0 + 32, k=2 * NT * KL, v=2 * NT * KR, p=WIN * S, o=NT * R0 + 32)),
) for n, r in group.items()}


def _kernel(q_hbm, k_hbm, v_hbm, sk_hbm, h_hbm, d_hbm, x_hbm, w_hbm, wo_hbm, tab_hbm, out_hbm,
            ha, xa, wraw, taps, tab, sem_in, sem_out, *raw):
    *raw, sk_ref, d_ref = raw
    raw = dict(zip(_BUFS, raw))
    bufs = {n: b.bitcast(U32) if _BUFS[n][0] == BF16 else b for n, b in raw.items()}

    spec = _BUFS

    def ld(name, row, n=8, z=0):
        assert 0 <= row and row + n <= views[name][z].shape[0]
        return views[name][z][pl.ds(row, n), :]

    def st(name, row, val):
        assert 0 <= row and row + val.shape[0] <= views[name][3].shape[0]
        views[name][3][pl.ds(row, val.shape[0]), :] = val

    def st16(name, row, val):
        assert 0 <= row and 2 * row + val.shape[0] <= views[name][4].shape[0]
        views[name][4][pl.ds(2 * row, val.shape[0]), :] = val.astype(BF16)

    def window(name, row, n):
        return bufs[name].at[pl.ds(pl.multiple_of(row, 8), n), :]

    def window16(name, row, n):
        return raw[name].at[pl.ds(pl.multiple_of(2 * row, 16), 2 * n), :]

    def cols(a):
        return pl.ds(pl.multiple_of(a * 128, 128), 128)

    def rows(j):
        return pl.ds(pl.multiple_of(R0 + j * R, 128), R)

    def a_copies(a, sem):
        return [pltpu.make_async_copy(src, dst, sem) for src, dst in (
            (h_hbm.at[cols(a), :], ha.at[a]),
            (k_hbm.at[:, cols(a)], window16("ka", a * KA + 32, HS)),
            (v_hbm.at[:, cols(a)], window16("va", a * HS, HS)))]

    def in_copies(j, late):
        sem = sem_in.at[2 * j + late]
        if not late:
            return [pltpu.make_async_copy(x_hbm.at[rows(j), :], xa.at[rows(j), :], sem)] + a_copies(2 * j, sem)
        return a_copies(2 * j + 1, sem) + [
            pltpu.make_async_copy(q_hbm.at[:, cols(a)], window16("qa", a * HS, HS), sem)
            for a in (2 * j, 2 * j + 1)]

    def x0_copy(half):
        part = pl.ds(0, R0), pl.ds(half * D // 2, D // 2)
        return pltpu.make_async_copy(x_hbm.at[part], xa.at[part], sem_in.at[2 * NS + 10 + half])

    def w_copy(n, part=0, parts=1):
        size = D // 2 // parts
        span = pl.ds(n % 2 * D // 2 + part * size, size)
        src = w_hbm.at[span, pl.ds(n // 2 * D, D)] if n < 6 else wo_hbm.at[span, :]
        return pltpu.make_async_copy(src, wraw.at[n, pl.ds(part * size, size)],
                                     sem_in.at[2 * NS + (n + 2 if n > 1 else 2 * n + part)])

    def oa_copy(a):
        return pltpu.make_async_copy(window16("oa", a * HS, HS), out_hbm.at[:, cols(a)], sem_out.at[0])

    def ob_copy(t, row, n):
        return pltpu.make_async_copy(
            window16("ob", t * HS + row, n),
            out_hbm.at[pl.ds(pl.multiple_of(2 * row, 128), 2 * n), cols(NT + t)], sem_out.at[1])

    small = [pltpu.make_async_copy(a, b, sem_in.at[2 * NS + 13])
             for a, b in ((tab_hbm.at[pl.ds(5 * T // 2, 8)], tab.at[pl.ds(5 * T // 2, 8)]),
                          (sk_hbm, sk_ref), (d_hbm, d_ref))]
    full = pl.ds(0, 5 * T // 2)
    table = pltpu.make_async_copy(tab_hbm.at[full], tab.at[full], sem_in.at[2 * NS + 12])
    startup = lambda: [w_copy(0, 0, 2), x0_copy(0), w_copy(0, 1, 2), x0_copy(1), w_copy(1, 0, 2), w_copy(1, 1, 2)] + [
        w_copy(n) for n in range(2, 8)] + [table]
    _start(small + startup())
    _wait(small)
    unit = pltpu.bitcast(tab[pl.ds(5 * T // 2, 8), :], jnp.int32)
    zs = [pl.multiple_of(unit[i, 0] * 8, 8) for i in range(3)]
    views = {n: [b.at[pl.ds(z, spec[n][1]), :] for z in zs] + [b, raw[n]] for n, b in bufs.items()}

    for a in range(NT):
        st("ka", a * KA + 24, jnp.zeros((8, 128), U32))
    for t in range(2 * NT):
        st("k", t * KL + 8, jnp.zeros((WIN, 128), F32))
    skf = sk_ref[...].astype(F32)
    df = d_ref[...].astype(F32)
    for t in range(NT):
        for i in range(4):
            taps[t, i] = jnp.broadcast_to(skf[i:i + 1, t * 128:(t + 1) * 128], (8, 128))
        taps[t, 4] = jnp.broadcast_to(df[t:t + 1, :], (8, 128))

    def step(j, first=False, last=False):
        memo = {}
        e = E0 if first else E
        never = tab[pl.ds(5 * T // 2, 8), :] != 0

        def once(key, fn):
            if key not in memo:
                memo[key] = fn()
            return memo[key]

        def fresh():
            memo["fresh"] = memo.get("fresh", 1) + 1
            return pl.multiple_of(zs[0] * memo["fresh"], 8)

        def pace(val):
            clock = memo.get("clock")
            if clock is None:
                return val
            if val.dtype != F32:
                clock = pltpu.bitcast(clock, val.dtype)
            return lax.select(never, clock, val)

        def paced(x):
            return jnp.concatenate([pace(x[:8]), x[8:]], axis=0)

        def wait(copies):
            memo["clock"] = None
            _wait(copies)

        def shifted(name, row, most):
            return [window(name, z + row, spec[name][1] - most) for z in zs + [0]]

        def perm_in(w, u, t):
            tt = paced(pltpu.bitcast(w[pl.ds(u * 256, 256), pl.ds(t * 128, 128)], U32)).T
            for hh in range(4):
                st(f"t{u}", (4 * t + hh) * PITCH, tt[hh * DH:(hh + 1) * DH])

        def perm_out(p, h, u, t):
            g = jnp.concatenate(
                [bufs[f"t{u}"][pl.ds(zs[0] + 4 * t + i, 32, stride=PITCH), :] for i in range(4)], axis=0)
            st(f"w{p}", (h * NT + t) * KW + u * 128, paced(g).T)

        def perm_list(n, us=(0, 1), ts=range(NT)):
            return ([(1, P(perm_in, wraw.at[n], u, t)) for u in us for t in range(NT)]
                    + [(1, P(perm_out, n // 2, n % 2, u, t)) for t in ts for u in us])

        def wo_in(w, t, hh):
            w = pltpu.bitcast(w[pl.ds(hh * DH, DH), pl.ds(t * 128, 128)], U32)
            st("wp", (16 * t + hh) * WP, _rows(pace(w[:8]), pace(w[8:])))

        def wo_list(w):
            return [(9, P(wo_in, w, t, hh)) for t in range(NT) for hh in range(16)]

        LEFT = ((2, add, 3), (3,), (0, add, 1), (0,), (0, add, 3), (1, sub, 3), (2, sub, 0))
        RIGHT = ((0,), (2, sub, 0), (3,), (1, sub, 3), (0, add, 3), (2, add, 3), (0, add, 1))

        def wo_out(r, t, dh):
            b = [bufs["wp"][pl.ds(zs[dh % 2] + 16 * (t + n % 2 * 4) * WP + n // 2 * 8 + dh // 2, 16, stride=WP), :]
                 for n in range(4)]
            b = [(_lo, _hi)[dh % 2](w) for w in [paced(b[0])] + b[1:]]
            for i, (b0, *rest) in enumerate(RIGHT):
                name, n = ("ws3", 4 * (i - 1 - (i > 2))) if rest else ("w3", i * 2)
                st16(name, (n + t) * KW + 16 * dh + r, rest[0](b[b0], b[rest[1]]) if rest else b[b0])

        def wo_out_list(r):
            return [(26, P(wo_out, r, t, dh)) for t in range(4) for dh in range(16)]

        def right2(p, r, i):
            u, m = divmod(r, KW // 2)
            w = [factor(p, i, u + c % 2 * 2, c // 2 * KW // 2 + m, 8, 1) for c in range(4)]
            w[0], w[3] = pace(w[0]), pace(w[3])
            b = [pltpu.bitcast(x, BF16).astype(F32) for x in w]
            for k in (1, 3, 4, 5, 6):
                st16(f"wt{p}", (5 * i + k - 1 - (k > 2)) * KW + r, RIGHT[k][1](b[RIGHT[k][0]], b[RIGHT[k][2]]))

        def right2_list(p, step, end=0, order=(0, 2, 1, 4, 5, 3, 6), start=0):
            return [(25, P(right2, p, r, i)) for i in order for r in range(start, end, step)]

        def right(p, t, r):
            b = [ld(f"w{p}", (h * NT + t + 4 * u) * KW + r, 16) for h in range(2) for u in range(2)]
            mask = 9 if p else 9
            b = [_rows(pace(x[:8]), pace(x[8:])) if mask >> c & 1 else x for c, x in enumerate(b)]
            b11, b12, b21, b22 = (pltpu.bitcast(x, BF16).astype(F32) for x in b)
            for i, val in enumerate((sub(b21, b11), sub(b12, b22), add(b11, b22),
                                     add(b21, b22), add(b11, b12))):
                st16(f"ws{p}", (4 * i + t) * KW + r, val)

        def right_list(p):
            return [(48, P(right, p, t, r)) for t in range(4) for r in range(0, KW, 16)]

        def ld_kv(c, row, n, z=0):
            return ld(f"kv{c // 4}", c % 4 * (T // 2) + row, n, z)

        def a1(i, r):
            a = once(("a", i), lambda: 2 * j + i)
            w0, w1, w2, w3 = once(("taps", i), lambda: [taps[a, u] for u in range(4)])
            k32 = once(("ka", i), lambda: window("ka", a * KA, KA))
            v32 = once(("va", i), lambda: window("va", a * (S // 2), S // 2))
            c0, c1, c2 = (k32[pl.ds(8 * r + 32 - u, 8), :] for u in range(3))
            vv = v32[pl.ds(8 * r, 8), :]
            e0, o0, e1, o1, o2 = _lo(c0), _hi(c0), _lo(c1), _hi(c1), _hi(c2)
            ke = _tree([mul(e0, w0), mul(o1, w1), mul(e1, w2), mul(o2, w3)])
            ko = _tree([mul(o0, w0), mul(e0, w1), mul(o1, w2), mul(e1, w3)])
            st16(f"kv{r // 32}", 8 * (r % 32), _rows(mul(ke, _lo(vv)), pace(mul(ko, _hi(vv)))))

        def a1_list(i, c0, c1):
            return [(24, P(a1, i, r)) for r in range(8 * c0, 8 * c1)]

        def freq(c, im, m):
            return c * FP + im * (T + 8) + m

        def dft(i, name, c0, m):
            def mm():
                f = pltpu.bitcast(tab[pl.ds(fresh() + T * (name == "xf"), T), :], BF16)
                if name == "hf":
                    a = once(("a", i), lambda: 2 * j + i)
                    rhs = jnp.concatenate(
                        [ha[a, :, pl.ds(c * T, T)] for c in range(c0, c0 + 4)], axis=0)
                    return lax.dot_general(f, rhs, (((1,), (1,)), ((), ())),
                                           preferred_element_type=F32)
                rhs = jnp.concatenate(
                    [pltpu.bitcast(ld_kv(c, 0, T // 2, i % 2), BF16) for c in range(c0, c0 + 4)], axis=1)
                return jnp.dot(f, rhs, preferred_element_type=F32)
            res = once((name, i, c0), mm)
            for u in range(4):
                val = res[m:m + 16, u * 128:(u + 1) * 128]
                if name == "hf" and c0 + u == 0 and m < T:
                    val = add(val, once(("dd", i), lambda: _rows(*[taps[memo["a", i], 4]] * 2)))
                st(name, freq(c0 + u, m // T, m % T), val)
            memo["clock"] = res[m + 8:m + 16, 384:]

        def dft_list(i, name, *c0s):
            return [(16, P(dft, i, name, c0, m)) for c0 in c0s for m in range(0, 2 * T, 16)]

        def a3(i, g, plane, upper, n):
            def opnd(name, c):
                re = lambda: ld(name, freq(c, 0, 8 * g), z=plane)
                im = lambda: ld(name, freq(c, 1, 8 * g), z=plane)
                if name == "xf":
                    val = add(re(), im()) if plane == 0 else re() if plane == 1 else im()
                    return pace(val) if c >= 8 else val
                return pace(re() if plane == 0 else (sub, add)[plane - 1](im(), re()))
            get = lambda name, c: once((name, i, g, plane, c), P(opnd, name, c))
            done = pace if n % 4 == 3 else lambda v: v
            cs = range(8, n + 1) if upper else range(min(n, 7) + 1)
            terms = [mul(get("xf", n - c), get("hf", c)) for c in cs]
            if upper:
                st("up", 8 * n, done(_tree(terms)))
                return
            if n >= 8:
                terms.append(ld("up", 8 * n))
            if plane == 0:
                st("k1", 8 * n, done(_tree(terms)))
            elif plane == 1:
                st("pi", 8 * n, done(_tree(terms + [ld("k1", 8 * n)])))
            else:
                pr = sub(ld("k1", 8 * n, z=1), _tree(terms))
                pi = ld("pi", 8 * n)
                zr, zi = pr, pi
                if n > 0:
                    qr, qi = memo["prev"]
                    zr, zi = sub(pr, qi), add(pi, qr)
                memo["prev"] = (pr, pi)
                if g % 2 == 0:
                    st("zr", 8 * n, done(zr))
                    st("zi", 8 * n, zi)
                else:
                    st16("z", n * T + 4 * (g - 1), _rows(ld("zr", 8 * n), done(zr)))
                    st16("z", n * T + T // 2 + 4 * (g - 1), _rows(ld("zi", 8 * n), zi))

        def a3_list(i):
            out = []
            for g in range(T // 8):
                for plane in range(3):
                    out += [(2 * (n - 8) + 4, P(a3, i, g, plane, True, n)) for n in range(8, NC)]
                    out += [(2 * min(n, 7) + 4 + 2 * (plane == 2), P(a3, i, g, plane, False, n))
                            for n in range(NC)]
            return out

        def idft(i, c0, odd, m):
            def mm():
                rhs = jnp.concatenate([pltpu.bitcast(ld("z", c * T + odd * T // 2, T // 2, i), BF16)
                                       for c in range(c0, c0 + 4)], axis=1)
                f = tab[pl.ds(fresh() + 2 * T + odd * T // 4, T // 4), :]
                return jnp.dot(pltpu.bitcast(f, BF16), rhs, preferred_element_type=F32)
            y = once(("y", i, c0, odd), mm)
            a = once(("a", i), lambda: 2 * j + i)
            q16 = once(("qa", i), lambda: window16("qa", a * (S // 2), S // 2))
            o16 = once(("oa", i), lambda: window16("oa", a * (S // 2), S // 2))
            flip = lambda w: jnp.take_along_axis(
                w, 7 - lax.broadcasted_iota(jnp.int32, (8, 128), 0), axis=0, mode="promise_in_bounds")
            for u in range(4):
                val = y[m:m + 16, u * 128:(u + 1) * 128]
                if not odd:
                    st("even", u * T // 2 + m, val)
                    continue
                even, mid = ld("even", u * T // 2 + m, 16), (c0 + u) * T + T // 2
                low = add(even, val)
                for row, out in ((mid + m, sub(even, val)),
                                 (mid - 16 - m, _rows(flip(low[8:]), flip(low[:8])))):
                    o16[pl.ds(row, 16), :] = mul(q16[pl.ds(row, 16), :].astype(F32), out).astype(BF16)
            memo["clock"] = y[m + 8:m + 16, 384:]

        def idft_list(i, *c0s):
            return [(16, P(idft, i, c0, odd, m)) for c0 in c0s
                    for odd in range(2) for m in range(0, T // 2, 16)]

        def xprep(x, u, r):
            halves = []
            for m in (r, r + 8):
                a, b = (pltpu.bitcast(x[pl.ds(2 * m, 16), pl.ds(t * 128, 128)], U32)
                        for t in (u, u + 4))
                a = pace(a)
                a11, a12, a21, a22 = _lo(a), _lo(b), _hi(a), _hi(b)
                halves.append(_left(a11, a12, a21, a22))
            for i, pair in enumerate(zip(*halves)):
                st16("xs", ((4 * i + u) * E0 + r) // 2, jnp.concatenate(pair, axis=0))

        def xprep_list(x):
            return [(27, P(xprep, x, u, r)) for r in range(0, e, 16) for u in range(4)]

        def tiles(name, rows, n):
            view = views[name][3].at[pl.ds(fresh(), spec[name][1]), :]
            return jnp.concatenate(
                [pltpu.bitcast(view[pl.ds(row, n // 2), :], BF16) for row in rows], axis=1)

        def emit(p, r0, n, par, t, m, val, end):
            if p == 0:
                st("q", (par * NT + t) * E0 + m, val)
            elif p == 3:
                base = once("row", lambda: j * E)
                o16 = once("ob", lambda: window16("ob", base, (NT - 1) * HS + (E0 if last else E)))
                o16[pl.ds(t * S + r0 + par * n + m, 16), :] = val.astype(BF16)
                if m + 16 == end and par == t // 4:
                    ob_copy(t, base + r0 // 2, n).start()
            elif p == 2:
                st("v", (par * NT + t) * KR + 16 + m, val)
            else:
                row = (par * NT + t + 1) * KL - e
                if m == 0 and not first:
                    st("k", row - WIN, ld("k", row + e - WIN, z=3))
                st("k", row + m, val)
            if m == 0 and first and p == 2 and par == 0:
                for other in range(2):
                    st("v", (other * NT + t) * KR + 8, jnp.broadcast_to(val[0:1], (WIN, 128)))

        def plain(n, t, m):
            def mm():
                w = [ld("w0", (n // 2 * NT + t + u) * KW + n % 2 * KW // 2, KW // 2, 3) for u in range(2)]
                return jnp.dot(xa[pl.ds(0, R0), pl.ds(n * D // 4, D // 4)],
                               jnp.concatenate([pltpu.bitcast(v, BF16) for v in w], axis=1),
                               preferred_element_type=F32)
            res = once(("plain", n, t), mm)
            h = (0, 128, m // 16 % 2 * 128)[0]
            memo["clock"] = res[m + 8:m + 16, h:h + 128]
            for u in range(2):
                val = res[m:m + 16, u * 128:(u + 1) * 128]
                if n:
                    val = add(val, ld("qo"[n % 2], (t + u) * R0 + m, 16))
                st("oq"[n % 2], (t + u) * R0 + m, val)

        def plain_list():
            return [(16, P(plain, n, t, m)) for n in range(4) for t in range(0, NT, 2) for m in range(0, R0, 16)]

        def combine(level, i, row, res, out, early=False):
            get = lambda name, z=0: ld(name + level, row, 16, z)
            if i % 2 == 0 and i < 6:
                st("abc"[i // 2] + level, row, res)
            elif i == 1:
                st("d" + level, row, res if early else sub(res, get("b")))
                out(1, 0, add(get("a"), res))
            elif i == 3:
                st("e" + level, row, sub(res, get("a", 1)))
                out(0, 1, add(get("b", 1), res))
            else:
                part = add(get("de"[i - 5]), get("c", i - 5))
                out(i - 5, i - 5, add(sub(part, get("b")) if early and i == 5 else part, res))

        def factor(p, i, t, r=0, n=KW, z=3):
            if i in (0, 2):
                return ld(f"w{p}", (t + (4 if p == 3 else NT + 4) * i // 2) * KW + r, n, z)
            return ld(f"ws{p}", (4 * (i - 1 - (i > 2)) + t) * KW + r, n, z)

        def product(p, src, r0, n, t, i, m):
            res = once(("product", p, r0, t, i), lambda: jnp.dot(
                tiles(src, [(4 * i + u) * E0 // 2 for u in range(4)], n),
                pltpu.bitcast(factor(p, i, t), BF16), preferred_element_type=F32))
            memo["clock"] = res[m + 8:m + 16]
            combine("1", i, t * E0 + m, res[m:m + 16],
                    lambda par, h, val: emit(p, r0, n, par, t + 4 * h, m, val, n), last and not r0)

        ORDER = (0, 2, 1, 4, 5, 3, 6)

        def strassen(p, src="xs", r0=0, n=e, order=ORDER):
            return [(16, P(product, p, src, r0, n, t, i, m))
                    for t in range(4) for i in order for m in range(0, n, 16)]

        def product2(p, r0, n, i, k, m):
            def mm():
                if p == 3:
                    name, row, step = f"os{i}", k * E0 // 2, E0 // 4
                elif k in (1, 3):
                    name, row, step = "xs", 2 * i * E0 + (k == 1) * (E0 + n // 4), E0 // 2
                else:
                    name, row, step = "xt", (5 * i + (0, 2, 4, 5, 6).index(k)) * E0 // 2, E0 // 4
                if k in (0, 2):
                    w = [factor(p, i, k + u, k * KW // 4, KW // 2) for u in range(2)]
                else:
                    w = [ld(f"wt{p}", ((5 * i + k - 1 - (k > 2)) * 2 + u) * KW // 2, KW // 2, 3) for u in range(2)]
                return jnp.dot(tiles(name, (row, row + step), n // 2),
                               jnp.concatenate([pltpu.bitcast(v, BF16) for v in w], axis=1),
                               preferred_element_type=F32)
            res = once(("product2", p, i, k), mm)
            memo["clock"] = res[m + 8:m + 16, 128:]

            def out(u, r2, c2, val):
                t, row = 2 * c2 + u, r2 * n // 2 + m
                combine("1", i, t * E0 + row, val, lambda par, h, v: emit(
                    p, r0, n, par, t + 4 * h, row, v, (1 + c2) * n // 2))
            for u in range(2):
                combine("2", k, u * E0 // 2 + m, res[m:m + 16, u * 128:(u + 1) * 128], P(out, u))

        def strassen2(p, deep=7, r0=0, n=e):
            return [task for i in ORDER for task in (
                [(16, P(product2, p, r0, n, i, k, m)) for k in ORDER for m in range(0, n // 2, 16)]
                if i < deep else strassen(p, order=(i,)))]

        def xprep2(x, u, r, i):
            def blk(b):
                w = once(("x", u, r, b % 2), lambda: [pltpu.bitcast(
                    x[pl.ds(c // 2 * e + 2 * r, 32), pl.ds((u + c % 2 * 2 + b % 2 * 4) * 128, 128)], U32)
                    for c in range(4)])
                return [(_lo, _hi)[b // 2](v) for v in w]
            b0, *rest = LEFT[i]
            a = list(once(("left", u, r, b0), P(blk, b0)))
            a[0], a[3] = paced(a[0]), paced(a[3])
            if rest:
                a = list(map(rest[0], a, once(("left", u, r, rest[1]), P(blk, rest[1]))))
            for n, k in enumerate((0, 2, 4, 5, 6)):
                st16("xt", ((5 * i + n) * 2 + u) * E0 // 4 + r // 2, LEFT[k][1](a[LEFT[k][0]], a[LEFT[k][2]]))

        def xprep2_list(x):
            return [(c, P(xprep2, x, u, r, i)) for r in range(0, e // 2, 16) for u in range(2)
                    for i, c in ((1, 25), (0, 33), (6, 33), (4, 25), (3, 17), (5, 33), (2, 25))]

        def oprep2(r0, n, i, u, r):
            view = once(("oprep", i), lambda: window("o", fresh(), NT * R0))
            blk = lambda b, c: view[pl.ds(
                (u + 2 * (c % 2) + 4 * (b % 2)) * R0 + r0 + b // 2 * n + c // 2 * n // 2 + r, 16), :]
            b0, *rest = LEFT[i]
            a = [blk(b0, c) for c in range(4)]
            a[3] = paced(a[3])
            a[0] = paced(a[0])
            if rest:
                a = [rest[0](x, blk(rest[1], c)) for c, x in enumerate(a)]
            for k, val in enumerate(_left(*a)):
                st16(f"os{i}", (k * 2 + u) * E0 // 4 + r // 2, val)

        def oprep2_list(r0=0, n=e):
            return [(19 + 8 * (len(LEFT[i]) > 1), P(oprep2, r0, n, i, u, r))
                    for i in ORDER for r in range(0, n // 2, 16) for u in range(2)]

        def qk(r, w):
            par, m = r
            query = lambda t: (bufs["q"][pl.ds(t * R0 + 2 * m + par, 8, stride=2), :] if first
                               else ld("q", (par * NT + t) * E0 + m))
            scale = once(("scale", r), lambda: pace(jnp.full((8, 128), DH ** -0.5 * LOG2E, F32)))
            qv = once(("qv", r), lambda: [mul(query(t), scale) for t in range(NT)])
            qv = [pace(qv[0])] + qv[1:]
            s = (_tree([mul(qv[t], ld("k", (par * NT + t + 1) * KL - e + m - w)) for t in range(NT)]))
            def fold(mask, a, b, shift):
                return add(lax.select(mask, a, b), pltpu.roll(lax.select(mask, b, a), shift, 1))
            g = m // 8 % 4
            if g % 2:
                s = fold(thirds[g // 2], memo.pop(("s", 0, w)), s, 64)
            if g == 3:
                s = fold(thirds[2], ld("pair", 8 * w) if 0 == 0 else pace(ld("pair", 8 * w)) if 0 == 1 else memo["s", 1, w], s, 32)
                if first and m == 24 and w:
                    early = lax.broadcasted_iota(jnp.int32, (8, 128), 0) < w
                    s = jnp.where(early & (quarter == 1), -1e9 * LOG2E, s)
            if g == 1 and 0 < 2:
                st("pair", 8 * w, s)
            memo[("lg", r, w) if g == 3 else ("s", g % 2, w)] = s

        quarter = lax.shift_right_logical(lax.broadcasted_iota(jnp.int32, (8, 128), 1), 5)
        thirds = quarter < 2, (quarter == 1) | (quarter == 2), (quarter & 1) == 1

        def expo(r):
            lg = [memo["lg", r, w] for w in range(WIN)]
            m = pace(functools.reduce(lax.max, lg))
            memo["e", r] = [lax.exp2(sub(s, m)) for s in lg]

        def norm(r):
            total = pace(_tree(memo["e", r]))
            memo["inv", r] = total, pl.reciprocal(total, approx=True)

        def probs(r):
            total, inv = memo["inv", r]
            inv = pace(inv)
            inv = mul(inv, sub(np.float32(2), mul(total, inv)))
            for w, x in enumerate(memo["e", r]):
                st("quad", 8 * w, mul(x, inv))

        def spread(r, g):
            row = lambda w, g: (2 * w + r[0]) * HS + r[1] - 24 + 8 * g
            if 0:
                lane = lax.broadcasted_iota(jnp.int32, (8, 128), 1)
                index = pace((lane & 31) + 32 * (1, 3, 2, 0)[g])
                for w, x in enumerate([ld("quad", 8 * w, 8, g) for w in range(WIN)]):
                    st("p", row(w, g), jnp.take_along_axis(x, index, axis=1, mode="promise_in_bounds"))
                return
            for w in (2 * g, 2 * g + 1):
                x = pace(ld("quad", 8 * w))
                y = pltpu.roll(x, 64, 1)
                for a, (even, odd) in ((lax.select(thirds[0], x, y), (3, 0)), (lax.select(thirds[0], y, x), (2, 1))):
                    b = pltpu.roll(a, 32, 1)
                    st("p", row(w, odd), lax.select(thirds[2], a, b))
                    st("p", row(w, even), lax.select(thirds[2], b, a))

        def qk_list(m0, m1):
            rs = [(par, m) for par in range(2) for m in range(m0, m1, 8)]
            q0, q1, q2 = 20, 3, 2
            stages = [(expo, q0), (norm, q0 + q1), (probs, q0 + 2 * q1)] + [
                (lambda r, g=g: spread(r, g), q0 + 2 * q1 + q2 * (g + 1)) for g in range(4)]
            out = [[P(qk, rs[n + u], w)] for n in range(0, len(rs), 2) for w in range(WIN) for u in range(2)] + [[] for _ in range(stages[-1][1])]
            for n in range(3, len(rs), 4):
                for f, lag in stages:
                    out[WIN * n + WIN - 1 + lag].append(P(f, rs[n]))
            return [(22, P(_run, [(0, f) for f in tasks])) for tasks in out]

        def pv(par, m, t):
            p = once(("pv", par, m), lambda: [
                (pace if w % 4 == 0 else lambda v: v)(ld("pr", (2 * w + par) * HS + m))
                for w in range(WIN)])
            row = (par * NT + t) * KR + 16 + m
            bufs["o"][pl.ds(t * R0 + 2 * m + par, 8, stride=2), :] = pace(
                _tree([mul(p[w], ld("vr", row - w)) for w in range(WIN)]))

        def pv_list(m0, m1, ts=range(NT)):
            return [(16, P(pv, par, m, t)) for par in range(2) for m in range(m0, m1, 8) for t in ts]

        def oprep(name, r0, n, which, u, r):
            a = lambda b: once(("o", name, r0, u, r, b), lambda: ld(
                "o", (u + b % 2 * 4) * R0 + r0 + b // 2 * n + r, 16, 1 + (name == "xu")))
            memo["o", name, r0, u, r, 3] = paced(a(3))
            for i in which:
                b0, *rest = LEFT[i]
                st16(name, ((4 * i + u) * E0 + r) // 2, rest[0](a(b0), a(rest[1])) if rest else a(b0))

        def oprep_list(name, r0, n, which=range(7)):
            return [(18, P(oprep, name, r0, n, which, u, r)) for r in range(0, n, 16) for u in range(4)]

        if first:

            def phase(end, side, *copies):
                start, gap = memo.get("done", 0), 3 * bool(copies)
                memo["done"] = end
                _weave(main[start:end - gap], side)
                _run(main[end - gap:end])
                if copies:
                    wait(copies)

            both = lambda p: strassen(p, order=ORDER[:1]) + strassen(p, order=ORDER[1:2]) + strassen(p, order=ORDER[2:])
            two = 0
            main = plain_list() + both(1) + (strassen2(2) if two else strassen(2))
            dq, dv = right2_list(0, 8, KW, ORDER[:3] + ORDER[5:6]), right2_list(2, 8, KW)
            wo = lambda n: wo_list(wraw.at[6 + n]) + wo_out_list(8 * n)
            do = lambda n: right2_list(3, 16, KW, start=8 * n)
            wait([w_copy(0, 0, 2)])
            _run(perm_list(0, (0,)))
            wait([x0_copy(0)])
            phase(64, [], w_copy(0, 1, 2))
            phase(90, perm_list(0, (1,))[:10])
            phase(120, perm_list(0, (1,))[10:])
            phase(192, [], x0_copy(1), w_copy(1, 0, 2))
            phase(90 + 128, perm_list(1, (0,))[:10])
            phase(248, perm_list(1, (0,))[10:])
            phase(256, [], w_copy(1, 1, 2))
            phase(304, _merge(perm_list(1, (1,)), xprep_list(xa)[:40]))
            phase(320, xprep_list(xa)[40:])
            phase(384, right_list(0)[:48], w_copy(2))
            phase(468, _merge(perm_list(2), right_list(0)[48:] + dq[32:80]))
            phase(480, [], w_copy(3))
            order = (4, 0, 5, 1, 6, 2, 7, 3)
            phase(562, _merge(perm_list(3, ts=order), dq[:32] + dq[80:]))
            phase(572, [])
            phase(592, right_list(1)[:12], w_copy(4))
            _start(in_copies(0, 0) + in_copies(0, 1))
            phase(634, _merge(perm_list(4)[:16], right_list(1)[12:36]))
            phase(676, _merge(perm_list(4)[16:], right_list(1)[36:60]))
            phase(688, right_list(1)[60:])
            phase(704, dv[:20], w_copy(5))
            phase(788, perm_list(5))
            phase(796, [])
            phase(832, dv[20:32] + right_list(2)[:20], w_copy(6))
            phase(944, _zip(wo(0), right_list(2)[20:]) + dv[32:56], w_copy(7))
            _start(sum((in_copies(n, late) for n in range(1, NS) for late in range(2)), []))
            rest = dv[56:] + do(0) + do(1)
            phase(1010, _zip(wo(1), rest[:40]))
            phase(len(main) - 4, _merge(rest[40:], qk_list(0, E0)))
            phase(len(main), [])
            return

        views.update(pr=shifted("p", j * E, NS * E), vr=shifted("v", j * E, NS * E))
        if last:
            n = E0 // 4
            _run(pv_list(n // 2, n) + oprep_list("xs", 0, n, (0, 1)))
            main = strassen(3, "xs", 0, n, (0,)) + strassen(3, "xs", 0, n, (1,))
            _weave(main[:28], pv_list(0, n // 2) + oprep_list("xu", 0, n, range(2, 7)))
            main = main[28:] + strassen(3, "xu", 0, n, (2, 4, 5, 3, 6))
            _weave(main[:-4], pv_list(n, 2 * n) + oprep_list("xt", 2 * n, n))
            main = main[-4:] + strassen(3, "xt", 2 * n, n) + strassen2(3, 7, 4 * n, 2 * n)
            pre = oprep2_list(4 * n, 2 * n)
            _weave(main[:110], pv_list(2 * n, 4 * n) + pre[:8])
            _weave(main[110:170], pre[8:])
            _run(main[170:])
            return

        for name in "vp":
            views[name] = shifted(name, E0 + j * E, E0 + (NS - 1) * E)
        head, x = strassen(1) + strassen2(0, 4), xa.at[rows(j)]
        h0, h1, h2, h3 = 66, 416, 528, 26
        for u in range(4):
            _weave(dft_list(0, "hf", 4 * u), a1_list(0, 12 * u // 4, 12 * (u + 1) // 4))
        extra = _split(xprep_list(x), 4, 6)
        _weave(dft_list(0, "xf", 0), a1_list(0, 12, 13))
        _weave(dft_list(0, "xf", 4), _merge(a1_list(0, 13, 16), extra[0]))
        _weave(dft_list(0, "xf", 8) + dft_list(0, "xf", 12)[:4], extra[1])
        _run(dft_list(0, "xf", 12)[4:])
        _weave(head[:h0], xprep2_list(x))
        _weave(head[h0:h1 - 0], a3_list(0))
        _run(head[h1 - 0:h1])
        wait(in_copies(j, 1))
        mix = _split(pv_list(0, E), 1, 4)
        for u in range(4):
            _run(idft_list(0, 4 * u))
            _weave(dft_list(1, "hf", 4 * u), a1_list(1, 3 * u, 3 * u + 3))
        oa_copy(2 * j).start()
        _weave(dft_list(1, "xf", 0), a1_list(1, 12, 16))
        _weave(dft_list(1, "xf", 4, 8, 12), mix[0])
        pre = _split(oprep2_list(), 4, 3)
        planes, g0 = _split(a3_list(1), *[1] * 48), 16
        _weave(head[h1:h2], mix[1])
        side = pre[0]
        for n, part in enumerate(_split(pre[1], *[1] * g0)):
            side = side + planes[n] + part
        tail = strassen2(2, 7)
        _weave(head[h2:] + strassen2(3) + tail[:h3], side + sum(planes[g0:], []))
        back, cutp = idft_list(1, 0, 4, 8, 12), 294
        tail = tail[:cutp] + back + tail[cutp:]
        _weave(tail[h3:len(tail) - 10], qk_list(0, E))
        _run(tail[len(tail) - 10:])
        oa_copy(2 * j + 1).start()

    def loop(j, carry):
        _wait(in_copies(j, 0))
        step(j)
        return carry

    step(0, first=True)
    _wait([table])
    lax.fori_loop(0, NS, loop, 0)
    step(NS, last=True)
    for i, name in enumerate(("oa", "ob")):
        pltpu.make_async_copy(raw[name], raw[name], sem_out.at[i]).wait()


@jax.jit
def pallas_concat_heads__ssm_conv_h3__sliding_local_dilated__prompt_kernel(
    A_q, A_k, A_v, A_shift_k, A_ssm_k, A_ssm_D, B_x, B_wqkv, B_wo,
):
    hbm = pl.BlockSpec(memory_space=pl.ANY)
    out = pl.pallas_call(
        _kernel,
        in_specs=[hbm] * 10,
        out_specs=hbm,
        out_shape=jax.ShapeDtypeStruct((S, 2 * D), BF16),
        scratch_shapes=[
            pltpu.VMEM((NT, 128, S), BF16),
            pltpu.VMEM((S, D), BF16),
            pltpu.VMEM((8, D // 2, D), BF16),
            pltpu.VMEM((NT, 5, 8, 128), F32),
            pltpu.VMEM(_TABLE.shape, U32),
            pltpu.SemaphoreType.DMA((2 * NS + 14,)),
            pltpu.SemaphoreType.DMA((2,)),
        ] + [pltpu.VMEM((r * 4 // np.dtype(t).itemsize, 128), t) for t, r in _BUFS.values()]
        + [pltpu.VMEM((4, D), BF16), pltpu.VMEM((8, 128), BF16)],
        compiler_params=pltpu.CompilerParams(vmem_limit_bytes=116 * 1024 * 1024,
                                             disable_bounds_checks=True,
                                             disable_semaphore_checks=True),
        name="fused",
    )(A_q[0], A_k[0], A_v[0], A_shift_k.T, A_ssm_k,
      A_ssm_D.reshape(8, 128), B_x[0], B_wqkv, B_wo, _TABLE)
    return out[None]
```

```python
import functools

import jax
import jax.numpy as jnp
import numpy as np
from jax import lax
from jax.experimental import pallas as pl
import jax.experimental.pallas.tpu as pltpu


S = 2048
D = 1024
T = 128
NC = S // T
NT = D // 128
NS = 4
R0 = 512
R = (S - R0) // NS
E0, E, HS = R0 // 2, R // 2, S // 2
WIN, DH = 8, 32
LOG2E = float(np.log2(np.e))
PITCH = 33
WP = 33
KR, KL = HS + 16, E0 + 16
FP = 2 * T + 16
KW = D // 4
KA = S // 2 + 32

F32, BF16, U32 = jnp.float32, jnp.bfloat16, jnp.uint32
P = functools.partial
add, sub, mul = lax.add, lax.sub, lax.mul


def _pack_rows(m):
    b = m.astype(jnp.bfloat16).view(np.uint16).astype(np.uint32)
    return np.ascontiguousarray(b[0::2] | (b[1::2] << 16))


def _dft_table():
    th = 2.0 * np.pi * (np.arange(T) + 0.25) / T
    dft = lambda t: np.concatenate([np.cos(np.outer(th, t)), -np.sin(np.outer(th, t))], axis=0)
    paired = np.arange(T).reshape(-1, 8, 2).transpose(0, 2, 1).reshape(-1)
    ph = np.outer(np.arange(T // 2) + 0.5, th)
    mats = (dft(np.arange(T)), dft(paired - (T - 1) / 2), np.cos(ph) / T, np.sin(ph) / T)
    return np.concatenate([_pack_rows(m) for m in mats] + [np.zeros((32, T), np.uint32)], axis=0)


_TABLE = _dft_table()


def _lo(w):
    return pltpu.bitcast(lax.shift_left(w, np.uint32(16)), F32)


def _hi(w):
    return pltpu.bitcast(lax.bitwise_and(w, np.uint32(0xFFFF0000)), F32)


def _rows(first, second):
    return jnp.concatenate([first, second], axis=0)


def _tree(xs):
    while len(xs) > 1:
        xs = [add(xs[i], xs[i + 1]) if i + 1 < len(xs) else xs[i] for i in range(0, len(xs), 2)]
    return xs[0]


def _left(a11, a12, a21, a22):
    return [add(a21, a22), a22, add(a11, a12), a11, add(a11, a22), sub(a12, a22), sub(a21, a11)]


def _merge(main, side):
    if not main:
        return side
    total_m = sum(c for c, _ in main)
    total_s = sum(c for c, _ in side)
    done_m, done_s, i, out = 0, 0, 0, []
    for c, f in main:
        out.append((c * total_s, f))
        done_m += c
        while i < len(side) and (done_s + side[i][0]) * total_m <= done_m * total_s:
            done_s += side[i][0]
            out.append((side[i][0] * total_m, side[i][1]))
            i += 1
    assert i == len(side)
    return out


def _zip(main, side):
    cost = {id(f): c for c, f in main + side}
    return [(cost[id(f)], f) for _, f in _merge(main, side)]


def _run(tasks):
    for _, f in tasks:
        f()


def _weave(main, side):
    _run(_merge(main, side))


def _split(tasks, *weights):
    ends = np.cumsum((0,) + weights) * len(tasks) // sum(weights)
    return [tasks[a:b] for a, b in zip(ends[:-1], ends[1:])]


def _start(copies):
    for c in copies:
        c.start()


def _wait(copies):
    for c in copies:
        c.wait()


_BUFS = {n: (t, r) for t, group in (
    (BF16, dict(qa=NT * HS, ka=NT * KA, va=NT * HS, oa=NT * HS, ob=NT * HS,
                xs=14 * E0, xt=35 * E0 // 2, **{f"os{i}": 7 * E0 // 2 for i in range(7)},
                kv0=S // 8, kv1=S // 8, kv2=S // 8, kv3=S // 8, z=NC * T, w3=NT * KW, xu=14 * E0,
                **{f"ws{p}": 20 * KW for p in range(4)}, wt0=20 * KW, wt2=35 * KW, wt3=35 * KW)),
    (U32, dict(**{f"w{p}": 2 * NT * KW for p in range(3)}, t0=34 * DH, t1=34 * DH, wp=4 * WP * DH)),
    (F32, dict(hf=NC * FP, xf=NC * FP, up=8 * NC, k1=8 * NC, pi=8 * NC, zr=8 * NC, zi=8 * NC,
               even=2 * T, quad=8 * WIN, **{n + "1": 4 * E0 for n in "abcde"}, **{n + "2": E0 for n in "abcde"},
               q=NT * R0 + 32, k=2 * NT * KL, v=2 * NT * KR, p=WIN * S, o=NT * R0 + 32)),
) for n, r in group.items()}


def _kernel(q_hbm, k_hbm, v_hbm, sk_hbm, h_hbm, d_hbm, x_hbm, w_hbm, wo_hbm, tab_hbm, out_hbm,
            ha, xa, wraw, taps, tab, sem_in, sem_out, *raw):
    *raw, sk_ref, d_ref = raw
    raw = dict(zip(_BUFS, raw))
    bufs = {n: b.bitcast(U32) if _BUFS[n][0] == BF16 else b for n, b in raw.items()}

    spec = _BUFS

    def ld(name, row, n=8, z=0):
        assert 0 <= row and row + n <= views[name][z].shape[0]
        return views[name][z][pl.ds(row, n), :]

    def st(name, row, val):
        assert 0 <= row and row + val.shape[0] <= views[name][3].shape[0]
        views[name][3][pl.ds(row, val.shape[0]), :] = val

    def st16(name, row, val):
        assert 0 <= row and 2 * row + val.shape[0] <= views[name][4].shape[0]
        views[name][4][pl.ds(2 * row, val.shape[0]), :] = val.astype(BF16)

    def window(name, row, n):
        return bufs[name].at[pl.ds(pl.multiple_of(row, 8), n), :]

    def window16(name, row, n):
        return raw[name].at[pl.ds(pl.multiple_of(2 * row, 16), 2 * n), :]

    def cols(a):
        return pl.ds(pl.multiple_of(a * 128, 128), 128)

    def rows(j):
        return pl.ds(pl.multiple_of(R0 + j * R, 128), R)

    def a_copies(a, sem):
        return [pltpu.make_async_copy(src, dst, sem) for src, dst in (
            (h_hbm.at[cols(a), :], ha.at[a]),
            (k_hbm.at[:, cols(a)], window16("ka", a * KA + 32, HS)),
            (v_hbm.at[:, cols(a)], window16("va", a * HS, HS)))]

    def in_copies(j, late):
        sem = sem_in.at[2 * j + late]
        if not late:
            return [pltpu.make_async_copy(x_hbm.at[rows(j), :], xa.at[rows(j), :], sem)] + a_copies(2 * j, sem)
        return a_copies(2 * j + 1, sem) + [
            pltpu.make_async_copy(q_hbm.at[:, cols(a)], window16("qa", a * HS, HS), sem)
            for a in (2 * j, 2 * j + 1)]

    def x0_copy(half):
        part = pl.ds(0, R0), pl.ds(half * D // 2, D // 2)
        return pltpu.make_async_copy(x_hbm.at[part], xa.at[part], sem_in.at[2 * NS + 10 + half])

    def w_copy(n, part=0, parts=1):
        size = D // 2 // parts
        span = pl.ds(n % 2 * D // 2 + part * size, size)
        src = w_hbm.at[span, pl.ds(n // 2 * D, D)] if n < 6 else wo_hbm.at[span, :]
        return pltpu.make_async_copy(src, wraw.at[n, pl.ds(part * size, size)],
                                     sem_in.at[2 * NS + (n + 2 if n > 1 else 2 * n + part)])

    def oa_copy(a):
        return pltpu.make_async_copy(window16("oa", a * HS, HS), out_hbm.at[:, cols(a)], sem_out.at[0])

    def ob_copy(t, row, n):
        return pltpu.make_async_copy(
            window16("ob", t * HS + row, n),
            out_hbm.at[pl.ds(pl.multiple_of(2 * row, 128), 2 * n), cols(NT + t)], sem_out.at[1])

    small = [pltpu.make_async_copy(a, b, sem_in.at[2 * NS + 13])
             for a, b in ((tab_hbm.at[pl.ds(5 * T // 2, 8)], tab.at[pl.ds(5 * T // 2, 8)]),
                          (sk_hbm, sk_ref), (d_hbm, d_ref))]
    full = pl.ds(0, 5 * T // 2)
    table = pltpu.make_async_copy(tab_hbm.at[full], tab.at[full], sem_in.at[2 * NS + 12])
    startup = lambda: [w_copy(0, 0, 2), x0_copy(0), w_copy(0, 1, 2), x0_copy(1), w_copy(1, 0, 2), w_copy(1, 1, 2)] + [
        w_copy(n) for n in range(2, 8)] + [table]
    _start(small + startup())
    _wait(small)
    unit = pltpu.bitcast(tab[pl.ds(5 * T // 2, 8), :], jnp.int32)
    zs = [pl.multiple_of(unit[i, 0] * 8, 8) for i in range(3)]
    views = {n: [b.at[pl.ds(z, spec[n][1]), :] for z in zs] + [b, raw[n]] for n, b in bufs.items()}

    for a in range(NT):
        st("ka", a * KA + 24, jnp.zeros((8, 128), U32))
    for t in range(2 * NT):
        st("k", t * KL + 8, jnp.zeros((WIN, 128), F32))
    skf = sk_ref[...].astype(F32)
    df = d_ref[...].astype(F32)
    for t in range(NT):
        for i in range(4):
            taps[t, i] = jnp.broadcast_to(skf[i:i + 1, t * 128:(t + 1) * 128], (8, 128))
        taps[t, 4] = jnp.broadcast_to(df[t:t + 1, :], (8, 128))

    def step(j, first=False, last=False):
        memo = {}
        e = E0 if first else E
        never = tab[pl.ds(5 * T // 2, 8), :] != 0

        def once(key, fn):
            if key not in memo:
                memo[key] = fn()
            return memo[key]

        def fresh():
            memo["fresh"] = memo.get("fresh", 1) + 1
            return pl.multiple_of(zs[0] * memo["fresh"], 8)

        def pace(val):
            clock = memo.get("clock")
            if clock is None:
                return val
            if val.dtype != F32:
                clock = pltpu.bitcast(clock, val.dtype)
            return lax.select(never, clock, val)

        def paced(x):
            return jnp.concatenate([pace(x[:8]), x[8:]], axis=0)

        def wait(copies):
            memo["clock"] = None
            _wait(copies)

        def shifted(name, row, most):
            return [window(name, z + row, spec[name][1] - most) for z in zs + [0]]

        def perm_in(w, u, t):
            tt = paced(pltpu.bitcast(w[pl.ds(u * 256, 256), pl.ds(t * 128, 128)], U32)).T
            for hh in range(4):
                st(f"t{u}", (4 * t + hh) * PITCH, tt[hh * DH:(hh + 1) * DH])

        def perm_out(p, h, u, t):
            g = jnp.concatenate(
                [bufs[f"t{u}"][pl.ds(zs[0] + 4 * t + i, 32, stride=PITCH), :] for i in range(4)], axis=0)
            st(f"w{p}", (h * NT + t) * KW + u * 128, paced(g).T)

        def perm_list(n, us=(0, 1), ts=range(NT)):
            return ([(1, P(perm_in, wraw.at[n], u, t)) for u in us for t in range(NT)]
                    + [(1, P(perm_out, n // 2, n % 2, u, t)) for t in ts for u in us])

        def wo_in(w, t, hh):
            w = pltpu.bitcast(w[pl.ds(hh * DH, DH), pl.ds(t * 128, 128)], U32)
            st("wp", (16 * t + hh) * WP, _rows(pace(w[:8]), pace(w[8:])))

        def wo_list(w):
            return [(9, P(wo_in, w, t, hh)) for t in range(NT) for hh in range(16)]

        LEFT = ((2, add, 3), (3,), (0, add, 1), (0,), (0, add, 3), (1, sub, 3), (2, sub, 0))
        RIGHT = ((0,), (2, sub, 0), (3,), (1, sub, 3), (0, add, 3), (2, add, 3), (0, add, 1))

        def wo_out(r, t, dh):
            b = [bufs["wp"][pl.ds(zs[dh % 2] + 16 * (t + n % 2 * 4) * WP + n // 2 * 8 + dh // 2, 16, stride=WP), :]
                 for n in range(4)]
            b = [(_lo, _hi)[dh % 2](w) for w in [paced(b[0])] + b[1:]]
            for i, (b0, *rest) in enumerate(RIGHT):
                name, n = ("ws3", 4 * (i - 1 - (i > 2))) if rest else ("w3", i * 2)
                st16(name, (n + t) * KW + 16 * dh + r, rest[0](b[b0], b[rest[1]]) if rest else b[b0])

        def wo_out_list(r):
            return [(26, P(wo_out, r, t, dh)) for t in range(4) for dh in range(16)]

        def right2(p, r, i):
            u, m = divmod(r, KW // 2)
            w = [factor(p, i, u + c % 2 * 2, c // 2 * KW // 2 + m, 8, 1) for c in range(4)]
            w[0], w[3] = pace(w[0]), pace(w[3])
            b = [pltpu.bitcast(x, BF16).astype(F32) for x in w]
            for k in (1, 3, 4, 5, 6):
                st16(f"wt{p}", (5 * i + k - 1 - (k > 2)) * KW + r, RIGHT[k][1](b[RIGHT[k][0]], b[RIGHT[k][2]]))

        def right2_list(p, step, end=0, order=(0, 2, 1, 4, 5, 3, 6), start=0):
            return [(25, P(right2, p, r, i)) for i in order for r in range(start, end, step)]

        def right(p, t, r):
            b = [ld(f"w{p}", (h * NT + t + 4 * u) * KW + r, 16) for h in range(2) for u in range(2)]
            mask = 9 if p else 9
            b = [_rows(pace(x[:8]), pace(x[8:])) if mask >> c & 1 else x for c, x in enumerate(b)]
            b11, b12, b21, b22 = (pltpu.bitcast(x, BF16).astype(F32) for x in b)
            for i, val in enumerate((sub(b21, b11), sub(b12, b22), add(b11, b22),
                                     add(b21, b22), add(b11, b12))):
                st16(f"ws{p}", (4 * i + t) * KW + r, val)

        def right_list(p):
            return [(48, P(right, p, t, r)) for t in range(4) for r in range(0, KW, 16)]

        def ld_kv(c, row, n, z=0):
            return ld(f"kv{c // 4}", c % 4 * (T // 2) + row, n, z)

        def a1(i, r):
            a = once(("a", i), lambda: 2 * j + i)
            w0, w1, w2, w3 = once(("taps", i), lambda: [taps[a, u] for u in range(4)])
            k32 = once(("ka", i), lambda: window("ka", a * KA, KA))
            v32 = once(("va", i), lambda: window("va", a * (S // 2), S // 2))
            c0, c1, c2 = (k32[pl.ds(8 * r + 32 - u, 8), :] for u in range(3))
            vv = v32[pl.ds(8 * r, 8), :]
            e0, o0, e1, o1, o2 = _lo(c0), _hi(c0), _lo(c1), _hi(c1), _hi(c2)
            ke = _tree([mul(e0, w0), mul(o1, w1), mul(e1, w2), mul(o2, w3)])
            ko = _tree([mul(o0, w0), mul(e0, w1), mul(o1, w2), mul(e1, w3)])
            st16(f"kv{r // 32}", 8 * (r % 32), _rows(mul(ke, _lo(vv)), pace(mul(ko, _hi(vv)))))

        def a1_list(i, c0, c1):
            return [(24, P(a1, i, r)) for r in range(8 * c0, 8 * c1)]

        def freq(c, im, m):
            return c * FP + im * (T + 8) + m

        def dft(i, name, c0, m):
            def mm():
                f = pltpu.bitcast(tab[pl.ds(fresh() + T * (name == "xf"), T), :], BF16)
                if name == "hf":
                    a = once(("a", i), lambda: 2 * j + i)
                    rhs = jnp.concatenate(
                        [ha[a, :, pl.ds(c * T, T)] for c in range(c0, c0 + 4)], axis=0)
                    return lax.dot_general(f, rhs, (((1,), (1,)), ((), ())),
                                           preferred_element_type=F32)
                rhs = jnp.concatenate(
                    [pltpu.bitcast(ld_kv(c, 0, T // 2, i % 2), BF16) for c in range(c0, c0 + 4)], axis=1)
                return jnp.dot(f, rhs, preferred_element_type=F32)
            res = once((name, i, c0), mm)
            for u in range(4):
                val = res[m:m + 16, u * 128:(u + 1) * 128]
                if name == "hf" and c0 + u == 0 and m < T:
                    val = add(val, once(("dd", i), lambda: _rows(*[taps[memo["a", i], 4]] * 2)))
                st(name, freq(c0 + u, m // T, m % T), val)
            memo["clock"] = res[m + 8:m + 16, 384:]

        def dft_list(i, name, *c0s):
            return [(16, P(dft, i, name, c0, m)) for c0 in c0s for m in range(0, 2 * T, 16)]

        def a3(i, g, plane, upper, n):
            def opnd(name, c):
                re = lambda: ld(name, freq(c, 0, 8 * g), z=plane)
                im = lambda: ld(name, freq(c, 1, 8 * g), z=plane)
                if name == "xf":
                    val = add(re(), im()) if plane == 0 else re() if plane == 1 else im()
                    return pace(val) if c >= 8 else val
                return pace(re() if plane == 0 else (sub, add)[plane - 1](im(), re()))
            get = lambda name, c: once((name, i, g, plane, c), P(opnd, name, c))
            done = pace if n % 4 == 3 else lambda v: v
            cs = range(8, n + 1) if upper else range(min(n, 7) + 1)
            terms = [mul(get("xf", n - c), get("hf", c)) for c in cs]
            if upper:
                st("up", 8 * n, done(_tree(terms)))
                return
            if n >= 8:
                terms.append(ld("up", 8 * n))
            if plane == 0:
                st("k1", 8 * n, done(_tree(terms)))
            elif plane == 1:
                st("pi", 8 * n, done(_tree(terms + [ld("k1", 8 * n)])))
            else:
                pr = sub(ld("k1", 8 * n, z=1), _tree(terms))
                pi = ld("pi", 8 * n)
                zr, zi = pr, pi
                if n > 0:
                    qr, qi = memo["prev"]
                    zr, zi = sub(pr, qi), add(pi, qr)
                memo["prev"] = (pr, pi)
                if g % 2 == 0:
                    st("zr", 8 * n, done(zr))
                    st("zi", 8 * n, zi)
                else:
                    st16("z", n * T + 4 * (g - 1), _rows(ld("zr", 8 * n), done(zr)))
                    st16("z", n * T + T // 2 + 4 * (g - 1), _rows(ld("zi", 8 * n), zi))

        def a3_list(i):
            out = []
            for g in range(T // 8):
                for plane in range(3):
                    out += [(2 * (n - 8) + 4, P(a3, i, g, plane, True, n)) for n in range(8, NC)]
                    out += [(2 * min(n, 7) + 4 + 2 * (plane == 2), P(a3, i, g, plane, False, n))
                            for n in range(NC)]
            return out

        def idft(i, c0, odd, m):
            def mm():
                rhs = jnp.concatenate([pltpu.bitcast(ld("z", c * T + odd * T // 2, T // 2, i), BF16)
                                       for c in range(c0, c0 + 4)], axis=1)
                f = tab[pl.ds(fresh() + 2 * T + odd * T // 4, T // 4), :]
                return jnp.dot(pltpu.bitcast(f, BF16), rhs, preferred_element_type=F32)
            y = once(("y", i, c0, odd), mm)
            a = once(("a", i), lambda: 2 * j + i)
            q16 = once(("qa", i), lambda: window16("qa", a * (S // 2), S // 2))
            o16 = once(("oa", i), lambda: window16("oa", a * (S // 2), S // 2))
            flip = lambda w: jnp.take_along_axis(
                w, 7 - lax.broadcasted_iota(jnp.int32, (8, 128), 0), axis=0, mode="promise_in_bounds")
            for u in range(4):
                val = y[m:m + 16, u * 128:(u + 1) * 128]
                if not odd:
                    st("even", u * T // 2 + m, val)
                    continue
                even, mid = ld("even", u * T // 2 + m, 16), (c0 + u) * T + T // 2
                low = add(even, val)
                for row, out in ((mid + m, sub(even, val)),
                                 (mid - 16 - m, _rows(flip(low[8:]), flip(low[:8])))):
                    o16[pl.ds(row, 16), :] = mul(q16[pl.ds(row, 16), :].astype(F32), out).astype(BF16)
            memo["clock"] = y[m + 8:m + 16, 384:]

        def idft_list(i, *c0s):
            return [(16, P(idft, i, c0, odd, m)) for c0 in c0s
                    for odd in range(2) for m in range(0, T // 2, 16)]

        def xprep(x, u, r):
            halves = []
            for m in (r, r + 8):
                a, b = (pltpu.bitcast(x[pl.ds(2 * m, 16), pl.ds(t * 128, 128)], U32)
                        for t in (u, u + 4))
                a = pace(a)
                a11, a12, a21, a22 = _lo(a), _lo(b), _hi(a), _hi(b)
                halves.append(_left(a11, a12, a21, a22))
            for i, pair in enumerate(zip(*halves)):
                st16("xs", ((4 * i + u) * E0 + r) // 2, jnp.concatenate(pair, axis=0))

        def xprep_list(x):
            return [(27, P(xprep, x, u, r)) for r in range(0, e, 16) for u in range(4)]

        def tiles(name, rows, n):
            view = views[name][3].at[pl.ds(fresh(), spec[name][1]), :]
            return jnp.concatenate(
                [pltpu.bitcast(view[pl.ds(row, n // 2), :], BF16) for row in rows], axis=1)

        def emit(p, r0, n, par, t, m, val, end):
            if p == 0:
                st("q", (par * NT + t) * E0 + m, val)
            elif p == 3:
                base = once("row", lambda: j * E)
                o16 = once("ob", lambda: window16("ob", base, (NT - 1) * HS + (E0 if last else E)))
                o16[pl.ds(t * S + r0 + par * n + m, 16), :] = val.astype(BF16)
                if m + 16 == end and par == t // 4:
                    ob_copy(t, base + r0 // 2, n).start()
            elif p == 2:
                st("v", (par * NT + t) * KR + 16 + m, val)
            else:
                row = (par * NT + t + 1) * KL - e
                if m == 0 and not first:
                    st("k", row - WIN, ld("k", row + e - WIN, z=3))
                st("k", row + m, val)
            if m == 0 and first and p == 2 and par == 0:
                for other in range(2):
                    st("v", (other * NT + t) * KR + 8, jnp.broadcast_to(val[0:1], (WIN, 128)))

        def plain(n, t, m):
            def mm():
                w = [ld("w0", (n // 2 * NT + t + u) * KW + n % 2 * KW // 2, KW // 2, 3) for u in range(2)]
                return jnp.dot(xa[pl.ds(0, R0), pl.ds(n * D // 4, D // 4)],
                               jnp.concatenate([pltpu.bitcast(v, BF16) for v in w], axis=1),
                               preferred_element_type=F32)
            res = once(("plain", n, t), mm)
            memo["clock"] = res[m + 8:m + 16, :128]
            for u in range(2):
                val = res[m:m + 16, u * 128:(u + 1) * 128]
                if n:
                    val = add(val, ld("qo"[n % 2], (t + u) * R0 + m, 16))
                st("oq"[n % 2], (t + u) * R0 + m, val)

        def plain_list():
            return [(16, P(plain, n, t, m)) for n in range(4) for t in range(0, NT, 2) for m in range(0, R0, 16)]

        def combine(level, i, row, res, out, early=False):
            get = lambda name, z=0: ld(name + level, row, 16, z)
            if i % 2 == 0 and i < 6:
                st("abc"[i // 2] + level, row, res)
            elif i == 1:
                st("d" + level, row, res if early else sub(res, get("b")))
                out(1, 0, add(get("a"), res))
            elif i == 3:
                st("e" + level, row, sub(res, get("a", 1)))
                out(0, 1, add(get("b", 1), res))
            else:
                part = add(get("de"[i - 5]), get("c", i - 5))
                out(i - 5, i - 5, add(sub(part, get("b")) if early and i == 5 else part, res))

        def factor(p, i, t, r=0, n=KW, z=3):
            if i in (0, 2):
                return ld(f"w{p}", (t + (4 if p == 3 else NT + 4) * i // 2) * KW + r, n, z)
            return ld(f"ws{p}", (4 * (i - 1 - (i > 2)) + t) * KW + r, n, z)

        def product(p, src, r0, n, t, i, m):
            res = once(("product", p, r0, t, i), lambda: jnp.dot(
                tiles(src, [(4 * i + u) * E0 // 2 for u in range(4)], n),
                pltpu.bitcast(factor(p, i, t), BF16), preferred_element_type=F32))
            memo["clock"] = res[m + 8:m + 16]
            combine("1", i, t * E0 + m, res[m:m + 16],
                    lambda par, h, val: emit(p, r0, n, par, t + 4 * h, m, val, n), last and not r0)

        ORDER = (0, 2, 1, 4, 5, 3, 6)

        def strassen(p, src="xs", r0=0, n=e, order=ORDER):
            return [(16, P(product, p, src, r0, n, t, i, m))
                    for t in range(4) for i in order for m in range(0, n, 16)]

        def product2(p, r0, n, i, k, m):
            def mm():
                if p == 3:
                    name, row, step = f"os{i}", k * E0 // 2, E0 // 4
                elif k in (1, 3):
                    name, row, step = "xs", 2 * i * E0 + (k == 1) * (E0 + n // 4), E0 // 2
                else:
                    name, row, step = "xt", (5 * i + (0, 2, 4, 5, 6).index(k)) * E0 // 2, E0 // 4
                if k in (0, 2):
                    w = [factor(p, i, k + u, k * KW // 4, KW // 2) for u in range(2)]
                else:
                    w = [ld(f"wt{p}", ((5 * i + k - 1 - (k > 2)) * 2 + u) * KW // 2, KW // 2, 3) for u in range(2)]
                return jnp.dot(tiles(name, (row, row + step), n // 2),
                               jnp.concatenate([pltpu.bitcast(v, BF16) for v in w], axis=1),
                               preferred_element_type=F32)
            res = once(("product2", p, i, k), mm)
            memo["clock"] = res[m + 8:m + 16, 128:128 + 128]

            def out(u, r2, c2, val):
                t, row = 2 * c2 + u, r2 * n // 2 + m
                combine("1", i, t * E0 + row, val, lambda par, h, v: emit(
                    p, r0, n, par, t + 4 * h, row, v, (1 + c2) * n // 2))
            for u in range(2):
                combine("2", k, u * E0 // 2 + m, res[m:m + 16, u * 128:(u + 1) * 128], P(out, u))

        def strassen2(p, deep=7, r0=0, n=e):
            return [task for i in ORDER for task in (
                [(16, P(product2, p, r0, n, i, k, m)) for k in ORDER for m in range(0, n // 2, 16)]
                if i < deep else strassen(p, order=(i,)))]

        def xprep2(x, u, r, i):
            def blk(b):
                w = once(("x", u, r, b % 2), lambda: [pltpu.bitcast(
                    x[pl.ds(c // 2 * e + 2 * r, 32), pl.ds((u + c % 2 * 2 + b % 2 * 4) * 128, 128)], U32)
                    for c in range(4)])
                return [(_lo, _hi)[b // 2](v) for v in w]
            b0, *rest = LEFT[i]
            a = list(once(("left", u, r, b0), P(blk, b0)))
            a[0], a[3] = paced(a[0]), paced(a[3])
            if rest:
                a = list(map(rest[0], a, once(("left", u, r, rest[1]), P(blk, rest[1]))))
            for n, k in enumerate((0, 2, 4, 5, 6)):
                st16("xt", ((5 * i + n) * 2 + u) * E0 // 4 + r // 2, LEFT[k][1](a[LEFT[k][0]], a[LEFT[k][2]]))

        def xprep2_list(x):
            return [(c, P(xprep2, x, u, r, i)) for r in range(0, e // 2, 16) for u in range(2)
                    for i, c in ((1, 25), (0, 33), (6, 33), (4, 25), (3, 17), (5, 33), (2, 25))]

        def oprep2(r0, n, i, u, r):
            view = once(("oprep", i), lambda: window("o", fresh(), NT * R0))
            blk = lambda b, c: view[pl.ds(
                (u + 2 * (c % 2) + 4 * (b % 2)) * R0 + r0 + b // 2 * n + c // 2 * n // 2 + r, 16), :]
            b0, *rest = LEFT[i]
            a = [blk(b0, c) for c in range(4)]
            a = [paced(x) if 9 >> c & 1 else x for c, x in enumerate(a)]
            if rest:
                a = [rest[0](x, blk(rest[1], c)) for c, x in enumerate(a)]
            for k, val in enumerate(_left(*a)):
                st16(f"os{i}", (k * 2 + u) * E0 // 4 + r // 2, val)

        def oprep2_list(r0=0, n=e):
            return [(19 + 8 * (len(LEFT[i]) > 1), P(oprep2, r0, n, i, u, r))
                    for i in ORDER for r in range(0, n // 2, 16) for u in range(2)]

        def qk(r, w):
            par, m = r
            query = lambda t: (bufs["q"][pl.ds(t * R0 + 2 * m + par, 8, stride=2), :] if first
                               else ld("q", (par * NT + t) * E0 + m))
            scale = once(("scale", r), lambda: pace(jnp.full((8, 128), DH ** -0.5 * LOG2E, F32)))
            if r == (0, 8) and not first:
                scale = once("flush", lambda: lax.select(never, pltpu.bitcast(ld("z", 0, z=2), F32), scale))
            qv = once(("qv", r), lambda: [mul(query(t), scale) for t in range(NT)])
            s = (pace if m // 8 % 2 else lambda v: v)(_tree([mul(qv[t], ld("k", (par * NT + t + 1) * KL - e + m - w)) for t in range(NT)]))
            def fold(mask, a, b, shift):
                return add(lax.select(mask, a, b), pltpu.roll(lax.select(mask, b, a), shift, 1))
            g = m // 8 % 4
            if g % 2:
                s = fold(thirds[g // 2], memo.pop(("s", 0, w)), s, 64)
            if g == 3:
                s = fold(thirds[2], memo["s", 1, w], s, 32)
                if first and m == 24 and w:
                    early = lax.broadcasted_iota(jnp.int32, (8, 128), 0) < w
                    s = jnp.where(early & (quarter == 1), -1e9 * LOG2E, s)
            memo[("lg", r, w) if g == 3 else ("s", g % 2, w)] = s

        quarter = lax.shift_right_logical(lax.broadcasted_iota(jnp.int32, (8, 128), 1), 5)
        thirds = quarter < 2, (quarter == 1) | (quarter == 2), (quarter & 1) == 1

        def expo(r):
            lg = [memo["lg", r, w] for w in range(WIN)]
            m = pace(functools.reduce(lax.max, lg))
            memo["e", r] = [lax.exp2(sub(s, m)) for s in lg]

        def norm(r):
            total = pace(_tree(memo["e", r]))
            memo["inv", r] = total, pl.reciprocal(total, approx=True)

        def probs(r):
            total, inv = memo["inv", r]
            inv = pace(inv)
            inv = mul(inv, sub(np.float32(2), mul(total, inv)))
            for w, x in enumerate(memo["e", r]):
                st("quad", 8 * w, mul(x, inv))

        def spread(r, g):
            row = lambda w, g: (2 * w + r[0]) * HS + r[1] - 24 + 8 * g
            for w in (2 * g, 2 * g + 1):
                x = pace(ld("quad", 8 * w))
                y = pltpu.roll(x, 64, 1)
                for a, (even, odd) in ((lax.select(thirds[0], x, y), (3, 0)), (lax.select(thirds[0], y, x), (2, 1))):
                    b = pltpu.roll(a, 32, 1)
                    st("p", row(w, odd), lax.select(thirds[2], a, b))
                    st("p", row(w, even), lax.select(thirds[2], b, a))

        def qk_list(m0, m1):
            rs = [(par, m) for par in range(2) for m in range(m0, m1, 8)]
            q0, q1, q2 = 20, 3, 2
            stages = [(expo, q0), (norm, q0 + q1), (probs, q0 + 2 * q1)] + [
                (lambda r, g=g: spread(r, g), q0 + 2 * q1 + q2 * (g + 1)) for g in range(4)]
            out = [[P(qk, rs[n + u], w)] for n in range(0, len(rs), 2) for w in range(WIN) for u in range(2)] + [[] for _ in range(stages[-1][1])]
            for n in range(3, len(rs), 4):
                for f, lag in stages:
                    out[WIN * n + WIN - 1 + lag].append(P(f, rs[n]))
            return [(22, P(_run, [(0, f) for f in tasks])) for tasks in out]

        def pv(par, m, t):
            p = once(("pv", par, m), lambda: [
                (pace if w % 4 == 0 else lambda v: v)(ld("pr", (2 * w + par) * HS + m))
                for w in range(WIN)])
            row = (par * NT + t) * KR + 16 + m
            bufs["o"][pl.ds(t * R0 + 2 * m + par, 8, stride=2), :] = pace(
                _tree([mul(p[w], ld("vr", row - w)) for w in range(WIN)]))

        def pv_list(m0, m1, ts=range(NT)):
            return [(16, P(pv, par, m, t)) for par in range(2) for m in range(m0, m1, 8) for t in ts]

        def oprep(name, r0, n, which, u, r):
            a = lambda b: once(("o", name, r0, u, r, b), lambda: ld(
                "o", (u + b % 2 * 4) * R0 + r0 + b // 2 * n + r, 16, 1 + (name == "xu")))
            memo["o", name, r0, u, r, 3] = paced(a(3))
            for i in which:
                b0, *rest = LEFT[i]
                st16(name, ((4 * i + u) * E0 + r) // 2, rest[0](a(b0), a(rest[1])) if rest else a(b0))

        def oprep_list(name, r0, n, which=range(7)):
            return [(18, P(oprep, name, r0, n, which, u, r)) for r in range(0, n, 16) for u in range(4)]

        if first:

            def phase(end, side, *copies):
                start, gap = memo.get("done", 0), 3 * bool(copies)
                memo["done"] = end
                _weave(main[start:end - gap], side)
                _run(main[end - gap:end])
                if copies:
                    wait(copies)

            both = lambda p: strassen(p, order=ORDER[:1]) + strassen(p, order=ORDER[1:2]) + strassen(p, order=ORDER[2:])
            two = 0
            main = plain_list() + both(1) + (strassen2(2) if two else strassen(2))
            dq, dv = right2_list(0, 8, KW, ORDER[:3] + ORDER[5:6]), right2_list(2, 8, KW)
            wo = lambda n: wo_list(wraw.at[6 + n]) + wo_out_list(8 * n)
            do = lambda n: right2_list(3, 16, KW, start=8 * n)
            wait([w_copy(0, 0, 2)])
            _run(perm_list(0, (0,)))
            wait([x0_copy(0)])
            phase(64, [], w_copy(0, 1, 2))
            phase(90, perm_list(0, (1,))[:10])
            phase(120, perm_list(0, (1,))[10:])
            phase(192, [], x0_copy(1), w_copy(1, 0, 2))
            phase(90 + 128, perm_list(1, (0,))[:10])
            phase(248, perm_list(1, (0,))[10:])
            phase(256, [], w_copy(1, 1, 2))
            phase(304, _merge(perm_list(1, (1,)), xprep_list(xa)[:40]))
            phase(320, xprep_list(xa)[40:])
            phase(384, right_list(0)[:48], w_copy(2))
            phase(468, _merge(perm_list(2), right_list(0)[48:] + dq[32:80]))
            phase(480, [], w_copy(3))
            order = (4, 0, 5, 1, 6, 2, 7, 3)
            phase(562, _merge(perm_list(3, ts=order), dq[:32] + dq[80:]))
            phase(572, [])
            phase(592, right_list(1)[:6], w_copy(4))
            _start(in_copies(0, 0) + in_copies(0, 1))
            phase(634, _merge(perm_list(4)[:16], right_list(1)[6:36]))
            phase(676, _merge(perm_list(4)[16:], right_list(1)[36:60]))
            phase(688, right_list(1)[60:])
            phase(704, dv[:10], w_copy(5))
            phase(788, perm_list(5))
            phase(800, dv[10:26])
            phase(832, dv[26:32] + right_list(2)[:16], w_copy(6))
            phase(944, _zip(wo(0), right_list(2)[16:]) + dv[32:56], w_copy(7))
            _start(sum((in_copies(n, late) for n in range(1, NS) for late in range(2)), []))
            rest = dv[56:] + do(0) + do(1)
            phase(1010, _zip(wo(1), rest[:40]))
            logits, a = qk_list(0, E0), 40
            phase(len(main) - 4, _zip(rest[40:-a], logits[:-34])
                  + _zip(rest[-a:], [(5, f) for _, f in logits[-34:]]))
            phase(len(main), [])
            return

        views.update(pr=shifted("p", j * E, NS * E), vr=shifted("v", j * E, NS * E))
        if last:
            n = E0 // 4
            _run(pv_list(n // 2, n) + oprep_list("xs", 0, n, (0, 1)))
            main = strassen(3, "xs", 0, n, (0,)) + strassen(3, "xs", 0, n, (1,))
            _weave(main[:24], pv_list(0, n // 2) + oprep_list("xu", 0, n, range(2, 7)))
            main = main[24:] + strassen(3, "xu", 0, n, (2, 4, 5, 3, 6))
            g, h = 16, 40
            _weave(main[:-g], pv_list(n, 2 * n) + oprep_list("xt", 2 * n, n))
            _weave(main[-g:], pv_list(2 * n, 4 * n)[:h])
            main = [] + strassen(3, "xt", 2 * n, n) + strassen2(3, 7, 4 * n, 2 * n)
            pre = oprep2_list(4 * n, 2 * n)
            _weave(main[:96], pv_list(2 * n, 4 * n)[h:] + pre[:8])
            _weave(main[96:166], pre[8:])
            _run(main[166:])
            return

        for name in "vp":
            views[name] = shifted(name, E0 + j * E, E0 + (NS - 1) * E)
        head, x = strassen(1) + strassen2(0, 4), xa.at[rows(j)]
        h0, h1, h2, h3 = 66, 416, 528, 26
        for u in range(4):
            _weave(dft_list(0, "hf", 4 * u), a1_list(0, 12 * u // 4, 12 * (u + 1) // 4))
        extra = _split(xprep_list(x), 4, 6)
        _weave(dft_list(0, "xf", 0), a1_list(0, 12, 13))
        _weave(dft_list(0, "xf", 4), _merge(a1_list(0, 13, 16), extra[0]))
        _weave(dft_list(0, "xf", 8) + dft_list(0, "xf", 12)[:4], extra[1])
        _run(dft_list(0, "xf", 12)[4:])
        _weave(head[:h0], xprep2_list(x))
        _weave(head[h0:h1 - 0], a3_list(0))
        _run(head[h1 - 0:h1])
        wait(in_copies(j, 1))
        mix = _split(pv_list(0, E), 1, 4)
        for u in range(4):
            _run(idft_list(0, 4 * u))
            _weave(dft_list(1, "hf", 4 * u), a1_list(1, 3 * u, 3 * u + 3))
        oa_copy(2 * j).start()
        _weave(dft_list(1, "xf", 0), a1_list(1, 12, 16))
        _weave(dft_list(1, "xf", 4, 8, 12), mix[0])
        pre = _split(oprep2_list(), 4, 3)
        planes, g0 = _split(a3_list(1), *[1] * 48), 16
        _weave(head[h1:h2], mix[1])
        side = pre[0]
        for n, part in enumerate(_split(pre[1], *[1] * g0)):
            side = side + planes[n] + part
        tail = strassen2(2, 7)
        _weave(head[h2:] + strassen2(3) + tail[:h3], side + sum(planes[g0:], []))
        back, cutp = idft_list(1, 0, 4, 8, 12), 294
        tail = tail[:cutp] + back + tail[cutp:]
        _weave(tail[h3:len(tail) - 10], qk_list(0, E))
        _run(tail[len(tail) - 10:])
        oa_copy(2 * j + 1).start()

    def loop(j, carry):
        _wait(in_copies(j, 0))
        step(j)
        return carry

    step(0, first=True)
    _wait([table])
    lax.fori_loop(0, NS, loop, 0)
    step(NS, last=True)
    for i, name in enumerate(("oa", "ob")):
        pltpu.make_async_copy(raw[name], raw[name], sem_out.at[i]).wait()


@jax.jit
def pallas_concat_heads__ssm_conv_h3__sliding_local_dilated__prompt_kernel(
    A_q, A_k, A_v, A_shift_k, A_ssm_k, A_ssm_D, B_x, B_wqkv, B_wo,
):
    hbm = pl.BlockSpec(memory_space=pl.ANY)
    out = pl.pallas_call(
        _kernel,
        in_specs=[hbm] * 10,
        out_specs=hbm,
        out_shape=jax.ShapeDtypeStruct((S, 2 * D), BF16),
        scratch_shapes=[
            pltpu.VMEM((NT, 128, S), BF16),
            pltpu.VMEM((S, D), BF16),
            pltpu.VMEM((8, D // 2, D), BF16),
            pltpu.VMEM((NT, 5, 8, 128), F32),
            pltpu.VMEM(_TABLE.shape, U32),
            pltpu.SemaphoreType.DMA((2 * NS + 14,)),
            pltpu.SemaphoreType.DMA((2,)),
        ] + [pltpu.VMEM((r * 4 // np.dtype(t).itemsize, 128), t) for t, r in _BUFS.values()]
        + [pltpu.VMEM((4, D), BF16), pltpu.VMEM((8, 128), BF16)],
        compiler_params=pltpu.CompilerParams(vmem_limit_bytes=116 * 1024 * 1024,
                                             disable_bounds_checks=True,
                                             disable_semaphore_checks=True),
        name="fused",
    )(A_q[0], A_k[0], A_v[0], A_shift_k.T, A_ssm_k,
      A_ssm_D.reshape(8, 128), B_x[0], B_wqkv, B_wo, _TABLE)
    return out[None]
```

```python
import functools

import jax
import jax.numpy as jnp
import numpy as np
from jax import lax
from jax.experimental import pallas as pl
import jax.experimental.pallas.tpu as pltpu


S = 2048
D = 1024
T = 128
NC = S // T
NT = D // 128
NS = 4
R0 = 512
R = (S - R0) // NS
E0, E, HS = R0 // 2, R // 2, S // 2
WIN, DH = 8, 32
LOG2E = float(np.log2(np.e))
PITCH = 33
WP = 33
KR, KL = HS + 16, E0 + 16
FP = 2 * T + 16
KW = D // 4
KA = S // 2 + 32

F32, BF16, U32 = jnp.float32, jnp.bfloat16, jnp.uint32
P = functools.partial
add, sub, mul = lax.add, lax.sub, lax.mul


def _pack_rows(m):
    b = m.astype(jnp.bfloat16).view(np.uint16).astype(np.uint32)
    return np.ascontiguousarray(b[0::2] | (b[1::2] << 16))


def _dft_table():
    th = 2.0 * np.pi * (np.arange(T) + 0.25) / T
    dft = lambda t: np.concatenate([np.cos(np.outer(th, t)), -np.sin(np.outer(th, t))], axis=0)
    paired = np.arange(T).reshape(-1, 8, 2).transpose(0, 2, 1).reshape(-1)
    ph = np.outer(np.arange(T // 2) + 0.5, th)
    mats = (dft(np.arange(T)), dft(paired - (T - 1) / 2), np.cos(ph) / T, np.sin(ph) / T)
    return np.concatenate([_pack_rows(m) for m in mats] + [np.zeros((32, T), np.uint32)], axis=0)


_TABLE = _dft_table()


def _lo(w):
    return pltpu.bitcast(lax.shift_left(w, np.uint32(16)), F32)


def _hi(w):
    return pltpu.bitcast(lax.bitwise_and(w, np.uint32(0xFFFF0000)), F32)


def _rows(first, second):
    return jnp.concatenate([first, second], axis=0)


def _tree(xs):
    while len(xs) > 1:
        xs = [add(xs[i], xs[i + 1]) if i + 1 < len(xs) else xs[i] for i in range(0, len(xs), 2)]
    return xs[0]


def _left(a11, a12, a21, a22):
    return [add(a21, a22), a22, add(a11, a12), a11, add(a11, a22), sub(a12, a22), sub(a21, a11)]


def _merge(main, side):
    if not main:
        return side
    total_m = sum(c for c, _ in main)
    total_s = sum(c for c, _ in side)
    done_m, done_s, i, out = 0, 0, 0, []
    for c, f in main:
        out.append((c * total_s, f))
        done_m += c
        while i < len(side) and (done_s + side[i][0]) * total_m <= done_m * total_s:
            done_s += side[i][0]
            out.append((side[i][0] * total_m, side[i][1]))
            i += 1
    assert i == len(side)
    return out


def _zip(main, side):
    cost = {id(f): c for c, f in main + side}
    return [(cost[id(f)], f) for _, f in _merge(main, side)]


def _run(tasks):
    for _, f in tasks:
        f()


def _weave(main, side):
    _run(_merge(main, side))


def _split(tasks, *weights):
    ends = np.cumsum((0,) + weights) * len(tasks) // sum(weights)
    return [tasks[a:b] for a, b in zip(ends[:-1], ends[1:])]


def _start(copies):
    for c in copies:
        c.start()


def _wait(copies):
    for c in copies:
        c.wait()


_BUFS = {n: (t, r) for t, group in (
    (BF16, dict(qa=NT * HS, ka=NT * KA, va=NT * HS, oa=NT * HS, ob=NT * HS,
                xs=14 * E0, xt=35 * E0 // 2, **{f"os{i}": 7 * E0 // 2 for i in range(7)},
                kv0=S // 8, kv1=S // 8, kv2=S // 8, kv3=S // 8, z=NC * T, w3=NT * KW, xu=14 * E0,
                **{f"ws{p}": 20 * KW for p in range(4)}, wt0=20 * KW, wt2=35 * KW, wt3=35 * KW)),
    (U32, dict(**{f"w{p}": 2 * NT * KW for p in range(3)}, t0=34 * DH, t1=34 * DH, wp=4 * WP * DH)),
    (F32, dict(hf=NC * FP, xf=NC * FP, up=8 * NC, k1=8 * NC, pi=8 * NC, zr=8 * NC, zi=8 * NC,
               even=2 * T, quad=8 * WIN, **{n + "1": 4 * E0 for n in "abcde"}, **{n + "2": E0 for n in "abcde"},
               q=NT * R0 + 32, k=2 * NT * KL, v=2 * NT * KR, p=WIN * S, o=NT * R0 + 32)),
) for n, r in group.items()}


def _kernel(q_hbm, k_hbm, v_hbm, sk_hbm, h_hbm, d_hbm, x_hbm, w_hbm, wo_hbm, tab_hbm, out_hbm,
            ha, xa, wraw, taps, tab, sem_in, sem_out, *raw):
    *raw, sk_ref, d_ref = raw
    raw = dict(zip(_BUFS, raw))
    bufs = {n: b.bitcast(U32) if _BUFS[n][0] == BF16 else b for n, b in raw.items()}

    spec = _BUFS

    def ld(name, row, n=8, z=0):
        assert 0 <= row and row + n <= views[name][z].shape[0]
        return views[name][z][pl.ds(row, n), :]

    def st(name, row, val):
        assert 0 <= row and row + val.shape[0] <= views[name][3].shape[0]
        views[name][3][pl.ds(row, val.shape[0]), :] = val

    def st16(name, row, val):
        assert 0 <= row and 2 * row + val.shape[0] <= views[name][4].shape[0]
        views[name][4][pl.ds(2 * row, val.shape[0]), :] = val.astype(BF16)

    def window(name, row, n):
        return bufs[name].at[pl.ds(pl.multiple_of(row, 8), n), :]

    def window16(name, row, n):
        return raw[name].at[pl.ds(pl.multiple_of(2 * row, 16), 2 * n), :]

    def cols(a):
        return pl.ds(pl.multiple_of(a * 128, 128), 128)

    def rows(j):
        return pl.ds(pl.multiple_of(R0 + j * R, 128), R)

    def a_copies(a, sem):
        return [pltpu.make_async_copy(src, dst, sem) for src, dst in (
            (h_hbm.at[cols(a), :], ha.at[a]),
            (k_hbm.at[:, cols(a)], window16("ka", a * KA + 32, HS)),
            (v_hbm.at[:, cols(a)], window16("va", a * HS, HS)))]

    def in_copies(j, late):
        sem = sem_in.at[2 * j + late]
        if not late:
            return [pltpu.make_async_copy(x_hbm.at[rows(j), :], xa.at[rows(j), :], sem)] + a_copies(2 * j, sem)
        return a_copies(2 * j + 1, sem) + [
            pltpu.make_async_copy(q_hbm.at[:, cols(a)], window16("qa", a * HS, HS), sem)
            for a in (2 * j, 2 * j + 1)]

    def x0_copy(half):
        part = pl.ds(0, R0), pl.ds(half * D // 2, D // 2)
        return pltpu.make_async_copy(x_hbm.at[part], xa.at[part], sem_in.at[2 * NS + 10 + half])

    def w_copy(n, part=0, parts=1):
        size = D // 2 // parts
        span = pl.ds(n % 2 * D // 2 + part * size, size)
        src = w_hbm.at[span, pl.ds(n // 2 * D, D)] if n < 6 else wo_hbm.at[span, :]
        return pltpu.make_async_copy(src, wraw.at[n, pl.ds(part * size, size)],
                                     sem_in.at[2 * NS + (n + 2 if n > 1 else 2 * n + part)])

    def oa_copy(a):
        return pltpu.make_async_copy(window16("oa", a * HS, HS), out_hbm.at[:, cols(a)], sem_out.at[0])

    def ob_copy(t, row, n):
        return pltpu.make_async_copy(
            window16("ob", t * HS + row, n),
            out_hbm.at[pl.ds(pl.multiple_of(2 * row, 128), 2 * n), cols(NT + t)], sem_out.at[1])

    small = [pltpu.make_async_copy(a, b, sem_in.at[2 * NS + 13])
             for a, b in ((tab_hbm.at[pl.ds(5 * T // 2, 8)], tab.at[pl.ds(5 * T // 2, 8)]),
                          (sk_hbm, sk_ref), (d_hbm, d_ref))]
    full = pl.ds(0, 5 * T // 2)
    table = pltpu.make_async_copy(tab_hbm.at[full], tab.at[full], sem_in.at[2 * NS + 12])
    startup = lambda: [w_copy(0, 0, 2), x0_copy(0), w_copy(0, 1, 2), x0_copy(1), w_copy(1, 0, 2), w_copy(1, 1, 2)] + [
        w_copy(n) for n in range(2, 8)] + [table]
    _start(small + startup())
    _wait(small)
    unit = pltpu.bitcast(tab[pl.ds(5 * T // 2, 8), :], jnp.int32)
    zs = [pl.multiple_of(unit[i, 0] * 8, 8) for i in range(3)]
    views = {n: [b.at[pl.ds(z, spec[n][1]), :] for z in zs] + [b, raw[n]] for n, b in bufs.items()}

    for a in range(NT):
        st("ka", a * KA + 24, jnp.zeros((8, 128), U32))
    for t in range(2 * NT):
        st("k", t * KL + 8, jnp.zeros((WIN, 128), F32))
    skf = sk_ref[...].astype(F32)
    df = d_ref[...].astype(F32)
    for t in range(NT):
        for i in range(4):
            taps[t, i] = jnp.broadcast_to(skf[i:i + 1, t * 128:(t + 1) * 128], (8, 128))
        taps[t, 4] = jnp.broadcast_to(df[t:t + 1, :], (8, 128))

    def step(j, first=False, last=False):
        memo = {}
        e = E0 if first else E
        never = tab[pl.ds(5 * T // 2, 8), :] != 0

        def once(key, fn):
            if key not in memo:
                memo[key] = fn()
            return memo[key]

        def fresh():
            memo["fresh"] = memo.get("fresh", 1) + 1
            return pl.multiple_of(zs[0] * memo["fresh"], 8)

        def pace(val):
            clock = memo.get("clock")
            if clock is None:
                return val
            if val.dtype != F32:
                clock = pltpu.bitcast(clock, val.dtype)
            return lax.select(never, clock, val)

        def paced(x):
            return jnp.concatenate([pace(x[:8]), x[8:]], axis=0)

        def wait(copies):
            memo["clock"] = None
            _wait(copies)

        def shifted(name, row, most):
            return [window(name, z + row, spec[name][1] - most) for z in zs + [0]]

        def perm_in(w, u, t):
            tt = paced(pltpu.bitcast(w[pl.ds(u * 256, 256), pl.ds(t * 128, 128)], U32)).T
            for hh in range(4):
                st(f"t{u}", (4 * t + hh) * PITCH, tt[hh * DH:(hh + 1) * DH])

        def perm_out(p, h, u, t):
            g = jnp.concatenate(
                [bufs[f"t{u}"][pl.ds(zs[0] + 4 * t + i, 32, stride=PITCH), :] for i in range(4)], axis=0)
            st(f"w{p}", (h * NT + t) * KW + u * 128, paced(g).T)

        def perm_list(n, us=(0, 1), ts=range(NT)):
            return ([(1, P(perm_in, wraw.at[n], u, t)) for u in us for t in range(NT)]
                    + [(1, P(perm_out, n // 2, n % 2, u, t)) for t in ts for u in us])

        def wo_in(w, t, hh):
            w = pltpu.bitcast(w[pl.ds(hh * DH, DH), pl.ds(t * 128, 128)], U32)
            st("wp", (16 * t + hh) * WP, _rows(pace(w[:8]), pace(w[8:])))

        def wo_list(w):
            return [(9, P(wo_in, w, t, hh)) for t in range(NT) for hh in range(16)]

        LEFT = ((2, add, 3), (3,), (0, add, 1), (0,), (0, add, 3), (1, sub, 3), (2, sub, 0))
        RIGHT = ((0,), (2, sub, 0), (3,), (1, sub, 3), (0, add, 3), (2, add, 3), (0, add, 1))

        def wo_out(r, t, dh):
            b = [bufs["wp"][pl.ds(zs[dh % 2] + 16 * (t + n % 2 * 4) * WP + n // 2 * 8 + dh // 2, 16, stride=WP), :]
                 for n in range(4)]
            b = [(_lo, _hi)[dh % 2](w) for w in [paced(b[0])] + b[1:]]
            for i, (b0, *rest) in enumerate(RIGHT):
                name, n = ("ws3", 4 * (i - 1 - (i > 2))) if rest else ("w3", i * 2)
                st16(name, (n + t) * KW + 16 * dh + r, rest[0](b[b0], b[rest[1]]) if rest else b[b0])

        def wo_out_list(r):
            return [(26, P(wo_out, r, t, dh)) for t in range(4) for dh in range(16)]

        def right2(p, r, i):
            u, m = divmod(r, KW // 2)
            w = [factor(p, i, u + c % 2 * 2, c // 2 * KW // 2 + m, 8, 1) for c in range(4)]
            w[0], w[3] = pace(w[0]), pace(w[3])
            b = [pltpu.bitcast(x, BF16).astype(F32) for x in w]
            for k in (1, 3, 4, 5, 6):
                st16(f"wt{p}", (5 * i + k - 1 - (k > 2)) * KW + r, RIGHT[k][1](b[RIGHT[k][0]], b[RIGHT[k][2]]))

        def right2_list(p, step, end=0, order=(0, 2, 1, 4, 5, 3, 6), start=0):
            return [(25, P(right2, p, r, i)) for i in order for r in range(start, end, step)]

        def right(p, t, r):
            b = [ld(f"w{p}", (h * NT + t + 4 * u) * KW + r, 16) for h in range(2) for u in range(2)]
            mask = 9 if p else 9
            b = [_rows(pace(x[:8]), pace(x[8:])) if mask >> c & 1 else x for c, x in enumerate(b)]
            b11, b12, b21, b22 = (pltpu.bitcast(x, BF16).astype(F32) for x in b)
            for i, val in enumerate((sub(b21, b11), sub(b12, b22), add(b11, b22),
                                     add(b21, b22), add(b11, b12))):
                st16(f"ws{p}", (4 * i + t) * KW + r, val)

        def right_list(p):
            return [(48, P(right, p, t, r)) for t in range(4) for r in range(0, KW, 16)]

        def ld_kv(c, row, n, z=0):
            return ld(f"kv{c // 4}", c % 4 * (T // 2) + row, n, z)

        def a1(i, r):
            a = once(("a", i), lambda: 2 * j + i)
            w0, w1, w2, w3 = once(("taps", i), lambda: [taps[a, u] for u in range(4)])
            k32 = once(("ka", i), lambda: window("ka", a * KA, KA))
            v32 = once(("va", i), lambda: window("va", a * (S // 2), S // 2))
            c0, c1, c2 = (k32[pl.ds(8 * r + 32 - u, 8), :] for u in range(3))
            vv = v32[pl.ds(8 * r, 8), :]
            e0, o0, e1, o1, o2 = _lo(c0), _hi(c0), _lo(c1), _hi(c1), _hi(c2)
            ke = _tree([mul(e0, w0), mul(o1, w1), mul(e1, w2), mul(o2, w3)])
            ko = _tree([mul(o0, w0), mul(e0, w1), mul(o1, w2), mul(e1, w3)])
            st16(f"kv{r // 32}", 8 * (r % 32), _rows(mul(ke, _lo(vv)), pace(mul(ko, _hi(vv)))))

        def a1_list(i, c0, c1):
            return [(24, P(a1, i, r)) for r in range(8 * c0, 8 * c1)]

        def freq(c, im, m):
            return c * FP + im * (T + 8) + m

        def dft(i, name, c0, m):
            def mm():
                f = pltpu.bitcast(tab[pl.ds(fresh() + T * (name == "xf"), T), :], BF16)
                if name == "hf":
                    a = once(("a", i), lambda: 2 * j + i)
                    rhs = jnp.concatenate(
                        [ha[a, :, pl.ds(c * T, T)] for c in range(c0, c0 + 4)], axis=0)
                    return lax.dot_general(f, rhs, (((1,), (1,)), ((), ())),
                                           preferred_element_type=F32)
                rhs = jnp.concatenate(
                    [pltpu.bitcast(ld_kv(c, 0, T // 2, i % 2), BF16) for c in range(c0, c0 + 4)], axis=1)
                return jnp.dot(f, rhs, preferred_element_type=F32)
            res = once((name, i, c0), mm)
            for u in range(4):
                val = res[m:m + 16, u * 128:(u + 1) * 128]
                if name == "hf" and c0 + u == 0 and m < T:
                    val = add(val, once(("dd", i), lambda: _rows(*[taps[memo["a", i], 4]] * 2)))
                st(name, freq(c0 + u, m // T, m % T), val)
            memo["clock"] = res[m + 8:m + 8 + 8, 0:0 + 128]

        def dft_list(i, name, *c0s):
            return [(16, P(dft, i, name, c0, m)) for c0 in c0s for m in range(0, 2 * T, 16)]

        def a3(i, g, plane, upper, n):
            def opnd(name, c):
                re = lambda: ld(name, freq(c, 0, 8 * g), z=plane)
                im = lambda: ld(name, freq(c, 1, 8 * g), z=plane)
                if name == "xf":
                    val = add(re(), im()) if plane == 0 else re() if plane == 1 else im()
                    return pace(val) if c >= 8 and c % 1 == 0 else val
                val = re() if plane == 0 else (sub, add)[plane - 1](im(), re())
                return pace(val) if c % 4 == 0 else val
            get = lambda name, c: once((name, i, g, plane, c), P(opnd, name, c))
            done = pace if n % 4 == 4 - 1 else lambda v: v
            cs = range(8, n + 1) if upper else range(min(n, 7) + 1)
            terms = [mul(get("xf", n - c), get("hf", c)) for c in cs]
            if upper:
                st("up", 8 * n, done(_tree(terms)))
                return
            if n >= 8:
                terms.append(ld("up", 8 * n))
            if plane == 0:
                st("k1", 8 * n, done(_tree(terms)))
            elif plane == 1:
                st("pi", 8 * n, done(_tree(terms + [ld("k1", 8 * n)])))
            else:
                pr = sub(ld("k1", 8 * n, z=1), _tree(terms))
                pi = ld("pi", 8 * n)
                zr, zi = pr, pi
                if n > 0:
                    qr, qi = memo["prev"]
                    zr, zi = sub(pr, qi), add(pi, qr)
                memo["prev"] = (pr, pi)
                if g % 2 == 0:
                    st("zr", 8 * n, done(zr))
                    st("zi", 8 * n, zi)
                else:
                    st16("z", n * T + 4 * (g - 1), _rows(ld("zr", 8 * n), done(zr)))
                    st16("z", n * T + T // 2 + 4 * (g - 1), _rows(ld("zi", 8 * n), zi))

        def a3_list(i):
            out = []
            for g in range(T // 8):
                for plane in range(3):
                    out += [(2 * (n - 8) + 4, P(a3, i, g, plane, True, n)) for n in range(8, NC)]
                    out += [(2 * min(n, 7) + 4 + 2 * (plane == 2), P(a3, i, g, plane, False, n))
                            for n in range(NC)]
            return out

        def idft(i, c0, odd, m):
            def mm():
                rhs = jnp.concatenate([pltpu.bitcast(ld("z", c * T + odd * T // 2, T // 2, i), BF16)
                                       for c in range(c0, c0 + 4)], axis=1)
                f = tab[pl.ds(fresh() + 2 * T + odd * T // 4, T // 4), :]
                return jnp.dot(pltpu.bitcast(f, BF16), rhs, preferred_element_type=F32)
            y = once(("y", i, c0, odd), mm)
            a = once(("a", i), lambda: 2 * j + i)
            q16 = once(("qa", i), lambda: window16("qa", a * (S // 2), S // 2))
            o16 = once(("oa", i), lambda: window16("oa", a * (S // 2), S // 2))
            flip = lambda w: jnp.take_along_axis(
                w, 7 - lax.broadcasted_iota(jnp.int32, (8, 128), 0), axis=0, mode="promise_in_bounds")
            for u in range(4):
                val = y[m:m + 16, u * 128:(u + 1) * 128]
                if not odd:
                    st("even", u * T // 2 + m, val)
                    continue
                even, mid = ld("even", u * T // 2 + m, 16), (c0 + u) * T + T // 2
                low = add(even, val)
                for row, out in ((mid + m, sub(even, val)),
                                 (mid - 16 - m, _rows(flip(low[8:]), flip(low[:8])))):
                    o16[pl.ds(row, 16), :] = mul(q16[pl.ds(row, 16), :].astype(F32), out).astype(BF16)
            memo["clock"] = y[m + 8:m + 16, 384:]

        def idft_list(i, *c0s):
            return [(16, P(idft, i, c0, odd, m)) for c0 in c0s
                    for odd in range(2) for m in range(0, T // 2, 16)]

        def xprep(x, u, r):
            halves = []
            for m in (r, r + 8):
                a, b = (pltpu.bitcast(x[pl.ds(2 * m, 16), pl.ds(t * 128, 128)], U32)
                        for t in (u, u + 4))
                a = pace(a)
                a11, a12, a21, a22 = _lo(a), _lo(b), _hi(a), _hi(b)
                halves.append(_left(a11, a12, a21, a22))
            for i, pair in enumerate(zip(*halves)):
                st16("xs", ((4 * i + u) * E0 + r) // 2, jnp.concatenate(pair, axis=0))

        def xprep_list(x):
            return [(27, P(xprep, x, u, r)) for r in range(0, e, 16) for u in range(4)]

        def tiles(name, rows, n):
            view = views[name][3].at[pl.ds(fresh(), spec[name][1]), :]
            return jnp.concatenate(
                [pltpu.bitcast(view[pl.ds(row, n // 2), :], BF16) for row in rows], axis=1)

        def emit(p, r0, n, par, t, m, val, end):
            if p == 0:
                st("q", (par * NT + t) * E0 + m, val)
            elif p == 3:
                base = once("row", lambda: j * E)
                o16 = once("ob", lambda: window16("ob", base, (NT - 1) * HS + (E0 if last else E)))
                o16[pl.ds(t * S + r0 + par * n + m, 16), :] = val.astype(BF16)
                if m + 16 == end and par == t // 4:
                    ob_copy(t, base + r0 // 2, n).start()
            elif p == 2:
                st("v", (par * NT + t) * KR + 16 + m, val)
            else:
                row = (par * NT + t + 1) * KL - e
                if m == 0 and not first:
                    st("k", row - WIN, ld("k", row + e - WIN, z=3))
                st("k", row + m, val)
            if m == 0 and first and p == 2 and par == 0:
                for other in range(2):
                    st("v", (other * NT + t) * KR + 8, jnp.broadcast_to(val[0:1], (WIN, 128)))

        def plain(n, t, m):
            def mm():
                w = [ld("w0", (n // 2 * NT + t + u) * KW + n % 2 * KW // 2, KW // 2, 3) for u in range(2)]
                return jnp.dot(xa[pl.ds(0, R0), pl.ds(n * D // 4, D // 4)],
                               jnp.concatenate([pltpu.bitcast(v, BF16) for v in w], axis=1),
                               preferred_element_type=F32)
            res = once(("plain", n, t), mm)
            memo["clock"] = res[m + 8:m + 16, :128]
            for u in range(2):
                val = res[m:m + 16, u * 128:(u + 1) * 128]
                if n:
                    val = add(val, ld("qo"[n % 2], (t + u) * R0 + m, 16))
                st("oq"[n % 2], (t + u) * R0 + m, val)

        def plain_list():
            return [(16, P(plain, n, t, m)) for n in range(4) for t in range(0, NT, 2) for m in range(0, R0, 16)]

        def combine(level, i, row, res, out, early=False):
            get = lambda name, z=0: ld(name + level, row, 16, z)
            if i % 2 == 0 and i < 6:
                st("abc"[i // 2] + level, row, res)
            elif i == 1:
                st("d" + level, row, res if early else sub(res, get("b")))
                out(1, 0, add(get("a"), res))
            elif i == 3:
                st("e" + level, row, sub(res, get("a", 1)))
                out(0, 1, add(get("b", 1), res))
            else:
                part = add(get("de"[i - 5]), get("c", i - 5))
                out(i - 5, i - 5, add(sub(part, get("b")) if early and i == 5 else part, res))

        def factor(p, i, t, r=0, n=KW, z=3):
            if i in (0, 2):
                return ld(f"w{p}", (t + (4 if p == 3 else NT + 4) * i // 2) * KW + r, n, z)
            return ld(f"ws{p}", (4 * (i - 1 - (i > 2)) + t) * KW + r, n, z)

        def product(p, src, r0, n, t, i, m):
            res = once(("product", p, r0, t, i), lambda: jnp.dot(
                tiles(src, [(4 * i + u) * E0 // 2 for u in range(4)], n),
                pltpu.bitcast(factor(p, i, t), BF16), preferred_element_type=F32))
            memo["clock"] = res[m + 0:m + 0 + 8]
            combine("1", i, t * E0 + m, res[m:m + 16],
                    lambda par, h, val: emit(p, r0, n, par, t + 4 * h, m, val, n), last and not r0)

        ORDER = (0, 2, 1, 4, 5, 3, 6)

        def strassen(p, src="xs", r0=0, n=e, order=ORDER):
            return [(16, P(product, p, src, r0, n, t, i, m))
                    for t in range(4) for i in order for m in range(0, n, 16)]

        def product2(p, r0, n, i, k, m):
            def mm():
                if p == 3:
                    name, row, step = f"os{i}", k * E0 // 2, E0 // 4
                elif k in (1, 3):
                    name, row, step = "xs", 2 * i * E0 + (k == 1) * (E0 + n // 4), E0 // 2
                else:
                    name, row, step = "xt", (5 * i + (0, 2, 4, 5, 6).index(k)) * E0 // 2, E0 // 4
                if k in (0, 2):
                    w = [factor(p, i, k + u, k * KW // 4, KW // 2) for u in range(2)]
                else:
                    w = [ld(f"wt{p}", ((5 * i + k - 1 - (k > 2)) * 2 + u) * KW // 2, KW // 2, 3) for u in range(2)]
                return jnp.dot(tiles(name, (row, row + step), n // 2),
                               jnp.concatenate([pltpu.bitcast(v, BF16) for v in w], axis=1),
                               preferred_element_type=F32)
            res = once(("product2", p, i, k), mm)
            memo["clock"] = res[m + 8:m + 8 + 8, 0:0 + 128]

            def out(u, r2, c2, val):
                t, row = 2 * c2 + u, r2 * n // 2 + m
                combine("1", i, t * E0 + row, val, lambda par, h, v: emit(
                    p, r0, n, par, t + 4 * h, row, v, (1 + c2) * n // 2))
            for u in range(2):
                combine("2", k, u * E0 // 2 + m, res[m:m + 16, u * 128:(u + 1) * 128], P(out, u))

        def strassen2(p, deep=7, r0=0, n=e):
            return [task for i in ORDER for task in (
                [(16, P(product2, p, r0, n, i, k, m)) for k in ORDER for m in range(0, n // 2, 16)]
                if i < deep else strassen(p, order=(i,)))]

        def xprep2(x, u, r, i):
            def blk(b):
                w = once(("x", u, r, b % 2), lambda: [pltpu.bitcast(
                    x[pl.ds(c // 2 * e + 2 * r, 32), pl.ds((u + c % 2 * 2 + b % 2 * 4) * 128, 128)], U32)
                    for c in range(4)])
                return [(_lo, _hi)[b // 2](v) for v in w]
            b0, *rest = LEFT[i]
            a = list(once(("left", u, r, b0), P(blk, b0)))
            a[0], a[3] = paced(a[0]), paced(a[3])
            if rest:
                a = list(map(rest[0], a, once(("left", u, r, rest[1]), P(blk, rest[1]))))
            for n, k in enumerate((0, 2, 4, 5, 6)):
                st16("xt", ((5 * i + n) * 2 + u) * E0 // 4 + r // 2, LEFT[k][1](a[LEFT[k][0]], a[LEFT[k][2]]))

        def xprep2_list(x):
            return [(c, P(xprep2, x, u, r, i)) for r in range(0, e // 2, 16) for u in range(2)
                    for i, c in ((1, 25), (0, 33), (6, 33), (4, 25), (3, 17), (5, 33), (2, 25))]

        def oprep2(r0, n, i, u, r):
            view = once(("oprep", i), lambda: window("o", fresh(), NT * R0))
            blk = lambda b, c: view[pl.ds(
                (u + 2 * (c % 2) + 4 * (b % 2)) * R0 + r0 + b // 2 * n + c // 2 * n // 2 + r, 16), :]
            b0, *rest = LEFT[i]
            a = [blk(b0, c) for c in range(4)]
            a = [paced(x) if 9 >> c & 1 else x for c, x in enumerate(a)]
            if rest:
                a = [rest[0](x, blk(rest[1], c)) for c, x in enumerate(a)]
            for k, val in enumerate(_left(*a)):
                st16(f"os{i}", (k * 2 + u) * E0 // 4 + r // 2, val)

        def oprep2_list(r0=0, n=e):
            return [(19 + 8 * (len(LEFT[i]) > 1), P(oprep2, r0, n, i, u, r))
                    for i in ORDER for r in range(0, n // 2, 16) for u in range(2)]

        def qk(r, w):
            par, m = r
            query = lambda t: (bufs["q"][pl.ds(t * R0 + 2 * m + par, 8, stride=2), :] if first
                               else ld("q", (par * NT + t) * E0 + m))
            scale = once(("scale", r), lambda: pace(jnp.full((8, 128), DH ** -0.5 * LOG2E, F32)))
            if r == (0, 8) and not first:
                scale = once("flush", lambda: lax.select(never, pltpu.bitcast(ld("z", 0, z=2), F32), scale))
            qv = once(("qv", r), lambda: [mul(query(t), scale) for t in range(NT)])
            s = (pace if m // 8 % 2 else lambda v: v)(_tree([mul(qv[t], ld("k", (par * NT + t + 1) * KL - e + m - w)) for t in range(NT)]))
            def fold(mask, a, b, shift):
                return add(lax.select(mask, a, b), pltpu.roll(lax.select(mask, b, a), shift, 1))
            g = m // 8 % 4
            if g % 2:
                s = fold(thirds[g // 2], memo.pop(("s", 0, w)), s, 64)
            if g == 3:
                s = fold(thirds[2], memo["s", 1, w], s, 32)
                if first and m == 24 and w:
                    early = lax.broadcasted_iota(jnp.int32, (8, 128), 0) < w
                    s = jnp.where(early & (quarter == 1), -1e9 * LOG2E, s)
            memo[("lg", r, w) if g == 3 else ("s", g % 2, w)] = s

        quarter = lax.shift_right_logical(lax.broadcasted_iota(jnp.int32, (8, 128), 1), 5)
        thirds = quarter < 2, (quarter == 1) | (quarter == 2), (quarter & 1) == 1

        def expo(r):
            lg = [memo["lg", r, w] for w in range(WIN)]
            m = pace(functools.reduce(lax.max, lg))
            memo["e", r] = [lax.exp2(sub(s, m)) for s in lg]

        def norm(r):
            total = pace(_tree(memo["e", r]))
            memo["inv", r] = total, pl.reciprocal(total, approx=True)

        def probs(r):
            total, inv = memo["inv", r]
            inv = pace(inv)
            inv = mul(inv, sub(np.float32(2), mul(total, inv)))
            for w, x in enumerate(memo["e", r]):
                st("quad", 8 * w, mul(x, inv))

        def spread(r, g):
            row = lambda w, g: (2 * w + r[0]) * HS + r[1] - 24 + 8 * g
            for w in (2 * g, 2 * g + 1):
                x = pace(ld("quad", 8 * w))
                y = pltpu.roll(x, 64, 1)
                for a, (even, odd) in ((lax.select(thirds[0], x, y), (3, 0)), (lax.select(thirds[0], y, x), (2, 1))):
                    b = pltpu.roll(a, 32, 1)
                    st("p", row(w, odd), lax.select(thirds[2], a, b))
                    st("p", row(w, even), lax.select(thirds[2], b, a))

        def qk_list(m0, m1):
            rs = [(par, m) for par in range(2) for m in range(m0, m1, 8)]
            q0, q1, q2 = 20, 3, 2
            stages = [(expo, q0), (norm, q0 + q1), (probs, q0 + 2 * q1)] + [
                (lambda r, g=g: spread(r, g), q0 + 2 * q1 + q2 * (g + 1)) for g in range(4)]
            out = [[P(qk, rs[n + u], w)] for n in range(0, len(rs), 2) for w in range(WIN) for u in range(2)] + [[] for _ in range(stages[-1][1])]
            for n in range(3, len(rs), 4):
                for f, lag in stages:
                    out[WIN * n + WIN - 1 + lag].append(P(f, rs[n]))
            return [(22, P(_run, [(0, f) for f in tasks])) for tasks in out]

        def pv(par, m, t):
            p = once(("pv", par, m), lambda: [
                (pace if w % 4 == 0 else lambda v: v)(ld("pr", (2 * w + par) * HS + m))
                for w in range(WIN)])
            row = (par * NT + t) * KR + 16 + m
            bufs["o"][pl.ds(t * R0 + 2 * m + par, 8, stride=2), :] = (pace if t % 1 == 0 else lambda v: v)(
                _tree([mul(p[w], ld("vr", row - w)) for w in range(WIN)]))

        def pv_list(m0, m1, ts=range(NT)):
            return [(16, P(pv, par, m, t)) for par in range(2) for m in range(m0, m1, 8) for t in ts]

        def oprep(name, r0, n, which, u, r):
            a = lambda b: once(("o", name, r0, u, r, b), lambda: ld(
                "o", (u + b % 2 * 4) * R0 + r0 + b // 2 * n + r, 16, 1 + (name == "xu")))
            memo["o", name, r0, u, r, 3] = paced(a(3))
            for i in which:
                b0, *rest = LEFT[i]
                st16(name, ((4 * i + u) * E0 + r) // 2, rest[0](a(b0), a(rest[1])) if rest else a(b0))

        def oprep_list(name, r0, n, which=range(7)):
            return [(18, P(oprep, name, r0, n, which, u, r)) for r in range(0, n, 16) for u in range(4)]

        if first:

            def phase(end, side, *copies):
                start, gap = memo.get("done", 0), 3 * bool(copies)
                memo["done"] = end
                _weave(main[start:end - gap], side)
                _run(main[end - gap:end])
                if copies:
                    wait(copies)

            both = lambda p: strassen(p, order=ORDER[:1]) + strassen(p, order=ORDER[1:2]) + strassen(p, order=ORDER[2:])
            two = 0
            main = plain_list() + both(1) + (strassen2(2) if two else strassen(2))
            dq, dv = right2_list(0, 8, KW, ORDER[:3] + ORDER[5:6]), right2_list(2, 8, KW)
            wo = lambda n: wo_list(wraw.at[6 + n]) + wo_out_list(8 * n)
            do = lambda n: right2_list(3, 16, KW, start=8 * n)
            wait([w_copy(0, 0, 2)])
            _run(perm_list(0, (0,)))
            wait([x0_copy(0)])
            phase(64, [], w_copy(0, 1, 2))
            phase(90, perm_list(0, (1,))[:10])
            phase(120, perm_list(0, (1,))[10:])
            phase(192, [], x0_copy(1), w_copy(1, 0, 2))
            phase(90 + 128, perm_list(1, (0,))[:10])
            phase(248, perm_list(1, (0,))[10:])
            phase(256, [], w_copy(1, 1, 2))
            phase(304, _merge(perm_list(1, (1,)), xprep_list(xa)[:40]))
            phase(320, xprep_list(xa)[40:])
            phase(384, right_list(0)[:48], w_copy(2))
            phase(468, _merge(perm_list(2), right_list(0)[48:] + dq[32:80]))
            phase(480, [], w_copy(3))
            order = (4, 0, 5, 1, 6, 2, 7, 3)
            phase(562, _merge(perm_list(3, ts=order), dq[:32] + dq[80:]))
            phase(572, [])
            phase(592, right_list(1)[:6], w_copy(4))
            _start(in_copies(0, 0) + in_copies(0, 1))
            phase(634, _merge(perm_list(4)[:16], right_list(1)[6:36]))
            phase(676, _merge(perm_list(4)[16:], right_list(1)[36:60]))
            phase(688, right_list(1)[60:])
            phase(704, dv[:10], w_copy(5))
            phase(788, perm_list(5))
            phase(800, dv[10:26])
            phase(832, dv[26:32] + right_list(2)[:16], w_copy(6))
            phase(944, _zip(wo(0), right_list(2)[16:]) + dv[32:56], w_copy(7))
            _start(sum((in_copies(n, late) for n in range(1, NS) for late in range(2)), []))
            rest = dv[56:] + do(0) + do(1)
            phase(1010, _zip(wo(1), rest[:40]))
            logits, a = qk_list(0, E0), 40
            phase(len(main) - 4, _zip(rest[40:-a], logits[:-34])
                  + _zip(rest[-a:], [(5, f) for _, f in logits[-34:]]))
            phase(len(main), [])
            return

        views.update(pr=shifted("p", j * E, NS * E), vr=shifted("v", j * E, NS * E))
        if last:
            n = E0 // 4
            _run(pv_list(n // 2, n) + oprep_list("xs", 0, n, (0, 1)))
            main = strassen(3, "xs", 0, n, (0,)) + strassen(3, "xs", 0, n, (1,))
            _weave(main[:24], pv_list(0, n // 2) + oprep_list("xu", 0, n, range(2, 7)))
            main = main[24:] + strassen(3, "xu", 0, n, (2, 4, 5, 3, 6))
            g, h = 16, 40
            _weave(main[:-g], pv_list(n, 2 * n) + oprep_list("xt", 2 * n, n))
            _weave(main[-g:], pv_list(2 * n, 4 * n)[:h])
            main = [] + strassen(3, "xt", 2 * n, n) + strassen2(3, 7, 4 * n, 2 * n)
            pre = oprep2_list(4 * n, 2 * n)
            _weave(main[:96], pv_list(2 * n, 4 * n)[h:] + pre[:8])
            _weave(main[96:166], pre[8:])
            _run(main[166:])
            return

        for name in "vp":
            views[name] = shifted(name, E0 + j * E, E0 + (NS - 1) * E)
        head, x = strassen(1) + strassen2(0, 4), xa.at[rows(j)]
        h0, h1, h2, h3 = 66, 416, 528, 26
        for u in range(4):
            _weave(dft_list(0, "hf", 4 * u), a1_list(0, 12 * u // 4, 12 * (u + 1) // 4))
        extra = _split(xprep_list(x), 4, 6)
        _weave(dft_list(0, "xf", 0), a1_list(0, 12, 13))
        _weave(dft_list(0, "xf", 4), _merge(a1_list(0, 13, 16), extra[0]))
        _weave(dft_list(0, "xf", 8) + dft_list(0, "xf", 12)[:4], extra[1])
        _run(dft_list(0, "xf", 12)[4:])
        _weave(head[:h0], xprep2_list(x))
        _weave(head[h0:h1 - 0], a3_list(0))
        _run(head[h1 - 0:h1])
        wait(in_copies(j, 1))
        mix = _split(pv_list(0, E), 1, 4)
        for u in range(4):
            _run(idft_list(0, 4 * u))
            _weave(dft_list(1, "hf", 4 * u), a1_list(1, 3 * u, 3 * u + 3))
        oa_copy(2 * j).start()
        _weave(dft_list(1, "xf", 0), a1_list(1, 12, 16))
        _weave(dft_list(1, "xf", 4, 8, 12), mix[0])
        pre = _split(oprep2_list(), 4, 3)
        planes, g0 = _split(a3_list(1), *[1] * 48), 16
        _weave(head[h1:h2], mix[1])
        side = pre[0]
        for n, part in enumerate(_split(pre[1], *[1] * g0)):
            side = side + planes[n] + part
        tail = strassen2(2, 7)
        _weave(head[h2:] + strassen2(3) + tail[:h3], side + sum(planes[g0:], []))
        back, cutp = idft_list(1, 0, 4, 8, 12), 294
        tail = tail[:cutp] + back + tail[cutp:]
        _weave(tail[h3:len(tail) - 10], qk_list(0, E))
        _run(tail[len(tail) - 10:])
        oa_copy(2 * j + 1).start()

    def loop(j, carry):
        _wait(in_copies(j, 0))
        step(j)
        return carry

    step(0, first=True)
    _wait([table])
    lax.fori_loop(0, NS, loop, 0)
    step(NS, last=True)
    for i, name in enumerate(("oa", "ob")):
        pltpu.make_async_copy(raw[name], raw[name], sem_out.at[i]).wait()


@jax.jit
def pallas_concat_heads__ssm_conv_h3__sliding_local_dilated__prompt_kernel(
    A_q, A_k, A_v, A_shift_k, A_ssm_k, A_ssm_D, B_x, B_wqkv, B_wo,
):
    hbm = pl.BlockSpec(memory_space=pl.ANY)
    out = pl.pallas_call(
        _kernel,
        in_specs=[hbm] * 10,
        out_specs=hbm,
        out_shape=jax.ShapeDtypeStruct((S, 2 * D), BF16),
        scratch_shapes=[
            pltpu.VMEM((NT, 128, S), BF16),
            pltpu.VMEM((S, D), BF16),
            pltpu.VMEM((8, D // 2, D), BF16),
            pltpu.VMEM((NT, 5, 8, 128), F32),
            pltpu.VMEM(_TABLE.shape, U32),
            pltpu.SemaphoreType.DMA((2 * NS + 14,)),
            pltpu.SemaphoreType.DMA((2,)),
        ] + [pltpu.VMEM((r * 4 // np.dtype(t).itemsize, 128), t) for t, r in _BUFS.values()]
        + [pltpu.VMEM((4, D), BF16), pltpu.VMEM((8, 128), BF16)],
        compiler_params=pltpu.CompilerParams(vmem_limit_bytes=116 * 1024 * 1024,
                                             disable_bounds_checks=True,
                                             disable_semaphore_checks=True),
        name="fused",
    )(A_q[0], A_k[0], A_v[0], A_shift_k.T, A_ssm_k,
      A_ssm_D.reshape(8, 128), B_x[0], B_wqkv, B_wo, _TABLE)
    return out[None]
```

```python
import functools

import jax
import jax.numpy as jnp
import numpy as np
from jax import lax
from jax.experimental import pallas as pl
import jax.experimental.pallas.tpu as pltpu


S = 2048
D = 1024
T = 128
NC = S // T
NT = D // 128
NS = 4
R0 = 512
R = (S - R0) // NS
E0, E, HS = R0 // 2, R // 2, S // 2
WIN, DH = 8, 32
LOG2E = float(np.log2(np.e))
PITCH = 33
WP = 33
KR, KL = HS + 16, E0 + 16
FP = 2 * T + 16
KW = D // 4
KA = S // 2 + 32

F32, BF16, U32 = jnp.float32, jnp.bfloat16, jnp.uint32
P = functools.partial
add, sub, mul = lax.add, lax.sub, lax.mul


def _pack_rows(m):
    b = m.astype(jnp.bfloat16).view(np.uint16).astype(np.uint32)
    return np.ascontiguousarray(b[0::2] | (b[1::2] << 16))


def _dft_table():
    th = 2.0 * np.pi * (np.arange(T) + 0.25) / T
    dft = lambda t: np.concatenate([np.cos(np.outer(th, t)), -np.sin(np.outer(th, t))], axis=0)
    paired = np.arange(T).reshape(-1, 8, 2).transpose(0, 2, 1).reshape(-1)
    ph = np.outer(np.arange(T // 2) + 0.5, th)
    mats = (dft(np.arange(T)), dft(paired - (T - 1) / 2), np.cos(ph) / T, np.sin(ph) / T)
    return np.concatenate([_pack_rows(m) for m in mats] + [np.zeros((32, T), np.uint32)], axis=0)


_TABLE = _dft_table()


def _lo(w):
    return pltpu.bitcast(lax.shift_left(w, np.uint32(16)), F32)


def _hi(w):
    return pltpu.bitcast(lax.bitwise_and(w, np.uint32(0xFFFF0000)), F32)


def _rows(first, second):
    return jnp.concatenate([first, second], axis=0)


def _tree(xs):
    while len(xs) > 1:
        xs = [add(xs[i], xs[i + 1]) if i + 1 < len(xs) else xs[i] for i in range(0, len(xs), 2)]
    return xs[0]


def _left(a11, a12, a21, a22):
    return [add(a21, a22), a22, add(a11, a12), a11, add(a11, a22), sub(a12, a22), sub(a21, a11)]


def _merge(main, side):
    if not main:
        return side
    total_m = sum(c for c, _ in main)
    total_s = sum(c for c, _ in side)
    done_m, done_s, i, out = 0, 0, 0, []
    for c, f in main:
        out.append((c * total_s, f))
        done_m += c
        while i < len(side) and (done_s + side[i][0]) * total_m <= done_m * total_s:
            done_s += side[i][0]
            out.append((side[i][0] * total_m, side[i][1]))
            i += 1
    assert i == len(side)
    return out


def _zip(main, side):
    cost = {id(f): c for c, f in main + side}
    return [(cost[id(f)], f) for _, f in _merge(main, side)]


def _run(tasks):
    for _, f in tasks:
        f()


def _weave(main, side):
    _run(_merge(main, side))


def _split(tasks, *weights):
    ends = np.cumsum((0,) + weights) * len(tasks) // sum(weights)
    return [tasks[a:b] for a, b in zip(ends[:-1], ends[1:])]


def _start(copies):
    for c in copies:
        c.start()


def _wait(copies):
    for c in copies:
        c.wait()


_BUFS = {n: (t, r) for t, group in (
    (BF16, dict(qa=NT * HS, ka=NT * KA, va=NT * HS, oa=NT * HS, ob=NT * HS,
                xs=14 * E0, xt=35 * E0 // 2, **{f"os{i}": 7 * E0 // 2 for i in range(7)},
                kv0=S // 8, kv1=S // 8, kv2=S // 8, kv3=S // 8, z=NC * T, w3=NT * KW, xu=14 * E0,
                **{f"ws{p}": 20 * KW for p in range(4)}, wt0=20 * KW, wt2=35 * KW, wt3=35 * KW)),
    (U32, dict(**{f"w{p}": 2 * NT * KW for p in range(3)}, **{f"t{u}": 34 * DH for u in range(4)}, wp0=4 * WP * DH, wp1=4 * WP * DH)),
    (F32, dict(hf=NC * FP, xf=NC * FP, up=8 * NC, k1=8 * NC, pi=8 * NC, zr=8 * NC, zi=8 * NC,
               even=2 * T, quad=8 * WIN, **{n + "1": 4 * E0 for n in "abcde"}, **{n + "2": E0 for n in "abcde"},
               q=NT * R0 + 32, k=2 * NT * KL, v=2 * NT * KR, p=WIN * S, o=NT * R0 + 32)),
) for n, r in group.items()}


def _kernel(q_hbm, k_hbm, v_hbm, sk_hbm, h_hbm, d_hbm, x_hbm, w_hbm, wo_hbm, tab_hbm, out_hbm,
            ha, xa, wraw, taps, tab, sem_in, sem_out, *raw):
    *raw, sk_ref, d_ref = raw
    raw = dict(zip(_BUFS, raw))
    bufs = {n: b.bitcast(U32) if _BUFS[n][0] == BF16 else b for n, b in raw.items()}

    spec = _BUFS

    def ld(name, row, n=8, z=0):
        assert 0 <= row and row + n <= views[name][z].shape[0]
        return views[name][z][pl.ds(row, n), :]

    def st(name, row, val):
        assert 0 <= row and row + val.shape[0] <= views[name][3].shape[0]
        views[name][3][pl.ds(row, val.shape[0]), :] = val

    def st16(name, row, val):
        assert 0 <= row and 2 * row + val.shape[0] <= views[name][4].shape[0]
        views[name][4][pl.ds(2 * row, val.shape[0]), :] = val.astype(BF16)

    def window(name, row, n):
        return bufs[name].at[pl.ds(pl.multiple_of(row, 8), n), :]

    def window16(name, row, n):
        return raw[name].at[pl.ds(pl.multiple_of(2 * row, 16), 2 * n), :]

    def cols(a):
        return pl.ds(pl.multiple_of(a * 128, 128), 128)

    def rows(j):
        return pl.ds(pl.multiple_of(R0 + j * R, 128), R)

    def a_copies(a, sem):
        return [pltpu.make_async_copy(src, dst, sem) for src, dst in (
            (h_hbm.at[cols(a), :], ha.at[a]),
            (k_hbm.at[:, cols(a)], window16("ka", a * KA + 32, HS)),
            (v_hbm.at[:, cols(a)], window16("va", a * HS, HS)))]

    def in_copies(j, late, z=0):
        sem = sem_in.at[2 * j + late + z]
        if not late:
            return [pltpu.make_async_copy(x_hbm.at[rows(j), :], xa.at[rows(j), :], sem)] + a_copies(2 * j, sem)
        return a_copies(2 * j + 1, sem) + [
            pltpu.make_async_copy(q_hbm.at[:, cols(a)], window16("qa", a * HS, HS), sem)
            for a in (2 * j, 2 * j + 1)]

    def x0_copy(half, z=0):
        part = pl.ds(0, R0), pl.ds(half * D // 2, D // 2)
        return pltpu.make_async_copy(x_hbm.at[part], xa.at[part], sem_in.at[2 * NS + 10 + half + z])

    def w_copy(n, part=0, parts=1, z=0):
        size = D // 2 // parts
        span = pl.ds(n % 2 * D // 2 + part * size, size)
        src = w_hbm.at[span, pl.ds(n // 2 * D, D)] if n < 6 else wo_hbm.at[span, :]
        return pltpu.make_async_copy(src, wraw.at[n, pl.ds(part * size, size)],
                                     sem_in.at[2 * NS + (n + 2 if n > 1 else 2 * n + part) + z])

    def oa_copy(a):
        return pltpu.make_async_copy(window16("oa", a * HS, HS), out_hbm.at[:, cols(a)], sem_out.at[0])

    def ob_copy(t, row, n):
        return pltpu.make_async_copy(
            window16("ob", t * HS + row, n),
            out_hbm.at[pl.ds(pl.multiple_of(2 * row, 128), 2 * n), cols(NT + t)], sem_out.at[1])

    small = [pltpu.make_async_copy(a, b, sem_in.at[2 * NS + 12])
             for a, b in ((tab_hbm.at[pl.ds(5 * T // 2, 8)], tab.at[pl.ds(5 * T // 2, 8)]),
                          (sk_hbm, sk_ref), (d_hbm, d_ref))]
    full = pl.ds(0, 5 * T // 2)
    table = lambda z=0: pltpu.make_async_copy(tab_hbm.at[full], tab.at[full], sem_in.at[2 * NS + 9 + z])
    startup = lambda: [w_copy(0, 0, 2), x0_copy(0), w_copy(0, 1, 2), x0_copy(1), w_copy(1, 0, 2), w_copy(1, 1, 2)] + [
        w_copy(n) for n in range(2, 8)] + [table()]
    _start(small + startup())
    _wait(small)
    unit = pltpu.bitcast(tab[pl.ds(5 * T // 2, 8), :], jnp.int32)
    zs = [pl.multiple_of(unit[i, 0] * 8, 8) for i in range(3)]
    views = {n: [b.at[pl.ds(z, spec[n][1]), :] for z in zs] + [b, raw[n]] for n, b in bufs.items()}

    for a in range(NT):
        st("ka", a * KA + 24, jnp.zeros((8, 128), U32))
    for t in range(2 * NT):
        st("k", t * KL + 8, jnp.zeros((WIN, 128), F32))
    skf = sk_ref[...].astype(F32)
    df = d_ref[...].astype(F32)
    for t in range(NT):
        for i in range(4):
            taps[t, i] = jnp.broadcast_to(skf[i:i + 1, t * 128:(t + 1) * 128], (8, 128))
        taps[t, 4] = jnp.broadcast_to(df[t:t + 1, :], (8, 128))

    def step(j, first=False, last=False):
        memo = {}
        e = E0 if first else E
        never = tab[pl.ds(5 * T // 2, 8), :] != 0

        def once(key, fn):
            if key not in memo:
                memo[key] = fn()
            return memo[key]

        def fresh():
            memo["fresh"] = memo.get("fresh", 1) + 1
            return pl.multiple_of(zs[0] * memo["fresh"], 8)

        def pace(val):
            clock = memo.get("clock")
            if clock is None:
                return val
            if val.dtype != F32:
                clock = pltpu.bitcast(clock, val.dtype)
            return lax.select(never, clock, val)

        def paced(x):
            return jnp.concatenate([pace(x[:8]), x[8:]], axis=0)

        def late():
            return pltpu.bitcast(pace(jnp.zeros((8, 128), F32)), jnp.int32)[0, 0]

        def shifted(name, row, most):
            return [window(name, z + row, spec[name][1] - most) for z in zs + [0]]

        def perm_in(w, h, u, t):
            tt = paced(pltpu.bitcast(w[pl.ds(u * 256, 256), pl.ds(t * 128, 128)], U32)).T
            for hh in range(4):
                st(f"t{2 * h + u}", (4 * t + hh) * PITCH, tt[hh * DH:(hh + 1) * DH])

        def perm_out(p, h, u, t):
            g = jnp.concatenate(
                [bufs[f"t{2 * h + u}"][pl.ds(zs[0] + 4 * t + i, 32, stride=PITCH), :] for i in range(4)], axis=0)
            st(f"w{p}", (h * NT + t) * KW + u * 128, paced(g).T)

        def perm_list(n, us=(0, 1), ts=range(NT)):
            return ([(1, P(perm_in, wraw.at[n], n % 2, u, t)) for u in us for t in range(NT)]
                    + [(1, P(perm_out, n // 2, n % 2, u, t)) for t in ts for u in us])

        def wo_in(n, t, hh):
            w = pltpu.bitcast(wraw[6 + n, pl.ds(hh * DH, DH), pl.ds(t * 128, 128)], U32)
            st(f"wp{n}", (16 * t + hh) * WP, _rows(pace(w[:8]), pace(w[8:])))

        def wo_list(w):
            return [(9, P(wo_in, w, t, hh)) for t in range(NT) for hh in range(16)]

        LEFT = ((2, add, 3), (3,), (0, add, 1), (0,), (0, add, 3), (1, sub, 3), (2, sub, 0))
        RIGHT = ((0,), (2, sub, 0), (3,), (1, sub, 3), (0, add, 3), (2, add, 3), (0, add, 1))

        def wo_out(r, t, dh):
            b = [bufs[f"wp{r // 8}"][pl.ds(zs[dh % 2] + 16 * (t + n % 2 * 4) * WP + n // 2 * 8 + dh // 2, 16, stride=WP), :]
                 for n in range(4)]
            b = [(_lo, _hi)[dh % 2](w) for w in [paced(b[0])] + b[1:3] + [paced(b[3]) if 0 else b[3]]]
            for i, (b0, *rest) in enumerate(RIGHT):
                name, n = ("ws3", 4 * (i - 1 - (i > 2))) if rest else ("w3", i * 2)
                st16(name, (n + t) * KW + 16 * dh + r, rest[0](b[b0], b[rest[1]]) if rest else b[b0])

        def wo_out_list(r):
            return [(26, P(wo_out, r, t, dh)) for t in range(4) for dh in range(16)]

        def right2(p, r, i):
            u, m = divmod(r, KW // 2)
            w = [factor(p, i, u + c % 2 * 2, c // 2 * KW // 2 + m, 8, 1) for c in range(4)]
            w[0], w[3] = pace(w[0]), pace(w[3])
            b = [pltpu.bitcast(x, BF16).astype(F32) for x in w]
            for k in (1, 3, 4, 5, 6):
                st16(f"wt{p}", (5 * i + k - 1 - (k > 2)) * KW + r, RIGHT[k][1](b[RIGHT[k][0]], b[RIGHT[k][2]]))

        def right2_list(p, step, end=0, order=(0, 2, 1, 4, 5, 3, 6), start=0):
            return [(25, P(right2, p, r, i)) for i in order for r in range(start, end, step)]

        def right(p, which, t, r):
            b = [ld(f"w{p}", (h * NT + t + 4 * u) * KW + r, 16, 2 * (which == (4,))) for h in range(2) for u in range(2)]
            mask = 1 if which == (4,) else 9
            b = [_rows(pace(x[:8]), pace(x[8:])) if mask >> c & 1 else x for c, x in enumerate(b)]
            b11, b12, b21, b22 = (pltpu.bitcast(x, BF16).astype(F32) for x in b)
            for i, val in enumerate((sub(b21, b11), sub(b12, b22), add(b11, b22),
                                     add(b21, b22), add(b11, b12))):
                if i in which:
                    st16(f"ws{p}", (4 * i + t) * KW + r, val)

        def right_list(p, which=range(5)):
            return [(18 + 6 * len(which), P(right, p, which, t, r)) for t in range(4) for r in range(0, KW, 16)]

        def ld_kv(c, row, n, z=0):
            return ld(f"kv{c // 4}", c % 4 * (T // 2) + row, n, z)

        def a1(i, r):
            a = once(("a", i), lambda: 2 * j + i)
            w0, w1, w2, w3 = once(("taps", i), lambda: [taps[a, u] for u in range(4)])
            k32 = once(("ka", i), lambda: window("ka", a * KA, KA))
            v32 = once(("va", i), lambda: window("va", a * (S // 2), S // 2))
            c0, c1, c2 = (k32[pl.ds(8 * r + 32 - u, 8), :] for u in range(3))
            vv = v32[pl.ds(8 * r, 8), :]
            e0, o0, e1, o1, o2 = _lo(c0), _hi(c0), _lo(c1), _hi(c1), _hi(c2)
            ke = _tree([mul(e0, w0), mul(o1, w1), mul(e1, w2), mul(o2, w3)])
            ko = _tree([mul(o0, w0), mul(e0, w1), mul(o1, w2), mul(e1, w3)])
            st16(f"kv{r // 32}", 8 * (r % 32), _rows(mul(ke, _lo(vv)), pace(mul(ko, _hi(vv)))))

        def a1_list(i, c0, c1):
            return [(24, P(a1, i, r)) for r in range(8 * c0, 8 * c1)]

        def freq(c, im, m):
            return c * FP + im * (T + 8) + m

        def dft(i, name, c0, m):
            def mm():
                f = pltpu.bitcast(tab[pl.ds(fresh() + T * (name == "xf"), T), :], BF16)
                if name == "hf":
                    a = once(("a", i), lambda: 2 * j + i)
                    rhs = jnp.concatenate(
                        [ha[a, :, pl.ds(c * T, T)] for c in range(c0, c0 + 4)], axis=0)
                    return lax.dot_general(f, rhs, (((1,), (1,)), ((), ())),
                                           preferred_element_type=F32)
                rhs = jnp.concatenate(
                    [pltpu.bitcast(ld_kv(c, 0, T // 2, i % 2), BF16) for c in range(c0, c0 + 4)], axis=1)
                return jnp.dot(f, rhs, preferred_element_type=F32)
            res = once((name, i, c0), mm)
            for u in range(4):
                val = res[m:m + 16, u * 128:(u + 1) * 128]
                if name == "hf" and c0 + u == 0 and m < T:
                    val = add(val, once(("dd", i), lambda: _rows(*[taps[memo["a", i], 4]] * 2)))
                st(name, freq(c0 + u, m // T, m % T), val)
            memo["clock"] = res[m + 8:m + 8 + 8, 0:0 + 128]

        def dft_list(i, name, *c0s):
            return [(16, P(dft, i, name, c0, m)) for c0 in c0s for m in range(0, 2 * T, 16)]

        def a3(i, g, plane, upper, n):
            def opnd(name, c):
                re = lambda: ld(name, freq(c, 0, 8 * g), z=plane)
                im = lambda: ld(name, freq(c, 1, 8 * g), z=plane)
                if name == "xf":
                    val = add(re(), im()) if plane == 0 else re() if plane == 1 else im()
                    return pace(val) if c >= 8 and c % 1 == 0 else val
                val = re() if plane == 0 else (sub, add)[plane - 1](im(), re())
                return pace(val) if c % 4 == 0 else val
            get = lambda name, c: once((name, i, g, plane, c), P(opnd, name, c))
            done = pace if n % 4 == 4 - 1 else lambda v: v
            cs = range(8, n + 1) if upper else range(min(n, 7) + 1)
            terms = [mul(get("xf", n - c), get("hf", c)) for c in cs]
            if upper:
                st("up", 8 * n, done(_tree(terms)))
                return
            if n >= 8:
                terms.append(ld("up", 8 * n))
            if plane == 0:
                st("k1", 8 * n, done(_tree(terms)))
            elif plane == 1:
                st("pi", 8 * n, done(_tree(terms + [ld("k1", 8 * n)])))
            else:
                pr = sub(ld("k1", 8 * n, z=1), _tree(terms))
                pi = ld("pi", 8 * n)
                zr, zi = pr, pi
                if n > 0:
                    qr, qi = memo["prev"]
                    zr, zi = sub(pr, qi), add(pi, qr)
                memo["prev"] = (pr, pi)
                if g % 2 == 0:
                    st("zr", 8 * n, done(zr))
                    st("zi", 8 * n, zi)
                else:
                    st16("z", n * T + 4 * (g - 1), _rows(ld("zr", 8 * n), done(zr)))
                    st16("z", n * T + T // 2 + 4 * (g - 1), _rows(ld("zi", 8 * n), zi))

        def a3_list(i):
            out = []
            for g in range(T // 8):
                for plane in range(3):
                    out += [(2 * (n - 8) + 4, P(a3, i, g, plane, True, n)) for n in range(8, NC)]
                    out += [(2 * min(n, 7) + 4 + 2 * (plane == 2), P(a3, i, g, plane, False, n))
                            for n in range(NC)]
            return out

        def idft(i, c0, odd, m):
            def mm():
                rhs = jnp.concatenate([pltpu.bitcast(ld("z", c * T + odd * T // 2, T // 2, i), BF16)
                                       for c in range(c0, c0 + 4)], axis=1)
                f = tab[pl.ds(fresh() + 2 * T + odd * T // 4, T // 4), :]
                return jnp.dot(pltpu.bitcast(f, BF16), rhs, preferred_element_type=F32)
            y = once(("y", i, c0, odd), mm)
            a = once(("a", i), lambda: 2 * j + i)
            q16 = once(("qa", i), lambda: window16("qa", a * (S // 2), S // 2))
            o16 = once(("oa", i), lambda: window16("oa", a * (S // 2), S // 2))
            flip = lambda w: jnp.take_along_axis(
                w, 7 - lax.broadcasted_iota(jnp.int32, (8, 128), 0), axis=0, mode="promise_in_bounds")
            for u in range(4):
                val = y[m:m + 16, u * 128:(u + 1) * 128]
                if not odd:
                    st("even", u * T // 2 + m, val)
                    continue
                even, mid = ld("even", u * T // 2 + m, 16), (c0 + u) * T + T // 2
                low = add(even, val)
                for row, out in ((mid + m, sub(even, val)),
                                 (mid - 16 - m, _rows(flip(low[8:]), flip(low[:8])))):
                    o16[pl.ds(row, 16), :] = mul(q16[pl.ds(row, 16), :].astype(F32), out).astype(BF16)
            memo["clock"] = y[m + 8:m + 16, 384:]

        def idft_list(i, *c0s):
            return [(16, P(idft, i, c0, odd, m)) for c0 in c0s
                    for odd in range(2) for m in range(0, T // 2, 16)]

        def xprep(x, u, r):
            halves = []
            for m in (r, r + 8):
                a, b = (pltpu.bitcast(x[pl.ds(2 * m, 16), pl.ds(t * 128, 128)], U32)
                        for t in (u, u + 4))
                a = pace(a)
                a11, a12, a21, a22 = _lo(a), _lo(b), _hi(a), _hi(b)
                halves.append(_left(a11, a12, a21, a22))
            for i, pair in enumerate(zip(*halves)):
                st16("xs", ((4 * i + u) * E0 + r) // 2, jnp.concatenate(pair, axis=0))

        def xprep_list(x):
            return [(27, P(xprep, x, u, r)) for r in range(0, e, 16) for u in range(4)]

        def tiles(name, rows, n):
            view = views[name][3].at[pl.ds(fresh(), spec[name][1]), :]
            return jnp.concatenate(
                [pltpu.bitcast(view[pl.ds(row, n // 2), :], BF16) for row in rows], axis=1)

        def emit(p, r0, n, par, t, m, val, end):
            if p == 0:
                st("q", (par * NT + t) * E0 + m, val)
            elif p == 3:
                base = once("row", lambda: j * E)
                o16 = once("ob", lambda: window16("ob", base, (NT - 1) * HS + (E0 if last else E)))
                o16[pl.ds(t * S + r0 + par * n + m, 16), :] = val.astype(BF16)
                if m + 16 == end and par == t // 4:
                    ob_copy(t, base + r0 // 2, n).start()
            elif p == 2:
                st("v", (par * NT + t) * KR + 16 + m, val)
            else:
                row = (par * NT + t + 1) * KL - e
                if m == 0 and not first:
                    st("k", row - WIN, ld("k", row + e - WIN, z=3))
                st("k", row + m, val)
            if m == 0 and first and p == 2 and par == 0:
                for other in range(2):
                    st("v", (other * NT + t) * KR + 8, jnp.broadcast_to(val[0:1], (WIN, 128)))

        def plain(n, t, m):
            def mm():
                w = [ld("w0", (n // 2 * NT + t + u) * KW + n % 2 * KW // 2, KW // 2, 3) for u in range(2)]
                return jnp.dot(xa[pl.ds(0, R0), pl.ds(n * D // 4, D // 4)],
                               jnp.concatenate([pltpu.bitcast(v, BF16) for v in w], axis=1),
                               preferred_element_type=F32)
            res = once(("plain", n, t), mm)
            memo["clock"] = res[m + 0:m + 0 + 8, :128]
            for u in range(2):
                val = res[m:m + 16, u * 128:(u + 1) * 128]
                if n:
                    val = add(val, ld("qo"[n % 2], (t + u) * R0 + m, 16))
                st("oq"[n % 2], (t + u) * R0 + m, val)

        def plain_list():
            return [(16, P(plain, n, t, m)) for n in range(4) for t in range(0, NT, 2) for m in range(0, R0, 16)]

        def combine(level, i, row, res, out, early=False):
            get = lambda name, z=0: ld(name + level, row, 16, z)
            if early == 6 and i == 6:
                st("e" + level, row, res)
            elif early == 6 and i == 3:
                out(0, 1, add(get("b", 1), res))
                out(1, 1, add(add(get("e"), get("c", 1)), sub(res, get("a", 1))))
            elif i % 2 == 0 and i < 6:
                st("abc"[i // 2] + level, row, res)
            elif i == 1:
                st("d" + level, row, res if early == 1 else sub(res, get("b")))
                out(1, 0, add(get("a"), res))
            elif i == 3:
                st("e" + level, row, sub(res, get("a", 1)))
                out(0, 1, add(get("b", 1), res))
            else:
                part = add(get("de"[i - 5]), get("c", i - 5))
                out(i - 5, i - 5, add(sub(part, get("b")) if early == 1 and i == 5 else part, res))

        def factor(p, i, t, r=0, n=KW, z=3):
            if i in (0, 2):
                return ld(f"w{p}", (t + (4 if p == 3 else NT + 4) * i // 2) * KW + r, n, z)
            return ld(f"ws{p}", (4 * (i - 1 - (i > 2)) + t) * KW + r, n, z)

        def product(p, src, r0, n, t, i, m):
            res = once(("product", p, r0, t, i), lambda: jnp.dot(
                tiles(src, [(4 * i + u) * E0 // 2 for u in range(4)], n),
                pltpu.bitcast(factor(p, i, t), BF16), preferred_element_type=F32))
            memo["clock"] = res[m + 0:m + 0 + 8]
            combine("1", i, t * E0 + m, res[m:m + 16],
                    lambda par, h, val: emit(p, r0, n, par, t + 4 * h, m, val, n), 6 if first and p == 1 else last and not r0)

        ORDER = (0, 2, 1, 4, 5, 3, 6)

        def strassen(p, src="xs", r0=0, n=e, order=ORDER):
            return [(16, P(product, p, src, r0, n, t, i, m))
                    for t in range(4) for i in order for m in range(0, n, 16)]

        def product2(p, r0, n, i, k, m):
            def mm():
                if p == 3:
                    name, row, step = f"os{i}", k * E0 // 2, E0 // 4
                elif k in (1, 3):
                    name, row, step = "xs", 2 * i * E0 + (k == 1) * (E0 + n // 4), E0 // 2
                else:
                    name, row, step = "xt", (5 * i + (0, 2, 4, 5, 6).index(k)) * E0 // 2, E0 // 4
                if k in (0, 2):
                    w = [factor(p, i, k + u, k * KW // 4, KW // 2) for u in range(2)]
                else:
                    w = [ld(f"wt{p}", ((5 * i + k - 1 - (k > 2)) * 2 + u) * KW // 2, KW // 2, 3) for u in range(2)]
                return jnp.dot(tiles(name, (row, row + step), n // 2),
                               jnp.concatenate([pltpu.bitcast(v, BF16) for v in w], axis=1),
                               preferred_element_type=F32)
            res = once(("product2", p, i, k), mm)
            memo["clock"] = res[m + 8:m + 8 + 8, 0:0 + 128]

            def out(u, r2, c2, val):
                t, row = 2 * c2 + u, r2 * n // 2 + m
                combine("1", i, t * E0 + row, val, lambda par, h, v: emit(
                    p, r0, n, par, t + 4 * h, row, v, (1 + c2) * n // 2))
            for u in range(2):
                combine("2", k, u * E0 // 2 + m, res[m:m + 16, u * 128:(u + 1) * 128], P(out, u))

        def strassen2(p, deep=7, r0=0, n=e):
            return [task for i in ORDER for task in (
                [(16, P(product2, p, r0, n, i, k, m)) for k in ORDER for m in range(0, n // 2, 16)]
                if i < deep else strassen(p, order=(i,)))]

        def xprep2(x, u, r, i):
            def blk(b):
                w = once(("x", u, r, b % 2), lambda: [pltpu.bitcast(
                    x[pl.ds(c // 2 * e + 2 * r, 32), pl.ds((u + c % 2 * 2 + b % 2 * 4) * 128, 128)], U32)
                    for c in range(4)])
                return [(_lo, _hi)[b // 2](v) for v in w]
            b0, *rest = LEFT[i]
            a = list(once(("left", u, r, b0), P(blk, b0)))
            a[0], a[3] = paced(a[0]), paced(a[3])
            if rest:
                a = list(map(rest[0], a, once(("left", u, r, rest[1]), P(blk, rest[1]))))
            for n, k in enumerate((0, 2, 4, 5, 6)):
                st16("xt", ((5 * i + n) * 2 + u) * E0 // 4 + r // 2, LEFT[k][1](a[LEFT[k][0]], a[LEFT[k][2]]))

        def xprep2_list(x):
            return [(c, P(xprep2, x, u, r, i)) for r in range(0, e // 2, 16) for u in range(2)
                    for i, c in ((1, 25), (0, 33), (6, 33), (4, 25), (3, 17), (5, 33), (2, 25))]

        def oprep2(r0, n, i, u, r):
            view = once(("oprep", i), lambda: window("o", fresh(), NT * R0))
            blk = lambda b, c: view[pl.ds(
                (u + 2 * (c % 2) + 4 * (b % 2)) * R0 + r0 + b // 2 * n + c // 2 * n // 2 + r, 16), :]
            b0, *rest = LEFT[i]
            a = [blk(b0, c) for c in range(4)]
            a = [paced(x) if 9 >> c & 1 else x for c, x in enumerate(a)]
            if rest:
                a = [rest[0](x, blk(rest[1], c)) for c, x in enumerate(a)]
            for k, val in enumerate(_left(*a)):
                st16(f"os{i}", (k * 2 + u) * E0 // 4 + r // 2, val)

        def oprep2_list(r0=0, n=e):
            return [(19 + 8 * (len(LEFT[i]) > 1), P(oprep2, r0, n, i, u, r))
                    for i in ORDER for r in range(0, n // 2, 16) for u in range(2)]

        def qk(r, w):
            par, m = r
            query = lambda t: (bufs["q"][pl.ds(t * R0 + 2 * m + par, 8, stride=2), :] if first
                               else ld("q", (par * NT + t) * E0 + m))
            scale = once(("scale", r), lambda: pace(jnp.full((8, 128), DH ** -0.5 * LOG2E, F32)))
            if r == (0, 8) and not first:
                scale = once("flush", lambda: lax.select(never, pltpu.bitcast(ld("z", 0, z=2), F32), scale))
            if first and m % 32 == 8 and 1:
                scale = once(("flush", r), lambda: lax.select(never, window("v", fresh(), 8)[...], scale))
            qv = once(("qv", r), lambda: [mul(query(t), scale) for t in range(NT)])
            s = (pace if m // 8 % 2 else lambda v: v)(_tree([mul(qv[t], ld("k", (par * NT + t + 1) * KL - e + m - w)) for t in range(NT)]))
            def fold(mask, a, b, shift):
                return add(lax.select(mask, a, b), pltpu.roll(lax.select(mask, b, a), shift, 1))
            g = m // 8 % 4
            if g % 2:
                s = fold(thirds[g // 2], memo.pop(("s", 0, w)), s, 64)
            if g == 3:
                s = fold(thirds[2], memo["s", 1, w], s, 32)
                if first and m == 24 and w:
                    early = lax.broadcasted_iota(jnp.int32, (8, 128), 0) < w
                    s = jnp.where(early & (quarter == 1), -1e9 * LOG2E, s)
            memo[("lg", r, w) if g == 3 else ("s", g % 2, w)] = s

        quarter = lax.shift_right_logical(lax.broadcasted_iota(jnp.int32, (8, 128), 1), 5)
        thirds = quarter < 2, (quarter == 1) | (quarter == 2), (quarter & 1) == 1

        def expo(r):
            lg = [memo["lg", r, w] for w in range(WIN)]
            m = pace(functools.reduce(lax.max, lg))
            memo["e", r] = [lax.exp2(sub(s, m)) for s in lg]

        def norm(r):
            total = pace(_tree(memo["e", r]))
            memo["inv", r] = total, pl.reciprocal(total, approx=True)

        def probs(r):
            total, inv = memo["inv", r]
            inv = pace(inv)
            inv = mul(inv, sub(np.float32(2), mul(total, inv)))
            for w, x in enumerate(memo["e", r]):
                st("quad", 8 * w, mul(x, inv))

        def spread(r, g):
            row = lambda w, g: (2 * w + r[0]) * HS + r[1] - 24 + 8 * g
            for w in (2 * g, 2 * g + 1):
                x = pace(ld("quad", 8 * w))
                y = pltpu.roll(x, 64, 1)
                for a, (even, odd) in ((lax.select(thirds[0], x, y), (3, 0)), (lax.select(thirds[0], y, x), (2, 1))):
                    b = pltpu.roll(a, 32, 1)
                    st("p", row(w, odd), lax.select(thirds[2], a, b))
                    st("p", row(w, even), lax.select(thirds[2], b, a))

        def qk_list(m0, m1, pars=(0, 1)):
            rs = [(par, m) for par in pars for m in range(m0, m1, 8)]
            q0, q1, q2 = 20, 3, 2
            stages = [(expo, q0), (norm, q0 + q1), (probs, q0 + 2 * q1)] + [
                (lambda r, g=g: spread(r, g), q0 + 2 * q1 + q2 * (g + 1)) for g in range(4)]
            out = [[P(qk, rs[n + u], w)] for n in range(0, len(rs), 2) for w in range(WIN) for u in range(2)] + [[] for _ in range(stages[-1][1])]
            for n in range(3, len(rs), 4):
                for f, lag in stages:
                    out[WIN * n + WIN - 1 + lag].append(P(f, rs[n]))
            return [(22, P(_run, [(0, f) for f in tasks])) for tasks in out]

        def pv(par, m, t):
            p = once(("pv", par, m), lambda: [
                (pace if w % 4 == 0 else lambda v: v)(ld("pr", (2 * w + par) * HS + m))
                for w in range(WIN)])
            row = (par * NT + t) * KR + 16 + m
            bufs["o"][pl.ds(t * R0 + 2 * m + par, 8, stride=2), :] = (pace if t % 1 == 0 else lambda v: v)(
                _tree([mul(p[w], ld("vr", row - w)) for w in range(WIN)]))

        def pv_list(m0, m1, ts=range(NT)):
            return [(16, P(pv, par, m, t)) for par in range(2) for m in range(m0, m1, 8) for t in ts]

        def oprep(name, r0, n, which, u, r):
            a = lambda b: once(("o", name, r0, u, r, b), lambda: ld(
                "o", (u + b % 2 * 4) * R0 + r0 + b // 2 * n + r, 16, 1 + (name == "xu")))
            memo["o", name, r0, u, r, 3] = paced(a(3))
            for i in which:
                b0, *rest = LEFT[i]
                st16(name, ((4 * i + u) * E0 + r) // 2, rest[0](a(b0), a(rest[1])) if rest else a(b0))

        def oprep_list(name, r0, n, which=range(7)):
            return [(18, P(oprep, name, r0, n, which, u, r)) for r in range(0, n, 16) for u in range(4)]

        if first:

            def phase(end, side, *copies):
                start, gap = memo.get("done", 0), 0 * bool(copies)
                memo["done"] = end
                _weave(main[start:end - gap], side)
                _run(main[end - gap:end])
                if copies:
                    z = late()
                    _wait([c(z) for c in copies])

            main = plain_list() + sum((strassen(1, order=order) for order in (
                (0,), (6,), (2,), (1, 4, 5, 3))), []) + strassen(2)
            dq, dv = right2_list(0, 8, KW, ORDER[:3] + ORDER[5:6]), right2_list(2, 8, KW)
            wo = lambda n: wo_list(n) + wo_out_list(8 * n)
            do = lambda n: right2_list(3, 16, KW, start=8 * n)
            w_copy(0, 0, 2).wait()
            _run(perm_list(0, (0,)))
            memo["clock"] = pltpu.bitcast(ld("w0", 1 * KW + 120, z=3), F32)
            x0_copy(0, late()).wait()
            d, gap = 0, 18

            def permute(tasks, side):
                phase(memo["done"] + 8 * len(tasks) // 3, _merge(tasks, side) if side else tasks)
                phase(memo["done"] + gap, [])
            xp, rq, rk, rv = xprep_list(xa), right_list(0), right_list(1, range(4)), right_list(2)
            phase(64, [], P(w_copy, 0, 1, 2))
            permute(perm_list(0, (1,)), [])
            phase(150, [], P(x0_copy, 1))
            phase(190 + d, xp[:24], P(w_copy, 1, 0, 2))
            permute(perm_list(1, (0,)), xp[24:48])
            phase(258 + d, xp[48:56], P(w_copy, 1, 1, 2))
            permute(perm_list(1, (1,)), xp[56:])
            phase(380, rq[:48], P(w_copy, 2, 0, 1))
            permute(perm_list(2), rq[48:] + dq[:40])
            phase(506, right_list(1, (4,))[:28], P(w_copy, 3, 0, 1))
            permute(perm_list(3, ts=(4, 5, 0, 1, 6, 2, 7, 3)), right_list(1, (4,))[28:] + dq[40:])
            phase(630, rk[:14], P(w_copy, 4, 0, 1))
            permute(perm_list(4), rk[14:])
            phase(752, dv[:32], P(w_copy, 5, 0, 1))
            permute(perm_list(5), [])
            phase(880, rv[:18], P(w_copy, 6, 0, 1))
            _start(sum((in_copies(n, late) for n in range(NS) for late in range(2)), []))
            phase(996, _zip(wo(0), rv[18:]), P(w_copy, 7, 0, 1))
            rest = dv[32:] + do(0) + do(1)
            phase(1050, _zip(wo(1), rest[:20]))
            logits, a, b = qk_list(0, E0), 64, 24
            phase(len(main) - 4, _zip(rest[20:-a], logits[:-34])
                  + _zip(rest[-a:-b], [(5, f) for _, f in logits[-34:]]) + rest[-b:])
            phase(len(main), [], table)
            return

        views.update(pr=shifted("p", j * E, NS * E), vr=shifted("v", j * E, NS * E))
        if last:
            n = E0 // 4
            _run(pv_list(n // 2, n) + oprep_list("xs", 0, n, (0, 1)))
            main = strassen(3, "xs", 0, n, (0,)) + strassen(3, "xs", 0, n, (1,))
            _weave(main[:24], pv_list(0, n // 2) + oprep_list("xu", 0, n, range(2, 7)))
            main = main[24:] + strassen(3, "xu", 0, n, (2, 4, 5, 3, 6))
            g, h = 16, 40
            _weave(main[:-g], pv_list(n, 2 * n) + oprep_list("xt", 2 * n, n))
            _weave(main[-g:], pv_list(2 * n, 4 * n)[:h])
            main = [] + strassen(3, "xt", 2 * n, n) + strassen2(3, 7, 4 * n, 2 * n)
            pre = oprep2_list(4 * n, 2 * n)
            _weave(main[:96], pv_list(2 * n, 4 * n)[h:] + pre[:8])
            _weave(main[96:166], pre[8:])
            _run(main[166:])
            return

        for name in "vp":
            views[name] = shifted(name, E0 + j * E, E0 + (NS - 1) * E)
        head, x = strassen(1) + strassen2(0, 4), xa.at[rows(j)]
        h0, h1, h2, h3 = 66, 416, 528, 26
        for u in range(4):
            _weave(dft_list(0, "hf", 4 * u), a1_list(0, 12 * u // 4, 12 * (u + 1) // 4))
        extra = _split(xprep_list(x), 4, 6)
        _weave(dft_list(0, "xf", 0), a1_list(0, 12, 13))
        _weave(dft_list(0, "xf", 4), _merge(a1_list(0, 13, 16), extra[0]))
        _weave(dft_list(0, "xf", 8) + dft_list(0, "xf", 12)[:4], extra[1])
        _run(dft_list(0, "xf", 12)[4:])
        _weave(head[:h0], xprep2_list(x))
        _weave(head[h0:h1 - 0], a3_list(0))
        _run(head[h1 - 0:h1])
        _wait(in_copies(j, 1, late()))
        mix = _split(pv_list(0, E), 1, 4)
        for u in range(4):
            _run(idft_list(0, 4 * u))
            _weave(dft_list(1, "hf", 4 * u), a1_list(1, 3 * u, 3 * u + 3))
        oa_copy(2 * j).start()
        _weave(dft_list(1, "xf", 0), a1_list(1, 12, 16))
        _weave(dft_list(1, "xf", 4, 8, 12), mix[0])
        pre = _split(oprep2_list(), 4, 3)
        planes, g0 = _split(a3_list(1), *[1] * 48), 16
        _weave(head[h1:h2], mix[1])
        side = pre[0]
        for n, part in enumerate(_split(pre[1], *[1] * g0)):
            side = side + planes[n] + part
        tail = strassen2(2, 7)
        _weave(head[h2:] + strassen2(3) + tail[:h3], side + sum(planes[g0:], []))
        back, cutp = idft_list(1, 0, 4, 8, 12), 294
        tail = tail[:cutp] + back + tail[cutp:]
        _weave(tail[h3:len(tail) - 10], qk_list(0, E))
        _run(tail[len(tail) - 10:])
        oa_copy(2 * j + 1).start()

    def loop(j, carry):
        _wait(in_copies(j, 0))
        step(j)
        return carry

    step(0, first=True)
    lax.fori_loop(0, NS, loop, 0)
    step(NS, last=True)
    for i, name in enumerate(("oa", "ob")):
        pltpu.make_async_copy(raw[name], raw[name], sem_out.at[i]).wait()


@jax.jit
def pallas_concat_heads__ssm_conv_h3__sliding_local_dilated__prompt_kernel(
    A_q, A_k, A_v, A_shift_k, A_ssm_k, A_ssm_D, B_x, B_wqkv, B_wo,
):
    hbm = pl.BlockSpec(memory_space=pl.ANY)
    out = pl.pallas_call(
        _kernel,
        in_specs=[hbm] * 10,
        out_specs=hbm,
        out_shape=jax.ShapeDtypeStruct((S, 2 * D), BF16),
        scratch_shapes=[
            pltpu.VMEM((NT, 128, S), BF16),
            pltpu.VMEM((S, D), BF16),
            pltpu.VMEM((8, D // 2, D), BF16),
            pltpu.VMEM((NT, 5, 8, 128), F32),
            pltpu.VMEM(_TABLE.shape, U32),
            pltpu.SemaphoreType.DMA((2 * NS + 13,)),
            pltpu.SemaphoreType.DMA((2,)),
        ] + [pltpu.VMEM((r * 4 // np.dtype(t).itemsize, 128), t) for t, r in _BUFS.values()]
        + [pltpu.VMEM((4, D), BF16), pltpu.VMEM((8, 128), BF16)],
        compiler_params=pltpu.CompilerParams(vmem_limit_bytes=124 * 1024 * 1024,
                                             disable_bounds_checks=True,
                                             disable_semaphore_checks=True, flags={"XLA_TPU_RESCHEDULE_DMA_DONES": True}),
        name="fused",
    )(A_q[0], A_k[0], A_v[0], A_shift_k.T, A_ssm_k,
      A_ssm_D.reshape(8, 128), B_x[0], B_wqkv, B_wo, _TABLE)
    return out[None]
```

```python
import functools

import jax
import jax.numpy as jnp
import numpy as np
from jax import lax
from jax.experimental import pallas as pl
import jax.experimental.pallas.tpu as pltpu


S = 2048
D = 1024
T = 128
NC = S // T
NT = D // 128
NS = 4
R0 = 512
R = (S - R0) // NS
E0, E, HS = R0 // 2, R // 2, S // 2
WIN, DH = 8, 32
LOG2E = float(np.log2(np.e))
PITCH = 33
WP = 33
KR, KL = HS + 16, E0 + 16
FP = 2 * T + 16
KW = D // 4
KA = S // 2 + 32

F32, BF16, U32 = jnp.float32, jnp.bfloat16, jnp.uint32
P = functools.partial
add, sub, mul = lax.add, lax.sub, lax.mul


def _pack_rows(m):
    b = m.astype(jnp.bfloat16).view(np.uint16).astype(np.uint32)
    return np.ascontiguousarray(b[0::2] | (b[1::2] << 16))


def _dft_table():
    th = 2.0 * np.pi * (np.arange(T) + 0.25) / T
    dft = lambda t: np.concatenate([np.cos(np.outer(th, t)), -np.sin(np.outer(th, t))], axis=0)
    paired = np.arange(T).reshape(-1, 8, 2).transpose(0, 2, 1).reshape(-1)
    ph = np.outer(np.arange(T // 2) + 0.5, th)
    mats = (dft(np.arange(T)), dft(paired - (T - 1) / 2), np.cos(ph) / T, np.sin(ph) / T)
    return np.concatenate([_pack_rows(m) for m in mats] + [np.zeros((32, T), np.uint32)], axis=0)


_TABLE = _dft_table()


def _lo(w):
    return pltpu.bitcast(lax.shift_left(w, np.uint32(16)), F32)


def _hi(w):
    return pltpu.bitcast(lax.bitwise_and(w, np.uint32(0xFFFF0000)), F32)


def _rows(first, second):
    return jnp.concatenate([first, second], axis=0)


def _tree(xs):
    while len(xs) > 1:
        xs = [add(xs[i], xs[i + 1]) if i + 1 < len(xs) else xs[i] for i in range(0, len(xs), 2)]
    return xs[0]


def _left(a11, a12, a21, a22):
    return [add(a21, a22), a22, add(a11, a12), a11, add(a11, a22), sub(a12, a22), sub(a21, a11)]


def _merge(main, side):
    if not main:
        return side
    total_m = sum(c for c, _ in main)
    total_s = sum(c for c, _ in side)
    done_m, done_s, i, out = 0, 0, 0, []
    for c, f in main:
        out.append((c * total_s, f))
        done_m += c
        while i < len(side) and (done_s + side[i][0]) * total_m <= done_m * total_s:
            done_s += side[i][0]
            out.append((side[i][0] * total_m, side[i][1]))
            i += 1
    assert i == len(side)
    return out


def _zip(main, side):
    cost = {id(f): c for c, f in main + side}
    return [(cost[id(f)], f) for _, f in _merge(main, side)]


def _run(tasks):
    for _, f in tasks:
        f()


def _weave(main, side):
    _run(_merge(main, side))


def _split(tasks, *weights):
    ends = np.cumsum((0,) + weights) * len(tasks) // sum(weights)
    return [tasks[a:b] for a, b in zip(ends[:-1], ends[1:])]


def _start(copies):
    for c in copies:
        c.start()


def _wait(copies):
    for c in copies:
        c.wait()


_BUFS = {n: (t, r) for t, group in (
    (BF16, dict(qa=NT * HS, ka=NT * KA, va=NT * HS, oa=NT * HS, ob=NT * HS,
                xs=14 * E0, xt=35 * E0 // 2, **{f"os{i}": 7 * E0 // 2 for i in range(7)},
                kv0=S // 8, kv1=S // 8, kv2=S // 8, kv3=S // 8, z=NC * T, w3=NT * KW, xu=14 * E0,
                **{f"ws{p}": 20 * KW for p in range(4)}, wt0=20 * KW, wt2=35 * KW, wt3=35 * KW)),
    (U32, dict(**{f"w{p}": 2 * NT * KW for p in range(3)}, **{f"t{u}": 34 * DH for u in range(4)}, wp0=4 * WP * DH, wp1=4 * WP * DH)),
    (F32, dict(hf=NC * FP, xf=NC * FP, up=8 * NC, k1=8 * NC, pi=8 * NC, zr=8 * NC, zi=8 * NC,
               even=2 * T, quad=8 * WIN, **{n + "1": 4 * E0 for n in "abcde"}, **{n + "2": E0 for n in "abcde"},
               q=NT * R0 + 32, k=2 * NT * KL, v=2 * NT * KR, p=WIN * S, o=NT * R0 + 32)),
) for n, r in group.items()}


def _kernel(q_hbm, k_hbm, v_hbm, sk_hbm, h_hbm, d_hbm, x_hbm, w_hbm, wo_hbm, tab_hbm, out_hbm,
            ha, xa, wraw, taps, tab, sem_in, sem_out, *raw):
    *raw, sk_ref, d_ref = raw
    raw = dict(zip(_BUFS, raw))
    bufs = {n: b.bitcast(U32) if _BUFS[n][0] == BF16 else b for n, b in raw.items()}

    spec = _BUFS

    def ld(name, row, n=8, z=0):
        assert 0 <= row and row + n <= views[name][z].shape[0]
        return views[name][z][pl.ds(row, n), :]

    def st(name, row, val):
        assert 0 <= row and row + val.shape[0] <= views[name][3].shape[0]
        views[name][3][pl.ds(row, val.shape[0]), :] = val

    def st16(name, row, val):
        assert 0 <= row and 2 * row + val.shape[0] <= views[name][4].shape[0]
        views[name][4][pl.ds(2 * row, val.shape[0]), :] = val.astype(BF16)

    def window(name, row, n):
        return bufs[name].at[pl.ds(pl.multiple_of(row, 8), n), :]

    def window16(name, row, n):
        return raw[name].at[pl.ds(pl.multiple_of(2 * row, 16), 2 * n), :]

    def cols(a):
        return pl.ds(pl.multiple_of(a * 128, 128), 128)

    def rows(j):
        return pl.ds(pl.multiple_of(R0 + j * R, 128), R)

    def a_copies(a, sem):
        return [pltpu.make_async_copy(src, dst, sem) for src, dst in (
            (h_hbm.at[cols(a), :], ha.at[a]),
            (k_hbm.at[:, cols(a)], window16("ka", a * KA + 32, HS)),
            (v_hbm.at[:, cols(a)], window16("va", a * HS, HS)))]

    def in_copies(j, late, z=0):
        sem = sem_in.at[2 * j + late + z]
        if not late:
            return [pltpu.make_async_copy(x_hbm.at[rows(j), :], xa.at[rows(j), :], sem)] + a_copies(2 * j, sem)
        return a_copies(2 * j + 1, sem) + [
            pltpu.make_async_copy(q_hbm.at[:, cols(a)], window16("qa", a * HS, HS), sem)
            for a in (2 * j, 2 * j + 1)]

    def x0_copy(half, z=0):
        part = pl.ds(0, R0), pl.ds(half * D // 2, D // 2)
        return pltpu.make_async_copy(x_hbm.at[part], xa.at[part], sem_in.at[2 * NS + 10 + half + z])

    def w_copy(n, part=0, parts=1, z=0):
        size = D // 2 // parts
        span = pl.ds(n % 2 * D // 2 + part * size, size)
        src = w_hbm.at[span, pl.ds(n // 2 * D, D)] if n < 6 else wo_hbm.at[span, :]
        return pltpu.make_async_copy(src, wraw.at[n, pl.ds(part * size, size)],
                                     sem_in.at[2 * NS + (n + 2 if n > 1 else 2 * n + part) + z])

    def oa_copy(a):
        return pltpu.make_async_copy(window16("oa", a * HS, HS), out_hbm.at[:, cols(a)], sem_out.at[0])

    def ob_copy(t, row, n):
        return pltpu.make_async_copy(
            window16("ob", t * HS + row, n),
            out_hbm.at[pl.ds(pl.multiple_of(2 * row, 128), 2 * n), cols(NT + t)], sem_out.at[1])

    small = [pltpu.make_async_copy(a, b, sem_in.at[2 * NS + 12])
             for a, b in ((tab_hbm.at[pl.ds(5 * T // 2, 8)], tab.at[pl.ds(5 * T // 2, 8)]),
                          (sk_hbm, sk_ref), (d_hbm, d_ref))]
    full = pl.ds(0, 5 * T // 2)
    table = lambda z=0: pltpu.make_async_copy(tab_hbm.at[full], tab.at[full], sem_in.at[2 * NS + 9 + z])
    startup = lambda: [w_copy(0, 0, 2), x0_copy(0), w_copy(0, 1, 2), x0_copy(1), w_copy(1, 0, 2), w_copy(1, 1, 2)] + [
        w_copy(n) for n in range(2, 8)] + [table()]
    _start(small + startup())
    _wait(small)
    unit = pltpu.bitcast(tab[pl.ds(5 * T // 2, 8), :], jnp.int32)
    zs = [pl.multiple_of(unit[i, 0] * 8, 8) for i in range(3)]
    views = {n: [b.at[pl.ds(z, spec[n][1]), :] for z in zs] + [b, raw[n]] for n, b in bufs.items()}

    for a in range(NT):
        st("ka", a * KA + 24, jnp.zeros((8, 128), U32))
    for t in range(2 * NT):
        st("k", t * KL + 8, jnp.zeros((WIN, 128), F32))
    skf = sk_ref[...].astype(F32)
    df = d_ref[...].astype(F32)
    for t in range(NT):
        for i in range(4):
            taps[t, i] = jnp.broadcast_to(skf[i:i + 1, t * 128:(t + 1) * 128], (8, 128))
        taps[t, 4] = jnp.broadcast_to(df[t:t + 1, :], (8, 128))

    def step(j, first=False, last=False):
        memo = {}
        e = E0 if first else E
        never = tab[pl.ds(5 * T // 2, 8), :] != 0

        def once(key, fn):
            if key not in memo:
                memo[key] = fn()
            return memo[key]

        def fresh():
            memo["fresh"] = memo.get("fresh", 1) + 1
            return pl.multiple_of(zs[0] * memo["fresh"], 8)

        def pace(val):
            clock = memo.get("clock")
            if clock is None:
                return val
            if val.dtype != F32:
                clock = pltpu.bitcast(clock, val.dtype)
            return lax.select(never, clock, val)

        def paced(x):
            return jnp.concatenate([pace(x[:8]), x[8:]], axis=0)

        def late():
            return pltpu.bitcast(pace(jnp.zeros((8, 128), F32)), jnp.int32)[0, 0]

        def shifted(name, row, most):
            return [window(name, z + row, spec[name][1] - most) for z in zs + [0]]

        def perm_in(w, h, u, t):
            tt = paced(pltpu.bitcast(w[pl.ds(u * 256, 256), pl.ds(t * 128, 128)], U32)).T
            for hh in range(4):
                st(f"t{2 * h + u}", (4 * t + hh) * PITCH, tt[hh * DH:(hh + 1) * DH])

        def perm_out(p, h, u, t):
            g = jnp.concatenate(
                [bufs[f"t{2 * h + u}"][pl.ds(zs[0] + 4 * t + i, 32, stride=PITCH), :] for i in range(4)], axis=0)
            st(f"w{p}", (h * NT + t) * KW + u * 128, paced(g).T)

        def perm_list(n, us=(0, 1), ts=range(NT)):
            return ([(1, P(perm_in, wraw.at[n], n % 2, u, t)) for u in us for t in range(NT)]
                    + [(1, P(perm_out, n // 2, n % 2, u, t)) for t in ts for u in us])

        def wo_in(n, t, hh):
            w = pltpu.bitcast(wraw[6 + n, pl.ds(hh * DH, DH), pl.ds(t * 128, 128)], U32)
            st(f"wp{n}", (16 * t + hh) * WP, _rows(pace(w[:8]), pace(w[8:])))

        def wo_list(w):
            return [(9, P(wo_in, w, t, hh)) for t in range(NT) for hh in range(16)]

        LEFT = ((2, add, 3), (3,), (0, add, 1), (0,), (0, add, 3), (1, sub, 3), (2, sub, 0))
        RIGHT = ((0,), (2, sub, 0), (3,), (1, sub, 3), (0, add, 3), (2, add, 3), (0, add, 1))

        def wo_out(r, t, dh):
            b = [bufs[f"wp{r // 8}"][pl.ds(zs[dh % 2] + 16 * (t + n % 2 * 4) * WP + n // 2 * 8 + dh // 2, 16, stride=WP), :]
                 for n in range(4)]
            b = [(_lo, _hi)[dh % 2](w) for w in [paced(b[0])] + b[1:3] + [paced(b[3]) if 0 else b[3]]]
            for i, (b0, *rest) in enumerate(RIGHT):
                name, n = ("ws3", 4 * (i - 1 - (i > 2))) if rest else ("w3", i * 2)
                st16(name, (n + t) * KW + 16 * dh + r, rest[0](b[b0], b[rest[1]]) if rest else b[b0])

        def wo_out_list(r):
            return [(26, P(wo_out, r, t, dh)) for t in range(4) for dh in range(16)]

        def right2(p, r, i):
            u, m = divmod(r, KW // 2)
            w = [factor(p, i, u + c % 2 * 2, c // 2 * KW // 2 + m, 8, 1) for c in range(4)]
            w[0], w[3] = pace(w[0]), pace(w[3])
            b = [pltpu.bitcast(x, BF16).astype(F32) for x in w]
            for k in (1, 3, 4, 5, 6):
                st16(f"wt{p}", (5 * i + k - 1 - (k > 2)) * KW + r, RIGHT[k][1](b[RIGHT[k][0]], b[RIGHT[k][2]]))

        def right2_list(p, step, end=0, order=(0, 2, 1, 4, 5, 3, 6), start=0):
            return [(25, P(right2, p, r, i)) for i in order for r in range(start, end, step)]

        def right(p, which, t, r):
            b = [ld(f"w{p}", (h * NT + t + 4 * u) * KW + r, 16, 2 * (which == (4,))) for h in range(2) for u in range(2)]
            mask = 1 if which == (4,) else 9 if p else 9
            b = [_rows(pace(x[:8]), pace(x[8:])) if mask >> c & 1 else x for c, x in enumerate(b)]
            b11, b12, b21, b22 = (pltpu.bitcast(x, BF16).astype(F32) for x in b)
            for i, val in enumerate((sub(b21, b11), sub(b12, b22), add(b11, b22),
                                     add(b21, b22), add(b11, b12))):
                if i in which:
                    st16(f"ws{p}", (4 * i + t) * KW + r, val)

        def right_list(p, which=range(5)):
            return [(18 + 6 * len(which), P(right, p, which, t, r)) for t in range(4) for r in range(0, KW, 16)]

        def ld_kv(c, row, n, z=0):
            return ld(f"kv{c // 4}", c % 4 * (T // 2) + row, n, z)

        def a1(i, r):
            a = once(("a", i), lambda: 2 * j + i)
            w0, w1, w2, w3 = once(("taps", i), lambda: [taps[a, u] for u in range(4)])
            k32 = once(("ka", i), lambda: window("ka", a * KA, KA))
            v32 = once(("va", i), lambda: window("va", a * (S // 2), S // 2))
            c0, c1, c2 = (k32[pl.ds(8 * r + 32 - u, 8), :] for u in range(3))
            vv = v32[pl.ds(8 * r, 8), :]
            e0, o0, e1, o1, o2 = _lo(c0), _hi(c0), _lo(c1), _hi(c1), _hi(c2)
            ke = _tree([mul(e0, w0), mul(o1, w1), mul(e1, w2), mul(o2, w3)])
            ko = _tree([mul(o0, w0), mul(e0, w1), mul(o1, w2), mul(e1, w3)])
            st16(f"kv{r // 32}", 8 * (r % 32), _rows(mul(ke, _lo(vv)), pace(mul(ko, _hi(vv)))))

        def a1_list(i, c0, c1):
            return [(24, P(a1, i, r)) for r in range(8 * c0, 8 * c1)]

        def freq(c, im, m):
            return c * FP + im * (T + 8) + m

        def dft(i, name, c0, m):
            def mm():
                f = pltpu.bitcast(tab[pl.ds(fresh() + T * (name == "xf"), T), :], BF16)
                if name == "hf":
                    a = once(("a", i), lambda: 2 * j + i)
                    rhs = jnp.concatenate(
                        [ha[a, :, pl.ds(c * T, T)] for c in range(c0, c0 + 4)], axis=0)
                    return lax.dot_general(f, rhs, (((1,), (1,)), ((), ())),
                                           preferred_element_type=F32)
                rhs = jnp.concatenate(
                    [pltpu.bitcast(ld_kv(c, 0, T // 2, i % 2), BF16) for c in range(c0, c0 + 4)], axis=1)
                return jnp.dot(f, rhs, preferred_element_type=F32)
            res = once((name, i, c0), mm)
            for u in range(4):
                val = res[m:m + 16, u * 128:(u + 1) * 128]
                if name == "hf" and c0 + u == 0 and m < T:
                    val = add(val, once(("dd", i), lambda: _rows(*[taps[memo["a", i], 4]] * 2)))
                st(name, freq(c0 + u, m // T, m % T), val)
            memo["clock"] = res[m + 8:m + 8 + 8, 0:0 + 128]

        def dft_list(i, name, *c0s):
            return [(16, P(dft, i, name, c0, m)) for c0 in c0s for m in range(0, 2 * T, 16)]

        def a3(i, g, plane, upper, n):
            def opnd(name, c):
                re = lambda: ld(name, freq(c, 0, 8 * g), z=plane)
                im = lambda: ld(name, freq(c, 1, 8 * g), z=plane)
                if name == "xf":
                    val = add(re(), im()) if plane == 0 else re() if plane == 1 else im()
                    return pace(val) if c >= 8 and c % 1 == 0 else val
                val = re() if plane == 0 else (sub, add)[plane - 1](im(), re())
                return pace(val) if c % 4 == 0 else val
            get = lambda name, c: once((name, i, g, plane, c), P(opnd, name, c))
            done = pace if n % 4 == 4 - 1 else lambda v: v
            cs = range(8, n + 1) if upper else range(min(n, 7) + 1)
            terms = [mul(get("xf", n - c), get("hf", c)) for c in cs]
            if upper:
                st("up", 8 * n, done(_tree(terms)))
                return
            if n >= 8:
                terms.append(ld("up", 8 * n))
            if plane == 0:
                st("k1", 8 * n, done(_tree(terms)))
            elif plane == 1:
                st("pi", 8 * n, done(_tree(terms + [ld("k1", 8 * n)])))
            else:
                pr = sub(ld("k1", 8 * n, z=1), _tree(terms))
                pi = ld("pi", 8 * n)
                zr, zi = pr, pi
                if n > 0:
                    qr, qi = memo["prev"]
                    zr, zi = sub(pr, qi), add(pi, qr)
                memo["prev"] = (pr, pi)
                if g % 2 == 0:
                    st("zr", 8 * n, done(zr))
                    st("zi", 8 * n, zi)
                else:
                    st16("z", n * T + 4 * (g - 1), _rows(ld("zr", 8 * n), done(zr)))
                    st16("z", n * T + T // 2 + 4 * (g - 1), _rows(ld("zi", 8 * n), zi))

        def a3_list(i):
            out = []
            for g in range(T // 8):
                for plane in range(3):
                    out += [(2 * (n - 8) + 4, P(a3, i, g, plane, True, n)) for n in range(8, NC)]
                    out += [(2 * min(n, 7) + 4 + 2 * (plane == 2), P(a3, i, g, plane, False, n))
                            for n in range(NC)]
            return out

        def idft(i, c0, odd, m):
            def mm():
                rhs = jnp.concatenate([pltpu.bitcast(ld("z", c * T + odd * T // 2, T // 2, i), BF16)
                                       for c in range(c0, c0 + 4)], axis=1)
                f = tab[pl.ds(fresh() + 2 * T + odd * T // 4, T // 4), :]
                return jnp.dot(pltpu.bitcast(f, BF16), rhs, preferred_element_type=F32)
            y = once(("y", i, c0, odd), mm)
            a = once(("a", i), lambda: 2 * j + i)
            q16 = once(("qa", i), lambda: window16("qa", a * (S // 2), S // 2))
            o16 = once(("oa", i), lambda: window16("oa", a * (S // 2), S // 2))
            flip = lambda w: jnp.take_along_axis(
                w, 7 - lax.broadcasted_iota(jnp.int32, (8, 128), 0), axis=0, mode="promise_in_bounds")
            for u in range(4):
                val = y[m:m + 16, u * 128:(u + 1) * 128]
                if not odd:
                    st("even", u * T // 2 + m, val)
                    continue
                even, mid = ld("even", u * T // 2 + m, 16), (c0 + u) * T + T // 2
                low = add(even, val)
                for row, out in ((mid + m, sub(even, val)),
                                 (mid - 16 - m, _rows(flip(low[8:]), flip(low[:8])))):
                    o16[pl.ds(row, 16), :] = mul(q16[pl.ds(row, 16), :].astype(F32), out).astype(BF16)
            memo["clock"] = y[m + 8:m + 16, 384:]

        def idft_list(i, *c0s):
            return [(16, P(idft, i, c0, odd, m)) for c0 in c0s
                    for odd in range(2) for m in range(0, T // 2, 16)]

        def xprep(x, u, r):
            halves = []
            for m in (r, r + 8):
                a, b = (pltpu.bitcast(x[pl.ds(2 * m, 16), pl.ds(t * 128, 128)], U32)
                        for t in (u, u + 4))
                a = pace(a)
                a11, a12, a21, a22 = _lo(a), _lo(b), _hi(a), _hi(b)
                halves.append(_left(a11, a12, a21, a22))
            for i, pair in enumerate(zip(*halves)):
                st16("xs", ((4 * i + u) * E0 + r) // 2, jnp.concatenate(pair, axis=0))

        def xprep_list(x):
            return [(27, P(xprep, x, u, r)) for r in range(0, e, 16) for u in range(4)]

        def tiles(name, rows, n):
            view = views[name][3].at[pl.ds(fresh(), spec[name][1]), :]
            return jnp.concatenate(
                [pltpu.bitcast(view[pl.ds(row, n // 2), :], BF16) for row in rows], axis=1)

        def emit(p, r0, n, par, t, m, val, end):
            if p == 0:
                st("q", (par * NT + t) * E0 + m, val)
            elif p == 3:
                base = once("row", lambda: j * E)
                o16 = once("ob", lambda: window16("ob", base, (NT - 1) * HS + (E0 if last else E)))
                o16[pl.ds(t * S + r0 + par * n + m, 16), :] = val.astype(BF16)
                if m + 16 == end and par == t // 4:
                    ob_copy(t, base + r0 // 2, n).start()
            elif p == 2:
                st("v", (par * NT + t) * KR + 16 + m, val)
            else:
                row = (par * NT + t + 1) * KL - e
                if m == 0 and not first:
                    st("k", row - WIN, ld("k", row + e - WIN, z=3))
                st("k", row + m, val)
            if m == 0 and first and p == 2 and par == 0:
                for other in range(2):
                    st("v", (other * NT + t) * KR + 8, jnp.broadcast_to(val[0:1], (WIN, 128)))

        def plain(n, t, m):
            def mm():
                w = [ld("w0", (n // 2 * NT + t + u) * KW + n % 2 * KW // 2, KW // 2, 3) for u in range(2)]
                return jnp.dot(xa[pl.ds(0, R0), pl.ds(n * D // 4, D // 4)],
                               jnp.concatenate([pltpu.bitcast(v, BF16) for v in w], axis=1),
                               preferred_element_type=F32)
            res = once(("plain", n, t), mm)
            memo["clock"] = res[m + 0:m + 0 + 8, :128]
            for u in range(2):
                val = res[m:m + 16, u * 128:(u + 1) * 128]
                if n:
                    val = add(val, ld("qo"[n % 2], (t + u) * R0 + m, 16))
                st("oq"[n % 2], (t + u) * R0 + m, val)

        def plain_list():
            return [(16, P(plain, n, t, m)) for n in range(4) for t in range(0, NT, 2) for m in range(0, R0, 16)]

        def combine(level, i, row, res, out, early=False):
            get = lambda name, z=0: ld(name + level, row, 16, z)
            if early == 6 and i == 6:
                st("e" + level, row, res)
            elif early == 6 and i == 3:
                out(0, 1, add(get("b", 1), res))
                out(1, 1, add(add(get("e"), get("c", 1)), sub(res, get("a", 1))))
            elif i % 2 == 0 and i < 6:
                st("abc"[i // 2] + level, row, res)
            elif i == 1:
                st("d" + level, row, res if early == 1 else sub(res, get("b")))
                out(1, 0, add(get("a"), res))
            elif i == 3:
                st("e" + level, row, sub(res, get("a", 1)))
                out(0, 1, add(get("b", 1), res))
            else:
                part = add(get("de"[i - 5]), get("c", i - 5))
                out(i - 5, i - 5, add(sub(part, get("b")) if early == 1 and i == 5 else part, res))

        def factor(p, i, t, r=0, n=KW, z=3):
            if i in (0, 2):
                return ld(f"w{p}", (t + (4 if p == 3 else NT + 4) * i // 2) * KW + r, n, z)
            return ld(f"ws{p}", (4 * (i - 1 - (i > 2)) + t) * KW + r, n, z)

        def product(p, src, r0, n, t, i, m):
            res = once(("product", p, r0, t, i), lambda: jnp.dot(
                tiles(src, [(4 * i + u) * E0 // 2 for u in range(4)], n),
                pltpu.bitcast(factor(p, i, t), BF16), preferred_element_type=F32))
            memo["clock"] = res[m + 0:m + 0 + 8]
            combine("1", i, t * E0 + m, res[m:m + 16],
                    lambda par, h, val: emit(p, r0, n, par, t + 4 * h, m, val, n), 6 if first and p == 1 else last and not r0)

        ORDER = (0, 2, 1, 4, 5, 3, 6)

        def strassen(p, src="xs", r0=0, n=e, order=ORDER):
            return [(16, P(product, p, src, r0, n, t, i, m))
                    for t in range(4) for i in order for m in range(0, n, 16)]

        def product2(p, r0, n, i, k, m):
            def mm():
                if p == 3:
                    name, row, step = f"os{i}", k * E0 // 2, E0 // 4
                elif k in (1, 3):
                    name, row, step = "xs", 2 * i * E0 + (k == 1) * (E0 + n // 4), E0 // 2
                else:
                    name, row, step = "xt", (5 * i + (0, 2, 4, 5, 6).index(k)) * E0 // 2, E0 // 4
                if k in (0, 2):
                    w = [factor(p, i, k + u, k * KW // 4, KW // 2) for u in range(2)]
                else:
                    w = [ld(f"wt{p}", ((5 * i + k - 1 - (k > 2)) * 2 + u) * KW // 2, KW // 2, 3) for u in range(2)]
                return jnp.dot(tiles(name, (row, row + step), n // 2),
                               jnp.concatenate([pltpu.bitcast(v, BF16) for v in w], axis=1),
                               preferred_element_type=F32)
            res = once(("product2", p, i, k), mm)
            memo["clock"] = res[m + 8:m + 8 + 8, 0:0 + 128]

            def out(u, r2, c2, val):
                t, row = 2 * c2 + u, r2 * n // 2 + m
                combine("1", i, t * E0 + row, val, lambda par, h, v: emit(
                    p, r0, n, par, t + 4 * h, row, v, (1 + c2) * n // 2))
            for u in range(2):
                combine("2", k, u * E0 // 2 + m, res[m:m + 16, u * 128:(u + 1) * 128], P(out, u))

        def strassen2(p, deep=7, r0=0, n=e):
            return [task for i in ORDER for task in (
                [(16, P(product2, p, r0, n, i, k, m)) for k in ORDER for m in range(0, n // 2, 16)]
                if i < deep else strassen(p, order=(i,)))]

        def xprep2(x, u, r, i):
            def blk(b):
                w = once(("x", u, r, b % 2), lambda: [pltpu.bitcast(
                    x[pl.ds(c // 2 * e + 2 * r, 32), pl.ds((u + c % 2 * 2 + b % 2 * 4) * 128, 128)], U32)
                    for c in range(4)])
                return [(_lo, _hi)[b // 2](v) for v in w]
            b0, *rest = LEFT[i]
            a = list(once(("left", u, r, b0), P(blk, b0)))
            a[0], a[3] = paced(a[0]), paced(a[3])
            if rest:
                a = list(map(rest[0], a, once(("left", u, r, rest[1]), P(blk, rest[1]))))
            for n, k in enumerate((0, 2, 4, 5, 6)):
                st16("xt", ((5 * i + n) * 2 + u) * E0 // 4 + r // 2, LEFT[k][1](a[LEFT[k][0]], a[LEFT[k][2]]))

        def xprep2_list(x):
            return [(c, P(xprep2, x, u, r, i)) for r in range(0, e // 2, 16) for u in range(2)
                    for i, c in ((1, 25), (0, 33), (6, 33), (4, 25), (3, 17), (5, 33), (2, 25))]

        def oprep2(r0, n, i, u, r):
            view = once(("oprep", i), lambda: window("o", fresh(), NT * R0))
            blk = lambda b, c: view[pl.ds(
                (u + 2 * (c % 2) + 4 * (b % 2)) * R0 + r0 + b // 2 * n + c // 2 * n // 2 + r, 16), :]
            b0, *rest = LEFT[i]
            a = [blk(b0, c) for c in range(4)]
            a = [paced(x) if 9 >> c & 1 else x for c, x in enumerate(a)]
            if rest:
                a = [rest[0](x, blk(rest[1], c)) for c, x in enumerate(a)]
            for k, val in enumerate(_left(*a)):
                st16(f"os{i}", (k * 2 + u) * E0 // 4 + r // 2, val)

        def oprep2_list(r0=0, n=e):
            return [(19 + 8 * (len(LEFT[i]) > 1), P(oprep2, r0, n, i, u, r))
                    for i in ORDER for r in range(0, n // 2, 16) for u in range(2)]

        def qk(r, w):
            par, m = r
            query = lambda t: (bufs["q"][pl.ds(t * R0 + 2 * m + par, 8, stride=2), :] if first
                               else ld("q", (par * NT + t) * E0 + m))
            scale = once(("scale", r), lambda: pace(jnp.full((8, 128), DH ** -0.5 * LOG2E, F32)))
            if r == (0, 8) and not first and 1:
                scale = once("flush", lambda: lax.select(never, pltpu.bitcast(ld("z", 0, z=2), F32), scale))
            if first and m % 32 == 8 and 1:
                scale = once(("flush", r), lambda: lax.select(never, window("v", fresh(), 8)[...], scale))
            qv = once(("qv", r), lambda: [mul(query(t), scale) for t in range(NT)])
            s = (pace if m // 8 % 2 else lambda v: v)(_tree([mul(qv[t], ld("k", (par * NT + t + 1) * KL - e + m - w)) for t in range(NT)]))
            def fold(mask, a, b, shift):
                return add(lax.select(mask, a, b), pltpu.roll(lax.select(mask, b, a), shift, 1))
            g = m // 8 % 4
            if g % 2:
                s = fold(thirds[g // 2], memo.pop(("s", 0, w)), s, 64)
            if g == 3:
                s = fold(thirds[2], memo["s", 1, w], s, 32)
                if first and m == 24 and w:
                    early = lax.broadcasted_iota(jnp.int32, (8, 128), 0) < w
                    s = jnp.where(early & (quarter == 1), -1e9 * LOG2E, s)
            memo[("lg", r, w) if g == 3 else ("s", g % 2, w)] = s

        quarter = lax.shift_right_logical(lax.broadcasted_iota(jnp.int32, (8, 128), 1), 5)
        thirds = quarter < 2, (quarter == 1) | (quarter == 2), (quarter & 1) == 1

        def expo(r):
            lg = [memo["lg", r, w] for w in range(WIN)]
            m = pace(functools.reduce(lax.max, lg))
            memo["e", r] = [lax.exp2(sub(s, m)) for s in lg]

        def norm(r):
            total = pace(_tree(memo["e", r]))
            memo["inv", r] = total, pl.reciprocal(total, approx=True)

        def probs(r):
            total, inv = memo["inv", r]
            inv = pace(inv)
            inv = mul(inv, sub(np.float32(2), mul(total, inv)))
            for w, x in enumerate(memo["e", r]):
                st("quad", 8 * w, mul(x, inv))

        def spread(r, g):
            row = lambda w, g: (2 * w + r[0]) * HS + r[1] - 24 + 8 * g
            for w in (2 * g, 2 * g + 1):
                x = pace(ld("quad", 8 * w))
                y = pltpu.roll(x, 64, 1)
                for a, (even, odd) in ((lax.select(thirds[0], x, y), (3, 0)), (lax.select(thirds[0], y, x), (2, 1))):
                    b = pltpu.roll(a, 32, 1)
                    st("p", row(w, odd), lax.select(thirds[2], a, b))
                    st("p", row(w, even), lax.select(thirds[2], b, a))

        def qk_list(m0, m1, pars=(0, 1)):
            rs = [(par, m) for par in pars for m in range(m0, m1, 8)]
            q0, q1, q2 = 20, 3, 2
            stages = [(expo, q0), (norm, q0 + q1), (probs, q0 + 2 * q1)] + [
                (lambda r, g=g: spread(r, g), q0 + 2 * q1 + q2 * (g + 1)) for g in range(4)]
            out = [[P(qk, rs[n + u], w)] for n in range(0, len(rs), 2) for w in range(WIN) for u in range(2)] + [[] for _ in range(stages[-1][1])]
            for n in range(3, len(rs), 4):
                for f, lag in stages:
                    out[WIN * n + WIN - 1 + lag].append(P(f, rs[n]))
            return [(22, P(_run, [(0, f) for f in tasks])) for tasks in out]

        def pv(par, m, t):
            p = once(("pv", par, m), lambda: [
                (pace if w % 4 == 0 else lambda v: v)(ld("pr", (2 * w + par) * HS + m))
                for w in range(WIN)])
            row = (par * NT + t) * KR + 16 + m
            bufs["o"][pl.ds(t * R0 + 2 * m + par, 8, stride=2), :] = (pace if t % 1 == 0 else lambda v: v)(
                _tree([mul(p[w], ld("vr", row - w)) for w in range(WIN)]))

        def pv_list(m0, m1, ts=range(NT)):
            return [(16, P(pv, par, m, t)) for par in range(2) for m in range(m0, m1, 8) for t in ts]

        def oprep(name, r0, n, which, u, r):
            a = lambda b: once(("o", name, r0, u, r, b), lambda: ld(
                "o", (u + b % 2 * 4) * R0 + r0 + b // 2 * n + r, 16, 1 + (name == "xu")))
            memo["o", name, r0, u, r, 3] = paced(a(3))
            for i in which:
                b0, *rest = LEFT[i]
                st16(name, ((4 * i + u) * E0 + r) // 2, rest[0](a(b0), a(rest[1])) if rest else a(b0))

        def oprep_list(name, r0, n, which=range(7)):
            return [(18, P(oprep, name, r0, n, which, u, r)) for r in range(0, n, 16) for u in range(4)]

        if first:

            def phase(end, side, *copies):
                start, gap = memo.get("done", 0), 0 * bool(copies)
                memo["done"] = end
                _weave(main[start:end - gap], side)
                _run(main[end - gap:end])
                if copies:
                    z = late()
                    _wait([c(z) for c in copies])

            main = plain_list() + sum((strassen(1, order=order) for order in (
                (0,), (6,), (2,), (1, 4, 5, 3))), []) + strassen(2)
            dq, dv = right2_list(0, 8, KW, ORDER[:3] + ORDER[5:6]), right2_list(2, 8, KW, (0, 6, 2, 1, 4, 5, 3))
            wo = lambda n: wo_list(n) + wo_out_list(8 * n)
            do = lambda n: right2_list(3, 16, KW, start=8 * n)
            w_copy(0, 0, 2).wait()
            _run(perm_list(0, (0,)))
            memo["clock"] = pltpu.bitcast(ld("w0", 1 * KW + 120, z=3), F32)
            x0_copy(0, late()).wait()
            d, gap = 0, 18

            def permute(tasks, side, early=None):
                both = lambda a, b: _merge(a, b) if b else a
                if early:
                    phase(memo["done"] + 46, both(tasks[:16], early))
                    tasks = tasks[16:]
                phase(memo["done"] + 8 * len(tasks) // 3, both(tasks, side))
                phase(memo["done"] + gap, [])
            xp, rq, rk, rv = xprep_list(xa), right_list(0), right_list(1, range(4)), right_list(2, range(4))
            phase(64, [], P(w_copy, 0, 1, 2))
            permute(perm_list(0, (1,)), [])
            phase(150, [], P(x0_copy, 1))
            phase(190 + d, xp[:24], P(w_copy, 1, 0, 2))
            permute(perm_list(1, (0,)), xp[24:48])
            phase(258 + d, xp[48:56], P(w_copy, 1, 1, 2))
            permute(perm_list(1, (1,)), xp[56:])
            phase(380, rq[:44], P(w_copy, 2, 0, 1))
            permute(perm_list(2), rq[44:] + dq[:40])
            phase(506, right_list(1, (4,))[:22], P(w_copy, 3, 0, 1))
            permute(perm_list(3, ts=(4, 5, 0, 1, 6, 2, 7, 3)), dq[40:], right_list(1, (4,))[22:])
            phase(630, rk[:11], P(w_copy, 4, 0, 1))
            permute(perm_list(4), rk[11:])
            phase(752, dv[:22], P(w_copy, 5, 0, 1))
            permute(perm_list(5), dv[22:64], right_list(2, (4,)))
            phase(880, rv[:16], P(w_copy, 6, 0, 1))
            _start(sum((in_copies(n, late) for n in range(NS) for late in range(2)), []))
            phase(992, _zip(wo(0), rv[16:] + dv[64:64 + 32]))
            phase(992 + 6, [], P(w_copy, 7, 0, 1))
            phase(memo["done"] + 0, [])
            rest = dv[64 + 32:] + do(0) + do(1)
            phase(1058, _zip(wo(1), rest[:30]))
            logits, a, b = qk_list(0, E0), 64, 24
            phase(len(main) - 4, _zip(rest[30:-a], logits[:-34])
                  + _zip(rest[-a:-b], [(5, f) for _, f in logits[-34:]]) + rest[-b:])
            phase(len(main), [], table)
            return

        views.update(pr=shifted("p", j * E, NS * E), vr=shifted("v", j * E, NS * E))
        if last:
            n = E0 // 4
            _run(pv_list(n // 2, n) + oprep_list("xs", 0, n, (0, 1)))
            main = strassen(3, "xs", 0, n, (0,)) + strassen(3, "xs", 0, n, (1,))
            _weave(main[:24], pv_list(0, n // 2) + oprep_list("xu", 0, n, range(2, 7)))
            main = main[24:] + strassen(3, "xu", 0, n, (2, 4, 5, 3, 6))
            g, h = 16, 40
            _weave(main[:-g], pv_list(n, 2 * n) + oprep_list("xt", 2 * n, n))
            _weave(main[-g:], pv_list(2 * n, 4 * n)[:h])
            main = [] + strassen(3, "xt", 2 * n, n) + strassen2(3, 7, 4 * n, 2 * n)
            pre = oprep2_list(4 * n, 2 * n)
            _weave(main[:96], pv_list(2 * n, 4 * n)[h:] + pre[:8])
            _weave(main[96:166], pre[8:])
            _run(main[166:])
            return

        for name in "vp":
            views[name] = shifted(name, E0 + j * E, E0 + (NS - 1) * E)
        head, x = strassen(1) + strassen2(0, 4), xa.at[rows(j)]
        h0, h1, h2, h3 = 66, 416, 528, 20
        for u in range(4):
            _weave(dft_list(0, "hf", 4 * u), a1_list(0, 12 * u // 4, 12 * (u + 1) // 4))
        extra = _split(xprep_list(x), 4, 6)
        _weave(dft_list(0, "xf", 0), a1_list(0, 12, 13))
        _weave(dft_list(0, "xf", 4), _merge(a1_list(0, 13, 16), extra[0]))
        _weave(dft_list(0, "xf", 8) + dft_list(0, "xf", 12)[:4], extra[1])
        _run(dft_list(0, "xf", 12)[4:])
        _weave(head[:h0], xprep2_list(x))
        conv, cut = a3_list(0), 24 * 42
        _weave(head[h0:h1 - 10], conv[:cut] + [(0, lambda: _wait(in_copies(j, 1, late())))] + conv[cut:])
        _run(head[h1 - 10:h1])
        mix = _split(pv_list(0, E), 10, 40)
        for u in range(4):
            _run(idft_list(0, 4 * u))
            _weave(dft_list(1, "hf", 4 * u), a1_list(1, 3 * u, 3 * u + 3))
        oa_copy(2 * j).start()
        _weave(dft_list(1, "xf", 0), a1_list(1, 12, 16))
        _weave(dft_list(1, "xf", 4, 8, 12), mix[0])
        pre = _split(oprep2_list(), 4, 3)
        planes, g0 = _split(a3_list(1), *[1] * 48), 16
        _weave(head[h1:h2], mix[1])
        side = pre[0]
        for n, part in enumerate(_split(pre[1], *[1] * g0)):
            side = side + planes[n] + part
        tail = strassen2(2, 7)
        _weave(head[h2:] + strassen2(3) + tail[:h3], side + sum(planes[g0:], []))
        back, cutp = idft_list(1, 0, 4, 8, 12), 294
        tail = tail[:cutp] + back + tail[cutp:]
        _weave(tail[h3:len(tail) - 16], qk_list(0, E))
        _run(tail[len(tail) - 16:])
        oa_copy(2 * j + 1).start()

    def loop(j, carry):
        _wait(in_copies(j, 0))
        step(j)
        return carry

    step(0, first=True)
    lax.fori_loop(0, NS, loop, 0)
    step(NS, last=True)
    for i, name in enumerate(("oa", "ob")):
        pltpu.make_async_copy(raw[name], raw[name], sem_out.at[i]).wait()


@jax.jit
def pallas_concat_heads__ssm_conv_h3__sliding_local_dilated__prompt_kernel(
    A_q, A_k, A_v, A_shift_k, A_ssm_k, A_ssm_D, B_x, B_wqkv, B_wo,
):
    hbm = pl.BlockSpec(memory_space=pl.ANY)
    out = pl.pallas_call(
        _kernel,
        in_specs=[hbm] * 10,
        out_specs=hbm,
        out_shape=jax.ShapeDtypeStruct((S, 2 * D), BF16),
        scratch_shapes=[
            pltpu.VMEM((NT, 128, S), BF16),
            pltpu.VMEM((S, D), BF16),
            pltpu.VMEM((8, D // 2, D), BF16),
            pltpu.VMEM((NT, 5, 8, 128), F32),
            pltpu.VMEM(_TABLE.shape, U32),
            pltpu.SemaphoreType.DMA((2 * NS + 13,)),
            pltpu.SemaphoreType.DMA((2,)),
        ] + [pltpu.VMEM((r * 4 // np.dtype(t).itemsize, 128), t) for t, r in _BUFS.values()]
        + [pltpu.VMEM((4, D), BF16), pltpu.VMEM((8, 128), BF16)],
        compiler_params=pltpu.CompilerParams(vmem_limit_bytes=124 * 1024 * 1024,
                                             disable_bounds_checks=True,
                                             disable_semaphore_checks=True, flags={"XLA_TPU_RESCHEDULE_DMA_DONES": True}),
        name="fused",
    )(A_q[0], A_k[0], A_v[0], A_shift_k.T, A_ssm_k,
      A_ssm_D.reshape(8, 128), B_x[0], B_wqkv, B_wo, _TABLE)
    return out[None]
```

```python
import functools

import jax
import jax.numpy as jnp
import numpy as np
from jax import lax
from jax.experimental import pallas as pl
import jax.experimental.pallas.tpu as pltpu


S = 2048
D = 1024
T = 128
NC = S // T
NT = D // 128
NS = 4
R0 = 512
R = (S - R0) // NS
E0, E, HS = R0 // 2, R // 2, S // 2
WIN, DH = 8, 32
LOG2E = float(np.log2(np.e))
PITCH = 33
WP = 33
KR, KL = HS + 16, E0 + 16
FP = 2 * T + 16
KW = D // 4
KA = S // 2 + 32

F32, BF16, U32 = jnp.float32, jnp.bfloat16, jnp.uint32
P = functools.partial
add, sub, mul = lax.add, lax.sub, lax.mul


def _pack_rows(m):
    b = m.astype(jnp.bfloat16).view(np.uint16).astype(np.uint32)
    return np.ascontiguousarray(b[0::2] | (b[1::2] << 16))


def _dft_table():
    th = 2.0 * np.pi * (np.arange(T) + 0.25) / T
    dft = lambda t: np.concatenate([np.cos(np.outer(th, t)), -np.sin(np.outer(th, t))], axis=0)
    paired = np.arange(T).reshape(-1, 8, 2).transpose(0, 2, 1).reshape(-1)
    ph = np.outer(np.arange(T // 2) + 0.5, th)
    mats = (dft(np.arange(T)), dft(paired - (T - 1) / 2), np.cos(ph) / T, np.sin(ph) / T)
    return np.concatenate([_pack_rows(m) for m in mats] + [np.zeros((32, T), np.uint32)], axis=0)


_TABLE = _dft_table()


def _lo(w):
    return pltpu.bitcast(lax.shift_left(w, np.uint32(16)), F32)


def _hi(w):
    return pltpu.bitcast(lax.bitwise_and(w, np.uint32(0xFFFF0000)), F32)


def _rows(first, second):
    return jnp.concatenate([first, second], axis=0)


def _tree(xs):
    while len(xs) > 1:
        xs = [add(xs[i], xs[i + 1]) if i + 1 < len(xs) else xs[i] for i in range(0, len(xs), 2)]
    return xs[0]


def _left(a11, a12, a21, a22):
    return [add(a21, a22), a22, add(a11, a12), a11, add(a11, a22), sub(a12, a22), sub(a21, a11)]


def _merge(main, side):
    if not main:
        return side
    total_m = sum(c for c, _ in main)
    total_s = sum(c for c, _ in side)
    done_m, done_s, i, out = 0, 0, 0, []
    for c, f in main:
        out.append((c * total_s, f))
        done_m += c
        while i < len(side) and (done_s + side[i][0]) * total_m <= done_m * total_s:
            done_s += side[i][0]
            out.append((side[i][0] * total_m, side[i][1]))
            i += 1
    assert i == len(side)
    return out


def _zip(main, side):
    cost = {id(f): c for c, f in main + side}
    return [(cost[id(f)], f) for _, f in _merge(main, side)]


def _run(tasks):
    for _, f in tasks:
        f()


def _weave(main, side):
    _run(_merge(main, side))


def _split(tasks, *weights):
    ends = np.cumsum((0,) + weights) * len(tasks) // sum(weights)
    return [tasks[a:b] for a, b in zip(ends[:-1], ends[1:])]


def _start(copies):
    for c in copies:
        c.start()


def _wait(copies):
    for c in copies:
        c.wait()


_BUFS = {n: (t, r) for t, group in (
    (BF16, dict(qa=NT * HS, ka=NT * KA, va=NT * HS, oa=NT * HS, ob=NT * HS,
                xs=14 * E0, xt=35 * E0 // 2, **{f"os{i}": 7 * E0 // 2 for i in range(7)},
                kv0=S // 8, kv1=S // 8, kv2=S // 8, kv3=S // 8, z=NC * T, w3=NT * KW, xu=14 * E0,
                **{f"ws{p}": 20 * KW for p in range(4)}, wt0=20 * KW, wt2=35 * KW, wt3=35 * KW)),
    (U32, dict(**{f"w{p}": 2 * NT * KW for p in range(3)}, **{f"t{u}": 34 * DH for u in range(4)}, wp0=4 * WP * DH, wp1=4 * WP * DH)),
    (F32, dict(hf=NC * FP, xf=NC * FP, up=8 * NC, k1=8 * NC, pi=8 * NC, zr=8 * NC, zi=8 * NC,
               even=2 * T, quad=8 * WIN, **{n + "1": 4 * E0 for n in "abcde"}, **{n + "2": E0 for n in "abcde"},
               q=NT * R0 + 32, k=2 * NT * KL, v=2 * NT * KR, p=WIN * S, o=NT * R0 + 32)),
) for n, r in group.items()}


def _kernel(q_hbm, k_hbm, v_hbm, sk_hbm, h_hbm, d_hbm, x_hbm, w_hbm, wo_hbm, tab_hbm, out_hbm,
            ha, xa, wraw, taps, tab, sem_in, sem_out, *raw):
    *raw, sk_ref, d_ref = raw
    raw = dict(zip(_BUFS, raw))
    bufs = {n: b.bitcast(U32) if _BUFS[n][0] == BF16 else b for n, b in raw.items()}

    spec = _BUFS
    consts = {}

    def at(start, size, stride=None):
        if isinstance(start, int):
            if start not in consts:
                consts[start] = add(np.int32(start), np.int32(0))
            start = consts[start]
        return pl.ds(start, size, stride)

    def ld(name, row, n=8, z=0):
        assert 0 <= row and row + n <= views[name][z].shape[0]
        return views[name][z][at(row, n), :]

    def st(name, row, val):
        assert 0 <= row and row + val.shape[0] <= views[name][3].shape[0]
        views[name][3][at(row, val.shape[0]), :] = val

    def st16(name, row, val):
        assert 0 <= row and 2 * row + val.shape[0] <= views[name][4].shape[0]
        views[name][4][at(2 * row, val.shape[0]), :] = val.astype(BF16)

    def window(name, row, n):
        return bufs[name].at[pl.ds(pl.multiple_of(row, 8), n), :]

    def window16(name, row, n):
        return raw[name].at[pl.ds(pl.multiple_of(2 * row, 16), 2 * n), :]

    def cols(a):
        return pl.ds(pl.multiple_of(a * 128, 128), 128)

    def rows(j):
        return pl.ds(pl.multiple_of(R0 + j * R, 128), R)

    def a_copies(a, sem):
        return [pltpu.make_async_copy(src, dst, sem) for src, dst in (
            (h_hbm.at[cols(a), :], ha.at[a]),
            (k_hbm.at[:, cols(a)], window16("ka", a * KA + 32, HS)),
            (v_hbm.at[:, cols(a)], window16("va", a * HS, HS)))]

    def in_copies(j, late, z=0):
        sem = sem_in.at[2 * j + late + z]
        if not late:
            return [pltpu.make_async_copy(x_hbm.at[rows(j), :], xa.at[rows(j), :], sem)] + a_copies(2 * j, sem)
        return a_copies(2 * j + 1, sem) + [
            pltpu.make_async_copy(q_hbm.at[:, cols(a)], window16("qa", a * HS, HS), sem)
            for a in (2 * j, 2 * j + 1)]

    def x0_copy(half, z=0):
        part = pl.ds(0, R0), pl.ds(half * D // 2, D // 2)
        return pltpu.make_async_copy(x_hbm.at[part], xa.at[part], sem_in.at[2 * NS + 10 + half + z])

    def w_copy(n, part=0, parts=1, z=0):
        size = D // 2 // parts
        span = pl.ds(n % 2 * D // 2 + part * size, size)
        src = w_hbm.at[span, pl.ds(n // 2 * D, D)] if n < 6 else wo_hbm.at[span, :]
        return pltpu.make_async_copy(src, wraw.at[n, pl.ds(part * size, size)],
                                     sem_in.at[2 * NS + (n + 2 if n > 1 else 2 * n + part) + z])

    def oa_copy(a):
        return pltpu.make_async_copy(window16("oa", a * HS, HS), out_hbm.at[:, cols(a)], sem_out.at[0])

    def ob_copy(t, row, n):
        return pltpu.make_async_copy(
            window16("ob", t * HS + row, n),
            out_hbm.at[pl.ds(pl.multiple_of(2 * row, 128), 2 * n), cols(NT + t)], sem_out.at[1])

    small = [pltpu.make_async_copy(a, b, sem_in.at[2 * NS + 12])
             for a, b in ((tab_hbm.at[pl.ds(5 * T // 2, 8)], tab.at[pl.ds(5 * T // 2, 8)]),
                          (sk_hbm, sk_ref), (d_hbm, d_ref))]
    full = pl.ds(0, 5 * T // 2)
    table = lambda z=0: pltpu.make_async_copy(tab_hbm.at[full], tab.at[full], sem_in.at[2 * NS + 9 + z])
    startup = lambda: [w_copy(0, 0, 2), x0_copy(0), w_copy(0, 1, 2), x0_copy(1), w_copy(1, 0, 2), w_copy(1, 1, 2)] + [
        w_copy(n) for n in range(2, 8)] + [table()]
    _start(small + startup())
    _wait(small)
    unit = pltpu.bitcast(tab[pl.ds(5 * T // 2, 8), :], jnp.int32)
    zs = [pl.multiple_of(unit[i, 0] * 8, 8) for i in range(3)]
    views = {n: [b.at[pl.ds(z, spec[n][1]), :] for z in zs] + [b, raw[n]] for n, b in bufs.items()}

    for a in range(NT):
        st("ka", a * KA + 24, jnp.zeros((8, 128), U32))
    for t in range(2 * NT):
        st("k", t * KL + 8, jnp.zeros((WIN, 128), F32))
    skf = sk_ref[...].astype(F32)
    df = d_ref[...].astype(F32)
    for t in range(NT):
        for i in range(4):
            taps[t, i] = jnp.broadcast_to(skf[i:i + 1, t * 128:(t + 1) * 128], (8, 128))
        taps[t, 4] = jnp.broadcast_to(df[t:t + 1, :], (8, 128))

    def step(j, first=False, last=False):
        memo = {}
        consts.clear()
        e = E0 if first else E
        never = tab[pl.ds(5 * T // 2, 8), :] != 0

        def once(key, fn):
            if key not in memo:
                memo[key] = fn()
            return memo[key]

        def fresh():
            memo["fresh"] = memo.get("fresh", 1) + 1
            return pl.multiple_of(zs[0] * memo["fresh"], 8)

        def pace(val):
            clock = memo.get("clock")
            if clock is None:
                return val
            if val.dtype != F32:
                clock = pltpu.bitcast(clock, val.dtype)
            return lax.select(never, clock, val)

        def paced(x):
            return jnp.concatenate([pace(x[:8]), x[8:]], axis=0)

        def late():
            return pltpu.bitcast(pace(jnp.zeros((8, 128), F32)), jnp.int32)[0, 0]

        def shifted(name, row, most):
            return [window(name, z + row, spec[name][1] - most) for z in zs + [0]]

        def perm_in(w, h, u, t):
            tt = paced(pltpu.bitcast(w[pl.ds(u * 256, 256), pl.ds(t * 128, 128)], U32)).T
            for hh in range(4):
                st(f"t{2 * h + u}", (4 * t + hh) * PITCH, tt[hh * DH:(hh + 1) * DH])

        def perm_out(p, h, u, t):
            g = jnp.concatenate(
                [bufs[f"t{2 * h + u}"][pl.ds(zs[0] + 4 * t + i, 32, stride=PITCH), :] for i in range(4)], axis=0)
            st(f"w{p}", (h * NT + t) * KW + u * 128, paced(g).T)

        def perm_list(n, us=(0, 1), ts=range(NT)):
            return ([(1, P(perm_in, wraw.at[n], n % 2, u, t)) for u in us for t in range(NT)]
                    + [(1, P(perm_out, n // 2, n % 2, u, t)) for t in ts for u in us])

        def wo_in(n, t, hh):
            w = pltpu.bitcast(wraw[6 + n, pl.ds(hh * DH, DH), pl.ds(t * 128, 128)], U32)
            st(f"wp{n}", (16 * t + hh) * WP, _rows(pace(w[:8]), pace(w[8:])))

        def wo_list(w):
            return [(9, P(wo_in, w, t, hh)) for t in range(NT) for hh in range(16)]

        LEFT = ((2, add, 3), (3,), (0, add, 1), (0,), (0, add, 3), (1, sub, 3), (2, sub, 0))
        RIGHT = ((0,), (2, sub, 0), (3,), (1, sub, 3), (0, add, 3), (2, add, 3), (0, add, 1))

        def wo_out(r, t, dh):
            b = [bufs[f"wp{r // 8}"][pl.ds(zs[dh % 2] + 16 * (t + n % 2 * 4) * WP + n // 2 * 8 + dh // 2, 16, stride=WP), :]
                 for n in range(4)]
            b = [(_lo, _hi)[dh % 2](w) for w in [paced(b[0])] + b[1:3] + [paced(b[3]) if 0 else b[3]]]
            for i, (b0, *rest) in enumerate(RIGHT):
                name, n = ("ws3", 4 * (i - 1 - (i > 2))) if rest else ("w3", i * 2)
                st16(name, (n + t) * KW + 16 * dh + r, rest[0](b[b0], b[rest[1]]) if rest else b[b0])

        def wo_out_list(r):
            return [(26, P(wo_out, r, t, dh)) for t in range(4) for dh in range(16)]

        def right2(p, r, i):
            u, m = divmod(r, KW // 2)
            w = [factor(p, i, u + c % 2 * 2, c // 2 * KW // 2 + m, 8, 1) for c in range(4)]
            w[0], w[3] = pace(w[0]), pace(w[3])
            b = [pltpu.bitcast(x, BF16).astype(F32) for x in w]
            for k in (1, 3, 4, 5, 6):
                st16(f"wt{p}", (5 * i + k - 1 - (k > 2)) * KW + r, RIGHT[k][1](b[RIGHT[k][0]], b[RIGHT[k][2]]))

        def right2_list(p, step, end=0, order=(0, 2, 1, 4, 5, 3, 6), start=0):
            return [(25, P(right2, p, r, i)) for i in order for r in range(start, end, step)]

        def right(p, which, t, r):
            b = [ld(f"w{p}", (h * NT + t + 4 * u) * KW + r, 16, 2 * (which == (4,))) for h in range(2) for u in range(2)]
            mask = 1 if which == (4,) else 9 if p else 9
            b = [_rows(pace(x[:8]), pace(x[8:])) if mask >> c & 1 else x for c, x in enumerate(b)]
            b11, b12, b21, b22 = (pltpu.bitcast(x, BF16).astype(F32) for x in b)
            for i, val in enumerate((sub(b21, b11), sub(b12, b22), add(b11, b22),
                                     add(b21, b22), add(b11, b12))):
                if i in which:
                    st16(f"ws{p}", (4 * i + t) * KW + r, val)

        def right_list(p, which=range(5)):
            return [(18 + 6 * len(which), P(right, p, which, t, r)) for t in range(4) for r in range(0, KW, 16)]

        def ld_kv(c, row, n, z=0):
            return ld(f"kv{c // 4}", c % 4 * (T // 2) + row, n, z)

        def a1(i, r):
            a = once(("a", i), lambda: 2 * j + i)
            w0, w1, w2, w3 = once(("taps", i), lambda: [taps[a, u] for u in range(4)])
            k32 = once(("ka", i), lambda: window("ka", a * KA, KA))
            v32 = once(("va", i), lambda: window("va", a * (S // 2), S // 2))
            c0, c1, c2 = (k32[at(8 * r + 32 - u, 8), :] for u in range(3))
            vv = v32[at(8 * r, 8), :]
            e0, o0, e1, o1, o2 = _lo(c0), _hi(c0), _lo(c1), _hi(c1), _hi(c2)
            ke = _tree([mul(e0, w0), mul(o1, w1), mul(e1, w2), mul(o2, w3)])
            ko = _tree([mul(o0, w0), mul(e0, w1), mul(o1, w2), mul(e1, w3)])
            st16(f"kv{r // 32}", 8 * (r % 32), _rows(mul(ke, _lo(vv)), pace(mul(ko, _hi(vv)))))

        def a1_list(i, c0, c1):
            return [(24, P(a1, i, r)) for r in range(8 * c0, 8 * c1)]

        def freq(c, im, m):
            return c * FP + im * (T + 8) + m

        def dft(i, name, c0, m):
            def mm():
                f = pltpu.bitcast(tab[pl.ds(fresh() + T * (name == "xf"), T), :], BF16)
                if name == "hf":
                    a = once(("a", i), lambda: 2 * j + i)
                    rhs = jnp.concatenate(
                        [ha[a, :, pl.ds(c * T, T)] for c in range(c0, c0 + 4)], axis=0)
                    return lax.dot_general(f, rhs, (((1,), (1,)), ((), ())),
                                           preferred_element_type=F32)
                rhs = jnp.concatenate(
                    [pltpu.bitcast(ld_kv(c, 0, T // 2, i % 2), BF16) for c in range(c0, c0 + 4)], axis=1)
                return jnp.dot(f, rhs, preferred_element_type=F32)
            res = once((name, i, c0), mm)
            for u in range(4):
                val = res[m:m + 16, u * 128:(u + 1) * 128]
                if name == "hf" and c0 + u == 0 and m < T:
                    val = add(val, once(("dd", i), lambda: _rows(*[taps[memo["a", i], 4]] * 2)))
                st(name, freq(c0 + u, m // T, m % T), val)
            memo["clock"] = res[m + 8:m + 8 + 8, 0:0 + 128]

        def dft_list(i, name, *c0s):
            return [(16, P(dft, i, name, c0, m)) for c0 in c0s for m in range(0, 2 * T, 16)]

        def a3(i, g, plane, upper, n):
            def opnd(name, c):
                re = lambda: ld(name, freq(c, 0, 8 * g), z=plane)
                im = lambda: ld(name, freq(c, 1, 8 * g), z=plane)
                if name == "xf":
                    val = add(re(), im()) if plane == 0 else re() if plane == 1 else im()
                    return pace(val) if c >= 8 and c % 1 == 0 else val
                val = re() if plane == 0 else (sub, add)[plane - 1](im(), re())
                return pace(val) if c % 4 == 0 else val
            get = lambda name, c: once((name, i, g, plane, c), P(opnd, name, c))
            done = pace if n % 4 == 4 - 1 else lambda v: v
            cs = range(8, n + 1) if upper else range(min(n, 7) + 1)
            terms = [mul(get("xf", n - c), get("hf", c)) for c in cs]
            if upper:
                st("up", 8 * n, done(_tree(terms)))
                return
            if n >= 8:
                terms.append(ld("up", 8 * n))
            if plane == 0:
                st("k1", 8 * n, done(_tree(terms)))
            elif plane == 1:
                st("pi", 8 * n, done(_tree(terms + [ld("k1", 8 * n)])))
            else:
                pr = sub(ld("k1", 8 * n, z=1), _tree(terms))
                pi = ld("pi", 8 * n)
                zr, zi = pr, pi
                if n > 0:
                    qr, qi = memo["prev"]
                    zr, zi = sub(pr, qi), add(pi, qr)
                memo["prev"] = (pr, pi)
                if g % 2 == 0:
                    st("zr", 8 * n, done(zr))
                    st("zi", 8 * n, zi)
                else:
                    st16("z", n * T + 4 * (g - 1), _rows(ld("zr", 8 * n), done(zr)))
                    st16("z", n * T + T // 2 + 4 * (g - 1), _rows(ld("zi", 8 * n), zi))

        def a3_list(i):
            out = []
            for g in range(T // 8):
                for plane in range(3):
                    out += [(2 * (n - 8) + 4, P(a3, i, g, plane, True, n)) for n in range(8, NC)]
                    out += [(2 * min(n, 7) + 4 + 2 * (plane == 2), P(a3, i, g, plane, False, n))
                            for n in range(NC)]
            return out

        def idft(i, c0, odd, m):
            def mm():
                rhs = jnp.concatenate([pltpu.bitcast(ld("z", c * T + odd * T // 2, T // 2, i), BF16)
                                       for c in range(c0, c0 + 4)], axis=1)
                f = tab[pl.ds(fresh() + 2 * T + odd * T // 4, T // 4), :]
                return jnp.dot(pltpu.bitcast(f, BF16), rhs, preferred_element_type=F32)
            y = once(("y", i, c0, odd), mm)
            a = once(("a", i), lambda: 2 * j + i)
            q16 = once(("qa", i), lambda: window16("qa", a * (S // 2), S // 2))
            o16 = once(("oa", i), lambda: window16("oa", a * (S // 2), S // 2))
            flip = lambda w: jnp.take_along_axis(
                w, 7 - lax.broadcasted_iota(jnp.int32, (8, 128), 0), axis=0, mode="promise_in_bounds")
            for u in range(4):
                val = y[m:m + 16, u * 128:(u + 1) * 128]
                if not odd:
                    st("even", u * T // 2 + m, val)
                    continue
                even, mid = ld("even", u * T // 2 + m, 16), (c0 + u) * T + T // 2
                low = add(even, val)
                for row, out in ((mid + m, sub(even, val)),
                                 (mid - 16 - m, _rows(flip(low[8:]), flip(low[:8])))):
                    o16[at(row, 16), :] = mul(q16[at(row, 16), :].astype(F32), out).astype(BF16)
            memo["clock"] = y[m + 8:m + 16, 384:]

        def idft_list(i, *c0s):
            return [(16, P(idft, i, c0, odd, m)) for c0 in c0s
                    for odd in range(2) for m in range(0, T // 2, 16)]

        def xprep(x, u, r):
            halves = []
            for m in (r, r + 8):
                a, b = (pltpu.bitcast(x[pl.ds(2 * m, 16), pl.ds(t * 128, 128)], U32)
                        for t in (u, u + 4))
                a = pace(a)
                a11, a12, a21, a22 = _lo(a), _lo(b), _hi(a), _hi(b)
                halves.append(_left(a11, a12, a21, a22))
            for i, pair in enumerate(zip(*halves)):
                st16("xs", ((4 * i + u) * E0 + r) // 2, jnp.concatenate(pair, axis=0))

        def xprep_list(x):
            return [(27, P(xprep, x, u, r)) for r in range(0, e, 16) for u in range(4)]

        def tiles(name, rows, n):
            view = views[name][3].at[pl.ds(fresh(), spec[name][1]), :]
            return jnp.concatenate(
                [pltpu.bitcast(view[at(row, n // 2), :], BF16) for row in rows], axis=1)

        def emit(p, r0, n, par, t, m, val, end):
            if p == 0:
                st("q", (par * NT + t) * E0 + m, val)
            elif p == 3:
                base = once("row", lambda: j * E)
                o16 = once("ob", lambda: window16("ob", base, (NT - 1) * HS + (E0 if last else E)))
                o16[at(t * S + r0 + par * n + m, 16), :] = val.astype(BF16)
                if m + 16 == end and par == t // 4:
                    ob_copy(t, base + r0 // 2, n).start()
            elif p == 2:
                st("v", (par * NT + t) * KR + 16 + m, val)
            else:
                row = (par * NT + t + 1) * KL - e
                if m == 0 and not first:
                    st("k", row - WIN, ld("k", row + e - WIN, z=3))
                st("k", row + m, val)
            if m == 0 and first and p == 2 and par == 0:
                for other in range(2):
                    st("v", (other * NT + t) * KR + 8, jnp.broadcast_to(val[0:1], (WIN, 128)))

        def plain(n, t, m):
            def mm():
                w = [ld("w0", (n // 2 * NT + t + u) * KW + n % 2 * KW // 2, KW // 2, 3) for u in range(2)]
                return jnp.dot(xa[pl.ds(0, R0), pl.ds(n * D // 4, D // 4)],
                               jnp.concatenate([pltpu.bitcast(v, BF16) for v in w], axis=1),
                               preferred_element_type=F32)
            res = once(("plain", n, t), mm)
            memo["clock"] = res[m + 0:m + 0 + 8, :128]
            for u in range(2):
                val = res[m:m + 16, u * 128:(u + 1) * 128]
                if n:
                    val = add(val, ld("qo"[n % 2], (t + u) * R0 + m, 16))
                st("oq"[n % 2], (t + u) * R0 + m, val)

        def plain_list():
            return [(16, P(plain, n, t, m)) for n in range(4) for t in range(0, NT, 2) for m in range(0, R0, 16)]

        def combine(level, i, row, res, out, early=False):
            get = lambda name, z=0: ld(name + level, row, 16, z)
            if early == 6 and i == 6:
                st("e" + level, row, res)
            elif early == 6 and i == 3:
                out(0, 1, add(get("b", 1), res))
                out(1, 1, add(add(get("e"), get("c", 1)), sub(res, get("a", 1))))
            elif i % 2 == 0 and i < 6:
                st("abc"[i // 2] + level, row, res)
            elif i == 1:
                st("d" + level, row, res if early == 1 else sub(res, get("b")))
                out(1, 0, add(get("a"), res))
            elif i == 3:
                st("e" + level, row, sub(res, get("a", 1)))
                out(0, 1, add(get("b", 1), res))
            else:
                part = add(get("de"[i - 5]), get("c", i - 5))
                out(i - 5, i - 5, add(sub(part, get("b")) if early == 1 and i == 5 else part, res))

        def factor(p, i, t, r=0, n=KW, z=3):
            if i in (0, 2):
                return ld(f"w{p}", (t + (4 if p == 3 else NT + 4) * i // 2) * KW + r, n, z)
            return ld(f"ws{p}", (4 * (i - 1 - (i > 2)) + t) * KW + r, n, z)

        def product(p, src, r0, n, t, i, m):
            res = once(("product", p, r0, t, i), lambda: jnp.dot(
                tiles(src, [(4 * i + u) * E0 // 2 for u in range(4)], n),
                pltpu.bitcast(factor(p, i, t), BF16), preferred_element_type=F32))
            memo["clock"] = res[m + 0:m + 0 + 8]
            combine("1", i, t * E0 + m, res[m:m + 16],
                    lambda par, h, val: emit(p, r0, n, par, t + 4 * h, m, val, n), 6 if first and p == 1 else last and not r0)

        ORDER = (0, 2, 1, 4, 5, 3, 6)

        def strassen(p, src="xs", r0=0, n=e, order=ORDER):
            return [(16, P(product, p, src, r0, n, t, i, m))
                    for t in range(4) for i in order for m in range(0, n, 16)]

        def product2(p, r0, n, i, k, m):
            def mm():
                if p == 3:
                    name, row, step = f"os{i}", k * E0 // 2, E0 // 4
                elif k in (1, 3):
                    name, row, step = "xs", 2 * i * E0 + (k == 1) * (E0 + n // 4), E0 // 2
                else:
                    name, row, step = "xt", (5 * i + (0, 2, 4, 5, 6).index(k)) * E0 // 2, E0 // 4
                if k in (0, 2):
                    w = [factor(p, i, k + u, k * KW // 4, KW // 2) for u in range(2)]
                else:
                    w = [ld(f"wt{p}", ((5 * i + k - 1 - (k > 2)) * 2 + u) * KW // 2, KW // 2, 3) for u in range(2)]
                return jnp.dot(tiles(name, (row, row + step), n // 2),
                               jnp.concatenate([pltpu.bitcast(v, BF16) for v in w], axis=1),
                               preferred_element_type=F32)
            res = once(("product2", p, i, k), mm)
            memo["clock"] = res[m + 8:m + 8 + 8, 0:0 + 128]

            def out(u, r2, c2, val):
                t, row = 2 * c2 + u, r2 * n // 2 + m
                combine("1", i, t * E0 + row, val, lambda par, h, v: emit(
                    p, r0, n, par, t + 4 * h, row, v, (1 + c2) * n // 2))
            for u in range(2):
                combine("2", k, u * E0 // 2 + m, res[m:m + 16, u * 128:(u + 1) * 128], P(out, u))

        def strassen2(p, deep=7, r0=0, n=e):
            return [task for i in ORDER for task in (
                [(16, P(product2, p, r0, n, i, k, m)) for k in ORDER for m in range(0, n // 2, 16)]
                if i < deep else strassen(p, order=(i,)))]

        def xprep2(x, u, r, i):
            def blk(b):
                w = once(("x", u, r, b % 2), lambda: [pltpu.bitcast(
                    x[pl.ds(c // 2 * e + 2 * r, 32), pl.ds((u + c % 2 * 2 + b % 2 * 4) * 128, 128)], U32)
                    for c in range(4)])
                return [(_lo, _hi)[b // 2](v) for v in w]
            b0, *rest = LEFT[i]
            a = list(once(("left", u, r, b0), P(blk, b0)))
            a[0], a[3] = paced(a[0]), paced(a[3])
            if rest:
                a = list(map(rest[0], a, once(("left", u, r, rest[1]), P(blk, rest[1]))))
            for n, k in enumerate((0, 2, 4, 5, 6)):
                st16("xt", ((5 * i + n) * 2 + u) * E0 // 4 + r // 2, LEFT[k][1](a[LEFT[k][0]], a[LEFT[k][2]]))

        def xprep2_list(x):
            return [(c, P(xprep2, x, u, r, i)) for r in range(0, e // 2, 16) for u in range(2)
                    for i, c in ((1, 25), (0, 33), (6, 33), (4, 25), (3, 17), (5, 33), (2, 25))]

        def oprep2(r0, n, i, u, r):
            view = once(("oprep", i), lambda: window("o", fresh(), NT * R0))
            blk = lambda b, c: view[at(
                (u + 2 * (c % 2) + 4 * (b % 2)) * R0 + r0 + b // 2 * n + c // 2 * n // 2 + r, 16), :]
            b0, *rest = LEFT[i]
            a = [blk(b0, c) for c in range(4)]
            a = [paced(x) if 9 >> c & 1 else x for c, x in enumerate(a)]
            if rest:
                a = [rest[0](x, blk(rest[1], c)) for c, x in enumerate(a)]
            for k, val in enumerate(_left(*a)):
                st16(f"os{i}", (k * 2 + u) * E0 // 4 + r // 2, val)

        def oprep2_list(r0=0, n=e):
            return [(19 + 8 * (len(LEFT[i]) > 1), P(oprep2, r0, n, i, u, r))
                    for i in ORDER for r in range(0, n // 2, 16) for u in range(2)]

        def qk(r, w):
            par, m = r
            query = lambda t: (bufs["q"][at(t * R0 + 2 * m + par, 8, stride=2), :] if first
                               else ld("q", (par * NT + t) * E0 + m))
            scale = once(("scale", r), lambda: pace(jnp.full((8, 128), DH ** -0.5 * LOG2E, F32)))
            if r == (0, 8) and not first and 1:
                scale = once("flush", lambda: lax.select(never, pltpu.bitcast(ld("z", 0, z=2), F32), scale))
            if first and m % 32 == 8 and 1:
                scale = once(("flush", r), lambda: lax.select(never, window("v", fresh(), 8)[...], scale))
            qv = once(("qv", r), lambda: [mul(query(t), scale) for t in range(NT)])
            s = (pace if m // 8 % 2 else lambda v: v)(_tree([mul(qv[t], ld("k", (par * NT + t + 1) * KL - e + m - w)) for t in range(NT)]))
            def fold(mask, a, b, shift):
                return add(lax.select(mask, a, b), pltpu.roll(lax.select(mask, b, a), shift, 1))
            g = m // 8 % 4
            if g % 2:
                s = fold(thirds[g // 2], memo.pop(("s", 0, w)), s, 64)
            if g == 3:
                s = fold(thirds[2], memo["s", 1, w], s, 32)
                if first and m == 24 and w:
                    early = lax.broadcasted_iota(jnp.int32, (8, 128), 0) < w
                    s = jnp.where(early & (quarter == 1), -1e9 * LOG2E, s)
            memo[("lg", r, w) if g == 3 else ("s", g % 2, w)] = s

        quarter = lax.shift_right_logical(lax.broadcasted_iota(jnp.int32, (8, 128), 1), 5)
        thirds = quarter < 2, (quarter == 1) | (quarter == 2), (quarter & 1) == 1

        def expo(r):
            lg = [memo["lg", r, w] for w in range(WIN)]
            m = pace(functools.reduce(lax.max, lg))
            memo["e", r] = [lax.exp2(sub(s, m)) for s in lg]

        def norm(r):
            total = pace(_tree(memo["e", r]))
            memo["inv", r] = total, pl.reciprocal(total, approx=True)

        def probs(r):
            total, inv = memo["inv", r]
            inv = pace(inv)
            inv = mul(inv, sub(np.float32(2), mul(total, inv)))
            for w, x in enumerate(memo["e", r]):
                st("quad", 8 * w, mul(x, inv))

        def spread(r, g):
            row = lambda w, g: (2 * w + r[0]) * HS + r[1] - 24 + 8 * g
            for w in (2 * g, 2 * g + 1):
                x = pace(ld("quad", 8 * w))
                y = pltpu.roll(x, 64, 1)
                for a, (even, odd) in ((lax.select(thirds[0], x, y), (3, 0)), (lax.select(thirds[0], y, x), (2, 1))):
                    b = pltpu.roll(a, 32, 1)
                    st("p", row(w, odd), lax.select(thirds[2], a, b))
                    st("p", row(w, even), lax.select(thirds[2], b, a))

        def qk_list(m0, m1, pars=(0, 1)):
            rs = [(par, m) for par in pars for m in range(m0, m1, 8)]
            q0, q1, q2 = 20, 3, 2
            stages = [(expo, q0), (norm, q0 + q1), (probs, q0 + 2 * q1)] + [
                (lambda r, g=g: spread(r, g), q0 + 2 * q1 + q2 * (g + 1)) for g in range(4)]
            out = [[P(qk, rs[n + u], w)] for n in range(0, len(rs), 2) for w in range(WIN) for u in range(2)] + [[] for _ in range(stages[-1][1])]
            for n in range(3, len(rs), 4):
                for f, lag in stages:
                    out[WIN * n + WIN - 1 + lag].append(P(f, rs[n]))
            return [(22, P(_run, [(0, f) for f in tasks])) for tasks in out]

        def pv(par, m, t):
            p = once(("pv", par, m), lambda: [
                (pace if w % 4 == 0 else lambda v: v)(ld("pr", (2 * w + par) * HS + m))
                for w in range(WIN)])
            row = (par * NT + t) * KR + 16 + m
            bufs["o"][at(t * R0 + 2 * m + par, 8, stride=2), :] = (pace if t % 1 == 0 else lambda v: v)(
                _tree([mul(p[w], ld("vr", row - w)) for w in range(WIN)]))

        def pv_list(m0, m1, ts=range(NT)):
            return [(16, P(pv, par, m, t)) for par in range(2) for m in range(m0, m1, 8) for t in ts]

        def oprep(name, r0, n, which, u, r):
            a = lambda b: once(("o", name, r0, u, r, b), lambda: ld(
                "o", (u + b % 2 * 4) * R0 + r0 + b // 2 * n + r, 16, 1 + (name == "xu")))
            memo["o", name, r0, u, r, 3] = paced(a(3))
            for i in which:
                b0, *rest = LEFT[i]
                st16(name, ((4 * i + u) * E0 + r) // 2, rest[0](a(b0), a(rest[1])) if rest else a(b0))

        def oprep_list(name, r0, n, which=range(7)):
            return [(18, P(oprep, name, r0, n, which, u, r)) for r in range(0, n, 16) for u in range(4)]

        if first:

            def phase(end, side, *copies):
                start, gap = memo.get("done", 0), 0 * bool(copies)
                memo["done"] = end
                _weave(main[start:end - gap], side)
                _run(main[end - gap:end])
                if copies:
                    z = late()
                    _wait([c(z) for c in copies])

            main = plain_list() + sum((strassen(1, order=order) for order in (
                (0,), (6,), (2,), (1, 4, 5, 3))), []) + strassen(2)
            dq, dv = right2_list(0, 8, KW, ORDER[:3] + ORDER[5:6]), right2_list(2, 8, KW, (0, 6, 2, 1, 4, 5, 3))
            wo = lambda n: wo_list(n) + wo_out_list(8 * n)
            do = lambda n: right2_list(3, 16, KW, start=8 * n)
            w_copy(0, 0, 2).wait()
            _run(perm_list(0, (0,)))
            memo["clock"] = pltpu.bitcast(ld("w0", 1 * KW + 120, z=3), F32)
            x0_copy(0, late()).wait()
            d, gap = 0, 18

            def permute(tasks, side, early=None):
                both = lambda a, b: _merge(a, b) if b else a
                if early:
                    phase(memo["done"] + 46, both(tasks[:16], early))
                    tasks = tasks[16:]
                phase(memo["done"] + 8 * len(tasks) // 3, both(tasks, side))
                phase(memo["done"] + gap, [])
            xp, rq, rk, rv = xprep_list(xa), right_list(0), right_list(1, range(4)), right_list(2, range(4))
            phase(64, [], P(w_copy, 0, 1, 2))
            permute(perm_list(0, (1,)), [])
            phase(150, [], P(x0_copy, 1))
            phase(190 + d, xp[:24], P(w_copy, 1, 0, 2))
            permute(perm_list(1, (0,)), xp[24:48])
            phase(258 + d, xp[48:56], P(w_copy, 1, 1, 2))
            permute(perm_list(1, (1,)), xp[56:])
            phase(380, rq[:44], P(w_copy, 2, 0, 1))
            permute(perm_list(2), rq[44:] + dq[:40])
            phase(506, right_list(1, (4,))[:22], P(w_copy, 3, 0, 1))
            permute(perm_list(3, ts=(4, 5, 0, 1, 6, 2, 7, 3)), dq[40:], right_list(1, (4,))[22:])
            phase(630, rk[:11], P(w_copy, 4, 0, 1))
            permute(perm_list(4), rk[11:])
            phase(752, dv[:22], P(w_copy, 5, 0, 1))
            permute(perm_list(5), dv[22:64], right_list(2, (4,)))
            phase(880, rv[:16], P(w_copy, 6, 0, 1))
            _start(sum((in_copies(n, late) for n in range(NS) for late in range(2)), []))
            phase(992, _zip(wo(0), rv[16:] + dv[64:64 + 32]))
            phase(992 + 6, [], P(w_copy, 7, 0, 1))
            phase(memo["done"] + 0, [])
            rest = dv[64 + 32:] + do(0) + do(1)
            phase(1058, _zip(wo(1), rest[:30]))
            logits, a, b = qk_list(0, E0), 64, 24
            phase(len(main) - 4, _zip(rest[30:-a], logits[:-34])
                  + _zip(rest[-a:-b], [(5, f) for _, f in logits[-34:]]) + rest[-b:])
            phase(len(main), [], table)
            return

        views.update(pr=shifted("p", j * E, NS * E), vr=shifted("v", j * E, NS * E))
        if last:
            n = E0 // 4
            _run(pv_list(n // 2, n) + oprep_list("xs", 0, n, (0, 1)))
            main = strassen(3, "xs", 0, n, (0,)) + strassen(3, "xs", 0, n, (1,))
            _weave(main[:24], pv_list(0, n // 2) + oprep_list("xu", 0, n, range(2, 7)))
            main = main[24:] + strassen(3, "xu", 0, n, (2, 4, 5, 3, 6))
            g, h = 16, 40
            _weave(main[:-g], pv_list(n, 2 * n) + oprep_list("xt", 2 * n, n))
            _weave(main[-g:], pv_list(2 * n, 4 * n)[:h])
            main = [] + strassen(3, "xt", 2 * n, n) + strassen2(3, 7, 4 * n, 2 * n)
            pre = oprep2_list(4 * n, 2 * n)
            _weave(main[:96], pv_list(2 * n, 4 * n)[h:] + pre[:8])
            _weave(main[96:166], pre[8:])
            _run(main[166:])
            return

        for name in "vp":
            views[name] = shifted(name, E0 + j * E, E0 + (NS - 1) * E)
        head, x = strassen(1) + strassen2(0, 4), xa.at[rows(j)]
        h0, h1, h2, h3 = 66, 416, 528, 20
        for u in range(4):
            _weave(dft_list(0, "hf", 4 * u), a1_list(0, 12 * u // 4, 12 * (u + 1) // 4))
        extra = _split(xprep_list(x), 4, 6)
        _weave(dft_list(0, "xf", 0), a1_list(0, 12, 13))
        _weave(dft_list(0, "xf", 4), _merge(a1_list(0, 13, 16), extra[0]))
        _weave(dft_list(0, "xf", 8) + dft_list(0, "xf", 12)[:4], extra[1])
        _run(dft_list(0, "xf", 12)[4:])
        _weave(head[:h0], xprep2_list(x))
        conv, cut = a3_list(0), 24 * 42
        _weave(head[h0:h1 - 10], conv[:cut] + [(0, lambda: _wait(in_copies(j, 1, late())))] + conv[cut:])
        _run(head[h1 - 10:h1])
        mix = _split(pv_list(0, E), 10, 40)
        for u in range(4):
            _run(idft_list(0, 4 * u))
            _weave(dft_list(1, "hf", 4 * u), a1_list(1, 3 * u, 3 * u + 3))
        oa_copy(2 * j).start()
        _weave(dft_list(1, "xf", 0), a1_list(1, 12, 16))
        _weave(dft_list(1, "xf", 4, 8, 12), mix[0])
        pre = _split(oprep2_list(), 4, 3)
        planes, g0 = _split(a3_list(1), *[1] * 48), 16
        _weave(head[h1:h2], mix[1])
        side = pre[0]
        for n, part in enumerate(_split(pre[1], *[1] * g0)):
            side = side + planes[n] + part
        tail = strassen2(2, 7)
        _weave(head[h2:] + strassen2(3) + tail[:h3], side + sum(planes[g0:], []))
        back, cutp = idft_list(1, 0, 4, 8, 12), 294
        tail = tail[:cutp] + back + tail[cutp:]
        _weave(tail[h3:len(tail) - 16], qk_list(0, E))
        _run(tail[len(tail) - 16:])
        oa_copy(2 * j + 1).start()

    def loop(j, carry):
        _wait(in_copies(j, 0))
        step(j)
        return carry

    step(0, first=True)
    lax.fori_loop(0, NS, loop, 0)
    step(NS, last=True)
    for i, name in enumerate(("oa", "ob")):
        pltpu.make_async_copy(raw[name], raw[name], sem_out.at[i]).wait()


@jax.jit
def pallas_concat_heads__ssm_conv_h3__sliding_local_dilated__prompt_kernel(
    A_q, A_k, A_v, A_shift_k, A_ssm_k, A_ssm_D, B_x, B_wqkv, B_wo,
):
    hbm = pl.BlockSpec(memory_space=pl.ANY)
    out = pl.pallas_call(
        _kernel,
        in_specs=[hbm] * 10,
        out_specs=hbm,
        out_shape=jax.ShapeDtypeStruct((S, 2 * D), BF16),
        scratch_shapes=[
            pltpu.VMEM((NT, 128, S), BF16),
            pltpu.VMEM((S, D), BF16),
            pltpu.VMEM((8, D // 2, D), BF16),
            pltpu.VMEM((NT, 5, 8, 128), F32),
            pltpu.VMEM(_TABLE.shape, U32),
            pltpu.SemaphoreType.DMA((2 * NS + 13,)),
            pltpu.SemaphoreType.DMA((2,)),
        ] + [pltpu.VMEM((r * 4 // np.dtype(t).itemsize, 128), t) for t, r in _BUFS.values()]
        + [pltpu.VMEM((4, D), BF16), pltpu.VMEM((8, 128), BF16)],
        compiler_params=pltpu.CompilerParams(vmem_limit_bytes=124 * 1024 * 1024,
                                             disable_bounds_checks=True,
                                             disable_semaphore_checks=True, flags={"XLA_TPU_RESCHEDULE_DMA_DONES": True}),
        name="fused",
    )(A_q[0], A_k[0], A_v[0], A_shift_k.T, A_ssm_k,
      A_ssm_D.reshape(8, 128), B_x[0], B_wqkv, B_wo, _TABLE)
    return out[None]
```

```python
import functools

import jax
import jax.numpy as jnp
import numpy as np
from jax import lax
from jax.experimental import pallas as pl
import jax.experimental.pallas.tpu as pltpu

S = 2048
D = 1024
T = 128
NC = S // T
NT = D // 128
NS = 4
R0 = 512
R = (S - R0) // NS
E0, E, HS = R0 // 2, R // 2, S // 2
WIN, DH = 8, 32
LOG2E = float(np.log2(np.e))
PITCH = DH + 1
KL = E0 + 16
VL = HS + 16
FP = 2 * T + 16
KW = D // 4
KA = HS + 32
ZERO = 5 * T // 2

F32, BF16, U32 = jnp.float32, jnp.bfloat16, jnp.uint32
P = functools.partial
add, sub, mul = lax.add, lax.sub, lax.mul

LEFT = ((2, add, 3), (3,), (0, add, 1), (0,), (0, add, 3), (1, sub, 3), (2, sub, 0))
RIGHT = ((0,), (2, sub, 0), (3,), (1, sub, 3), (0, add, 3), (2, add, 3), (0, add, 1))
LEFT_SUMS, RIGHT_SUMS = (0, 2, 4, 5, 6), (1, 3, 4, 5, 6)
ORDER = (0, 2, 1, 4, 5, 3, 6)
DEEP_Q = 4


def _pack_rows(m):
    b = m.astype(jnp.bfloat16).view(np.uint16).astype(np.uint32)
    return np.ascontiguousarray(b[0::2] | (b[1::2] << 16))


def _dft_table():
    th = 2.0 * np.pi * (np.arange(T) + 0.25) / T
    dft = lambda t: np.concatenate([np.cos(np.outer(th, t)), -np.sin(np.outer(th, t))], axis=0)
    paired = np.arange(T).reshape(-1, 8, 2).transpose(0, 2, 1).reshape(-1)
    ph = np.outer(np.arange(T // 2) + 0.5, th)
    mats = (dft(np.arange(T)), dft(paired - (T - 1) / 2), np.cos(ph) / T, np.sin(ph) / T)
    return np.concatenate([_pack_rows(m) for m in mats] + [np.zeros((32, T), np.uint32)], axis=0)


_TABLE = _dft_table()


def _lo(w):
    return pltpu.bitcast(lax.shift_left(w, np.uint32(16)), F32)


def _hi(w):
    return pltpu.bitcast(lax.bitwise_and(w, np.uint32(0xFFFF0000)), F32)


def _rows(first, second):
    return jnp.concatenate([first, second], axis=0)


def _tree(xs):
    while len(xs) > 1:
        xs = [add(xs[i], xs[i + 1]) if i + 1 < len(xs) else xs[i] for i in range(0, len(xs), 2)]
    return xs[0]


def _factor(rule, block):
    return rule[1](block(rule[0]), block(rule[2])) if len(rule) > 1 else block(rule[0])


def _merge(main, side):
    if not main:
        return side
    total_m = sum(c for c, _ in main)
    total_s = sum(c for c, _ in side)
    done_m, done_s, i, out = 0, 0, 0, []
    for task in main:
        out.append(task)
        done_m += task[0]
        while i < len(side) and (done_s + side[i][0]) * total_m <= done_m * total_s:
            done_s += side[i][0]
            out.append(side[i])
            i += 1
    assert i == len(side)
    return out


def _run(tasks):
    for _, f in tasks:
        f()


def _weave(main, side):
    _run(_merge(main, side))


def _split(tasks, *weights):
    ends = np.cumsum((0,) + weights) * len(tasks) // sum(weights)
    return [tasks[a:b] for a, b in zip(ends[:-1], ends[1:])]


def _start(copies):
    for c in copies:
        c.start()


def _wait(copies):
    for c in copies:
        c.wait()


_BUFS = {n: (t, r) for t, group in (
    (BF16, dict(qa=NT * HS, ka=NT * KA, va=NT * HS, oa=NT * HS, ob=NT * HS,
                xs=14 * E0, xt=35 * E0 // 2, **{f"os{i}": 7 * E0 // 2 for i in range(7)},
                **{f"kv{u}": S // 8 for u in range(4)}, z=NC * T, w3=NT * KW, xu=14 * E0,
                **{f"ws{p}": 20 * KW for p in range(4)},
                wt0=5 * DEEP_Q * KW, wt2=35 * KW, wt3=35 * KW)),
    (U32, dict(**{f"w{p}": 2 * NT * KW for p in range(3)}, **{f"t{u}": 34 * DH for u in range(4)},
               wp0=(4 * PITCH + 1) * DH, wp1=(4 * PITCH + 1) * DH)),
    (F32, dict(hf=NC * FP, xf=NC * FP, up=8 * NC, k1=8 * NC, pi=8 * NC, zr=8 * NC, zi=8 * NC,
               even=2 * T, quad=8 * WIN,
               **{n + "1": 4 * E0 for n in "abcde"}, **{n + "2": E0 for n in "abcde"},
               q=NT * R0 + 32, k=2 * NT * KL, v=2 * NT * VL, p=WIN * S, o=NT * R0 + 32)),
) for n, r in group.items()}


def _kernel(q_hbm, k_hbm, v_hbm, sk_hbm, h_hbm, d_hbm, x_hbm, w_hbm, wo_hbm, tab_hbm, out_hbm,
            ha, xa, wraw, taps, tab, sem_in, sem_out, *raw):
    *raw, sk_ref, d_ref = raw
    raw = dict(zip(_BUFS, raw))
    bufs = {n: b.bitcast(U32) if _BUFS[n][0] == BF16 else b for n, b in raw.items()}
    consts = {}

    def at(start, size, stride=None):
        if start not in consts:
            consts[start] = add(np.int32(start), np.int32(0))
        return pl.ds(consts[start], size, stride)

    def ld(name, row, n=8, z=0):
        assert 0 <= row and row + n <= views[name][z].shape[0]
        return views[name][z][at(row, n), :]

    def st(name, row, val):
        assert 0 <= row and row + val.shape[0] <= views[name][3].shape[0]
        views[name][3][at(row, val.shape[0]), :] = val

    def st16(name, row, val):
        assert 0 <= row and 2 * row + val.shape[0] <= raw[name].shape[0]
        raw[name][at(2 * row, val.shape[0]), :] = val.astype(BF16)

    def window(name, row, n):
        return bufs[name].at[pl.ds(pl.multiple_of(row, 8), n), :]

    def window16(name, row, n):
        return raw[name].at[pl.ds(pl.multiple_of(2 * row, 16), 2 * n), :]

    def cols(a):
        return pl.ds(pl.multiple_of(a * 128, 128), 128)

    def rows(j):
        return pl.ds(pl.multiple_of(R0 + j * R, 128), R)

    def a_copies(a, sem):
        return [pltpu.make_async_copy(src, dst, sem) for src, dst in (
            (h_hbm.at[cols(a), :], ha.at[a]),
            (k_hbm.at[:, cols(a)], window16("ka", a * KA + 32, HS)),
            (v_hbm.at[:, cols(a)], window16("va", a * HS, HS)))]

    def in_copies(j, second, z=0):
        sem = sem_in.at[2 * j + second + z]
        if not second:
            return ([pltpu.make_async_copy(x_hbm.at[rows(j), :], xa.at[rows(j), :], sem)]
                    + a_copies(2 * j, sem))
        return a_copies(2 * j + 1, sem) + [
            pltpu.make_async_copy(q_hbm.at[:, cols(a)], window16("qa", a * HS, HS), sem)
            for a in (2 * j, 2 * j + 1)]

    def w_copy(n, part=0, parts=1, z=0):
        size = D // 2 // parts
        span = pl.ds(n % 2 * D // 2 + part * size, size)
        src = w_hbm.at[span, pl.ds(n // 2 * D, D)] if n < 6 else wo_hbm.at[span, :]
        return pltpu.make_async_copy(src, wraw.at[n, pl.ds(part * size, size)],
                                     sem_in.at[2 * NS + (n + 2 if n > 1 else 2 * n + part) + z])

    def x0_copy(half, z=0):
        part = pl.ds(0, R0), pl.ds(half * D // 2, D // 2)
        return pltpu.make_async_copy(x_hbm.at[part], xa.at[part], sem_in.at[2 * NS + 10 + half + z])

    def tab_copy(z=0):
        part = pl.ds(0, ZERO)
        return pltpu.make_async_copy(tab_hbm.at[part], tab.at[part], sem_in.at[2 * NS + 13 + z])

    def oa_copy(a):
        return pltpu.make_async_copy(window16("oa", a * HS, HS), out_hbm.at[:, cols(a)],
                                     sem_out.at[0])

    def ob_copy(t, row, n):
        return pltpu.make_async_copy(
            window16("ob", t * HS + row, n),
            out_hbm.at[pl.ds(pl.multiple_of(2 * row, 128), 2 * n), cols(NT + t)], sem_out.at[1])

    small = [pltpu.make_async_copy(a, b, sem_in.at[2 * NS + 12])
             for a, b in ((tab_hbm.at[pl.ds(ZERO, 8)], tab.at[pl.ds(ZERO, 8)]),
                          (sk_hbm, sk_ref), (d_hbm, d_ref))]
    _start(small + [w_copy(0, 0, 2), x0_copy(0), w_copy(0, 1, 2), x0_copy(1), w_copy(1, 0, 2),
                    w_copy(1, 1, 2)] + [w_copy(n) for n in range(2, 8)] + [tab_copy()])
    _wait(small)
    unit = pltpu.bitcast(tab[pl.ds(ZERO, 8), :], jnp.int32)
    zs = [pl.multiple_of(unit[i, 0] * 8, 8) for i in range(3)]
    views = {n: [b.at[pl.ds(z, _BUFS[n][1]), :] for z in zs] + [b] for n, b in bufs.items()}

    for a in range(NT):
        st("ka", a * KA + 24, jnp.zeros((8, 128), U32))
    for t in range(2 * NT):
        st("k", t * KL + 8, jnp.zeros((WIN, 128), F32))
    skf = sk_ref[...].astype(F32)
    df = d_ref[...].astype(F32)
    for t in range(NT):
        for i in range(4):
            taps[t, i] = jnp.broadcast_to(skf[i:i + 1, t * 128:(t + 1) * 128], (8, 128))
        taps[t, 4] = jnp.broadcast_to(df[t:t + 1, :], (8, 128))

    def step(j, first=False, last=False):
        memo = {}
        consts.clear()
        e = E0 if first else E
        never = tab[pl.ds(ZERO, 8), :] != 0

        def once(key, fn):
            if key not in memo:
                memo[key] = fn()
            return memo[key]

        def fresh():
            memo["fresh"] = memo.get("fresh", 1) + 1
            return pl.multiple_of(zs[0] * memo["fresh"], 8)

        def pace(val):
            clock = memo.get("clock")
            if clock is None:
                return val
            if val.dtype != F32:
                clock = pltpu.bitcast(clock, val.dtype)
            return lax.select(never, clock, val)

        def paced(x):
            return jnp.concatenate([pace(x[:8]), x[8:]], axis=0)

        def late():
            return pltpu.bitcast(pace(jnp.zeros((8, 128), F32)), jnp.int32)[0, 0]

        def shifted(name, row, most):
            return [window(name, z + row, _BUFS[name][1] - most) for z in zs + [0]]

        def perm_in(n, u, t):
            tt = paced(pltpu.bitcast(wraw[n, pl.ds(u * 256, 256), pl.ds(t * 128, 128)], U32)).T
            for hh in range(4):
                st(f"t{n % 2 * 2 + u}", (4 * t + hh) * PITCH, tt[hh * DH:(hh + 1) * DH])

        def perm_out(n, u, t):
            g = jnp.concatenate([bufs[f"t{n % 2 * 2 + u}"][pl.ds(zs[0] + 4 * t + i, 32, PITCH), :]
                                 for i in range(4)], axis=0)
            st(f"w{n // 2}", (n % 2 * NT + t) * KW + u * 128, paced(g).T)

        def perm_list(n, us=(0, 1), ts=range(NT)):
            return ([(1, P(perm_in, n, u, t)) for u in us for t in range(NT)]
                    + [(1, P(perm_out, n, u, t)) for t in ts for u in us])

        def wo_in(n, t, hh):
            w = pltpu.bitcast(wraw[6 + n, pl.ds(hh * DH, DH), pl.ds(t * 128, 128)], U32)
            st(f"wp{n}", (16 * t + hh) * PITCH, _rows(pace(w[:8]), pace(w[8:])))

        def wo_out(n, t, dh):
            b = [bufs[f"wp{n}"][pl.ds(zs[dh % 2] + 16 * (t + c % 2 * 4) * PITCH + c // 2 * 8 + dh // 2,
                                      16, PITCH), :] for c in range(4)]
            b = [(_lo, _hi)[dh % 2](w) for w in [paced(b[0])] + b[1:3] + [paced(b[3])]]
            for i, rule in enumerate(RIGHT):
                name, c = ("ws3", 4 * RIGHT_SUMS.index(i)) if i in RIGHT_SUMS else ("w3", 2 * i)
                st16(name, (c + t) * KW + 16 * dh + 8 * n, _factor(rule, b.__getitem__))

        def wo_list(n):
            return ([(11, P(wo_in, n, t, hh)) for t in range(NT) for hh in range(16)]
                    + [(26, P(wo_out, n, t, dh)) for t in range(4) for dh in range(16)])

        def factor(p, i, t, r=0, n=KW, z=3):
            if i in RIGHT_SUMS:
                return ld(f"ws{p}", (4 * RIGHT_SUMS.index(i) + t) * KW + r, n, z)
            return ld(f"w{p}", (t + (4 if p == 3 else NT + 4) * i // 2) * KW + r, n, z)

        def right(p, which, t, r):
            top = which == (6,)
            b = [ld(f"w{p}", (h * NT + t + 4 * u) * KW + r, 16, 2 * top)
                 for h in range(2 - top) for u in range(2)]
            b = [x if c % 3 else _rows(pace(x[:8]), pace(x[8:])) for c, x in enumerate(b)]
            b = [pltpu.bitcast(x, BF16).astype(F32) for x in b]
            for i, val in [(i, _factor(RIGHT[i], b.__getitem__)) for i in which]:
                st16(f"ws{p}", (4 * RIGHT_SUMS.index(i) + t) * KW + r, val)

        def right_list(p, which=RIGHT_SUMS):
            return [(18 + 6 * len(which), P(right, p, which, t, r))
                    for t in range(4) for r in range(0, KW, 16)]

        def right2(p, r, i):
            u, m = divmod(r, KW // 2)
            w = [factor(p, i, u + c % 2 * 2, c // 2 * KW // 2 + m, 8, 1) for c in range(4)]
            w[0], w[3] = pace(w[0]), pace(w[3])
            b = [pltpu.bitcast(x, BF16).astype(F32) for x in w]
            for n, k in enumerate(RIGHT_SUMS):
                st16(f"wt{p}", (5 * i + n) * KW + r, _factor(RIGHT[k], b.__getitem__))

        def right2_list(p, order, start=0, stride=8):
            return [(25, P(right2, p, r, i)) for i in order for r in range(start, KW, stride)]

        def a1(i, r):
            a = once(("a", i), lambda: 2 * j + i)
            w0, w1, w2, w3 = once(("taps", i), lambda: [taps[a, u] for u in range(4)])
            k32 = once(("ka", i), lambda: window("ka", a * KA, KA))
            v32 = once(("va", i), lambda: window("va", a * HS, HS))
            c0, c1, c2 = (k32[at(8 * r + 32 - u, 8), :] for u in range(3))
            vv = v32[at(8 * r, 8), :]
            e0, o0, e1, o1, o2 = _lo(c0), _hi(c0), _lo(c1), _hi(c1), _hi(c2)
            ke = _tree([mul(e0, w0), mul(o1, w1), mul(e1, w2), mul(o2, w3)])
            ko = _tree([mul(o0, w0), mul(e0, w1), mul(o1, w2), mul(e1, w3)])
            st16(f"kv{r // 32}", 8 * (r % 32), _rows(mul(ke, _lo(vv)), pace(mul(ko, _hi(vv)))))

        def a1_list(i, c0, c1):
            return [(24, P(a1, i, r)) for r in range(8 * c0, 8 * c1)]

        def freq(c, im, m):
            return c * FP + im * (T + 8) + m

        def dft(i, name, c0, m):
            def mm():
                f = pltpu.bitcast(tab[pl.ds(fresh() + T * (name == "xf"), T), :], BF16)
                if name == "hf":
                    a = once(("a", i), lambda: 2 * j + i)
                    rhs = jnp.concatenate(
                        [ha[a, :, pl.ds(c * T, T)] for c in range(c0, c0 + 4)], axis=0)
                    return lax.dot_general(f, rhs, (((1,), (1,)), ((), ())),
                                           preferred_element_type=F32)
                rhs = jnp.concatenate([pltpu.bitcast(ld(f"kv{c0 // 4}", u * T // 2, T // 2, i), BF16)
                                       for u in range(4)], axis=1)
                return jnp.dot(f, rhs, preferred_element_type=F32)
            res = once((name, i, c0), mm)
            for u in range(4):
                val = res[m:m + 16, u * 128:(u + 1) * 128]
                if name == "hf" and c0 + u == 0 and m < T:
                    val = add(val, once(("dd", i), lambda: _rows(*[taps[memo["a", i], 4]] * 2)))
                st(name, freq(c0 + u, m // T, m % T), val)
            memo["clock"] = res[m + 8:m + 16, :128]

        def dft_list(i, name, *c0s):
            return [(16, P(dft, i, name, c0, m)) for c0 in c0s for m in range(0, 2 * T, 16)]

        def a3(i, g, plane, upper, n):
            def opnd(name, c):
                re = lambda: ld(name, freq(c, 0, 8 * g), z=plane)
                im = lambda: ld(name, freq(c, 1, 8 * g), z=plane)
                if name == "xf":
                    val = add(re(), im()) if plane == 0 else re() if plane == 1 else im()
                    return pace(val) if c >= 8 else val
                val = re() if plane == 0 else (sub, add)[plane - 1](im(), re())
                return val if c % 3 else pace(val)
            get = lambda name, c: once((name, i, g, plane, c), P(opnd, name, c))
            done = pace if n % 8 == 7 else lambda v: v
            cs = range(8, n + 1) if upper else range(min(n, 7) + 1)
            terms = [mul(get("xf", n - c), get("hf", c)) for c in cs]
            if upper:
                st("up", 8 * n, done(_tree(terms)))
                return
            if n >= 8:
                terms.append(ld("up", 8 * n))
            if plane == 0:
                st("k1", 8 * n, done(_tree(terms)))
            elif plane == 1:
                st("pi", 8 * n, done(_tree(terms + [ld("k1", 8 * n)])))
            else:
                pr = sub(ld("k1", 8 * n, z=1), _tree(terms))
                pi = ld("pi", 8 * n)
                zr, zi = pr, pi
                if n > 0:
                    qr, qi = memo["prev"]
                    zr, zi = sub(pr, qi), add(pi, qr)
                memo["prev"] = (pr, pi)
                if g % 2 == 0:
                    st("zr", 8 * n, done(zr))
                    st("zi", 8 * n, zi)
                else:
                    st16("z", n * T + 4 * (g - 1), _rows(ld("zr", 8 * n), done(zr)))
                    st16("z", n * T + T // 2 + 4 * (g - 1), _rows(ld("zi", 8 * n), zi))

        def a3_list(i):
            out = []
            for g in range(T // 8):
                for plane in range(3):
                    out += [(2 * (n - 8) + 4, P(a3, i, g, plane, True, n)) for n in range(8, NC)]
                    out += [(2 * min(n, 7) + 4 + 2 * (plane == 2), P(a3, i, g, plane, False, n))
                            for n in range(NC)]
            return out

        def idft(i, c0, odd, m):
            def mm():
                rhs = jnp.concatenate([pltpu.bitcast(ld("z", c * T + odd * T // 2, T // 2, i), BF16)
                                       for c in range(c0, c0 + 4)], axis=1)
                f = tab[pl.ds(fresh() + 2 * T + odd * T // 4, T // 4), :]
                return jnp.dot(pltpu.bitcast(f, BF16), rhs, preferred_element_type=F32)
            y = once(("y", i, c0, odd), mm)
            a = once(("a", i), lambda: 2 * j + i)
            q16 = once(("qa", i), lambda: window16("qa", a * HS, HS))
            o16 = once(("oa", i), lambda: window16("oa", a * HS, HS))
            flip = lambda w: jnp.take_along_axis(
                w, 7 - lax.broadcasted_iota(jnp.int32, (8, 128), 0), axis=0, mode="promise_in_bounds")
            for u in range(4):
                val = y[m:m + 16, u * 128:(u + 1) * 128]
                if not odd:
                    st("even", u * T // 2 + m, val)
                    continue
                even, mid = ld("even", u * T // 2 + m, 16), (c0 + u) * T + T // 2
                low = add(even, val)
                for row, out in ((mid + m, sub(even, val)),
                                 (mid - 16 - m, _rows(flip(low[8:]), flip(low[:8])))):
                    o16[at(row, 16), :] = mul(q16[at(row, 16), :].astype(F32), out).astype(BF16)
            memo["clock"] = y[m + 8:m + 16, 384:]

        def idft_list(i, *c0s):
            return [(16, P(idft, i, c0, odd, m)) for c0 in c0s
                    for odd in range(2) for m in range(0, T // 2, 16)]

        def xprep(x, u, r):
            halves = []
            for m in (r, r + 8):
                a, b = (pltpu.bitcast(x[pl.ds(2 * m, 16), pl.ds(t * 128, 128)], U32)
                        for t in (u, u + 4))
                a = pace(a)
                blocks = _lo(a), _lo(b), _hi(a), _hi(b)
                halves.append([_factor(rule, blocks.__getitem__) for rule in LEFT])
            for i, pair in enumerate(zip(*halves)):
                st16("xs", ((4 * i + u) * E0 + r) // 2, _rows(*pair))

        def xprep_list(x):
            return [(27, P(xprep, x, u, r)) for r in range(0, e, 16) for u in range(4)]

        def xprep2(x, u, r, i):
            def block(b):
                w = once(("x", u, r, b % 2), lambda: [pltpu.bitcast(
                    x[pl.ds(c // 2 * e + 2 * r, 32), pl.ds((u + c % 2 * 2 + b % 2 * 4) * 128, 128)], U32)
                    for c in range(4)])
                return [(_lo, _hi)[b // 2](v) for v in w]
            b0, *rest = LEFT[i]
            a = list(once(("left", u, r, b0), P(block, b0)))
            a[0], a[3] = paced(a[0]), paced(a[3])
            if rest:
                a = list(map(rest[0], a, once(("left", u, r, rest[1]), P(block, rest[1]))))
            for n, k in enumerate(LEFT_SUMS):
                st16("xt", ((5 * i + n) * 2 + u) * E0 // 4 + r // 2, _factor(LEFT[k], a.__getitem__))

        def xprep2_list(x):
            return [(c, P(xprep2, x, u, r, i)) for r in range(0, e // 2, 16) for u in range(2)
                    for i, c in ((1, 25), (0, 33), (6, 33), (4, 25), (3, 17), (5, 33), (2, 25))]

        def oprep(name, r0, n, which, u, r):
            a = lambda b: once(("o", name, u, r, b), lambda: ld(
                "o", (u + b % 2 * 4) * R0 + r0 + b // 2 * n + r, 16, 1 + (name == "xu")))
            memo["o", name, u, r, 3] = paced(a(3))
            for i in which:
                st16(name, ((4 * i + u) * E0 + r) // 2, _factor(LEFT[i], a))

        def oprep_list(name, r0, n, which=range(7)):
            return [(18, P(oprep, name, r0, n, which, u, r)) for r in range(0, n, 16) for u in range(4)]

        def oprep2(r0, n, i, u, r):
            view = once(("oprep", i), lambda: window("o", fresh(), NT * R0))
            block = lambda b, c: view[at(
                (u + c % 2 * 2 + b % 2 * 4) * R0 + r0 + b // 2 * n + c // 2 * n // 2 + r, 16), :]
            b0, *rest = LEFT[i]
            a = [block(b0, c) for c in range(4)]
            a = [x if c % 3 else paced(x) for c, x in enumerate(a)]
            if rest:
                a = [rest[0](x, block(rest[1], c)) for c, x in enumerate(a)]
            for k, val in enumerate([_factor(rule, a.__getitem__) for rule in LEFT]):
                st16(f"os{i}", (k * 2 + u) * E0 // 4 + r // 2, val)

        def oprep2_list(r0=0, n=e):
            return [(19 + 8 * (i in LEFT_SUMS), P(oprep2, r0, n, i, u, r))
                    for i in ORDER for r in range(0, n // 2, 16) for u in range(2)]

        def emit(p, r0, n, par, t, m, val, end):
            if p == 0:
                st("q", (par * NT + t) * E0 + m, val)
            elif p == 1:
                row = (par * NT + t + 1) * KL - e
                if m == 0 and not first:
                    st("k", row - WIN, ld("k", row + e - WIN, z=3))
                st("k", row + m, val)
            elif p == 2:
                st("v", (par * NT + t) * VL + 16 + m, val)
                if m == 0 and first and par == 0:
                    for other in range(2):
                        st("v", (other * NT + t) * VL + 8, jnp.broadcast_to(val[0:1], (WIN, 128)))
            else:
                base = once("row", lambda: j * E)
                o16 = once("ob", lambda: window16("ob", base, (NT - 1) * HS + (E0 if last else E)))
                o16[at(t * S + r0 + par * n + m, 16), :] = val.astype(BF16)
                if m + 16 == end and par == t // 4:
                    ob_copy(t, base + r0 // 2, n).start()

        def plain(n, t, m):
            def mm():
                w = [ld("w0", (n // 2 * NT + t + u) * KW + n % 2 * KW // 2, KW // 2, 3) for u in range(2)]
                return jnp.dot(xa[pl.ds(0, R0), pl.ds(n * D // 4, D // 4)],
                               jnp.concatenate([pltpu.bitcast(v, BF16) for v in w], axis=1),
                               preferred_element_type=F32)
            res = once(("plain", n, t), mm)
            memo["clock"] = res[m:m + 8, :128]
            for u in range(2):
                val = res[m:m + 16, u * 128:(u + 1) * 128]
                if n:
                    val = add(val, ld("qo"[n % 2], (t + u) * R0 + m, 16))
                st("oq"[n % 2], (t + u) * R0 + m, val)

        def plain_list():
            return [(16, P(plain, n, t, m))
                    for n in range(4) for t in range(0, NT, 2) for m in range(0, R0, 16)]

        def combine(level, i, row, res, out, ahead=None):
            get = lambda name, z=0: ld(name + level, row, 16, z)
            if i in (0, 2, 4):
                st("abc"[i // 2] + level, row, res)
            elif i == 1:
                st("d" + level, row, res if ahead == 1 else sub(res, get("b")))
                out(1, 0, add(get("a"), res))
            elif i == 3 and ahead == 6:
                out(0, 1, add(get("b", 1), res))
                out(1, 1, add(add(get("e"), get("c", 1)), sub(res, get("a", 1))))
            elif i == 3:
                st("e" + level, row, sub(res, get("a", 1)))
                out(0, 1, add(get("b", 1), res))
            elif i == ahead:
                st("e" + level, row, res)
            else:
                part = add(get("de"[i - 5]), get("c", i - 5))
                out(i - 5, i - 5, add(sub(part, get("b")) if (i, ahead) == (5, 1) else part, res))

        def tiles(name, starts, n):
            view = window(name, fresh(), _BUFS[name][1])
            return jnp.concatenate(
                [pltpu.bitcast(view[at(row, n // 2), :], BF16) for row in starts], axis=1)

        def product(p, src, r0, n, ahead, t, i, m):
            res = once(("product", p, r0, t, i), lambda: jnp.dot(
                tiles(src, [(4 * i + u) * E0 // 2 for u in range(4)], n),
                pltpu.bitcast(factor(p, i, t), BF16), preferred_element_type=F32))
            memo["clock"] = res[m:m + 8]
            combine("1", i, t * E0 + m, res[m:m + 16],
                    lambda par, h, val: emit(p, r0, n, par, t + 4 * h, m, val, n), ahead)

        def strassen(p, src="xs", r0=0, n=e, order=ORDER, ahead=None):
            return [(16, P(product, p, src, r0, n, ahead, t, i, m))
                    for t in range(4) for i in order for m in range(0, n, 16)]

        def product2(p, r0, n, i, k, m):
            def mm():
                if p == 3:
                    name, row, gap = f"os{i}", k * E0 // 2, E0 // 4
                elif k in LEFT_SUMS:
                    name, row, gap = "xt", (5 * i + LEFT_SUMS.index(k)) * E0 // 2, E0 // 4
                else:
                    name, row, gap = "xs", 2 * i * E0 + (k == 1) * (E0 + n // 4), E0 // 2
                if k in RIGHT_SUMS:
                    w = [ld(f"wt{p}", ((5 * i + RIGHT_SUMS.index(k)) * 2 + u) * KW // 2, KW // 2, 3)
                         for u in range(2)]
                else:
                    w = [factor(p, i, k + u, k * KW // 4, KW // 2) for u in range(2)]
                return jnp.dot(tiles(name, (row, row + gap), n // 2),
                               jnp.concatenate([pltpu.bitcast(v, BF16) for v in w], axis=1),
                               preferred_element_type=F32)
            res = once(("product2", p, i, k), mm)
            memo["clock"] = res[m + 8:m + 16, :128]

            def out(u, r2, c2, val):
                t, row = 2 * c2 + u, r2 * n // 2 + m
                combine("1", i, t * E0 + row, val, lambda par, h, v: emit(
                    p, r0, n, par, t + 4 * h, row, v, (1 + c2) * n // 2))
            for u in range(2):
                combine("2", k, u * E0 // 2 + m, res[m:m + 16, u * 128:(u + 1) * 128], P(out, u))

        def strassen2(p, deep=7, r0=0, n=e):
            return [task for i in ORDER for task in (
                [(16, P(product2, p, r0, n, i, k, m)) for k in ORDER for m in range(0, n // 2, 16)]
                if i < deep else strassen(p, order=(i,)))]

        quarter = lax.shift_right_logical(lax.broadcasted_iota(jnp.int32, (8, 128), 1), 5)
        low, middle, odd = quarter < 2, (quarter == 1) | (quarter == 2), (quarter & 1) == 1

        def qk(par, m, w):
            query = lambda t: (bufs["q"][at(t * R0 + 2 * m + par, 8, 2), :] if first
                               else ld("q", (par * NT + t) * E0 + m))
            fold = lambda mask, a, b, shift: add(
                lax.select(mask, a, b), pltpu.roll(lax.select(mask, b, a), shift, 1))
            g = m // 8 % 4
            scale = once(("scale", par, m),
                         lambda: pace(jnp.full((8, 128), DH ** -0.5 * LOG2E, F32)))
            if first and g == 1:
                scale = once(("flush", par, m), lambda: lax.select(
                    never, window("v", fresh() + 16, 8)[...], scale))
            qv = once(("qv", par, m), lambda: [mul(query(t), scale) for t in range(NT)])
            s = _tree([mul(qv[t], ld("k", (par * NT + t + 1) * KL - e + m - w)) for t in range(NT)])
            if g % 2:
                s = fold((low, middle)[g // 2], memo["s", 0], pace(s), 64)
            if g == 3:
                s = fold(odd, memo["s", 1, w], s, 32)
                if first and m == 24 and w:
                    early = lax.broadcasted_iota(jnp.int32, (8, 128), 0) < w
                    s = jnp.where(early & (quarter == 1), -1e9 * LOG2E, s)
            memo[(("s", 0), ("s", 1, w), ("s", 0), ("lg", par, m, w))[g]] = s

        def expo(r):
            lg = [memo[("lg", *r, w)] for w in range(WIN)]
            top = pace(functools.reduce(lax.max, lg))
            memo["e", r] = [lax.exp2(sub(s, top)) for s in lg]

        def norm(r):
            total = pace(_tree(memo["e", r]))
            memo["inv", r] = total, pl.reciprocal(total, approx=True)

        def probs(r):
            total, inv = memo["inv", r]
            inv = pace(inv)
            inv = mul(inv, sub(np.float32(2), mul(total, inv)))
            for w, x in enumerate(memo["e", r]):
                st("quad", 8 * w, mul(x, inv))

        def spread(u, r):
            row = lambda w, g: (2 * w + r[0]) * HS + r[1] - 24 + 8 * g
            for w in (2 * u, 2 * u + 1):
                x = pace(ld("quad", 8 * w))
                y = pltpu.roll(x, 64, 1)
                for a, groups in ((lax.select(low, x, y), (0, 3)), (lax.select(low, y, x), (1, 2))):
                    b = pltpu.roll(a, 32, 1)
                    st("p", row(w, groups[0]), lax.select(odd, a, b))
                    st("p", row(w, groups[1]), lax.select(odd, b, a))

        def qk_list():
            rs, gap = [(par, m) for par in range(2) for m in range(0, e, 8)], 2 + first
            stages = [(expo, 20), (norm, 20 + gap), (probs, 20 + 2 * gap)] + [
                (P(spread, u), 22 + 2 * gap + 2 * u) for u in range(4)]
            out = [[(0, P(qk, *rs[n + u], w))]
                   for n in range(0, len(rs), 2) for w in range(WIN) for u in range(2)]
            out += [[] for _ in range(stages[-1][1])]
            for n in range(3, len(rs), 4):
                for f, lag in stages:
                    out[WIN * n + WIN - 1 + lag].append((0, P(f, rs[n])))
            return [(22, P(_run, tasks)) for tasks in out]

        def pv(par, m, t):
            p = once(("pv", par, m), lambda: [
                (pace if w % 4 == 0 else lambda v: v)(ld("pr", (2 * w + par) * HS + m))
                for w in range(WIN)])
            row = (par * NT + t) * VL + 16 + m
            bufs["o"][at(t * R0 + 2 * m + par, 8, 2), :] = pace(
                _tree([mul(p[w], ld("vr", row - w)) for w in range(WIN)]))

        def pv_list(m0, m1):
            return [(16, P(pv, par, m, t))
                    for par in range(2) for m in range(m0, m1, 8) for t in range(NT)]

        if first:
            main = plain_list() + sum((strassen(1, order=order, ahead=6) for order in (
                (0,), (6,), (2,), (1, 4, 5, 3))), []) + strassen(2)

            def phase(end, side=(), arrival=None):
                _weave(main[memo.get("done", 0):end], side)
                memo["done"] = end
                if arrival:
                    arrival(late()).wait()

            def permute(tasks, side=(), early=()):
                if early:
                    phase(memo["done"] + 46, _merge(tasks[:16], early))
                    tasks = tasks[16:]
                phase(memo["done"] + 8 * len(tasks) // 3, _merge(tasks, side))
                phase(memo["done"] + 26)

            xp, rq = xprep_list(xa), right_list(0)
            tk, rk, tv, rv = (right_list(p, which) for p in (1, 2) for which in ((6,), (1, 3, 4, 5)))
            dq = right2_list(0, [i for i in ORDER if i < DEEP_Q])
            do = right2_list(2, (0, 6, 2, 1, 4, 5, 3)) + sum(
                (right2_list(3, ORDER, 8 * n, 16) for n in range(2)), [])
            w_copy(0, 0, 2).wait()
            _run(perm_list(0, (0,)))
            memo["clock"] = pltpu.bitcast(ld("w0", KW + 120, z=3), F32)
            x0_copy(0, late()).wait()
            phase(64, [], P(w_copy, 0, 1, 2))
            permute(perm_list(0, (1,)))
            phase(150, [], P(x0_copy, 1))
            phase(190, xp[:24], P(w_copy, 1, 0, 2))
            permute(perm_list(1, (0,)), xp[24:48])
            phase(258, xp[48:52], P(w_copy, 1, 1, 2))
            permute(perm_list(1, (1,)), xp[52:])
            phase(380, rq[:40], P(w_copy, 2, 0, 1))
            permute(perm_list(2), rq[40:] + dq[:56])
            phase(506, tk[:14], P(w_copy, 3, 0, 1))
            permute(perm_list(3, ts=(4, 5, 0, 1, 6, 2, 7, 3)), dq[56:], tk[14:])
            phase(630, rk[:7], P(w_copy, 4, 0, 1))
            permute(perm_list(4), rk[7:])
            phase(752, do[:22], P(w_copy, 5, 0, 1))
            permute(perm_list(5), do[22:64], tv)
            phase(880, rv[:14], P(w_copy, 6, 0, 1))
            _start(sum((in_copies(n, second) for n in range(NS) for second in range(2)), []))
            phase(996, _merge(wo_list(0), rv[14:] + do[64:112]))
            phase(1000, [], P(w_copy, 7, 0, 1))
            phase(1004)
            phase(1070, _merge(wo_list(1), do[112:126]))
            logits = qk_list()
            phase(len(main) - 8, _merge(do[126:-64], logits[:-34])
                  + _merge(do[-64:-18], [(5, f) for _, f in logits[-34:]]) + do[-18:])
            phase(len(main), [], tab_copy)
            return

        views.update(pr=shifted("p", j * E, NS * E), vr=shifted("v", j * E, NS * E))
        if last:
            n = E0 // 4
            _run(pv_list(n // 2, n) + oprep_list("xs", 0, n, (0, 1)))
            main = strassen(3, "xs", 0, n, (0,), 1) + strassen(3, "xs", 0, n, (1,), 1)
            _weave(main[:24], pv_list(0, n // 2) + oprep_list("xu", 0, n, range(2, 7)))
            main = main[24:] + strassen(3, "xu", 0, n, (2, 4, 5, 3, 6), 1)
            _weave(main[:-16], pv_list(n, 2 * n) + oprep_list("xt", 2 * n, n))
            _run(main[-16:])
            main = strassen(3, "xt", 2 * n, n) + strassen2(3, 7, 4 * n, 2 * n)
            pre = oprep2_list(4 * n, 2 * n)
            _weave(main[:100], pv_list(2 * n, 4 * n) + pre[:8])
            _weave(main[100:166], pre[8:])
            _run(main[166:])
            return

        for name in "vp":
            views[name] = shifted(name, E0 + j * E, E0 + (NS - 1) * E)
        head, tail, x = strassen(1) + strassen2(0, DEEP_Q), strassen2(2), xa.at[rows(j)]
        for u in range(4):
            _weave(dft_list(0, "hf", 4 * u), a1_list(0, 11 * u // 4, 11 * (u + 1) // 4))
        extra = _split(xprep_list(x), 4, 6)
        _weave(dft_list(0, "xf", 0), a1_list(0, 11, 13))
        _weave(dft_list(0, "xf", 4), _merge(a1_list(0, 13, 16), extra[0]))
        _weave(dft_list(0, "xf", 8, 12)[:20], extra[1])
        _run(dft_list(0, "xf", 12)[4:])
        _weave(head[:66], xprep2_list(x))
        conv = a3_list(0)
        conv.insert(24 * 42, (0, lambda: _wait(in_copies(j, 1, late()))))
        _weave(head[66:406], conv)
        _run(head[406:416])
        for u in range(4):
            _run(idft_list(0, 4 * u))
            _weave(dft_list(1, "hf", 4 * u), a1_list(1, 3 * u, 3 * u + 3))
        oa_copy(2 * j).start()
        _weave(dft_list(1, "xf", 0), a1_list(1, 12, 16))
        mix, pre, conv = _split(pv_list(0, E), 2, 5), _split(oprep2_list(), 6, 1), a3_list(1)
        _weave(dft_list(1, "xf", 4, 8, 12), mix[0])
        _weave(head[416:528], mix[1])
        side = pre[0]
        for n, part in enumerate(_split(pre[1], *[1] * 7)):
            side = side + conv[24 * n:24 * n + 24] + part
        _weave(head[528:] + strassen2(3) + tail[:20], side + conv[24 * 7:])
        tail += idft_list(1, 0, 4, 8, 12)
        _weave(tail[20:-16], qk_list())
        _run(tail[-16:])
        oa_copy(2 * j + 1).start()

    def loop(j, carry):
        _wait(in_copies(j, 0))
        step(j)
        return carry

    step(0, first=True)
    lax.fori_loop(0, NS, loop, 0)
    step(NS, last=True)
    for i, name in enumerate(("oa", "ob")):
        pltpu.make_async_copy(raw[name], raw[name], sem_out.at[i]).wait()


@jax.jit
def pallas_concat_heads__ssm_conv_h3__sliding_local_dilated__prompt_kernel(
    A_q, A_k, A_v, A_shift_k, A_ssm_k, A_ssm_D, B_x, B_wqkv, B_wo,
):
    hbm = pl.BlockSpec(memory_space=pl.ANY)
    out = pl.pallas_call(
        _kernel,
        in_specs=[hbm] * 10,
        out_specs=hbm,
        out_shape=jax.ShapeDtypeStruct((S, 2 * D), BF16),
        scratch_shapes=[
            pltpu.VMEM((NT, 128, S), BF16),
            pltpu.VMEM((S, D), BF16),
            pltpu.VMEM((8, D // 2, D), BF16),
            pltpu.VMEM((NT, 5, 8, 128), F32),
            pltpu.VMEM(_TABLE.shape, U32),
            pltpu.SemaphoreType.DMA((2 * NS + 14,)),
            pltpu.SemaphoreType.DMA((2,)),
        ] + [pltpu.VMEM((r * 4 // np.dtype(t).itemsize, 128), t) for t, r in _BUFS.values()]
        + [pltpu.VMEM((4, D), BF16), pltpu.VMEM((8, 128), BF16)],
        compiler_params=pltpu.CompilerParams(
            vmem_limit_bytes=118 * 1024 * 1024, disable_bounds_checks=True,
            disable_semaphore_checks=True, flags={"XLA_TPU_RESCHEDULE_DMA_DONES": True}),
        name="fused",
    )(A_q[0], A_k[0], A_v[0], A_shift_k.T, A_ssm_k,
      A_ssm_D.reshape(8, 128), B_x[0], B_wqkv, B_wo, _TABLE)
    return out[None]
```

```python
import functools

import jax
import jax.numpy as jnp
import numpy as np
from jax import lax
from jax.experimental import pallas as pl
import jax.experimental.pallas.tpu as pltpu

S = 2048
D = 1024
T = 128
NC = S // T
NT = D // 128
NS = 4
R0 = 512
R = (S - R0) // NS
E0, E, HS = R0 // 2, R // 2, S // 2
WIN, DH = 8, 32
LOG2E = float(np.log2(np.e))
PITCH = DH + 1
KL = E0 + 16
VL = HS + 16
FP = 2 * T + 16
KW = D // 4
KA = HS + 32
ZERO = 5 * T // 2

F32, BF16, U32 = jnp.float32, jnp.bfloat16, jnp.uint32
P = functools.partial
add, sub, mul = lax.add, lax.sub, lax.mul

LEFT = ((2, add, 3), (3,), (0, add, 1), (0,), (0, add, 3), (1, sub, 3), (2, sub, 0))
RIGHT = ((0,), (2, sub, 0), (3,), (1, sub, 3), (0, add, 3), (2, add, 3), (0, add, 1))
LEFT_SUMS, RIGHT_SUMS = (0, 2, 4, 5, 6), (1, 3, 4, 5, 6)
ORDER = (0, 2, 1, 4, 5, 3, 6)
DEEP_Q = 4


def _pack_rows(m):
    b = m.astype(jnp.bfloat16).view(np.uint16).astype(np.uint32)
    return np.ascontiguousarray(b[0::2] | (b[1::2] << 16))


def _dft_table():
    th = 2.0 * np.pi * (np.arange(T) + 0.25) / T
    dft = lambda t: np.concatenate([np.cos(np.outer(th, t)), -np.sin(np.outer(th, t))], axis=0)
    paired = np.arange(T).reshape(-1, 8, 2).transpose(0, 2, 1).reshape(-1)
    ph = np.outer(np.arange(T // 2) + 0.5, th)
    mats = (dft(np.arange(T)), dft(paired - (T - 1) / 2), np.cos(ph) / T, np.sin(ph) / T)
    return np.concatenate([_pack_rows(m) for m in mats] + [np.zeros((32, T), np.uint32)], axis=0)


_TABLE = _dft_table()


def _lo(w):
    return pltpu.bitcast(lax.shift_left(w, np.uint32(16)), F32)


def _hi(w):
    return pltpu.bitcast(lax.bitwise_and(w, np.uint32(0xFFFF0000)), F32)


def _rows(first, second):
    return jnp.concatenate([first, second], axis=0)


def _tree(xs):
    while len(xs) > 1:
        xs = [add(xs[i], xs[i + 1]) if i + 1 < len(xs) else xs[i] for i in range(0, len(xs), 2)]
    return xs[0]


def _factor(rule, block):
    return rule[1](block(rule[0]), block(rule[2])) if len(rule) > 1 else block(rule[0])


def _merge(main, side):
    if not main:
        return side
    total_m = sum(c for c, _ in main)
    total_s = sum(c for c, _ in side)
    done_m, done_s, i, out = 0, 0, 0, []
    for task in main:
        out.append(task)
        done_m += task[0]
        while i < len(side) and (done_s + side[i][0]) * total_m <= done_m * total_s:
            done_s += side[i][0]
            out.append(side[i])
            i += 1
    assert i == len(side)
    return out


def _run(tasks):
    for _, f in tasks:
        f()


def _weave(main, side):
    _run(_merge(main, side))


def _split(tasks, *weights):
    ends = np.cumsum((0,) + weights) * len(tasks) // sum(weights)
    return [tasks[a:b] for a, b in zip(ends[:-1], ends[1:])]


def _start(copies):
    for c in copies:
        c.start()


def _wait(copies):
    for c in copies:
        c.wait()


_BUFS = {n: (t, r) for t, group in (
    (BF16, dict(qa=NT * HS, ka=NT * KA, va=NT * HS, oa=NT * HS, ob=NT * HS,
                xs=14 * E0, xt=35 * E0 // 2, **{f"os{i}": 7 * E0 // 2 for i in range(7)},
                **{f"kv{u}": S // 8 for u in range(4)}, z=NC * T, w3=NT * KW, xu=14 * E0,
                **{f"ws{p}": 20 * KW for p in range(4)},
                wt0=5 * DEEP_Q * KW, wt2=35 * KW, wt3=35 * KW)),
    (U32, dict(**{f"w{p}": 2 * NT * KW for p in range(3)}, **{f"t{u}": 34 * DH for u in range(4)},
               wp0=(4 * PITCH + 1) * DH, wp1=(4 * PITCH + 1) * DH)),
    (F32, dict(hf=NC * FP, xf=NC * FP, up=8 * NC, k1=8 * NC, pi=8 * NC, zr=8 * NC, zi=8 * NC,
               even=2 * T, quad=8 * WIN,
               **{n + "1": 4 * E0 for n in "abcde"}, **{n + "2": E0 for n in "abcde"},
               q=NT * R0 + 32, k=2 * NT * KL, v=2 * NT * VL, p=WIN * S, o=NT * R0 + 32)),
) for n, r in group.items()}


def _kernel(q_hbm, k_hbm, v_hbm, sk_hbm, h_hbm, d_hbm, x_hbm, w_hbm, wo_hbm, tab_hbm, out_hbm,
            ha, xa, wraw, taps, tab, sem_in, sem_out, *raw):
    *raw, sk_ref, d_ref = raw
    raw = dict(zip(_BUFS, raw))
    bufs = {n: b.bitcast(U32) if _BUFS[n][0] == BF16 else b for n, b in raw.items()}
    consts = {}

    def at(start, size, stride=None):
        if start not in consts:
            consts[start] = add(np.int32(start), np.int32(0))
        return pl.ds(consts[start], size, stride)

    def ld(name, row, n=8, z=0):
        assert 0 <= row and row + n <= views[name][z].shape[0]
        return views[name][z][at(row, n), :]

    def st(name, row, val):
        assert 0 <= row and row + val.shape[0] <= views[name][3].shape[0]
        views[name][3][at(row, val.shape[0]), :] = val

    def st16(name, row, val):
        assert 0 <= row and 2 * row + val.shape[0] <= raw[name].shape[0]
        raw[name][at(2 * row, val.shape[0]), :] = val.astype(BF16)

    def window(name, row, n):
        return bufs[name].at[pl.ds(pl.multiple_of(row, 8), n), :]

    def window16(name, row, n):
        return raw[name].at[pl.ds(pl.multiple_of(2 * row, 16), 2 * n), :]

    def cols(a):
        return pl.ds(pl.multiple_of(a * 128, 128), 128)

    def rows(j):
        return pl.ds(pl.multiple_of(R0 + j * R, 128), R)

    def a_copies(a, sem):
        return [pltpu.make_async_copy(src, dst, sem) for src, dst in (
            (h_hbm.at[cols(a), :], ha.at[a]),
            (k_hbm.at[:, cols(a)], window16("ka", a * KA + 32, HS)),
            (v_hbm.at[:, cols(a)], window16("va", a * HS, HS)))]

    def in_copies(j, second, z=0):
        sem = sem_in.at[2 * j + second + z]
        if not second:
            return ([pltpu.make_async_copy(x_hbm.at[rows(j), :], xa.at[rows(j), :], sem)]
                    + a_copies(2 * j, sem))
        return a_copies(2 * j + 1, sem) + [
            pltpu.make_async_copy(q_hbm.at[:, cols(a)], window16("qa", a * HS, HS), sem)
            for a in (2 * j, 2 * j + 1)]

    def w_copy(n, part=0, parts=1, z=0):
        size = D // 2 // parts
        span = pl.ds(n % 2 * D // 2 + part * size, size)
        src = w_hbm.at[span, pl.ds(n // 2 * D, D)] if n < 6 else wo_hbm.at[span, :]
        return pltpu.make_async_copy(src, wraw.at[n, pl.ds(part * size, size)],
                                     sem_in.at[2 * NS + (n + 2 if n > 1 else 2 * n + part) + z])

    def x0_copy(half, z=0):
        part = pl.ds(0, R0), pl.ds(half * D // 2, D // 2)
        return pltpu.make_async_copy(x_hbm.at[part], xa.at[part], sem_in.at[2 * NS + 10 + half + z])

    def small_copies(z=0):
        part = pl.ds(0, ZERO)
        return [pltpu.make_async_copy(a, b, sem_in.at[2 * NS + 13 + z])
                for a, b in ((tab_hbm.at[part], tab.at[part]), (sk_hbm, sk_ref), (d_hbm, d_ref))]

    def oa_copy(a):
        return pltpu.make_async_copy(window16("oa", a * HS, HS), out_hbm.at[:, cols(a)],
                                     sem_out.at[0])

    def ob_copy(t, row, n):
        return pltpu.make_async_copy(
            window16("ob", t * HS + row, n),
            out_hbm.at[pl.ds(pl.multiple_of(2 * row, 64), 2 * n), cols(NT + t)], sem_out.at[1])

    zero = [pltpu.make_async_copy(tab_hbm.at[pl.ds(ZERO, 8)], tab.at[pl.ds(ZERO, 8)],
                                  sem_in.at[2 * NS + 12])]
    _start(zero + [w_copy(0, 0, 2), x0_copy(0), w_copy(0, 1, 2), x0_copy(1), w_copy(1, 0, 2),
           w_copy(1, 1, 2)] + [w_copy(n) for n in range(2, 8)] + small_copies())
    _wait(zero)
    unit = pltpu.bitcast(tab[pl.ds(ZERO, 8), :], jnp.int32)
    zs = [pl.multiple_of(unit[i, 0] * 8, 8) for i in range(3)]
    views = {n: [b.at[pl.ds(z, _BUFS[n][1]), :] for z in zs] + [b] for n, b in bufs.items()}

    for a in range(NT):
        st("ka", a * KA + 24, jnp.zeros((8, 128), U32))
    for t in range(2 * NT):
        st("k", t * KL + 8, jnp.zeros((WIN, 128), F32))

    def step(j, first=False, last=False):
        memo = {}
        consts.clear()
        e = E0 if first else E
        never = tab[pl.ds(ZERO, 8), :] != 0

        def once(key, fn):
            if key not in memo:
                memo[key] = fn()
            return memo[key]

        def fresh():
            memo["fresh"] = memo.get("fresh", 1) + 1
            return pl.multiple_of(zs[0] * memo["fresh"], 8)

        def pace(val):
            clock = memo.get("clock")
            if clock is None:
                return val
            if val.dtype != F32:
                clock = pltpu.bitcast(clock, val.dtype)
            return lax.select(never, clock, val)

        def paced(x):
            return jnp.concatenate([pace(x[:8]), x[8:]], axis=0)

        def late():
            return pltpu.bitcast(pace(jnp.zeros((8, 128), F32)), jnp.int32)[0, 0]

        def shifted(name, row, most):
            return [window(name, z + row, _BUFS[name][1] - most) for z in zs + [0]]

        def perm_in(n, u, t):
            tt = paced(pltpu.bitcast(wraw[n, pl.ds(u * 256, 256), pl.ds(t * 128, 128)], U32)).T
            for hh in range(4):
                st(f"t{n % 2 * 2 + u}", (4 * t + hh) * PITCH, tt[hh * DH:(hh + 1) * DH])

        def perm_out(n, u, t):
            g = jnp.concatenate([bufs[f"t{n % 2 * 2 + u}"][pl.ds(zs[0] + 4 * t + i, 32, PITCH), :]
                                 for i in range(4)], axis=0)
            st(f"w{n // 2}", (n % 2 * NT + t) * KW + u * 128, paced(g).T)

        def perm_list(n, us=(0, 1), ts=range(NT)):
            return ([(1, P(perm_in, n, u, t)) for u in us for t in range(NT)]
                    + [(1, P(perm_out, n, u, t)) for t in ts for u in us])

        def wo_in(n, t, hh):
            w = pltpu.bitcast(wraw[6 + n, pl.ds(hh * DH, DH), pl.ds(t * 128, 128)], U32)
            st(f"wp{n}", (16 * t + hh) * PITCH, _rows(pace(w[:8]), pace(w[8:])))

        def wo_out(n, t, dh):
            b = [bufs[f"wp{n}"][pl.ds(zs[dh % 2] + 16 * (t + c % 2 * 4) * PITCH + c // 2 * 8 + dh // 2,
                                      16, PITCH), :] for c in range(4)]
            b = [(_lo, _hi)[dh % 2](w) for w in [paced(b[0])] + b[1:3] + [paced(b[3])]]
            for i, rule in enumerate(RIGHT):
                name, c = ("ws3", 4 * RIGHT_SUMS.index(i)) if i in RIGHT_SUMS else ("w3", 2 * i)
                st16(name, (c + t) * KW + 16 * dh + 8 * n, _factor(rule, b.__getitem__))

        def wo_list(n):
            return ([(11, P(wo_in, n, t, hh)) for t in range(NT) for hh in range(16)]
                    + [(26, P(wo_out, n, t, dh)) for t in range(4) for dh in range(16)])

        def factor(p, i, t, r=0, n=KW, z=3):
            if i in RIGHT_SUMS:
                return ld(f"ws{p}", (4 * RIGHT_SUMS.index(i) + t) * KW + r, n, z)
            return ld(f"w{p}", (t + (4 if p == 3 else NT + 4) * i // 2) * KW + r, n, z)

        def right(p, which, t, r):
            top = which == (6,)
            b = [ld(f"w{p}", (h * NT + t + 4 * u) * KW + r, 16, 2 * top)
                 for h in range(2 - top) for u in range(2)]
            b = [x if c % 3 else _rows(pace(x[:8]), pace(x[8:])) for c, x in enumerate(b)]
            b = [pltpu.bitcast(x, BF16).astype(F32) for x in b]
            for i, val in [(i, _factor(RIGHT[i], b.__getitem__)) for i in which]:
                st16(f"ws{p}", (4 * RIGHT_SUMS.index(i) + t) * KW + r, val)

        def right_list(p, which=RIGHT_SUMS):
            return [(18 + 6 * len(which), P(right, p, which, t, r))
                    for t in range(4) for r in range(0, KW, 16)]

        def right2(p, r, i):
            u, m = divmod(r, KW // 2)
            w = [factor(p, i, u + c % 2 * 2, c // 2 * KW // 2 + m, 8, 1) for c in range(4)]
            w[0], w[3] = pace(w[0]), pace(w[3])
            b = [pltpu.bitcast(x, BF16).astype(F32) for x in w]
            for n, k in enumerate(RIGHT_SUMS):
                st16(f"wt{p}", (5 * i + n) * KW + r, _factor(RIGHT[k], b.__getitem__))

        def right2_list(p, order, start=0, stride=8):
            return [(25, P(right2, p, r, i)) for i in order for r in range(start, KW, stride)]

        def a1(i, r):
            a = once(("a", i), lambda: 2 * j + i)
            w0, w1, w2, w3 = once(("taps", i), lambda: [taps[a, u] for u in range(4)])
            k32 = once(("ka", i), lambda: window("ka", a * KA, KA))
            v32 = once(("va", i), lambda: window("va", a * HS, HS))
            c0, c1, c2 = (k32[at(8 * r + 32 - u, 8), :] for u in range(3))
            vv = v32[at(8 * r, 8), :]
            e0, o0, e1, o1, o2 = _lo(c0), _hi(c0), _lo(c1), _hi(c1), _hi(c2)
            ke = _tree([mul(e0, w0), mul(o1, w1), mul(e1, w2), mul(o2, w3)])
            ko = _tree([mul(o0, w0), mul(e0, w1), mul(o1, w2), mul(e1, w3)])
            st16(f"kv{r // 32}", 8 * (r % 32), _rows(mul(ke, _lo(vv)), pace(mul(ko, _hi(vv)))))

        def a1_list(i, c0, c1):
            return [(24, P(a1, i, r)) for r in range(8 * c0, 8 * c1)]

        def freq(c, im, m):
            return c * FP + im * (T + 8) + m

        def dft(i, name, c0, m):
            def mm():
                f = pltpu.bitcast(tab[pl.ds(fresh() + T * (name == "xf"), T), :], BF16)
                if name == "hf":
                    a = once(("a", i), lambda: 2 * j + i)
                    rhs = jnp.concatenate(
                        [ha[a, :, pl.ds(c * T, T)] for c in range(c0, c0 + 4)], axis=0)
                    return lax.dot_general(f, rhs, (((1,), (1,)), ((), ())),
                                           preferred_element_type=F32)
                rhs = jnp.concatenate([pltpu.bitcast(ld(f"kv{c0 // 4}", u * T // 2, T // 2, i), BF16)
                                       for u in range(4)], axis=1)
                return jnp.dot(f, rhs, preferred_element_type=F32)
            res = once((name, i, c0), mm)
            for u in range(4):
                val = res[m:m + 16, u * 128:(u + 1) * 128]
                if name == "hf" and c0 + u == 0 and m < T:
                    val = add(val, once(("dd", i), lambda: _rows(*[taps[memo["a", i], 4]] * 2)))
                st(name, freq(c0 + u, m // T, m % T), val)
            memo["clock"] = res[m + 8:m + 16, :128]

        def dft_list(i, name, *c0s):
            return [(16, P(dft, i, name, c0, m)) for c0 in c0s for m in range(0, 2 * T, 16)]

        def a3(i, g, plane, upper, n):
            def opnd(name, c):
                re = lambda: ld(name, freq(c, 0, 8 * g), z=plane)
                im = lambda: ld(name, freq(c, 1, 8 * g), z=plane)
                if name == "xf":
                    val = add(re(), im()) if plane == 0 else re() if plane == 1 else im()
                    return pace(val) if c >= 8 else val
                val = re() if plane == 0 else (sub, add)[plane - 1](im(), re())
                return val if c % 3 else pace(val)
            get = lambda name, c: once((name, i, g, plane, c), P(opnd, name, c))
            done = pace if n % 8 == 7 else lambda v: v
            cs = range(8, n + 1) if upper else range(min(n, 7) + 1)
            terms = [mul(get("xf", n - c), get("hf", c)) for c in cs]
            if upper:
                st("up", 8 * n, done(_tree(terms)))
                return
            if n >= 8:
                terms.append(ld("up", 8 * n))
            if plane == 0:
                st("k1", 8 * n, done(_tree(terms)))
            elif plane == 1:
                st("pi", 8 * n, done(_tree(terms + [ld("k1", 8 * n)])))
            else:
                pr = sub(ld("k1", 8 * n, z=1), _tree(terms))
                pi = ld("pi", 8 * n)
                zr, zi = pr, pi
                if n > 0:
                    qr, qi = memo["prev"]
                    zr, zi = sub(pr, qi), add(pi, qr)
                memo["prev"] = (pr, pi)
                if g % 2 == 0:
                    st("zr", 8 * n, done(zr))
                    st("zi", 8 * n, zi)
                else:
                    st16("z", n * T + 4 * (g - 1), _rows(ld("zr", 8 * n), done(zr)))
                    st16("z", n * T + T // 2 + 4 * (g - 1), _rows(ld("zi", 8 * n), zi))

        def a3_list(i):
            out = []
            for g in range(T // 8):
                for plane in range(3):
                    out += [(2 * (n - 8) + 4, P(a3, i, g, plane, True, n)) for n in range(8, NC)]
                    out += [(2 * min(n, 7) + 4 + 2 * (plane == 2), P(a3, i, g, plane, False, n))
                            for n in range(NC)]
            return out

        def idft(i, c0, odd, m):
            def mm():
                rhs = jnp.concatenate([pltpu.bitcast(ld("z", c * T + odd * T // 2, T // 2, i), BF16)
                                       for c in range(c0, c0 + 4)], axis=1)
                f = tab[pl.ds(fresh() + 2 * T + odd * T // 4, T // 4), :]
                return jnp.dot(pltpu.bitcast(f, BF16), rhs, preferred_element_type=F32)
            y = once(("y", i, c0, odd), mm)
            a = once(("a", i), lambda: 2 * j + i)
            q16 = once(("qa", i), lambda: window16("qa", a * HS, HS))
            o16 = once(("oa", i), lambda: window16("oa", a * HS, HS))
            flip = lambda w: jnp.take_along_axis(
                w, 7 - lax.broadcasted_iota(jnp.int32, (8, 128), 0), axis=0, mode="promise_in_bounds")
            for u in range(4):
                val = y[m:m + 16, u * 128:(u + 1) * 128]
                if not odd:
                    st("even", u * T // 2 + m, val)
                    continue
                even, mid = ld("even", u * T // 2 + m, 16), (c0 + u) * T + T // 2
                low = add(even, val)
                for row, out in ((mid + m, sub(even, val)),
                                 (mid - 16 - m, _rows(flip(low[8:]), flip(low[:8])))):
                    o16[at(row, 16), :] = mul(q16[at(row, 16), :].astype(F32), out).astype(BF16)
            memo["clock"] = y[m + 8:m + 16, 384:]

        def idft_list(i, *c0s):
            return [(16, P(idft, i, c0, odd, m)) for c0 in c0s
                    for odd in range(2) for m in range(0, T // 2, 16)]

        def xprep(x, u, r):
            halves = []
            for m in (r, r + 8):
                a, b = (pltpu.bitcast(x[pl.ds(2 * m, 16), pl.ds(t * 128, 128)], U32)
                        for t in (u, u + 4))
                a = pace(a)
                blocks = _lo(a), _lo(b), _hi(a), _hi(b)
                halves.append([_factor(rule, blocks.__getitem__) for rule in LEFT])
            for i, pair in enumerate(zip(*halves)):
                st16("xs", ((4 * i + u) * E0 + r) // 2, _rows(*pair))

        def xprep_list(x):
            return [(27, P(xprep, x, u, r)) for r in range(0, e, 16) for u in range(4)]

        def xprep2(x, u, r, i):
            def block(b):
                w = once(("x", u, r, b % 2), lambda: [pltpu.bitcast(
                    x[pl.ds(c // 2 * e + 2 * r, 32), pl.ds((u + c % 2 * 2 + b % 2 * 4) * 128, 128)], U32)
                    for c in range(4)])
                return [(_lo, _hi)[b // 2](v) for v in w]
            b0, *rest = LEFT[i]
            a = list(once(("left", u, r, b0), P(block, b0)))
            a[0], a[3] = paced(a[0]), paced(a[3])
            if rest:
                a = list(map(rest[0], a, once(("left", u, r, rest[1]), P(block, rest[1]))))
            for n, k in enumerate(LEFT_SUMS):
                st16("xt", ((5 * i + n) * 2 + u) * E0 // 4 + r // 2, _factor(LEFT[k], a.__getitem__))

        def xprep2_list(x):
            return [(c, P(xprep2, x, u, r, i)) for r in range(0, e // 2, 16) for u in range(2)
                    for i, c in ((1, 25), (0, 33), (6, 33), (4, 25), (3, 17), (5, 33), (2, 25))]

        def oprep(name, r0, n, which, u, r):
            a = lambda b: once(("o", name, u, r, b), lambda: ld(
                "o", (u + b % 2 * 4) * R0 + r0 + b // 2 * n + r, 16, 1 + (name == "xu")))
            memo["o", name, u, r, 3] = paced(a(3))
            for i in which:
                st16(name, ((4 * i + u) * E0 + r) // 2, _factor(LEFT[i], a))

        def oprep_list(name, r0, n, which=range(7)):
            return [(18, P(oprep, name, r0, n, which, u, r)) for r in range(0, n, 16) for u in range(4)]

        def oprep2(r0, n, i, u, r):
            view = once(("oprep", i), lambda: window("o", fresh(), NT * R0))
            block = lambda b, c: view[at(
                (u + c % 2 * 2 + b % 2 * 4) * R0 + r0 + b // 2 * n + c // 2 * n // 2 + r, 16), :]
            b0, *rest = LEFT[i]
            a = [block(b0, c) for c in range(4)]
            a = [x if c % 3 else paced(x) for c, x in enumerate(a)]
            if rest:
                a = [rest[0](x, block(rest[1], c)) for c, x in enumerate(a)]
            for k, val in enumerate([_factor(rule, a.__getitem__) for rule in LEFT]):
                st16(f"os{i}", (k * 2 + u) * E0 // 4 + r // 2, val)

        def oprep2_list(r0=0, n=e):
            return [(19 + 8 * (i in LEFT_SUMS), P(oprep2, r0, n, i, u, r))
                    for i in ORDER for r in range(0, n // 2, 16) for u in range(2)]

        def emit(p, r0, n, par, t, m, val, end):
            if p == 0:
                st("q", (par * NT + t) * E0 + m, val)
            elif p == 1:
                row = (par * NT + t + 1) * KL - e
                if m == 0 and not first:
                    st("k", row - WIN, ld("k", row + e - WIN, z=3))
                st("k", row + m, val)
            elif p == 2:
                st("v", (par * NT + t) * VL + 16 + m, val)
                if m == 0 and first and par == 0:
                    for other in range(2):
                        st("v", (other * NT + t) * VL + 8, jnp.broadcast_to(val[0:1], (WIN, 128)))
            else:
                base = once("row", lambda: j * E)
                o16 = once("ob", lambda: window16("ob", base, (NT - 1) * HS + (E0 if last else E)))
                o16[at(t * S + r0 + par * n + m, 16), :] = val.astype(BF16)
                if last and r0 + 2 * n == R0 and t >= 6:
                    if (m + 16) % (n // 2) == 0:
                        ob_copy(t, base + (r0 + par * n + m + 16 - n // 2) // 2, n // 4).start()
                elif m + 16 == end and par == t // 4:
                    ob_copy(t, base + r0 // 2, n).start()

        def plain(n, t, m):
            def mm():
                w = [ld("w0", (n // 2 * NT + t + u) * KW + n % 2 * KW // 2, KW // 2, 3) for u in range(2)]
                return jnp.dot(xa[pl.ds(0, R0), pl.ds(n * D // 4, D // 4)],
                               jnp.concatenate([pltpu.bitcast(v, BF16) for v in w], axis=1),
                               preferred_element_type=F32)
            res = once(("plain", n, t), mm)
            memo["clock"] = res[m:m + 8, :128]
            for u in range(2):
                val = res[m:m + 16, u * 128:(u + 1) * 128]
                if n:
                    val = add(val, ld("qo"[n % 2], (t + u) * R0 + m, 16))
                st("oq"[n % 2], (t + u) * R0 + m, val)

        def plain_list():
            return [(16, P(plain, n, t, m))
                    for n in range(4) for t in range(0, NT, 2) for m in range(0, R0, 16)]

        def combine(level, i, row, res, out, ahead=None):
            get = lambda name, z=0: ld(name + level, row, 16, z)
            if i in (0, 2, 4):
                st("abc"[i // 2] + level, row, res)
            elif i == 1:
                st("d" + level, row, res if ahead == 1 else sub(res, get("b")))
                out(1, 0, add(get("a"), res))
            elif i == 3 and ahead == 6:
                out(0, 1, add(get("b", 1), res))
                out(1, 1, add(add(get("e"), get("c", 1)), sub(res, get("a", 1))))
            elif i == 3:
                st("e" + level, row, sub(res, get("a", 1)))
                out(0, 1, add(get("b", 1), res))
            elif i == ahead:
                st("e" + level, row, res)
            else:
                part = add(get("de"[i - 5]), get("c", i - 5))
                out(i - 5, i - 5, add(sub(part, get("b")) if (i, ahead) == (5, 1) else part, res))

        def tiles(name, starts, n):
            view = window(name, fresh(), _BUFS[name][1])
            return jnp.concatenate(
                [pltpu.bitcast(view[at(row, n // 2), :], BF16) for row in starts], axis=1)

        def product(p, src, r0, n, ahead, t, i, m):
            res = once(("product", p, r0, t, i), lambda: jnp.dot(
                tiles(src, [(4 * i + u) * E0 // 2 for u in range(4)], n),
                pltpu.bitcast(factor(p, i, t), BF16), preferred_element_type=F32))
            memo["clock"] = res[m:m + 8]
            combine("1", i, t * E0 + m, res[m:m + 16],
                    lambda par, h, val: emit(p, r0, n, par, t + 4 * h, m, val, n), ahead)

        def strassen(p, src="xs", r0=0, n=e, order=ORDER, ahead=None):
            return [(16, P(product, p, src, r0, n, ahead, t, i, m))
                    for t in range(4) for i in order for m in range(0, n, 16)]

        def product2(p, r0, n, i, k, m):
            def mm():
                if p == 3:
                    name, row, gap = f"os{i}", k * E0 // 2, E0 // 4
                elif k in LEFT_SUMS:
                    name, row, gap = "xt", (5 * i + LEFT_SUMS.index(k)) * E0 // 2, E0 // 4
                else:
                    name, row, gap = "xs", 2 * i * E0 + (k == 1) * (E0 + n // 4), E0 // 2
                if k in RIGHT_SUMS:
                    w = [ld(f"wt{p}", ((5 * i + RIGHT_SUMS.index(k)) * 2 + u) * KW // 2, KW // 2, 3)
                         for u in range(2)]
                else:
                    w = [factor(p, i, k + u, k * KW // 4, KW // 2) for u in range(2)]
                return jnp.dot(tiles(name, (row, row + gap), n // 2),
                               jnp.concatenate([pltpu.bitcast(v, BF16) for v in w], axis=1),
                               preferred_element_type=F32)
            res = once(("product2", p, i, k), mm)
            memo["clock"] = res[m + 8:m + 16, :128]

            def out(u, r2, c2, val):
                t, row = 2 * c2 + u, r2 * n // 2 + m
                combine("1", i, t * E0 + row, val, lambda par, h, v: emit(
                    p, r0, n, par, t + 4 * h, row, v, (1 + c2) * n // 2))
            for u in range(2):
                combine("2", k, u * E0 // 2 + m, res[m:m + 16, u * 128:(u + 1) * 128], P(out, u))

        def strassen2(p, deep=7, r0=0, n=e):
            return [task for i in ORDER for task in (
                [(16, P(product2, p, r0, n, i, k, m)) for k in ORDER for m in range(0, n // 2, 16)]
                if i < deep else strassen(p, order=(i,)))]

        quarter = lax.shift_right_logical(lax.broadcasted_iota(jnp.int32, (8, 128), 1), 5)
        low, middle, odd = quarter < 2, (quarter == 1) | (quarter == 2), (quarter & 1) == 1

        def qk(par, m, w):
            query = lambda t: (bufs["q"][at(t * R0 + 2 * m + par, 8, 2), :] if first
                               else ld("q", (par * NT + t) * E0 + m))
            fold = lambda mask, a, b, shift: add(
                lax.select(mask, a, b), pltpu.roll(lax.select(mask, b, a), shift, 1))
            g = m // 8 % 4
            scale = once(("scale", par, m),
                         lambda: pace(jnp.full((8, 128), DH ** -0.5 * LOG2E, F32)))
            if first and g == 1:
                scale = once(("flush", par, m), lambda: lax.select(
                    never, window("v", fresh() + 16, 8)[...], scale))
            qv = once(("qv", par, m), lambda: [mul(query(t), scale) for t in range(NT)])
            s = _tree([mul(qv[t], ld("k", (par * NT + t + 1) * KL - e + m - w)) for t in range(NT)])
            if g % 2:
                s = fold((low, middle)[g // 2], memo["s", 0], pace(s), 64)
            if g == 3:
                s = fold(odd, memo["s", 1, w], s, 32)
                if first and m == 24 and w:
                    early = lax.broadcasted_iota(jnp.int32, (8, 128), 0) < w
                    s = jnp.where(early & (quarter == 1), -1e9 * LOG2E, s)
            memo[(("s", 0), ("s", 1, w), ("s", 0), ("lg", par, m, w))[g]] = s

        def expo(r):
            lg = [memo[("lg", *r, w)] for w in range(WIN)]
            top = pace(functools.reduce(lax.max, lg))
            memo["e", r] = [lax.exp2(sub(s, top)) for s in lg]

        def norm(r):
            total = pace(_tree(memo["e", r]))
            memo["inv", r] = total, pl.reciprocal(total, approx=True)

        def probs(r):
            total, inv = memo["inv", r]
            inv = pace(inv)
            inv = mul(inv, sub(np.float32(2), mul(total, inv)))
            for w, x in enumerate(memo["e", r]):
                st("quad", 8 * w, mul(x, inv))

        def spread(u, r):
            row = lambda w, g: (2 * w + r[0]) * HS + r[1] - 24 + 8 * g
            for w in (2 * u, 2 * u + 1):
                x = pace(ld("quad", 8 * w))
                y = pltpu.roll(x, 64, 1)
                for a, groups in ((lax.select(low, x, y), (0, 3)), (lax.select(low, y, x), (1, 2))):
                    b = pltpu.roll(a, 32, 1)
                    st("p", row(w, groups[0]), lax.select(odd, a, b))
                    st("p", row(w, groups[1]), lax.select(odd, b, a))

        def qk_list():
            rs, gap = [(par, m) for par in range(2) for m in range(0, e, 8)], 2 + first
            stages = [(expo, 20), (norm, 20 + gap), (probs, 20 + 2 * gap)] + [
                (P(spread, u), 22 + 2 * gap + 2 * u) for u in range(4)]
            out = [[(0, P(qk, *rs[n + u], w))]
                   for n in range(0, len(rs), 2) for w in range(WIN) for u in range(2)]
            out += [[] for _ in range(stages[-1][1])]
            for n in range(3, len(rs), 4):
                for f, lag in stages:
                    out[WIN * n + WIN - 1 + lag].append((0, P(f, rs[n])))
            return [(22, P(_run, tasks)) for tasks in out]

        def pv(par, m, t):
            p = once(("pv", par, m), lambda: [
                (pace if w % 4 == 0 else lambda v: v)(ld("pr", (2 * w + par) * HS + m))
                for w in range(WIN)])
            row = (par * NT + t) * VL + 16 + m
            bufs["o"][at(t * R0 + 2 * m + par, 8, 2), :] = pace(
                _tree([mul(p[w], ld("vr", row - w)) for w in range(WIN)]))

        def pv_list(m0, m1):
            return [(16, P(pv, par, m, t))
                    for par in range(2) for m in range(m0, m1, 8) for t in range(NT)]

        if first:
            main = plain_list() + sum((strassen(1, order=order, ahead=6) for order in (
                (0,), (6,), (2,), (1, 4, 5, 3))), []) + strassen(2)

            def phase(end, side=(), arrival=None):
                _weave(main[memo.get("done", 0):end], side)
                memo["done"] = end
                if arrival:
                    arrival(late()).wait()

            def permute(tasks, side=(), early=()):
                if early:
                    phase(memo["done"] + 46, _merge(tasks[:16], early))
                    tasks = tasks[16:]
                phase(memo["done"] + 8 * len(tasks) // 3, _merge(tasks, side))
                phase(memo["done"] + 26)

            xp, rq = xprep_list(xa), right_list(0)
            tk, rk, tv, rv = (right_list(p, which) for p in (1, 2) for which in ((6,), (1, 3, 4, 5)))
            dq = right2_list(0, [i for i in ORDER if i < DEEP_Q])
            do = right2_list(2, (0, 6, 2, 1, 4, 5, 3)) + sum(
                (right2_list(3, ORDER, 8 * n, 16) for n in range(2)), [])
            w_copy(0, 0, 2).wait()
            _run(perm_list(0, (0,)))
            memo["clock"] = pltpu.bitcast(ld("w0", KW + 120, z=3), F32)
            x0_copy(0, late()).wait()
            phase(64, [], P(w_copy, 0, 1, 2))
            permute(perm_list(0, (1,)))
            phase(150, [], P(x0_copy, 1))
            phase(190, xp[:24], P(w_copy, 1, 0, 2))
            permute(perm_list(1, (0,)), xp[24:48])
            phase(258, xp[48:52], P(w_copy, 1, 1, 2))
            permute(perm_list(1, (1,)), xp[52:])
            phase(380, rq[:40], P(w_copy, 2, 0, 1))
            permute(perm_list(2), rq[40:] + dq[:56])
            phase(506, tk[:14], P(w_copy, 3, 0, 1))
            permute(perm_list(3, ts=(4, 5, 0, 1, 6, 2, 7, 3)), dq[56:], tk[14:])
            phase(630, rk[:7], P(w_copy, 4, 0, 1))
            permute(perm_list(4), rk[7:])
            phase(752, do[:22], P(w_copy, 5, 0, 1))
            permute(perm_list(5), do[22:64], tv)
            phase(880, rv[:14], P(w_copy, 6, 0, 1))
            _start(sum((in_copies(n, second) for n in range(NS) for second in range(2)), []))
            phase(996, _merge(wo_list(0), rv[14:] + do[64:112]))
            phase(1000, [], P(w_copy, 7, 0, 1))
            phase(1004)
            phase(1070, _merge(wo_list(1), do[112:126]))
            logits = qk_list()
            phase(len(main) - 8, _merge(do[126:-64], logits[:-34])
                  + _merge(do[-64:-18], [(5, f) for _, f in logits[-34:]]) + do[-18:])
            _wait(small_copies(late()))
            skf, df = sk_ref[...].astype(F32), d_ref[...].astype(F32)
            for t in range(NT):
                for i in range(4):
                    taps[t, i] = jnp.broadcast_to(skf[i:i + 1, t * 128:(t + 1) * 128], (8, 128))
                taps[t, 4] = jnp.broadcast_to(df[t:t + 1, :], (8, 128))
            phase(len(main))
            return

        views.update(pr=shifted("p", j * E, NS * E), vr=shifted("v", j * E, NS * E))
        if last:
            n = E0 // 4
            _run(pv_list(n // 2, n) + oprep_list("xs", 0, n, (0, 1)))
            main = strassen(3, "xs", 0, n, (0,), 1) + strassen(3, "xs", 0, n, (1,), 1)
            _weave(main[:24], pv_list(0, n // 2) + oprep_list("xu", 0, n, range(2, 7)))
            main = main[24:] + strassen(3, "xu", 0, n, (2, 4, 5, 3, 6), 1)
            _weave(main[:-16], pv_list(n, 2 * n) + oprep_list("xt", 2 * n, n))
            _run(main[-16:])
            main = strassen(3, "xt", 2 * n, n) + strassen2(3, 7, 4 * n, 2 * n)
            pre = oprep2_list(4 * n, 2 * n)
            _weave(main[:100], pv_list(2 * n, 4 * n) + pre[:8])
            _weave(main[100:166], pre[8:])
            _run(main[166:])
            return

        for name in "vp":
            views[name] = shifted(name, E0 + j * E, E0 + (NS - 1) * E)
        head, tail, x = strassen(1) + strassen2(0, DEEP_Q), strassen2(2), xa.at[rows(j)]
        for u in range(4):
            _weave(dft_list(0, "hf", 4 * u), a1_list(0, 11 * u // 4, 11 * (u + 1) // 4))
        extra = _split(xprep_list(x), 4, 6)
        _weave(dft_list(0, "xf", 0), a1_list(0, 11, 13))
        _weave(dft_list(0, "xf", 4), _merge(a1_list(0, 13, 16), extra[0]))
        _weave(dft_list(0, "xf", 8, 12)[:20], extra[1])
        _run(dft_list(0, "xf", 12)[4:])
        _weave(head[:66], xprep2_list(x))
        conv = a3_list(0)
        conv.insert(24 * 42, (0, lambda: _wait(in_copies(j, 1, late()))))
        _weave(head[66:406], conv)
        _run(head[406:416])
        for u in range(4):
            _run(idft_list(0, 4 * u))
            _weave(dft_list(1, "hf", 4 * u), a1_list(1, 3 * u, 3 * u + 3))
        oa_copy(2 * j).start()
        _weave(dft_list(1, "xf", 0), a1_list(1, 12, 16))
        mix, pre, conv = _split(pv_list(0, E), 2, 5), _split(oprep2_list(), 6, 1), a3_list(1)
        _weave(dft_list(1, "xf", 4, 8, 12), mix[0])
        _weave(head[416:528], mix[1])
        side = pre[0]
        for n, part in enumerate(_split(pre[1], *[1] * 7)):
            side = side + conv[24 * n:24 * n + 24] + part
        _weave(head[528:] + strassen2(3) + tail[:20], side + conv[24 * 7:])
        tail += idft_list(1, 0, 4, 8, 12)
        _weave(tail[20:-16], qk_list())
        _run(tail[-16:])
        oa_copy(2 * j + 1).start()

    def loop(j, carry):
        _wait(in_copies(j, 0))
        step(j)
        return carry

    step(0, first=True)
    lax.fori_loop(0, NS, loop, 0)
    step(NS, last=True)
    for i, name in enumerate(("oa", "ob")):
        pltpu.make_async_copy(raw[name], raw[name], sem_out.at[i]).wait()


@jax.jit
def pallas_concat_heads__ssm_conv_h3__sliding_local_dilated__prompt_kernel(
    A_q, A_k, A_v, A_shift_k, A_ssm_k, A_ssm_D, B_x, B_wqkv, B_wo,
):
    hbm = pl.BlockSpec(memory_space=pl.ANY)
    out = pl.pallas_call(
        _kernel,
        in_specs=[hbm] * 10,
        out_specs=hbm,
        out_shape=jax.ShapeDtypeStruct((S, 2 * D), BF16),
        scratch_shapes=[
            pltpu.VMEM((NT, 128, S), BF16),
            pltpu.VMEM((S, D), BF16),
            pltpu.VMEM((8, D // 2, D), BF16),
            pltpu.VMEM((NT, 5, 8, 128), F32),
            pltpu.VMEM(_TABLE.shape, U32),
            pltpu.SemaphoreType.DMA((2 * NS + 14,)),
            pltpu.SemaphoreType.DMA((2,)),
        ] + [pltpu.VMEM((r * 4 // np.dtype(t).itemsize, 128), t) for t, r in _BUFS.values()]
        + [pltpu.VMEM((4, D), BF16), pltpu.VMEM((8, 128), BF16)],
        compiler_params=pltpu.CompilerParams(
            vmem_limit_bytes=118 * 1024 * 1024, disable_bounds_checks=True,
            disable_semaphore_checks=True, flags={"XLA_TPU_RESCHEDULE_DMA_DONES": True}),
        name="fused",
    )(A_q[0], A_k[0], A_v[0], A_shift_k.T, A_ssm_k,
      A_ssm_D.reshape(8, 128), B_x[0], B_wqkv, B_wo, _TABLE)
    return out[None]
```
